```python
import jax
import jax.numpy as jnp

def _softmax(x, axis=-1):
    return jax.nn.softmax(x, axis=axis)
def _gelu(x):
    return jax.nn.gelu(x, approximate=True)
def _silu(x):
    return jax.nn.silu(x)
def _sigmoid(x):
    return jax.nn.sigmoid(x)
def _layernorm(x, axis=-1, eps=1e-5):
    m = jnp.mean(x, axis=axis, keepdims=True)
    v = jnp.var(x, axis=axis, keepdims=True)
    return (x - m) / jnp.sqrt(v + eps)
def _scatter_add(tgt, idx, src, axis=0):
    return tgt.at[idx].add(src)
def _segment_sum(src, seg, n):
    return jax.ops.segment_sum(src, seg, n)
class _Rng:
    def __init__(self, key):
        self._k = key
    def _next(self):
        self._k, sub = jax.random.split(self._k)
        return sub
    def normal(self, shape):
        return jax.random.normal(self._next(), shape, dtype=jnp.bfloat16)
    def randint(self, lo, hi, shape):
        return jax.random.randint(self._next(), shape, lo, hi, dtype=jnp.int32)
    def uniform(self, shape, lo=0.0, hi=1.0):
        return jax.random.uniform(self._next(), shape, jnp.bfloat16, lo, hi)
    def permutation(self, n):
        return jax.random.permutation(self._next(), n)


kernel_name = 'concat_heads__sliding_local_dilated__compressed_kv_cla__prompt'

def setup_inputs():
    _rng = _Rng(jax.random.key(int.from_bytes(__import__("os").urandom(4), "little")))
    _w = (lambda a: (lambda t: t.astype(jnp.bfloat16) if jnp.issubdtype(t.dtype, jnp.floating) else t)(jnp.asarray(a)))
    def _A_setup():
        B, S, D = 1, 2048, 1024
        return {
            "x": _w((lambda *s: _rng.normal(s) * 0.05)(B, S, D)),
            "wqkv": _w((lambda *s: _rng.normal(s) * 0.05)(D, 3 * D)),
            "wo": _w((lambda *s: _rng.normal(s) * 0.05)(D, D)),
        }
    _A_in = _A_setup()

    def _B_setup():
        B, H, Sq, Sk, D, M = 1, 32, 2048, 2048, 128, 1024
        Dc = 4 * D
        return {
            "x": _w((lambda *s: _rng.normal(s) * 0.05)(B, Sq, M)),
            "c_kv": _w((lambda *s: _rng.normal(s) * 0.05)(B, Sk, Dc)),
            "w_q": _w((lambda *s: _rng.normal(s) * 0.05)(M, H, D) * (M ** -0.5)),
            "w_uk": _w((lambda *s: _rng.normal(s) * 0.05)(Dc, H, D) * (Dc ** -0.5)),
            "w_uv": _w((lambda *s: _rng.normal(s) * 0.05)(Dc, H, D) * (Dc ** -0.5)),
            "w_o": _w((lambda *s: _rng.normal(s) * 0.05)(H, D, M) * ((H * D) ** -0.5)),
        }
    _B_in = _B_setup()

    return {
        "A_x": _A_in["x"],
        "A_wqkv": _A_in["wqkv"],
        "A_wo": _A_in["wo"],
        "B_x": _B_in["x"],
        "B_c_kv": _B_in["c_kv"],
        "B_w_q": _B_in["w_q"],
        "B_w_uk": _B_in["w_uk"],
        "B_w_uv": _B_in["w_uv"],
        "B_w_o": _B_in["w_o"],
    }

def reference(A_x, A_wqkv, A_wo, B_x, B_c_kv, B_w_q, B_w_uk, B_w_uv, B_w_o):
    def _A_ref(x, wqkv, wo):
        B, S, D = x.shape
        H = 32; Dh = D // H
        W, dil = 8, 2
        qkv = (lambda x, *d: x.transpose(*d))((x @ wqkv).reshape(B, S, 3, H, Dh), 2, 0, 3, 1, 4)
        q, k, v = qkv[0], qkv[1], qkv[2]
        scale = Dh ** -0.5
        pos = jnp.arange(S)
        off = jnp.arange(W) * dil
        idx = pos[:, None] - off[None, :]
        mask = idx >= 0
        idx_c = jnp.where(mask, idx, 0).reshape(-1)
        kg = k[:, :, idx_c, :].reshape(B, H, S, W, Dh)
        vg = v[:, :, idx_c, :].reshape(B, H, S, W, Dh)
        logits = jnp.einsum("bhsd,bhswd->bhsw", q, kg) * scale
        logits = jnp.where(mask[None, None, :, :], logits, -1e9)
        attn = _softmax(logits, axis=-1)
        o = jnp.einsum("bhsw,bhswd->bhsd", attn, vg)
        return (lambda x, *d: x.transpose(*d))(o, 0, 2, 1, 3).reshape(B, S, D) @ wo

    def _B_ref(x, c_kv, w_q, w_uk, w_uv, w_o):
        B, Sq, M = x.shape[0], x.shape[1], x.shape[2]
        Sk = c_kv.shape[1]
        H, D = w_q.shape[1], w_q.shape[2]
        q = jnp.einsum("bqm,mhd->bhqd", x, w_q)
        k = jnp.einsum("bkc,chd->bhkd", c_kv, w_uk)
        v = jnp.einsum("bkc,chd->bhkd", c_kv, w_uv)
        scores = jnp.einsum("bhqd,bhkd->bhqk", q, k) * (D ** -0.5)
        off = Sk - Sq
        qi = jnp.arange(Sq)[:, None]
        kj = jnp.arange(Sk)[None, :]
        cmask = kj <= (qi + off)
        scores = jnp.where(cmask[None, None], scores, -1e9)
        p = _softmax(scores, axis=-1)
        ctx = jnp.einsum("bhqk,bhkd->bhqd", p, v)
        return jnp.einsum("bhqd,hdm->bqm", ctx, w_o)

    a = _A_ref(A_x, A_wqkv, A_wo)
    b = _B_ref(B_x, B_c_kv, B_w_q, B_w_uk, B_w_uv, B_w_o)
    return jnp.concatenate([a, b], axis=-1)
```

```python
import functools

import jax
import jax.numpy as jnp
from jax import lax
import jax.experimental.pallas as pl
import jax.experimental.pallas.tpu as pltpu

S = 2048
DM = 1024
LANES = 128
A_HEADS, A_DH, A_WIN, A_DIL = 32, 32, 8, 2
HALO = 16
B_HEADS, B_DH, B_DC = 32, 128, 512

LOG2E = 1.4426950408889634
NEG = -1e9
NT_DIMS = (((1,), (1,)), ((), ()))


def _dot(a, b):
    return jnp.dot(a, b, preferred_element_type=jnp.float32)


def _dot_nt(a, b):
    return lax.dot_general(a, b, NT_DIMS, preferred_element_type=jnp.float32)


def _swap_group_and_lane_bits(groups):
    lane = lax.broadcasted_iota(jnp.int32, groups[0].shape, 1)
    groups = list(groups)
    for t in range(3):
        shift = 4 << t
        low = (lane & shift) == 0
        for g in range(8):
            if g & (1 << t):
                continue
            x, y = groups[g], groups[g | (1 << t)]
            groups[g] = jnp.where(low, x, pltpu.roll(y, shift, 1))
            groups[g | (1 << t)] = jnp.where(low, pltpu.roll(x, LANES - shift, 1), y)
    return groups


def _kernel(xa_hbm, wqkv_hbm, woa_hbm, xb_hbm, c_hbm, wq_hbm, wuk_hbm, wuv_hbm, wob_hbm,
            out_hbm,
            xb, cb, wq_raw, wuk_raw, wuv_raw, wq_s, wkv_s, q_s, k_s, v_s, ctx,
            xa, wqkv_raw, wqkv_s, woa, wob, ka, va, obuf,
            sem_x, sem_w, sem_p, sem_o, *, cfg):
    BQ = cfg["bq"]
    BR = cfg["br"]
    NB = S // BQ
    NR = S // BR
    PROWS = DM // B_HEADS

    wq_u = wq_hbm.bitcast(jnp.uint32)
    wuk_u = wuk_hbm.bitcast(jnp.uint32)
    wuv_u = wuv_hbm.bitcast(jnp.uint32)

    def pair_copies(j, slot):
        return (
            pltpu.make_async_copy(wuk_u.at[:, j, :], wuk_raw.at[slot], sem_w.at[slot, 0]),
            pltpu.make_async_copy(wuv_u.at[:, j, :], wuv_raw.at[slot], sem_w.at[slot, 1]),
            pltpu.make_async_copy(wq_u.at[:, j, :], wq_raw.at[slot], sem_w.at[slot, 2]),
        )

    def wqkv_copy(h):
        rows = pl.ds(pl.multiple_of(h * PROWS, PROWS), PROWS)
        return pltpu.make_async_copy(wqkv_hbm.at[rows, :], wqkv_raw.at[h % 2], sem_p.at[h % 2])

    late = (
        pltpu.make_async_copy(wob_hbm, wob, sem_x.at[2]),
        pltpu.make_async_copy(xa_hbm, xa, sem_x.at[3]),
        pltpu.make_async_copy(woa_hbm, woa, sem_x.at[4]),
    )
    cp_c = pltpu.make_async_copy(c_hbm, cb, sem_x.at[0])
    cp_x = pltpu.make_async_copy(xb_hbm, xb, sem_x.at[1])

    for cp in pair_copies(0, 0):
        cp.start()
    cp_c.start()
    cp_x.start()
    wqkv_copy(0).start()

    def unpack_weights(h):
        slot = (h // 2) % 2
        sh = (16 * (1 - h % 2)).astype(jnp.uint32)

        def half(u):
            return pltpu.bitcast((u << sh) & jnp.uint32(0xFFFF0000), jnp.float32).astype(jnp.bfloat16)

        wkv_s[:, 0:B_DH] = half(wuk_raw[slot])
        wkv_s[:, B_DH:2 * B_DH] = half(wuv_raw[slot])
        wq_s[...] = half(wq_raw[slot])

    def project(i):
        rows = slice(i * BQ, (i + 1) * BQ)
        kv = _dot(cb[rows, :], wkv_s[...])
        k_s[rows, :] = kv[:, :B_DH].astype(jnp.bfloat16)
        v_s[rows, :] = kv[:, B_DH:].astype(jnp.bfloat16)
        q = _dot(xb[rows, :], wq_s[...])
        q_s[rows, :] = (q * (B_DH ** -0.5 * LOG2E)).astype(jnp.bfloat16)

    def scores(i):
        row = lax.broadcasted_iota(jnp.int32, (LANES, LANES), 0)
        col = lax.broadcasted_iota(jnp.int32, (LANES, LANES), 1)
        r0 = i * BQ
        full = _dot_nt(q_s[r0:r0 + BQ, :], k_s[0:r0, :]) if i else None
        diag = []
        for a in range(BQ // LANES):
            d = _dot_nt(q_s[r0 + a * LANES:r0 + (a + 1) * LANES, :], k_s[r0:r0 + (a + 1) * LANES, :])
            last = jnp.where(col <= row, d[:, a * LANES:], NEG)
            diag.append(jnp.concatenate([d[:, :a * LANES], last], axis=1) if a else last)
        return full, diag

    def softmax(i, sc):
        full, diag = sc
        nsub = BQ // LANES
        ms = []
        for a in range(nsub):
            m = jnp.max(diag[a], axis=1, keepdims=True)
            if full is not None:
                m = jnp.maximum(m, jnp.max(full[a * LANES:(a + 1) * LANES], axis=1, keepdims=True))
            ms.append(m)
        pd = [jnp.exp2(diag[a] - ms[a]) for a in range(nsub)]
        ls = [jnp.sum(p, axis=1, keepdims=True) for p in pd]
        pf = None
        if full is not None:
            pf = jnp.exp2(full - (jnp.concatenate(ms, axis=0) if nsub > 1 else ms[0]))
            lf = jnp.sum(pf, axis=1, keepdims=True)
            ls = [ls[a] + lf[a * LANES:(a + 1) * LANES] for a in range(nsub)]
            pf = pf.astype(jnp.bfloat16)
        return pf, [p.astype(jnp.bfloat16) for p in pd], ls

    def context(h, i, sm):
        pf, pd, ls = sm
        r0 = i * BQ
        of = _dot(pf, v_s[0:r0, :]) if pf is not None else None
        for a in range(BQ // LANES):
            o = _dot(pd[a], v_s[r0:r0 + (a + 1) * LANES, :])
            if of is not None:
                o = o + of[a * LANES:(a + 1) * LANES]
            ctx[h, r0 + a * LANES:r0 + (a + 1) * LANES, :] = (o * (1.0 / ls[a])).astype(jnp.bfloat16)

    def relayout_wqkv(h):
        raw = wqkv_raw[h % 2]
        rows = pl.ds(pl.multiple_of(h * PROWS, PROWS), PROWS)
        for part in range(3):
            groups = [pltpu.bitcast(raw[:, part * DM + g * LANES:part * DM + (g + 1) * LANES], jnp.uint32)
                      for g in range(8)]
            groups = _swap_group_and_lane_bits(groups)
            for g in range(8):
                wqkv_s[rows, part * DM + g * LANES:part * DM + (g + 1) * LANES] = pltpu.bitcast(
                    groups[g], jnp.bfloat16)

    def stage_dma(h):
        @pl.when(h % 2 == 0)
        def _():
            for cp in pair_copies(h // 2, (h // 2) % 2):
                cp.wait()

            @pl.when(h + 2 < B_HEADS)
            def _():
                for cp in pair_copies(h // 2 + 1, (h // 2 + 1) % 2):
                    cp.start()

    cp_c.wait()
    cp_x.wait()

    if cfg["order"] == "asc":
        def head(h, carry):
            stage_dma(h)

            @pl.when(h == 0)
            def _():
                for cp in late:
                    cp.start()

            wqkv_copy(h).wait()

            @pl.when(h + 1 < B_HEADS)
            def _():
                wqkv_copy(h + 1).start()

            unpack_weights(h)
            la = cfg["ahead"]
            for i in range(min(la, NB)):
                project(i)
            sc = scores(0)
            for i in range(NB):
                if i + la < NB:
                    project(i + la)
                nxt = scores(i + 1) if i + 1 < NB else None
                context(h, i, softmax(i, sc))
                sc = nxt
            relayout_wqkv(h)
            return carry

        lax.fori_loop(0, B_HEADS, head, 0)
    else:
        stage_dma(jnp.int32(0))
        unpack_weights(jnp.int32(0))
        for i in range(NB):
            project(i)

        def head(h, carry):
            hn = jnp.minimum(h + 1, B_HEADS - 1)

            @pl.when(h + 1 < B_HEADS)
            def _():
                stage_dma(h + 1)

            @pl.when(h == 0)
            def _():
                for cp in late:
                    cp.start()

            wqkv_copy(h).wait()

            @pl.when(h + 1 < B_HEADS)
            def _():
                wqkv_copy(h + 1).start()

            unpack_weights(hn)
            sc = scores(NB - 1)
            for i in range(NB - 1, -1, -1):
                nxt = scores(i - 1) if i else None
                context(h, i, softmax(i, sc))
                project(i)
                sc = nxt
            relayout_wqkv(h)
            return carry

        lax.fori_loop(0, B_HEADS, head, 0)

    for cp in late:
        cp.wait()

    ka[:, 0:HALO, :] = jnp.zeros((8, HALO, LANES), jnp.float32)
    va[:, 0:HALO, :] = jnp.zeros((8, HALO, LANES), jnp.float32)

    def out_copy(r):
        rows = pl.ds(pl.multiple_of(r * BR, BR), BR)
        return pltpu.make_async_copy(obuf.at[r % 2], out_hbm.at[rows, :], sem_o.at[r % 2])

    def row_block(r, carry):
        slot = r % 2
        rows = pl.ds(pl.multiple_of(r * BR, BR), BR)

        @pl.when(r >= 2)
        def _():
            out_copy(r - 2).wait()

        x = xa[rows, :]
        kf = _dot(x, wqkv_s[:, DM:2 * DM])
        for g in range(8):
            ka[g, HALO:HALO + BR, :] = kf[:, g * LANES:(g + 1) * LANES]
        qf = _dot(x, wqkv_s[:, 0:DM]) * (A_DH ** -0.5 * LOG2E)
        vf = _dot(x, wqkv_s[:, 2 * DM:3 * DM])
        for g in range(8):
            va[g, HALO:HALO + BR, :] = vf[:, g * LANES:(g + 1) * LANES]

        cx = jnp.concatenate([ctx[hh, rows, :] for hh in range(B_HEADS)], axis=1)
        obuf[slot, :, DM:2 * DM] = _dot(cx, wob[...]).astype(jnp.bfloat16)

        CH = cfg["ch"]
        lane = lax.broadcasted_iota(jnp.int32, (CH, LANES), 1)
        odd1 = (lane & 1) != 0
        odd2 = (lane & 2) != 0
        o_chunks = []
        for c0 in range(0, BR, CH):
            qg = [qf[c0:c0 + CH, g * LANES:(g + 1) * LANES] for g in range(8)]
            logits = []
            for w in range(A_WIN):
                b0 = HALO + c0 - A_DIL * w
                acc = qg[0] * ka[0, b0:b0 + CH, :]
                for g in range(1, 8):
                    acc = acc + qg[g] * ka[g, b0:b0 + CH, :]
                acc = acc + jnp.where(odd1, pltpu.roll(acc, 1, 1), pltpu.roll(acc, LANES - 1, 1))
                acc = acc + jnp.where(odd2, pltpu.roll(acc, 2, 1), pltpu.roll(acc, LANES - 2, 1))
                if c0 < A_DIL * w:
                    pos = r * BR + c0 + lax.broadcasted_iota(jnp.int32, (CH, LANES), 0)
                    acc = jnp.where(pos >= A_DIL * w, acc, NEG * LOG2E)
                logits.append(acc)
            m = functools.reduce(jnp.maximum, logits)
            ps = [jnp.exp2(l - m) for l in logits]
            inv = 1.0 / functools.reduce(lambda a, b: a + b, ps)
            ps = [p * inv for p in ps]
            og = []
            for g in range(8):
                acc = None
                for w in range(A_WIN):
                    b0 = HALO + c0 - A_DIL * w
                    t = ps[w] * va[g, b0:b0 + CH, :]
                    acc = t if acc is None else acc + t
                og.append(pltpu.bitcast(acc.astype(jnp.bfloat16), jnp.uint32))
            og = _swap_group_and_lane_bits(og)
            o_chunks.append(jnp.concatenate([pltpu.bitcast(t, jnp.bfloat16) for t in og], axis=1))
        o = jnp.concatenate(o_chunks, axis=0)
        obuf[slot, :, 0:DM] = _dot(o, woa[...]).astype(jnp.bfloat16)

        ka[:, 0:HALO, :] = ka[:, BR:BR + HALO, :]
        va[:, 0:HALO, :] = va[:, BR:BR + HALO, :]
        out_copy(r).start()
        return carry

    lax.fori_loop(0, NR, row_block, 0)
    out_copy(NR - 2).wait()
    out_copy(NR - 1).wait()


DEFAULT_CFG = dict(bq=256, br=256, ch=16, order="asc", ahead=2)


def build(cfg=None):
    cfg = dict(DEFAULT_CFG, **(cfg or {}))
    BR = cfg["br"]

    def fn(A_x, A_wqkv, A_wo, B_x, B_c_kv, B_w_q, B_w_uk, B_w_uv, B_w_o):
        bf16, f32, u32 = jnp.bfloat16, jnp.float32, jnp.uint32
        out = pl.pallas_call(
            functools.partial(_kernel, cfg=cfg),
            out_shape=jax.ShapeDtypeStruct((S, 2 * DM), bf16),
            in_specs=[pl.BlockSpec(memory_space=pl.ANY)] * 9,
            out_specs=pl.BlockSpec(memory_space=pl.ANY),
            scratch_shapes=[
                pltpu.VMEM((S, DM), bf16),
                pltpu.VMEM((S, B_DC), bf16),
                pltpu.VMEM((2, DM, B_DH), u32),
                pltpu.VMEM((2, B_DC, B_DH), u32),
                pltpu.VMEM((2, B_DC, B_DH), u32),
                pltpu.VMEM((DM, B_DH), bf16),
                pltpu.VMEM((B_DC, 2 * B_DH), bf16),
                pltpu.VMEM((S, B_DH), bf16),
                pltpu.VMEM((S, B_DH), bf16),
                pltpu.VMEM((S, B_DH), bf16),
                pltpu.VMEM((B_HEADS, S, B_DH), bf16),
                pltpu.VMEM((S, DM), bf16),
                pltpu.VMEM((2, DM // B_HEADS, 3 * DM), bf16),
                pltpu.VMEM((DM, 3 * DM), bf16),
                pltpu.VMEM((DM, DM), bf16),
                pltpu.VMEM((B_HEADS * B_DH, DM), bf16),
                pltpu.VMEM((8, HALO + BR, LANES), f32),
                pltpu.VMEM((8, HALO + BR, LANES), f32),
                pltpu.VMEM((2, BR, 2 * DM), bf16),
                pltpu.SemaphoreType.DMA((5,)),
                pltpu.SemaphoreType.DMA((2, 3)),
                pltpu.SemaphoreType.DMA((2,)),
                pltpu.SemaphoreType.DMA((2,)),
            ],
            compiler_params=pltpu.CompilerParams(vmem_limit_bytes=120 * 2 ** 20),
            name="fused_local_and_latent_attention",
        )(A_x.reshape(S, DM), A_wqkv, A_wo, B_x.reshape(S, DM), B_c_kv.reshape(S, B_DC),
          B_w_q, B_w_uk, B_w_uv, B_w_o.reshape(B_HEADS * B_DH, DM))
        return out.reshape(1, S, 2 * DM)

    return jax.jit(fn)


@jax.jit
def pallas_concat_heads__sliding_local_dilated__compressed_kv_cla__prompt_kernel(
    A_x: jax.Array,
    A_wqkv: jax.Array,
    A_wo: jax.Array,
    B_x: jax.Array,
    B_c_kv: jax.Array,
    B_w_q: jax.Array,
    B_w_uk: jax.Array,
    B_w_uv: jax.Array,
    B_w_o: jax.Array,
):
    return build(dict(order='asc'))(A_x, A_wqkv, A_wo, B_x, B_c_kv, B_w_q, B_w_uk, B_w_uv, B_w_o)
```

```python
import functools

import jax
import jax.numpy as jnp
from jax import lax
import jax.experimental.pallas as pl
import jax.experimental.pallas.tpu as pltpu

S = 2048
DM = 1024
LANES = 128
A_DH, A_WIN, A_DIL = 32, 8, 2
HALO = 16
B_HEADS, B_DH, B_DC = 32, 128, 512

LOG2E = 1.4426950408889634
NEG = -1e9
F32, BF16, U32 = jnp.float32, jnp.bfloat16, jnp.uint32

A_TERMS = (((1, 0, 0), (1, 1, 1)), ((1, 1, 0), (1, 1, 1)), ((1, 0, 0),), ((1, 1, 1),),
           ((1, 0, 0), (1, 0, 1)), ((1, 1, 0), (-1, 0, 0)), ((1, 0, 1), (-1, 1, 1)))
B_TERMS = (((1, 0, 0), (1, 1, 1)), ((1, 0, 0),), ((1, 0, 1), (-1, 1, 1)), ((1, 1, 0), (-1, 0, 0)),
           ((1, 1, 1),), ((1, 0, 0), (1, 0, 1)), ((1, 1, 0), (1, 1, 1)))
C_USES = ((0, ((1, 0, 0), (1, 1, 1))), (3, ((1, 0, 0), (1, 1, 0))), (4, ((-1, 0, 0), (1, 0, 1))),
          (6, ((1, 0, 0),)), (1, ((1, 1, 0), (-1, 1, 1))), (2, ((1, 0, 1), (1, 1, 1))),
          (5, ((1, 1, 1),)))


def _pack(x):
    return pltpu.bitcast(x.astype(BF16), U32)


def _unpack(x):
    return pltpu.bitcast(x, BF16)


def _expand(blocks, terms, level):
    if level == 0:
        return [blocks[0][0].astype(BF16)]
    n = 1 << (level - 1)
    out = []
    for combo in terms:
        def entry(a, b):
            (_, i, k), *rest = combo
            acc = blocks[i * n + a][k * n + b]
            for sign, i, k in rest:
                other = blocks[i * n + a][k * n + b].astype(F32)
                acc = acc.astype(F32) + other if sign > 0 else acc.astype(F32) - other
            return acc
        out += _expand([[entry(a, b) for b in range(n)] for a in range(n)], terms, level - 1)
    return out


def _combine(product, level, base=0):
    if level == 0:
        return [[product(base)]]
    n = 1 << (level - 1)
    c = [[None] * (2 * n) for _ in range(2 * n)]
    for r, uses in C_USES:
        m = _combine(product, level - 1, base + r * 7 ** (level - 1))
        for sign, i, j in uses:
            for a in range(n):
                for b in range(n):
                    cur = c[i * n + a][j * n + b]
                    c[i * n + a][j * n + b] = (
                        m[a][b] if cur is None else cur + m[a][b] if sign > 0 else cur - m[a][b])
    return c


def _grid(get, rows, cols, level):
    n = 1 << level
    dr, dc = rows // n, cols // n
    return [[get(i * dr, (i + 1) * dr, k * dc, (k + 1) * dc) for k in range(n)] for i in range(n)]


def _swap_group_and_lane_bits(groups):
    lane = lax.broadcasted_iota(jnp.int32, groups[0].shape, 1)
    groups = list(groups)
    for t in range(3):
        shift = 4 << t
        low = (lane & shift) == 0
        for g in range(8):
            if g & (1 << t):
                continue
            x, y = groups[g], groups[g | (1 << t)]
            groups[g] = jnp.where(low, x, pltpu.roll(y, shift, 1))
            groups[g | (1 << t)] = jnp.where(low, pltpu.roll(x, LANES - shift, 1), y)
    return groups


def _reciprocal(x):
    r = pl.reciprocal(x, approx=True)
    return r * (2.0 - x * r)


def _kernel(xa_hbm, wqkv_hbm, woa_hbm, xb_hbm, c_hbm, wq_hbm, wuk_hbm, wuv_hbm, wob_hbm,
            out_hbm,
            xb_raw, c_raw, xs, cks, cvs, wq_raw, wuk_raw, wuv_raw, wqs, wks, wvs,
            q_s, k_s, v_s, ctx,
            wqkv_raw, woa_raw, wob_raw, wqkvs, woas, wobs, xa_raw, ka, va, obuf,
            sem_x, sem_w, sem_s, sem_a, sem_o, *, cfg):
    BQ, BR, G = cfg["bq"], cfg["br"], cfg["g"]
    LQ, LK, LV, LOB, LA, LOA = (cfg[n] for n in ("lq", "lk", "lv", "lob", "la", "loa"))
    NB, NR, NG = S // BQ, S // BR, B_HEADS // G
    PAIRS = G // 2
    if LK == LV:
        cvs = cks

    wq_u = wq_hbm.bitcast(U32)
    wuk_u = wuk_hbm.bitcast(U32)
    wuv_u = wuv_hbm.bitcast(U32)

    def head_weight_copies(g):
        slot = g % 2
        cps = []
        for p in range(PAIRS):
            j = g * PAIRS + p
            cps += [
                pltpu.make_async_copy(wuk_u.at[:, j, :], wuk_raw.at[slot, p], sem_w.at[slot, 3 * p]),
                pltpu.make_async_copy(wuv_u.at[:, j, :], wuv_raw.at[slot, p], sem_w.at[slot, 3 * p + 1]),
                pltpu.make_async_copy(wq_u.at[:, j, :], wq_raw.at[slot, p], sem_w.at[slot, 3 * p + 2]),
            ]
        return cps

    streams = ((wqkv_hbm, wqkv_raw, LA), (woa_hbm, woa_raw, LOA), (wob_hbm, wob_raw, LOB))

    def stream_copies(g):
        slot = g % 2
        cps = []
        for s, (src, dst, level) in enumerate(streams):
            part = src.shape[0] >> level
            rows = part // NG
            for k in range(1 << level):
                r0 = pl.multiple_of(k * part + g * rows, rows)
                cps.append(pltpu.make_async_copy(
                    src.at[pl.ds(r0, rows), :], dst.at[slot, k], sem_s.at[slot, 4 * s + k]))
        return cps

    def input_copies(i):
        rows = pl.ds(pl.multiple_of(i * BQ, BQ), BQ)
        return [pltpu.make_async_copy(c_hbm.at[rows, :], c_raw.at[i], sem_x.at[0, i]),
                pltpu.make_async_copy(xb_hbm.at[rows, :], xb_raw.at[i], sem_x.at[1, i])]

    def xa_copy(r):
        rows = pl.ds(pl.multiple_of(r * BR, BR), BR)
        return pltpu.make_async_copy(xa_hbm.at[rows, :], xa_raw.at[r % 2], sem_a.at[r % 2])

    def out_copy(r):
        rows = pl.ds(pl.multiple_of(r * BR, BR), BR)
        return pltpu.make_async_copy(obuf.at[r % 2], out_hbm.at[rows, :], sem_o.at[r % 2])

    def start(cps):
        for cp in cps:
            cp.start()

    def wait(cps):
        for cp in cps:
            cp.wait()

    def prepare_head_weights(g):
        slot = g % 2
        for raw, dst, level in ((wuk_raw, wks, LK), (wuv_raw, wvs, LV), (wq_raw, wqs, LQ)):
            n = 1 << level
            depth = raw.shape[2] // n
            for j0 in range(0, G, n):
                def block(k, j):
                    word = raw[slot, (j0 + j) // 2, k * depth:(k + 1) * depth, :]
                    word = word & U32(0xFFFF0000) if (j0 + j) % 2 else word << 16
                    return pltpu.bitcast(word, F32)
                ops = _expand([[block(k, j) for j in range(n)] for k in range(n)], B_TERMS, level)
                for r, op in enumerate(ops):
                    dst[j0 // n, r] = _pack(op)

    def prepare_inputs(i):
        for raw, dst, level in ((c_raw, cks, LK), (c_raw, cvs, LV), (xb_raw, xs, LQ))[
                (1 if LK == LV else 0):]:
            width = raw.shape[2]
            ops = _expand(_grid(lambda a, b, c, d: raw[i, a:b, c:d], BQ, width, level), A_TERMS, level)
            for r, op in enumerate(ops):
                dst[i, r] = _pack(op)

    def project(i, which):
        lhs, rhs, dst, level, scale = {
            "q": (xs, wqs, q_s, LQ, B_DH ** -0.5 * LOG2E),
            "k": (cks, wks, k_s, LK, None), "v": (cvs, wvs, v_s, LV, None)}[which]
        n = 1 << level
        rows = BQ // n
        for j0 in range(0, G, n):
            c = _combine(lambda r: jnp.dot(_unpack(lhs[i, r]), _unpack(rhs[j0 // n, r]),
                                           preferred_element_type=F32), level)
            for a in range(n):
                for b in range(n):
                    val = c[a][b] if scale is None else c[a][b] * scale
                    dst[j0 + b, pl.ds(pl.multiple_of((i * BQ + a * rows) // 2, rows // 2), rows // 2), :] = _pack(val)

    def head_rows(ref, h, r0, r1):
        return _unpack(ref[h, r0 // 2:r1 // 2, :])

    def scores(h, i):
        def nt(a, b):
            return lax.dot_general(a, b, (((1,), (1,)), ((), ())), preferred_element_type=F32)
        row = lax.broadcasted_iota(jnp.int32, (LANES, LANES), 0)
        col = lax.broadcasted_iota(jnp.int32, (LANES, LANES), 1)
        r0 = i * BQ
        full = nt(head_rows(q_s, h, r0, r0 + BQ), head_rows(k_s, h, 0, r0)) if i else None
        diag = []
        for a in range(BQ // LANES):
            d = nt(head_rows(q_s, h, r0 + a * LANES, r0 + (a + 1) * LANES),
                   head_rows(k_s, h, r0, r0 + (a + 1) * LANES))
            last = jnp.where(col <= row, d[:, a * LANES:], NEG)
            diag.append(jnp.concatenate([d[:, :a * LANES], last], axis=1) if a else last)
        return full, diag

    def softmax(i, sc):
        full, diag = sc
        ch, nf = cfg["chs"], i * BQ
        pf, pd, inv = [], [], []
        for a in range(BQ // LANES):
            pda, inva = [], []
            for c0 in range(0, LANES, ch):
                s = diag[a][c0:c0 + ch]
                if full is not None:
                    s = jnp.concatenate([full[a * LANES + c0:a * LANES + c0 + ch], s], axis=1)
                p = jnp.exp2(s - jnp.max(s, axis=1, keepdims=True))
                pb = p.astype(BF16)
                total = jnp.sum(pb.astype(F32) if cfg["sum16"] else p, axis=1, keepdims=True)
                if full is not None:
                    pf.append(pb[:, :nf])
                pda.append(pb[:, nf:])
                inva.append(_reciprocal(total))
            pd.append(jnp.concatenate(pda, axis=0))
            inv.append(jnp.concatenate(inva, axis=0))
        return (jnp.concatenate(pf, axis=0) if pf else None), pd, inv

    def context(g, h, i, sm):
        def pv(a, b):
            return jnp.dot(a, b, preferred_element_type=F32)
        pf, pd, inv = sm
        r0 = i * BQ
        of = pv(pf, head_rows(v_s, h, 0, r0)) if pf is not None else None
        for a in range(BQ // LANES):
            o = pv(pd[a], head_rows(v_s, h, r0, r0 + (a + 1) * LANES))
            if of is not None:
                o = o + of[a * LANES:(a + 1) * LANES]
            ctx[g * G + h, (r0 + a * LANES) // 2:(r0 + (a + 1) * LANES) // 2, :] = _pack(o * inv[a])

    def prepare_stream(g):
        slot = g % 2
        for raw, dst, level in ((woa_raw, woas, LOA), (wob_raw, wobs, LOB)):
            n = 1 << level
            rows, dc = raw.shape[2], DM // n
            ops = _expand([[raw[slot, k, :, j * dc:(j + 1) * dc] for j in range(n)] for k in range(n)],
                          B_TERMS, level)
            for r, op in enumerate(ops):
                dst[r, pl.ds(pl.multiple_of(g * (rows // 2), rows // 2), rows // 2), :] = _pack(op)
        n = 1 << LA
        rows = wqkv_raw.shape[2]
        for part in range(3):
            blocks = []
            for k in range(n):
                groups = _swap_group_and_lane_bits([
                    wqkv_raw[slot, k, :, part * DM + a * LANES:part * DM + (a + 1) * LANES].astype(F32)
                    for a in range(8)])
                per = 8 // n
                blocks.append([jnp.concatenate(groups[j * per:(j + 1) * per], axis=1) for j in range(n)])
            for r, op in enumerate(_expand(blocks, B_TERMS, LA)):
                wqkvs[part, r, pl.ds(pl.multiple_of(g * (rows // 2), rows // 2), rows // 2), :] = _pack(op)

    first = head_weight_copies(0)
    start(first[:2])
    start(input_copies(0))
    start(first[2:])
    wait(first)
    start(input_copies(1))
    prepare_head_weights(0)

    def first_projection(i, carry):
        wait(input_copies(i))

        @pl.when(i + 2 < NB)
        def _():
            start(input_copies(i + 2))

        @pl.when(i + 2 == NB)
        def _():
            start(head_weight_copies(1))

        @pl.when(i + 1 == NB)
        def _():
            start(stream_copies(0))

        prepare_inputs(i)
        for which in "kvq":
            project(i, which)
        return carry

    with jax.named_scope("prologue"):
        lax.fori_loop(0, NB, first_projection, 0)
    start(stream_copies(1))
    start(head_weight_copies(2))

    def head_group(g, project_next):
        wait(stream_copies(g))
        if project_next:
            wait(head_weight_copies(g + 1))
            prepare_head_weights(g + 1)
        else:
            xa_copy(0).start()
            xa_copy(1).start()
        proj = project if project_next else (lambda i, which: None)
        order = cfg["order"]
        for i in range(NB - 1, -1, -1):
            sc, sm = {}, {}
            for tok in order:
                if tok[0] == "s":
                    sc[int(tok[1])] = scores(int(tok[1]), i)
                elif tok[0] == "c":
                    h = int(tok[1])
                    context(g, h, i, softmax(i, sc[h]))
                elif tok == "q":
                    proj(i, "q")
                elif i + 1 < NB:
                    proj(i + 1, tok)
        proj(0, "k")
        proj(0, "v")
        prepare_stream(g)
        if project_next:
            @pl.when(g + 3 < NG)
            def _():
                start(head_weight_copies(g + 3))

            @pl.when(g + 2 < NG)
            def _():
                start(stream_copies(g + 2))

    def loop_body(g, carry):
        with jax.named_scope("group"):
            head_group(g, True)
        return carry

    with jax.named_scope("phase1"):
        lax.fori_loop(0, NG - 1, loop_body, 0)
    with jax.named_scope("lastgroup"):
        if cfg.get("nolast"):
            wait(stream_copies(NG - 1))
            xa_copy(0).start()
            xa_copy(1).start()
        else:
            head_group(NG - 1, False)

    ka[:, 0:HALO, :] = jnp.zeros((8, HALO, LANES), F32)
    va[:, 0:HALO, :] = jnp.zeros((8, HALO, LANES), F32)

    def store_blocks(slot, col0, c):
        n = len(c)
        dr, dc = BR // n, DM // n
        for a in range(n):
            for b in range(n):
                obuf[slot, a * dr:(a + 1) * dr, col0 + b * dc:col0 + (b + 1) * dc] = c[a][b].astype(BF16)

    def row_block(r, carry):
        slot = r % 2
        xa_copy(r).wait()

        @pl.when(r >= 2)
        def _():
            out_copy(r - 2).wait()

        xops = _expand(_grid(lambda a, b, c, d: xa_raw[slot, a:b, c:d], BR, DM, LA), A_TERMS, LA)
        n = 1 << LA
        dr, per = BR // n, 8 // n

        def lane_groups(part):
            c = _combine(lambda t: jnp.dot(xops[t], _unpack(wqkvs[part, t]), preferred_element_type=F32), LA)
            return lambda a, g: c[a][g // per][:, (g % per) * LANES:(g % per + 1) * LANES]

        kf = lane_groups(1)
        for a in range(n):
            for g in range(8):
                ka[g, HALO + a * dr:HALO + (a + 1) * dr, :] = kf(a, g)
        qf = lane_groups(0)
        vf = lane_groups(2)
        for a in range(n):
            for g in range(8):
                va[g, HALO + a * dr:HALO + (a + 1) * dr, :] = vf(a, g)

        def ctx_block(a, b, c, d):
            rows = pl.ds(pl.multiple_of(r * (BR // 2) + a // 2, (b - a) // 2), (b - a) // 2)
            return _unpack(jnp.concatenate([ctx[h, rows, :] for h in range(c // B_DH, d // B_DH)], axis=1))

        cops = _expand(_grid(ctx_block, BR, B_HEADS * B_DH, LOB), A_TERMS, LOB)
        store_blocks(slot, DM, _combine(
            lambda t: jnp.dot(cops[t], _unpack(wobs[t]), preferred_element_type=F32), LOB))

        ch = cfg["cha"]
        lane = lax.broadcasted_iota(jnp.int32, (ch, LANES), 1)
        odd1 = (lane & 1) != 0
        odd2 = (lane & 2) != 0
        o_chunks = []
        for c0 in range(0, BR, ch):
            qg = [qf(c0 // dr, g)[c0 % dr:c0 % dr + ch] for g in range(8)]
            logits = []
            for w in range(A_WIN):
                b0 = HALO + c0 - A_DIL * w
                acc = qg[0] * ka[0, b0:b0 + ch, :]
                for g in range(1, 8):
                    acc = acc + qg[g] * ka[g, b0:b0 + ch, :]
                acc = acc + jnp.where(odd1, pltpu.roll(acc, 1, 1), pltpu.roll(acc, LANES - 1, 1))
                acc = acc + jnp.where(odd2, pltpu.roll(acc, 2, 1), pltpu.roll(acc, LANES - 2, 1))
                acc = acc * (A_DH ** -0.5 * LOG2E)
                if c0 < A_DIL * w:
                    pos = r * BR + c0 + lax.broadcasted_iota(jnp.int32, (ch, LANES), 0)
                    acc = jnp.where(pos >= A_DIL * w, acc, NEG * LOG2E)
                logits.append(acc)
            m = functools.reduce(jnp.maximum, logits)
            ps = [jnp.exp2(l - m) for l in logits]
            inv = _reciprocal(functools.reduce(lambda a, b: a + b, ps))
            ps = [p * inv for p in ps]
            og = []
            for g in range(8):
                acc = None
                for w in range(A_WIN):
                    b0 = HALO + c0 - A_DIL * w
                    t = ps[w] * va[g, b0:b0 + ch, :]
                    acc = t if acc is None else acc + t
                og.append(acc)
            o_chunks.append(jnp.concatenate(_swap_group_and_lane_bits(og), axis=1))
        o = jnp.concatenate(o_chunks, axis=0)
        oops = _expand(_grid(lambda a, b, c, d: o[a:b, c:d], BR, DM, LOA), A_TERMS, LOA)
        store_blocks(slot, 0, _combine(
            lambda t: jnp.dot(oops[t], _unpack(woas[t]), preferred_element_type=F32), LOA))

        ka[:, 0:HALO, :] = ka[:, BR:BR + HALO, :]
        va[:, 0:HALO, :] = va[:, BR:BR + HALO, :]
        out_copy(r).start()

        @pl.when(r + 2 < NR)
        def _():
            xa_copy(r + 2).start()

        return carry

    def row_scope(r, carry):
        with jax.named_scope("rowblk"):
            return row_block(r, carry)

    with jax.named_scope("phase2"):
        lax.fori_loop(0, NR, row_scope, 0)
    out_copy(NR - 2).wait()
    out_copy(NR - 1).wait()


DEFAULT_CFG = dict(bq=256, br=256, g=2, cha=16, chs=128, sum16=True,
                   lq=1, lk=1, lv=1, lob=1, la=1, loa=1,
                   order=("s0", "s1", "k", "v", "c0", "q", "c1"))


def build(cfg=None):
    cfg = dict(DEFAULT_CFG, **(cfg or {}))
    BQ, BR, G = cfg["bq"], cfg["br"], cfg["g"]
    LQ, LK, LV, LOB, LA, LOA = (cfg[n] for n in ("lq", "lk", "lv", "lob", "la", "loa"))
    NB, NG = S // BQ, B_HEADS // G
    vmem = pltpu.VMEM

    def lhs_ops(width, level):
        return vmem((NB, 7 ** level, (BQ // 2) >> level, width >> level), U32)

    def head_ops(depth, level):
        return vmem((G >> level, 7 ** level, (depth // 2) >> level, B_DH), U32)

    def stage(rows, cols, level):
        return vmem((2, 1 << level, (rows >> level) // NG, cols), BF16)

    def fn(A_x, A_wqkv, A_wo, B_x, B_c_kv, B_w_q, B_w_uk, B_w_uv, B_w_o):
        out = pl.pallas_call(
            functools.partial(_kernel, cfg=cfg),
            out_shape=jax.ShapeDtypeStruct((S, 2 * DM), BF16),
            in_specs=[pl.BlockSpec(memory_space=pl.ANY)] * 9,
            out_specs=pl.BlockSpec(memory_space=pl.ANY),
            scratch_shapes=[
                vmem((NB, BQ, DM), BF16),
                vmem((NB, BQ, B_DC), BF16),
                lhs_ops(DM, LQ), lhs_ops(B_DC, LK),
                lhs_ops(B_DC, LV) if LV != LK else vmem((8, LANES), F32),
                vmem((2, G // 2, DM, B_DH), U32),
                vmem((2, G // 2, B_DC, B_DH), U32),
                vmem((2, G // 2, B_DC, B_DH), U32),
                head_ops(DM, LQ), head_ops(B_DC, LK), head_ops(B_DC, LV),
                vmem((G, S // 2, B_DH), U32),
                vmem((G, S // 2, B_DH), U32),
                vmem((G, S // 2, B_DH), U32),
                vmem((B_HEADS, S // 2, B_DH), U32),
                stage(DM, 3 * DM, LA), stage(DM, DM, LOA), stage(B_HEADS * B_DH, DM, LOB),
                vmem((3, 7 ** LA, (DM // 2) >> LA, DM >> LA), U32),
                vmem((7 ** LOA, (DM // 2) >> LOA, DM >> LOA), U32),
                vmem((7 ** LOB, (B_HEADS * B_DH // 2) >> LOB, DM >> LOB), U32),
                vmem((2, BR, DM), BF16),
                vmem((8, HALO + BR, LANES), F32),
                vmem((8, HALO + BR, LANES), F32),
                vmem((2, BR, 2 * DM), BF16),
                pltpu.SemaphoreType.DMA((2, NB)),
                pltpu.SemaphoreType.DMA((2, 3 * G // 2)),
                pltpu.SemaphoreType.DMA((2, 12)),
                pltpu.SemaphoreType.DMA((2,)),
                pltpu.SemaphoreType.DMA((2,)),
            ],
            compiler_params=pltpu.CompilerParams(vmem_limit_bytes=124 * 2 ** 20, flags=cfg.get("flags"),
                                                 disable_bounds_checks=cfg.get("nobc", False)),
            name="fused_local_and_latent_attention",
        )(A_x.reshape(S, DM), A_wqkv, A_wo, B_x.reshape(S, DM), B_c_kv.reshape(S, B_DC),
          B_w_q, B_w_uk, B_w_uv, B_w_o.reshape(B_HEADS * B_DH, DM))
        return out.reshape(1, S, 2 * DM)

    return jax.jit(fn)


@jax.jit
def pallas_concat_heads__sliding_local_dilated__compressed_kv_cla__prompt_kernel(
    A_x: jax.Array,
    A_wqkv: jax.Array,
    A_wo: jax.Array,
    B_x: jax.Array,
    B_c_kv: jax.Array,
    B_w_q: jax.Array,
    B_w_uk: jax.Array,
    B_w_uv: jax.Array,
    B_w_o: jax.Array,
):
    return build(dict(nobc=True,order=('s0','k','s1','v','c0','q','c1')))(A_x, A_wqkv, A_wo, B_x, B_c_kv, B_w_q, B_w_uk, B_w_uv, B_w_o)
```

```python
import functools

import jax
import jax.numpy as jnp
from jax import lax
import jax.experimental.pallas as pl
import jax.experimental.pallas.tpu as pltpu

S = 2048
DM = 1024
HALF = DM // 2
LANES = 128
A_DH, A_WIN, A_DIL = 32, 8, 2
HALO = 16
B_HEADS, B_DH, B_DC = 32, 128, 512
PAIRS = B_HEADS // 2

BLK = 256
SUB = BLK // 2
NBLK = S // BLK

LOG2E = 1.4426950408889634
NEG = -1e9
F32, BF16, U32 = jnp.float32, jnp.bfloat16, jnp.uint32

A_TERMS = (((1, 0, 0), (1, 1, 1)), ((1, 1, 0), (1, 1, 1)), ((1, 0, 0),), ((1, 1, 1),),
           ((1, 0, 0), (1, 0, 1)), ((1, 1, 0), (-1, 0, 0)), ((1, 0, 1), (-1, 1, 1)))
B_TERMS = (((1, 0, 0), (1, 1, 1)), ((1, 0, 0),), ((1, 0, 1), (-1, 1, 1)), ((1, 1, 0), (-1, 0, 0)),
           ((1, 1, 1),), ((1, 0, 0), (1, 0, 1)), ((1, 1, 0), (1, 1, 1)))
C_USES = ((0, ((1, 0, 0), (1, 1, 1))), (3, ((1, 0, 0), (1, 1, 0))), (4, ((-1, 0, 0), (1, 0, 1))),
          (6, ((1, 0, 0),)), (1, ((1, 1, 0), (-1, 1, 1))), (2, ((1, 0, 1), (1, 1, 1))),
          (5, ((1, 1, 1),)))

POOL_X = 0
POOL_QKV = POOL_X + S // 4
POOL_OA = POOL_QKV + 3 * HALF // 2
POOL_OB = POOL_OA + HALF // 2
POOL_ROWS = POOL_OB + PAIRS * B_DH // 2


def _pack(x):
    return pltpu.bitcast(x.astype(BF16), U32)


def _unpack(x):
    return pltpu.bitcast(x, BF16)


def _operand_sums(block, terms):
    blocks = [[block(i, j) for j in range(2)] for i in range(2)]
    out = []
    for (_, i, j), *rest in terms:
        acc = blocks[i][j]
        for sign, i, j in rest:
            a, b = acc.astype(F32), blocks[i][j].astype(F32)
            acc = a + b if sign > 0 else a - b
        out.append(acc.astype(BF16))
    return out


def _block_product(product):
    c = [[None, None], [None, None]]
    for r, uses in C_USES:
        m = product(r)
        for sign, i, j in uses:
            c[i][j] = m if c[i][j] is None else c[i][j] + m if sign > 0 else c[i][j] - m
    return c


def _swap_group_and_lane_bits(groups):
    lane = lax.broadcasted_iota(jnp.int32, groups[0].shape, 1)
    groups = list(groups)
    for t in range(3):
        shift = 4 << t
        low = (lane & shift) == 0
        for g in range(8):
            if g & (1 << t):
                continue
            x, y = groups[g], groups[g | (1 << t)]
            groups[g] = jnp.where(low, x, pltpu.roll(y, shift, 1))
            groups[g | (1 << t)] = jnp.where(low, pltpu.roll(x, LANES - shift, 1), y)
    return groups


def _reciprocal(x):
    r = pl.reciprocal(x, approx=True)
    return r * (2.0 - x * r)


def _start(copies):
    for cp in copies:
        cp.start()


def _wait(copies):
    for cp in copies:
        cp.wait()


def _kernel(xa_hbm, wqkv_hbm, woa_hbm, xb_hbm, c_hbm, wq_hbm, wuk_hbm, wuv_hbm, wob_hbm,
            out_hbm,
            xb_raw, c_raw, pool, cs, wq_raw, wuk_raw, wuv_raw, wqs, wks, wvs,
            q_s, k_s, v_s, ctxs,
            wqkv_raw, woa_raw, wob_raw, xa_raw, ka, va, obuf,
            sem_x, sem_w, sem_s, sem_a, sem_o, *, cfg):
    wq_u = wq_hbm.bitcast(U32)
    wuk_u = wuk_hbm.bitcast(U32)
    wuv_u = wuv_hbm.bitcast(U32)

    def pair_copies(j):
        slot = j % 2
        return [pltpu.make_async_copy(wuk_u.at[:, j, :], wuk_raw.at[slot], sem_w.at[slot, 0]),
                pltpu.make_async_copy(wuv_u.at[:, j, :], wuv_raw.at[slot], sem_w.at[slot, 1]),
                pltpu.make_async_copy(wq_u.at[:, j, :], wq_raw.at[slot], sem_w.at[slot, 2])]

    def stream_copies(j):
        slot = j % 2
        rows = HALF // PAIRS
        cps = []
        for k in range(2):
            r0 = pl.multiple_of(k * HALF + j * rows, rows)
            cps.append(pltpu.make_async_copy(
                wqkv_hbm.at[pl.ds(r0, rows), :], wqkv_raw.at[slot, k], sem_s.at[slot, k]))
            cps.append(pltpu.make_async_copy(
                woa_hbm.at[pl.ds(r0, rows), :], woa_raw.at[slot, k], sem_s.at[slot, 2 + k]))
        cps.append(pltpu.make_async_copy(
            wob_hbm.at[pl.ds(2 * j, 2)], wob_raw.at[slot], sem_s.at[slot, 4]))
        return cps

    def input_copies(i):
        rows = pl.ds(pl.multiple_of(i * BLK, BLK), BLK)
        return [pltpu.make_async_copy(c_hbm.at[rows, :], c_raw.at[i], sem_x.at[0, i]),
                pltpu.make_async_copy(xb_hbm.at[rows, :], xb_raw.at[i], sem_x.at[1, i])]

    def xa_copy(i):
        rows = pl.ds(pl.multiple_of(i * BLK, BLK), BLK)
        return pltpu.make_async_copy(xa_hbm.at[rows, :], xa_raw.at[i % 2], sem_a.at[i % 2])

    def out_copy(i):
        rows = pl.ds(pl.multiple_of(i * BLK, BLK), BLK)
        return pltpu.make_async_copy(obuf.at[i % 2], out_hbm.at[rows, :], sem_o.at[i % 2])

    def packed_rows(start, size):
        return pl.ds(pl.multiple_of(start // 2, size // 2), size // 2)

    def prepare_pair_weights(j):
        slot = j % 2
        for raw, dst in ((wuk_raw, wks), (wuv_raw, wvs), (wq_raw, wqs)):
            depth = raw.shape[1] // 2

            def block(k, head):
                word = raw[slot, k * depth:(k + 1) * depth, :]
                return pltpu.bitcast(word & U32(0xFFFF0000) if head else word << 16, F32)

            for r, op in enumerate(_operand_sums(block, B_TERMS)):
                dst[r] = _pack(op)

    def prepare_inputs(i):
        ops = _operand_sums(
            lambda a, k: c_raw[i, a * SUB:(a + 1) * SUB, k * (B_DC // 2):(k + 1) * (B_DC // 2)], A_TERMS)
        for r, op in enumerate(ops):
            cs[r, packed_rows(i * SUB, SUB), :] = _pack(op)
        ops = _operand_sums(
            lambda a, k: xb_raw[i, a * SUB:(a + 1) * SUB, k * HALF:(k + 1) * HALF], A_TERMS)
        for r, op in enumerate(ops):
            pool[r, packed_rows(2 * POOL_X + i * SUB, SUB), :] = _pack(op)

    def project(i, which):
        lhs, base, rhs, dst = {"q": (pool, 2 * POOL_X, wqs, q_s), "k": (cs, 0, wks, k_s),
                               "v": (cs, 0, wvs, v_s)}[which]
        rows = packed_rows(base + i * SUB, SUB)
        c = _block_product(lambda r: jnp.dot(_unpack(lhs[r, rows, :]), _unpack(rhs[r]),
                                             preferred_element_type=F32))
        for a in range(2):
            for head in range(2):
                val = c[a][head] * (B_DH ** -0.5 * LOG2E) if which == "q" else c[a][head]
                dst[head, packed_rows(i * BLK + a * SUB, SUB), :] = _pack(val)

    def head_rows(ref, h, r0, r1):
        return _unpack(ref[h, r0 // 2:r1 // 2, :])

    def scores(h, i):
        def nt(a, b):
            return lax.dot_general(a, b, (((1,), (1,)), ((), ())), preferred_element_type=F32)
        row = lax.broadcasted_iota(jnp.int32, (SUB, SUB), 0)
        col = lax.broadcasted_iota(jnp.int32, (SUB, SUB), 1)
        r0 = i * BLK
        full = nt(head_rows(q_s, h, r0, r0 + BLK), head_rows(k_s, h, 0, r0)) if i else None
        diag = []
        for a in range(2):
            d = nt(head_rows(q_s, h, r0 + a * SUB, r0 + (a + 1) * SUB),
                   head_rows(k_s, h, r0, r0 + (a + 1) * SUB))
            last = jnp.where(col <= row, d[:, a * SUB:], NEG)
            diag.append(jnp.concatenate([d[:, :SUB], last], axis=1) if a else last)
        return full, diag

    def softmax(i, sc):
        full, diag = sc
        nf = i * BLK
        pf, pd, inv = [], [], []
        for a in range(2):
            s = diag[a]
            if full is not None:
                s = jnp.concatenate([full[a * SUB:(a + 1) * SUB], s], axis=1)
            p = jnp.exp2(s - jnp.max(s, axis=1, keepdims=True)).astype(BF16)
            inv.append(_reciprocal(jnp.sum(p.astype(F32), axis=1, keepdims=True)))
            if full is not None:
                pf.append(p[:, :nf])
            pd.append(p[:, nf:])
        return (jnp.concatenate(pf, axis=0) if pf else None), pd, inv

    def context(h, i, sm):
        def pv(a, b):
            return jnp.dot(a, b, preferred_element_type=F32)
        pf, pd, inv = sm
        r0 = i * BLK
        of = pv(pf, head_rows(v_s, h, 0, r0)) if pf is not None else None
        out = []
        for a in range(2):
            o = pv(pd[a], head_rows(v_s, h, r0, r0 + (a + 1) * SUB))
            if of is not None:
                o = o + of[a * SUB:(a + 1) * SUB]
            out.append(o * inv[a])
        return out

    def prepare_stream(j, piece):
        slot = j % 2
        if piece >= 4:
            size = B_DH // (len(cfg["pieces"]) - 4)
            r0 = (piece - 4) * size
            ops = _operand_sums(lambda k, n: wob_raw[slot, k, r0:r0 + size, n * HALF:(n + 1) * HALF], B_TERMS)
            rows = packed_rows(2 * POOL_OB + j * B_DH + r0, size)
        elif piece == 3:
            ops = _operand_sums(lambda k, n: woa_raw[slot, k, :, n * HALF:(n + 1) * HALF], B_TERMS)
            rows = packed_rows(2 * POOL_OA + j * (HALF // PAIRS), HALF // PAIRS)
        else:
            groups = [_swap_group_and_lane_bits([
                wqkv_raw[slot, k, :, piece * DM + a * LANES:piece * DM + (a + 1) * LANES].astype(F32)
                for a in range(8)]) for k in range(2)]
            ops = _operand_sums(lambda k, n: jnp.concatenate(groups[k][4 * n:4 * n + 4], axis=1), B_TERMS)
            rows = packed_rows(2 * POOL_QKV + piece * HALF + j * (HALF // PAIRS), HALF // PAIRS)
        for r, op in enumerate(ops):
            pool[r, rows, :] = _pack(op)

    first = pair_copies(0)
    _start(first[:2])
    _start(input_copies(0))
    _start(first[2:])
    _wait(first)
    _start(input_copies(1))
    prepare_pair_weights(0)

    def first_projection(i, carry):
        _wait(input_copies(i))

        @pl.when(i + 2 < NBLK)
        def _():
            _start(input_copies(i + 2))

        @pl.when(i + 2 == NBLK)
        def _():
            _start(pair_copies(1))
            _start(stream_copies(0))

        prepare_inputs(i)
        for which in "kvq":
            project(i, which)
        return carry

    only = cfg.get("only")
    with jax.named_scope("prologue"):
        if not only:
            lax.fori_loop(0, NBLK, first_projection, 0)
    _start(stream_copies(1))
    _start(pair_copies(2))

    def head_pair(j, project_next):
        _wait(stream_copies(j))
        if project_next:
            _wait(pair_copies(j + 1))
            prepare_pair_weights(j + 1)
        else:
            xa_copy(0).start()
            xa_copy(1).start()
        proj = project if project_next else (lambda i, which: None)
        for i in range(NBLK - 1, -1, -1):
            sc, o = {}, {}
            for tok in cfg["order"] if project_next else cfg["order_last"]:
                if tok[0] == "s":
                    sc[int(tok[1])] = scores(int(tok[1]), i)
                elif tok[0] == "c":
                    h = int(tok[1])
                    o[h] = context(h, i, softmax(i, sc[h]))
                elif tok == "q":
                    proj(i, "q")
                elif i + 1 < NBLK:
                    proj(i + 1, tok)
            for r, op in enumerate(_operand_sums(lambda a, head: o[head][a], A_TERMS)):
                ctxs[r, j, packed_rows(i * SUB, SUB), :] = _pack(op)
            for piece, at in enumerate(cfg["pieces"]):
                if at == i:
                    prepare_stream(j, piece)
        proj(0, "k")
        proj(0, "v")
        if project_next:
            @pl.when(j + 3 < PAIRS)
            def _():
                _start(pair_copies(j + 3))

            @pl.when(j + 2 < PAIRS)
            def _():
                _start(stream_copies(j + 2))

    def pair_step(j, carry):
        with jax.named_scope("group"):
            head_pair(j, True)
        return carry

    with jax.named_scope("phase1"):
        if only in (None, "p1"):
            lax.fori_loop(0, PAIRS - 1, pair_step, 0)
    with jax.named_scope("lastgroup"):
        if only in ("p1", "p2"):
            _wait(stream_copies(PAIRS - 1))
            xa_copy(0).start()
            xa_copy(1).start()
        else:
            head_pair(PAIRS - 1, False)

    ka[:, BLK:BLK + HALO, :] = jnp.zeros((8, HALO, LANES), F32)
    va[:, BLK:BLK + HALO, :] = jnp.zeros((8, HALO, LANES), F32)

    def store_blocks(slot, col0, c):
        for a in range(2):
            for n in range(2):
                obuf[slot, a * SUB:(a + 1) * SUB, col0 + n * HALF:col0 + (n + 1) * HALF] = c[a][n].astype(BF16)

    def row_block(i, carry):
        slot = i % 2
        xa_copy(i).wait()

        @pl.when(i >= 2)
        def _():
            out_copy(i - 2).wait()

        ka[:, 0:HALO, :] = ka[:, BLK:BLK + HALO, :]
        va[:, 0:HALO, :] = va[:, BLK:BLK + HALO, :]
        xops = _operand_sums(lambda a, k: xa_raw[slot, a * SUB:(a + 1) * SUB, k * HALF:(k + 1) * HALF], A_TERMS)

        def lane_groups(part):
            r0 = POOL_QKV + part * HALF // 2
            c = _block_product(lambda r: jnp.dot(xops[r], _unpack(pool[r, r0:r0 + HALF // 2, :]),
                                                 preferred_element_type=F32))
            return lambda a, g: c[a][g // 4][:, (g % 4) * LANES:(g % 4 + 1) * LANES]

        def out_b():
            rows = packed_rows(i * SUB, SUB)
            store_blocks(slot, DM, _block_product(lambda r: jnp.dot(
                _unpack(jnp.concatenate([ctxs[r, j, rows, :] for j in range(PAIRS)], axis=1)),
                _unpack(pool[r, POOL_OB:POOL_ROWS, :]), preferred_element_type=F32)))

        for part in cfg["aorder"]:
            if part == "b":
                out_b()
                continue
            f = lane_groups(part)
            if part == 0:
                qf = f
                continue
            dst = va if part == 2 else ka
            for a in range(2):
                for g in range(8):
                    dst[g, HALO + a * SUB:HALO + (a + 1) * SUB, :] = f(a, g)

        ch = cfg["cha"]
        lane = lax.broadcasted_iota(jnp.int32, (ch, LANES), 1)
        odd1 = (lane & 1) != 0
        odd2 = (lane & 2) != 0
        o_chunks = []
        for c0 in range(0, BLK, ch):
            qg = [qf(c0 // SUB, g)[c0 % SUB:c0 % SUB + ch] for g in range(8)]
            logits = []
            for w in range(A_WIN):
                b0 = HALO + c0 - A_DIL * w
                acc = qg[0] * ka[0, b0:b0 + ch, :]
                for g in range(1, 8):
                    acc = acc + qg[g] * ka[g, b0:b0 + ch, :]
                acc = acc + jnp.where(odd1, pltpu.roll(acc, 1, 1), pltpu.roll(acc, LANES - 1, 1))
                acc = acc + jnp.where(odd2, pltpu.roll(acc, 2, 1), pltpu.roll(acc, LANES - 2, 1))
                acc = acc * (A_DH ** -0.5 * LOG2E)
                if c0 < A_DIL * w:
                    pos = i * BLK + c0 + lax.broadcasted_iota(jnp.int32, (ch, LANES), 0)
                    acc = jnp.where(pos >= A_DIL * w, acc, NEG * LOG2E)
                logits.append(acc)
            m = functools.reduce(jnp.maximum, logits)
            ps = [jnp.exp2(l - m) for l in logits]
            inv = _reciprocal(functools.reduce(lambda a, b: a + b, ps))
            ps = [p * inv for p in ps]
            og = []
            for g in range(8):
                acc = None
                for w in range(A_WIN):
                    b0 = HALO + c0 - A_DIL * w
                    t = ps[w] * va[g, b0:b0 + ch, :]
                    acc = t if acc is None else acc + t
                og.append(acc)
            o_chunks.append(jnp.concatenate(_swap_group_and_lane_bits(og), axis=1))
        o = jnp.concatenate(o_chunks, axis=0)
        oops = _operand_sums(lambda a, k: o[a * SUB:(a + 1) * SUB, k * HALF:(k + 1) * HALF], A_TERMS)
        store_blocks(slot, 0, _block_product(lambda r: jnp.dot(
            oops[r], _unpack(pool[r, POOL_OA:POOL_OB, :]), preferred_element_type=F32)))

        out_copy(i).start()

        @pl.when(i + 2 < NBLK)
        def _():
            xa_copy(i + 2).start()

        return carry

    def row_step(i, carry):
        with jax.named_scope("rowblk"):
            return row_block(i, carry)

    with jax.named_scope("phase2"):
        if only in (None, "p2"):
            lax.fori_loop(0, NBLK, row_step, 0)
    out_copy(NBLK - 2).wait()
    out_copy(NBLK - 1).wait()


DEFAULT_CFG = dict(cha=16, order=('s0', 'k', 's1', 'v', 'c0', 'q', 'c1'), order_last=('s0', 's1', 'c0', 'c1'),
                   pieces=(6, 5, 4, 3, 6, 5, 4, 3), aorder=(1, 0, 2, "b"), nobc=True)


def build(cfg=None):
    cfg = dict(DEFAULT_CFG, **(cfg or {}))
    vmem = pltpu.VMEM

    def fn(A_x, A_wqkv, A_wo, B_x, B_c_kv, B_w_q, B_w_uk, B_w_uv, B_w_o):
        out = pl.pallas_call(
            functools.partial(_kernel, cfg=cfg),
            out_shape=jax.ShapeDtypeStruct((S, 2 * DM), BF16),
            in_specs=[pl.BlockSpec(memory_space=pl.ANY)] * 9,
            out_specs=pl.BlockSpec(memory_space=pl.ANY),
            scratch_shapes=[
                vmem((NBLK, BLK, DM), BF16),
                vmem((NBLK, BLK, B_DC), BF16),
                vmem((7, POOL_ROWS, HALF), U32),
                vmem((7, S // 4, B_DC // 2), U32),
                vmem((2, DM, B_DH), U32),
                vmem((2, B_DC, B_DH), U32),
                vmem((2, B_DC, B_DH), U32),
                vmem((7, DM // 4, B_DH), U32),
                vmem((7, B_DC // 4, B_DH), U32),
                vmem((7, B_DC // 4, B_DH), U32),
                vmem((2, S // 2, B_DH), U32),
                vmem((2, S // 2, B_DH), U32),
                vmem((2, S // 2, B_DH), U32),
                vmem((7, PAIRS, S // 4, B_DH), U32),
                vmem((2, 2, HALF // PAIRS, 3 * DM), BF16),
                vmem((2, 2, HALF // PAIRS, DM), BF16),
                vmem((2, 2, B_DH, DM), BF16),
                vmem((2, BLK, DM), BF16),
                vmem((8, HALO + BLK, LANES), F32),
                vmem((8, HALO + BLK, LANES), F32),
                vmem((2, BLK, 2 * DM), BF16),
                pltpu.SemaphoreType.DMA((2, NBLK)),
                pltpu.SemaphoreType.DMA((2, 3)),
                pltpu.SemaphoreType.DMA((2, 5)),
                pltpu.SemaphoreType.DMA((2,)),
                pltpu.SemaphoreType.DMA((2,)),
            ],
            compiler_params=pltpu.CompilerParams(vmem_limit_bytes=124 * 2 ** 20, flags=cfg.get("flags"),
                                                 disable_bounds_checks=cfg.get("nobc", False)),
            name="fused_local_and_latent_attention",
        )(A_x.reshape(S, DM), A_wqkv, A_wo, B_x.reshape(S, DM), B_c_kv.reshape(S, B_DC),
          B_w_q, B_w_uk, B_w_uv, B_w_o)
        return out.reshape(1, S, 2 * DM)

    return jax.jit(fn)


@jax.jit
def pallas_concat_heads__sliding_local_dilated__compressed_kv_cla__prompt_kernel(
    A_x: jax.Array,
    A_wqkv: jax.Array,
    A_wo: jax.Array,
    B_x: jax.Array,
    B_c_kv: jax.Array,
    B_w_q: jax.Array,
    B_w_uk: jax.Array,
    B_w_uv: jax.Array,
    B_w_o: jax.Array,
):
    return build(dict())(A_x, A_wqkv, A_wo, B_x, B_c_kv, B_w_q, B_w_uk, B_w_uv, B_w_o)
```

```python
import functools

import jax
import jax.numpy as jnp
from jax import lax
import jax.experimental.pallas as pl
import jax.experimental.pallas.tpu as pltpu

S = 2048
DM = 1024
HALF = DM // 2
LANES = 128
A_HEADS, A_DH, A_WIN, A_DIL = 32, 32, 8, 2
HALO = 16
B_HEADS, B_DH, B_DC = 32, 128, 512
PAIRS = B_HEADS // 2

BLK = 256
SUB = BLK // 2
NBLK = S // BLK

LOG2E = 1.4426950408889634
NEG = -1e9
F32, BF16, U32 = jnp.float32, jnp.bfloat16, jnp.uint32

A_TERMS = (((1, 0, 0), (1, 1, 1)), ((1, 1, 0), (1, 1, 1)), ((1, 0, 0),), ((1, 1, 1),),
           ((1, 0, 0), (1, 0, 1)), ((1, 1, 0), (-1, 0, 0)), ((1, 0, 1), (-1, 1, 1)))
B_TERMS = (((1, 0, 0), (1, 1, 1)), ((1, 0, 0),), ((1, 0, 1), (-1, 1, 1)), ((1, 1, 0), (-1, 0, 0)),
           ((1, 1, 1),), ((1, 0, 0), (1, 0, 1)), ((1, 1, 0), (1, 1, 1)))
C_USES = ((0, ((1, 0, 0), (1, 1, 1))), (3, ((1, 0, 0), (1, 1, 0))), (4, ((-1, 0, 0), (1, 0, 1))),
          (6, ((1, 0, 0),)), (1, ((1, 1, 0), (-1, 1, 1))), (2, ((1, 0, 1), (1, 1, 1))),
          (5, ((1, 1, 1),)))

POOL_X = 0
POOL_QKV = POOL_X + S // 4
POOL_OA = POOL_QKV + 3 * HALF // 2
POOL_OB = POOL_OA + HALF // 2
POOL_ROWS = POOL_OB
LOC_K, LOC_V, LOC_Q, LOC_PANELS = 0, 8, 16, 24


def _pack(x):
    return pltpu.bitcast(x.astype(BF16), U32)


def _unpack(x):
    return pltpu.bitcast(x, BF16)


def _operand_sums(block, terms):
    blocks = [[block(i, j) for j in range(2)] for i in range(2)]
    out = []
    for (_, i, j), *rest in terms:
        acc = blocks[i][j]
        for sign, i, j in rest:
            a, b = acc.astype(F32), blocks[i][j].astype(F32)
            acc = a + b if sign > 0 else a - b
        out.append(acc)
    return out


def _block_product(product):
    c = [[None, None], [None, None]]
    for r, uses in C_USES:
        m = product(r)
        for sign, i, j in uses:
            c[i][j] = m if c[i][j] is None else c[i][j] + m if sign > 0 else c[i][j] - m
    return c


def _operand_sums2(block, terms):
    outer = [[_operand_sums(lambda i, j: block(2 * i + a, 2 * j + b), terms) for b in range(2)] for a in range(2)]
    return [functools.partial(_operand_sums, lambda a, b, r=r: outer[a][b][r], terms) for r in range(7)]


def _join(c):
    return jnp.concatenate([jnp.concatenate(row, axis=1) for row in c], axis=0)


def _heads_to_lanes(groups):
    lane = lax.broadcasted_iota(jnp.int32, groups[0].shape, 1)
    groups = list(groups)
    for group_bit, lane_bit in ((2, 4), (1, 3), (0, 2), (2, 6), (2, 1), (1, 5), (1, 0)):
        shift = 1 << lane_bit
        low = (lane & shift) == 0
        for g in range(8):
            if g >> group_bit & 1:
                continue
            x, y = groups[g], groups[g | 1 << group_bit]
            groups[g] = jnp.where(low, x, pltpu.roll(y, shift, 1))
            groups[g | 1 << group_bit] = jnp.where(low, pltpu.roll(x, LANES - shift, 1), y)
    return [groups[(g & 1) << 2 | (g >> 2) << 1 | (g >> 1 & 1)] for g in range(8)]


def _word_half(word, hi):
    return pltpu.bitcast(word & U32(0xFFFF0000) if hi else word << 16, F32)


def _reciprocal(x):
    r = pl.reciprocal(x, approx=True)
    return r * (2.0 - x * r)


class _Timeline:
    def __init__(self, never):
        self.never, self.now, self.marks = never, 0.0, []

    def issue(self, cycles, results):
        for n, value in enumerate(results):
            self.marks.append((self.now + cycles * (n + 1) / len(results), value))
        self.now += cycles

    def after(self, cycle, value):
        ready = [v for t, v in self.marks if t <= cycle]
        if not ready:
            return value
        mark = ready[-1][0:8, 0:value.shape[1]]
        if value.shape[0] > 8:
            mark = jnp.concatenate([mark] * (value.shape[0] // 8), axis=0)
        return jnp.where(self.never, mark, value)


def _start(copies):
    for cp in copies:
        cp.start()


def _wait(copies):
    for cp in copies:
        cp.wait()


def _kernel(xa_hbm, wqkv_hbm, woa_hbm, xb_hbm, c_hbm, wq_hbm, wuk_hbm, wuv_hbm, wob_hbm,
            out_hbm,
            xb_raw, c_raw, pool, cs, wq_raw, wuk_raw, wuv_raw, wqs, wks, wvs,
            q_s, k_s, v_s, ctx, wobs,
            wqkv_raw, woa_raw, wob_raw, xa_raw, loc, obuf,
            sem_x, sem_w, sem_s, sem_a, sem_o, *, cfg):
    wq_u = wq_hbm.bitcast(U32)
    wuk_u = wuk_hbm.bitcast(U32)
    wuv_u = wuv_hbm.bitcast(U32)
    wqkv_u = wqkv_hbm.bitcast(U32)
    wob_u = wob_hbm.bitcast(U32)
    woa_u = woa_hbm.bitcast(U32)

    def pair_copies(j):
        slot = j % 2
        return [pltpu.make_async_copy(wuk_u.at[:, j, :], wuk_raw.at[slot], sem_w.at[slot, 0]),
                pltpu.make_async_copy(wuv_u.at[:, j, :], wuv_raw.at[slot], sem_w.at[slot, 1]),
                pltpu.make_async_copy(wq_u.at[:, j, :], wq_raw.at[slot], sem_w.at[slot, 2])]

    def stream_copies(j):
        slot = j % 2
        rows = HALF // PAIRS
        cps = []
        for k in range(2):
            cps.append(pltpu.make_async_copy(
                wqkv_u.at[packed_rows(k * HALF + j * rows, rows), :], wqkv_raw.at[slot, k], sem_s.at[slot, k]))
        cps.append(pltpu.make_async_copy(woa_u.at[:, j, :], woa_raw.at[slot], sem_s.at[slot, 2]))
        for k in range(4):
            cps.append(pltpu.make_async_copy(
                wob_u.at[packed_rows(k * DM + j * 64, 64), :], wob_raw.at[slot, k], sem_s.at[slot, 3 + k]))
        return cps

    def input_copies(i):
        rows = pl.ds(pl.multiple_of(i * BLK, BLK), BLK)
        return [pltpu.make_async_copy(c_hbm.at[rows, :], c_raw.at[i], sem_x.at[0, i]),
                pltpu.make_async_copy(xb_hbm.at[rows, :], xb_raw.at[i], sem_x.at[1, i])]

    def xa_copy(i):
        rows = pl.ds(pl.multiple_of(i * BLK, BLK), BLK)
        return pltpu.make_async_copy(xa_hbm.at[rows, :], xa_raw.at[i % 2], sem_a.at[i % 2])

    def out_copy(i):
        rows = pl.ds(pl.multiple_of(i * BLK, BLK), BLK)
        return pltpu.make_async_copy(obuf.at[i % 2], out_hbm.at[rows, :], sem_o.at[i % 2])

    def packed_rows(start, size):
        return pl.ds(pl.multiple_of(start // 2, size // 2), size // 2)

    def prepare_pair_weights(j, tl=None):
        slot = j % 2
        count, total = 0, (DM + 2 * B_DC) // 2
        for raw, dst in ((wq_raw, wqs), (wuk_raw, wks), (wuv_raw, wvs)):
            depth = raw.shape[1] // 2

            step = cfg["wch"]
            for r0 in range(0, depth, step):
                words = [raw[slot, k * depth + r0:k * depth + r0 + step, :] for k in range(2)]
                if tl is not None:
                    t = cfg["wspan"] * count / total
                    count += step
                    words = [pltpu.bitcast(tl.after(t, pltpu.bitcast(w, F32)), U32) for w in words]
                for r, op in enumerate(_operand_sums(lambda k, head: _word_half(words[k], head), B_TERMS)):
                    dst[r, r0 // 2:(r0 + step) // 2, :] = _pack(op)

    def prepare_inputs(i):
        ops = _operand_sums(
            lambda a, k: c_raw[i, a * SUB:(a + 1) * SUB, k * (B_DC // 2):(k + 1) * (B_DC // 2)], A_TERMS)
        for r, op in enumerate(ops):
            cs[r, packed_rows(i * SUB, SUB), :] = _pack(op)
        ops = _operand_sums(
            lambda a, k: xb_raw[i, a * SUB:(a + 1) * SUB, k * HALF:(k + 1) * HALF], A_TERMS)
        for r, op in enumerate(ops):
            pool[r, packed_rows(2 * POOL_X + i * SUB, SUB), :] = _pack(op)

    def project(i, which, tl=None):
        lhs, base, rhs, dst = {"q": (pool, 2 * POOL_X, wqs, q_s), "k": (cs, 0, wks, k_s),
                               "v": (cs, 0, wvs, v_s)}[which]
        rows = packed_rows(base + i * SUB, SUB)

        def product(r):
            m = jnp.dot(_unpack(lhs[r, rows, :]), _unpack(rhs[r]), preferred_element_type=F32)
            if tl is not None:
                tl.issue(SUB * rhs.shape[1] // 256, [m[SUB // 2 - 8:SUB // 2], m[SUB - 8:SUB]])
            return m

        c = _block_product(product)
        for a in range(2):
            for head in range(2):
                val = c[a][head] * (B_DH ** -0.5 * LOG2E) if which == "q" else c[a][head]
                dst[head, packed_rows(i * BLK + a * SUB, SUB), :] = _pack(val)

    def head_rows(ref, h, r0, r1):
        return _unpack(ref[h, r0 // 2:r1 // 2, :])

    def scores(h, i, tl):
        def nt(a, b):
            return lax.dot_general(a, b, (((1,), (1,)), ((), ())), preferred_element_type=F32)
        row = lax.broadcasted_iota(jnp.int32, (SUB, SUB), 0)
        col = lax.broadcasted_iota(jnp.int32, (SUB, SUB), 1)
        r0 = i * BLK
        full = nt(head_rows(q_s, h, r0, r0 + BLK), head_rows(k_s, h, 0, r0)) if i else None
        if i:
            tl.issue(BLK * i // 2, [full[t % BLK:t % BLK + 8, t // BLK * LANES:(t // BLK + 1) * LANES]
                                    for t in range(56, BLK * i // 2, 64)])
        diag = []
        for a in range(2):
            d = nt(head_rows(q_s, h, r0 + a * SUB, r0 + (a + 1) * SUB),
                   head_rows(k_s, h, r0, r0 + (a + 1) * SUB))
            tl.issue(32 * (a + 1), [d])
            last = jnp.where(col <= row, d[:, a * SUB:], NEG)
            diag.append(jnp.concatenate([d[:, :SUB], last], axis=1) if a else last)
        return full, diag, tl.now

    def softmax(i, sc, tl, h):
        full, diag, t0 = sc
        nf = i * BLK
        lo, hi = cfg["pace"][h]
        span = tl.now - t0
        step = cfg["pch"]
        pf, pd, inv = [], [], []
        for a in range(2):
            s = diag[a]
            if full is not None:
                s = jnp.concatenate([full[a * SUB:(a + 1) * SUB], s], axis=1)
            m = jnp.max(s, axis=1, keepdims=True)
            if step:
                m = jnp.concatenate([
                    tl.after(t0 + span * (lo + (hi - lo) * (a * SUB + c) / BLK), m[c:c + step])
                    for c in range(0, SUB, step)], axis=0)
            job = tl.jobs.get((i, h, a))
            if job is not None:
                done = pltpu.bitcast(job(), F32)[:, 0:1]
                m = jnp.concatenate([m[:SUB - 8], jnp.where(tl.never, done, m[SUB - 8:])], axis=0)
            p = jnp.exp2(s - m).astype(BF16)
            inv.append(_reciprocal(jnp.sum(p.astype(F32), axis=1, keepdims=True)))
            if full is not None:
                pf.append(p[:, :nf])
            pd.append(p[:, nf:])
        return (jnp.concatenate(pf, axis=0) if pf else None), pd, inv

    def context(h, i, sm, tl):
        def pv(a, b):
            return jnp.dot(a.astype(BF16), b, preferred_element_type=F32)
        pf, pd, inv = sm
        r0 = i * BLK
        of = None
        for k0 in range(0, r0, cfg["pvk"]):
            k1 = min(k0 + cfg["pvk"], r0)
            part = pv(pf[:, k0:k1], head_rows(v_s, h, k0, k1))
            of = part if of is None else of + part
            tl.issue((k1 - k0) // 2, [of[t:t + 8] for t in range(56, BLK, 64)])
        out = []
        for a in range(2):
            o = pv(pd[a], head_rows(v_s, h, r0, r0 + (a + 1) * SUB))
            tl.issue(32 * (a + 1), [o])
            if of is not None:
                o = o + of[a * SUB:(a + 1) * SUB]
            out.append(o * inv[a])
        return out

    def stream_jobs(j):
        slot = j % 2

        def emit(block, row0, col0=0):
            ops = [_pack(op) for op in _operand_sums(block, B_TERMS)]
            width = ops[0].shape[1]
            for r, op in enumerate(ops):
                pool[r, packed_rows(row0, 32), col0:col0 + width] = op
            return functools.reduce(jnp.bitwise_or, [op[8:, width - LANES:] for op in ops])

        def qkv(part):
            groups = [_heads_to_lanes([
                wqkv_raw[slot, k, :, part * DM + a * LANES:part * DM + (a + 1) * LANES]
                for a in range(8)]) for k in range(2)]
            return emit(lambda k, n: _unpack(jnp.concatenate(groups[k][4 * n:4 * n + 4], axis=1)),
                        2 * POOL_QKV + part * HALF + j * (HALF // PAIRS))

        def out_a(c0):
            return emit(lambda k, n: _word_half(woa_raw[slot, :, n * HALF + c0:n * HALF + c0 + 256], k),
                        2 * POOL_OA + ((j % 4) * 4 + j // 4) * A_HEADS, c0)

        def out_b(r0, c0):
            done = None
            for r, inner in enumerate(_operand_sums2(lambda k, n: _unpack(
                    wob_raw[slot, k, r0 // 2:r0 // 2 + 16, n * 256 + c0:n * 256 + c0 + LANES]), B_TERMS)):
                for t, op in enumerate(inner()):
                    op = _pack(op)
                    wobs[7 * r + t, packed_rows(j * 64 + r0, 32), c0:c0 + LANES] = op
                    if t in (0, 6):
                        done = op[8:] if done is None else done | op[8:]
            return done

        return ([functools.partial(qkv, part) for part in range(3)]
                + [functools.partial(out_a, c0) for c0 in (0, 256)]
                + [functools.partial(out_b, r0, c0) for r0 in (0, 32) for c0 in (0, LANES)])

    first = pair_copies(0)
    _start(first[:2])
    _start(input_copies(0))
    _start(first[2:])
    _wait(first)
    _start(input_copies(1))
    prepare_pair_weights(0)

    def first_projection(i, carry):
        _wait(input_copies(i))

        @pl.when(i + 2 < NBLK)
        def _():
            _start(input_copies(i + 2))

        @pl.when(i + 2 == NBLK)
        def _():
            _start(pair_copies(1))
            _start(stream_copies(0))

        prepare_inputs(i)
        for which in "kvq":
            project(i, which)
        return carry

    only = cfg.get("only")
    with jax.named_scope("prologue"):
        if not only:
            lax.fori_loop(0, NBLK, first_projection, 0)
    _start(stream_copies(1))
    _start(pair_copies(2))

    def head_pair(j, project_next):
        _wait(stream_copies(j))
        if project_next:
            _wait(pair_copies(j + 1))
            if not cfg["wspan"]:
                prepare_pair_weights(j + 1)
        else:
            xa_copy(0).start()
            xa_copy(1).start()
        tl = _Timeline(j < 0)
        jobs = stream_jobs(j)
        tl.jobs = dict(zip(cfg["jobslots"][:len(jobs)], jobs))
        assert len(tl.jobs) == len(jobs)
        proj = (lambda i, which: project(i, which, tl)) if project_next else (lambda i, which: None)
        for i in range(NBLK - 1, -1, -1):
            sc, o = {}, {}
            for tok in cfg["order"] if project_next else cfg["order_last"]:
                if tok[0] == "s":
                    sc[int(tok[1])] = scores(int(tok[1]), i, tl)
                elif tok[0] == "c":
                    if project_next and cfg["wspan"] and i == NBLK - 1 and tok == "c0":
                        prepare_pair_weights(j + 1, tl)
                    h = int(tok[1])
                    for a, val in enumerate(context(h, i, softmax(i, sc[h], tl, h), tl)):
                        ctx[2 * j + h, packed_rows(i * BLK + a * SUB, SUB), :] = _pack(val)
                elif tok == "q":
                    proj(i, "q")
                elif i + 1 < NBLK:
                    proj(i + 1, tok)
        proj(0, "k")
        proj(0, "v")
        if project_next:
            @pl.when(j + 3 < PAIRS)
            def _():
                _start(pair_copies(j + 3))

            @pl.when(j + 2 < PAIRS)
            def _():
                _start(stream_copies(j + 2))

    def pair_step(j, carry):
        with jax.named_scope("group"):
            head_pair(j, True)
        return carry

    with jax.named_scope("phase1"):
        if only in (None, "p1"):
            lax.fori_loop(0, PAIRS - 1, pair_step, 0)
    with jax.named_scope("lastgroup"):
        if only in ("p1", "p2"):
            _wait(stream_copies(PAIRS - 1))
            xa_copy(0).start()
            xa_copy(1).start()
        else:
            lax.fori_loop(PAIRS - 1, PAIRS, lambda j, c: (head_pair(j, False), c)[1], 0)

    loc[0:16, BLK:BLK + HALO, :] = jnp.zeros((16, HALO, LANES), F32)

    def store_blocks(slot, col0, c):
        for a in range(2):
            for n in range(2):
                obuf[slot, a * SUB:(a + 1) * SUB, col0 + n * HALF:col0 + (n + 1) * HALF] = c[a][n].astype(BF16)

    def row_block(i, carry):
        slot = i % 2
        xa_copy(i).wait()

        @pl.when(i >= 2)
        def _():
            out_copy(i - 2).wait()

        loc[0:16, 0:HALO, :] = loc[0:16, BLK:BLK + HALO, :]
        zero = i // NBLK if cfg["opaque"] else 0
        xops = [op.astype(BF16) for op in _operand_sums(
            lambda a, k: xa_raw[slot, a * SUB:(a + 1) * SUB, k * HALF:(k + 1) * HALF], A_TERMS)]

        def lane_groups(part):
            r0 = POOL_QKV + part * HALF // 2
            c = _block_product(lambda r: jnp.dot(xops[r], _unpack(pool[r, r0:r0 + HALF // 2, :]),
                                                 preferred_element_type=F32))
            return lambda a, g: c[a][g // 4][:, (g % 4) * LANES:(g % 4 + 1) * LANES]

        marks = []

        def out_b():
            quarter = B_HEADS // 4

            def block(a, k):
                rows = packed_rows(i * BLK + a * (BLK // 4), BLK // 4)
                return _unpack(jnp.concatenate(
                    [ctx[h, rows, :] for h in range(k * quarter, (k + 1) * quarter)], axis=1))

            lhs = _operand_sums2(block, A_TERMS)

            def outer(r):
                ops = lhs[r]()

                def product(t):
                    step = DM // cfg["ksplit"]
                    acc = None
                    for k0 in range(0, DM, step):
                        part = jnp.dot(ops[t][:, k0:k0 + step].astype(BF16),
                                       _unpack(wobs[7 * r + t, k0 // 2:(k0 + step) // 2, :]),
                                       preferred_element_type=F32)
                        acc = part if acc is None else acc + part
                        marks.append(acc)
                    return acc

                return _join(_block_product(product))

            store_blocks(slot, DM, _block_product(outer))

        for part in cfg["aorder"]:
            if part == "b":
                out_b()
                continue
            f = lane_groups(part)
            for a in range(2):
                for g in range(8):
                    loc[(LOC_Q, LOC_K, LOC_V)[part] + g, HALO + a * SUB:HALO + (a + 1) * SUB, :] = f(a, g)

        ch = cfg["cha"]

        stages = cfg["stages"]
        total = stages * BLK // ch
        count = [0]

        def paced(values):
            lo, hi = cfg["gate"]
            mark = marks[int((lo + (hi - lo) * count[0] / (total - 1)) * (len(marks) - 1))]
            count[0] += 1
            return [jnp.where(i < 0, mark[0:ch, 0:LANES], t) for t in values]

        def attend(c0):
            def rows(base, g, w):
                b0 = HALO + c0 - A_DIL * w
                return loc[zero + base + g, b0:b0 + ch, :]

            q0 = [rows(LOC_Q, g, 0) for g in range(8)]
            logits = []
            half = max(stages // 2, 1)
            for w in range(A_WIN):
                if w % (A_WIN // half) == 0:
                    q = paced(q0)
                acc = q[0] * rows(LOC_K, 0, w)
                for g in range(1, 8):
                    acc = acc + q[g] * rows(LOC_K, g, w)
                acc = acc + pltpu.roll(acc, 2 * A_HEADS, 1)
                acc = acc + pltpu.roll(acc, A_HEADS, 1)
                if c0 < A_DIL * w:
                    pos = i * BLK + c0 + lax.broadcasted_iota(jnp.int32, (ch, LANES), 0)
                    acc = jnp.where(pos >= A_DIL * w, acc, NEG * A_DH ** 0.5)
                logits.append(acc)
            m = functools.reduce(jnp.maximum, logits)
            ps = [jnp.exp2((l - m) * (A_DH ** -0.5 * LOG2E)) for l in logits]
            inv = _reciprocal(functools.reduce(lambda a, b: a + b, ps))
            ps = [p * inv for p in ps]
            out = []
            for g in range(8):
                if stages > 1 and g % (8 // half) == 0:
                    pg = paced(ps)
                elif stages == 1:
                    pg = ps
                out.append(functools.reduce(lambda a, b: a + b, [pg[w] * rows(LOC_V, g, w) for w in range(A_WIN)]))
            return out

        halves = [[], []]
        for c0 in range(0, SUB, ch):
            for a in range(2):
                halves[a].append(jnp.concatenate(attend(a * SUB + c0), axis=1))
        halves = [jnp.concatenate(h, axis=0) for h in halves]
        oops = _operand_sums(lambda a, k: halves[a][:, k * HALF:(k + 1) * HALF], A_TERMS)
        store_blocks(slot, 0, _block_product(lambda r: jnp.dot(
            oops[r].astype(BF16), _unpack(pool[r, POOL_OA:POOL_OB, :]), preferred_element_type=F32)))

        out_copy(i).start()

        @pl.when(i + 2 < NBLK)
        def _():
            xa_copy(i + 2).start()

        return carry

    def row_step(i, carry):
        with jax.named_scope("rowblk"):
            return row_block(i, carry)

    with jax.named_scope("phase2"):
        if only in (None, "p2"):
            lax.fori_loop(0, NBLK, row_step, 0)
    out_copy(NBLK - 2).wait()
    out_copy(NBLK - 1).wait()


DEFAULT_CFG = dict(cha=16, opaque=False, nsplit=4, ksplit=4, gate=(0, 0.93), stages=4, pace=((0, 0.7), (0.2, 0.8)), pch=0, sumgate=False, wch=32, wspan=0, pvk=512, jobslots=[(5, 1, 1), (4, 1, 1), (3, 1, 1), (5, 0, 1), (4, 0, 1), (5, 0, 0), (4, 0, 0), (3, 0, 0), (4, 1, 0)], order=('s0', 'k', 's1', 'v', 'c0', 'q', 'c1'), order_last=('s0', 's1', 'c0', 'c1'),
                   pieces=(6, 5, 4, 3, 6, 5, 4, 3), aorder=(1, 0, 2, "b"), nobc=True)


def build(cfg=None):
    cfg = dict(DEFAULT_CFG, **(cfg or {}))
    vmem = pltpu.VMEM

    def fn(A_x, A_wqkv, A_wo, B_x, B_c_kv, B_w_q, B_w_uk, B_w_uv, B_w_o):
        out = pl.pallas_call(
            functools.partial(_kernel, cfg=cfg),
            out_shape=jax.ShapeDtypeStruct((S, 2 * DM), BF16),
            in_specs=[pl.BlockSpec(memory_space=pl.ANY)] * 9,
            out_specs=pl.BlockSpec(memory_space=pl.ANY),
            scratch_shapes=[
                vmem((NBLK, BLK, DM), BF16),
                vmem((NBLK, BLK, B_DC), BF16),
                vmem((7, POOL_ROWS, HALF), U32),
                vmem((7, S // 4, B_DC // 2), U32),
                vmem((2, DM, B_DH), U32),
                vmem((2, B_DC, B_DH), U32),
                vmem((2, B_DC, B_DH), U32),
                vmem((7, DM // 4, B_DH), U32),
                vmem((7, B_DC // 4, B_DH), U32),
                vmem((7, B_DC // 4, B_DH), U32),
                vmem((2, S // 2, B_DH), U32),
                vmem((2, S // 2, B_DH), U32),
                vmem((2, S // 2, B_DH), U32),
                vmem((B_HEADS, S // 2, B_DH), U32),
                vmem((49, DM // 2, DM // 4), U32),
                vmem((2, 2, HALF // PAIRS // 2, 3 * DM), U32),
                vmem((2, A_HEADS, DM), U32),
                vmem((2, 4, 32, DM), U32),
                vmem((2, BLK, DM), BF16),
                vmem((LOC_PANELS, HALO + BLK, LANES), F32),
                vmem((2, BLK, 2 * DM), BF16),
                pltpu.SemaphoreType.DMA((2, NBLK)),
                pltpu.SemaphoreType.DMA((2, 3)),
                pltpu.SemaphoreType.DMA((2, 7)),
                pltpu.SemaphoreType.DMA((2,)),
                pltpu.SemaphoreType.DMA((2,)),
            ],
            compiler_params=pltpu.CompilerParams(vmem_limit_bytes=124 * 2 ** 20, flags=cfg.get("flags"),
                                                 disable_bounds_checks=cfg.get("nobc", False)),
            name="fused_local_and_latent_attention",
        )(A_x.reshape(S, DM), A_wqkv, A_wo.reshape(A_HEADS, A_DH, DM), B_x.reshape(S, DM), B_c_kv.reshape(S, B_DC),
          B_w_q, B_w_uk, B_w_uv, B_w_o.reshape(B_HEADS * B_DH, DM))
        return out.reshape(1, S, 2 * DM)

    return jax.jit(fn)


@jax.jit
def pallas_concat_heads__sliding_local_dilated__compressed_kv_cla__prompt_kernel(
    A_x: jax.Array,
    A_wqkv: jax.Array,
    A_wo: jax.Array,
    B_x: jax.Array,
    B_c_kv: jax.Array,
    B_w_q: jax.Array,
    B_w_uk: jax.Array,
    B_w_uv: jax.Array,
    B_w_o: jax.Array,
):
    return build(dict())(A_x, A_wqkv, A_wo, B_x, B_c_kv, B_w_q, B_w_uk, B_w_uv, B_w_o)
```

```python
import functools
import itertools

import jax
import jax.numpy as jnp
from jax import lax
import jax.experimental.pallas as pl
import jax.experimental.pallas.tpu as pltpu

S = 2048
DM = 1024
HALF = DM // 2
LANES = 128
A_HEADS, A_DH, A_WIN, A_DIL = 32, 32, 8, 2
HALO = 16
B_HEADS, B_DH, B_DC = 32, 128, 512
PAIRS = B_HEADS // 2

BLK = 256
SUB = BLK // 2
NBLK = S // BLK

LOG2E = 1.4426950408889634
NEG = -1e9
F32, BF16, U32 = jnp.float32, jnp.bfloat16, jnp.uint32

A_TERMS = (((1, 0, 0), (1, 1, 1)), ((1, 1, 0), (1, 1, 1)), ((1, 0, 0),), ((1, 1, 1),),
           ((1, 0, 0), (1, 0, 1)), ((1, 1, 0), (-1, 0, 0)), ((1, 0, 1), (-1, 1, 1)))
B_TERMS = (((1, 0, 0), (1, 1, 1)), ((1, 0, 0),), ((1, 0, 1), (-1, 1, 1)), ((1, 1, 0), (-1, 0, 0)),
           ((1, 1, 1),), ((1, 0, 0), (1, 0, 1)), ((1, 1, 0), (1, 1, 1)))
C_USES = ((0, ((1, 0, 0), (1, 1, 1))), (3, ((1, 0, 0), (1, 1, 0))), (4, ((-1, 0, 0), (1, 0, 1))),
          (6, ((1, 0, 0),)), (1, ((1, 1, 0), (-1, 1, 1))), (2, ((1, 0, 1), (1, 1, 1))),
          (5, ((1, 1, 1),)))

POOL_X = 0
POOL_QKV = POOL_X + S // 4
POOL_ROWS = POOL_QKV + 3 * HALF // 2
LOC_K, LOC_V, LOC_Q, LOC_PANELS = 0, 8, 16, 24


def _pack(x):
    return pltpu.bitcast(x.astype(BF16), U32)


def _unpack(x):
    return pltpu.bitcast(x, BF16)


def _operand_sums(block, terms):
    blocks = [[block(i, j) for j in range(2)] for i in range(2)]
    out = []
    for (_, i, j), *rest in terms:
        acc = blocks[i][j]
        for sign, i, j in rest:
            a, b = acc.astype(F32), blocks[i][j].astype(F32)
            acc = a + b if sign > 0 else a - b
        out.append(acc)
    return out


def _block_product(product):
    c = [[None, None], [None, None]]
    for r, uses in C_USES:
        m = product(r)
        for sign, i, j in uses:
            c[i][j] = m if c[i][j] is None else c[i][j] + m if sign > 0 else c[i][j] - m
    return c


def _operand_sums2(block, terms):
    outer = [[_operand_sums(lambda i, j: block(2 * i + a, 2 * j + b), terms) for b in range(2)] for a in range(2)]
    return [functools.partial(_operand_sums, lambda a, b, r=r: outer[a][b][r], terms) for r in range(7)]


def _join(c):
    return jnp.concatenate([jnp.concatenate(row, axis=1) for row in c], axis=0)


def _heads_to_lanes(groups):
    lane = lax.broadcasted_iota(jnp.int32, groups[0].shape, 1)
    groups = list(groups)
    for group_bit, lane_bit in ((2, 4), (1, 3), (0, 2), (2, 6), (2, 1), (1, 5), (1, 0)):
        shift = 1 << lane_bit
        low = (lane & shift) == 0
        for g in range(8):
            if g >> group_bit & 1:
                continue
            x, y = groups[g], groups[g | 1 << group_bit]
            groups[g] = jnp.where(low, x, pltpu.roll(y, shift, 1))
            groups[g | 1 << group_bit] = jnp.where(low, pltpu.roll(x, LANES - shift, 1), y)
    return [groups[(g & 1) << 2 | (g >> 2) << 1 | (g >> 1 & 1)] for g in range(8)]


def _word_half(word, hi):
    return pltpu.bitcast(word & U32(0xFFFF0000) if hi else word << 16, F32)


def _reciprocal(x):
    r = pl.reciprocal(x, approx=True)
    return r * (2.0 - x * r)


class _Timeline:
    def __init__(self, never):
        self.never, self.now, self.marks = never, 0.0, []

    def issue(self, cycles, results):
        for n, value in enumerate(results):
            self.marks.append((self.now + cycles * (n + 1) / len(results), value))
        self.now += cycles

    def after(self, cycle, value):
        ready = [v for t, v in self.marks if t <= cycle]
        if not ready:
            return value
        mark = ready[-1][0:8, 0:value.shape[1]]
        if value.shape[0] > 8:
            mark = jnp.concatenate([mark] * (value.shape[0] // 8), axis=0)
        return jnp.where(self.never, mark, value)


class _Background:
    def __init__(self, never):
        self.never, self.pending, self.credit, self.rate = never, iter(()), 0.0, 0.0

    def add(self, pieces, rate):
        self.pending, self.rate = itertools.chain(self.pending, pieces), rate

    def tie(self, words):
        self.credit += self.rate
        due = list(itertools.islice(self.pending, int(self.credit)))
        self.credit -= int(self.credit)
        if not due:
            return words
        mark = functools.reduce(jnp.bitwise_or, [pltpu.bitcast(d[-8:, -LANES:], U32) for d in due])
        top = jnp.where(self.never, mark, words[:8, :LANES])
        if words.shape[1] > LANES:
            top = jnp.concatenate([top, words[:8, LANES:]], axis=1)
        return jnp.concatenate([top, words[8:]], axis=0)

    def finish(self):
        for _ in self.pending:
            pass


def _start(copies):
    for cp in copies:
        cp.start()


def _wait(copies):
    for cp in copies:
        cp.wait()


def _kernel(xa_hbm, wqkv_hbm, woa_hbm, xb_hbm, c_hbm, wq_hbm, wuk_hbm, wuv_hbm, wob_hbm,
            out_hbm,
            xb_raw, c_raw, pool, cs, wq_raw, wuk_raw, wuv_raw, wqs, wks, wvs,
            q_s, k_s, v_s, ctx, wobs, woas,
            wqkv_raw, woa_raw, wob_raw, xa_raw, loc, obuf,
            sem_x, sem_w, sem_s, sem_a, sem_o, *, cfg):
    wq_u = wq_hbm.bitcast(U32)
    wuk_u = wuk_hbm.bitcast(U32)
    wuv_u = wuv_hbm.bitcast(U32)
    wqkv_u = wqkv_hbm.bitcast(U32)
    wob_u = wob_hbm.bitcast(U32)
    woa_u = woa_hbm.bitcast(U32)

    def pair_copies(j):
        slot = j % 2
        return [pltpu.make_async_copy(wuk_u.at[:, j, :], wuk_raw.at[slot], sem_w.at[slot, 0]),
                pltpu.make_async_copy(wuv_u.at[:, j, :], wuv_raw.at[slot], sem_w.at[slot, 1]),
                pltpu.make_async_copy(wq_u.at[:, j, :], wq_raw.at[slot], sem_w.at[slot, 2])]

    def stream_copies(j):
        slot = j % 2
        rows = HALF // PAIRS
        cps = []
        for k in range(2):
            cps.append(pltpu.make_async_copy(
                wqkv_u.at[packed_rows(k * HALF + j * rows, rows), :], wqkv_raw.at[slot, k], sem_s.at[slot, k]))
        for k in range(2):
            word = (j >> 1 & 1) | k << 1 | (j >> 2) << 2
            cps.append(pltpu.make_async_copy(woa_u.at[:, word, :], woa_raw.at[slot, k], sem_s.at[slot, 7 + k]))
        for k in range(4):
            cps.append(pltpu.make_async_copy(
                wob_u.at[packed_rows(k * DM + j * 64, 64), :], wob_raw.at[slot, k], sem_s.at[slot, 3 + k]))
        return cps

    def c_copy(i):
        rows = pl.ds(pl.multiple_of(i * BLK, BLK), BLK)
        return pltpu.make_async_copy(c_hbm.at[rows, :], c_raw.at[i], sem_x.at[0, i])

    def xb_copy(i):
        rows = pl.ds(pl.multiple_of(i * BLK, BLK), BLK)
        return pltpu.make_async_copy(xb_hbm.at[rows, :], xb_raw.at[i], sem_x.at[1, i])

    def xa_copy(i):
        rows = pl.ds(pl.multiple_of(i * BLK, BLK), BLK)
        return pltpu.make_async_copy(xa_hbm.at[rows, :], xa_raw.at[i % 2], sem_a.at[i % 2])

    def out_copy(i, part):
        r0, nr, c0, nc = (0, BLK, DM, DM) if part == 4 else (part // 2 * SUB, SUB, part % 2 * HALF, HALF)
        rows = pl.ds(pl.multiple_of(i * BLK + r0, SUB), nr)
        return pltpu.make_async_copy(obuf.at[i % 2, r0:r0 + nr, c0:c0 + nc], out_hbm.at[rows, c0:c0 + nc],
                                     sem_o.at[i % 2, part])

    def packed_rows(start, size):
        if isinstance(start, int):
            return pl.ds(start // 2, size // 2)
        return pl.ds(pl.multiple_of(start // 2, size // 2), size // 2)

    def prepare_pair_weights(j, which="qkv"):
        slot = j % 2
        for name in which:
            raw, dst = {"q": (wq_raw, wqs), "k": (wuk_raw, wks), "v": (wuv_raw, wvs)}[name]
            depth = raw.shape[1] // 2
            for r0 in range(0, depth, 32):
                words = [raw[slot, k * depth + r0:k * depth + r0 + 32, :] for k in range(2)]
                for r, op in enumerate(_operand_sums(lambda k, head: _word_half(words[k], head), B_TERMS)):
                    dst[r, r0 // 2:r0 // 2 + 16, :] = _pack(op)

    def prepare_inputs(i, raw, dst, base):
        width = raw.shape[2] // 2
        ops = _operand_sums(lambda a, k: raw[i, a * SUB:(a + 1) * SUB, k * width:(k + 1) * width], A_TERMS)
        for r, op in enumerate(ops):
            dst[r, packed_rows(base + i * SUB, SUB), :] = _pack(op)

    def project(i, which, tl=None):
        lhs, base, rhs, dst = {"q": (pool, 2 * POOL_X, wqs, q_s), "k": (cs, 0, wks, k_s),
                               "v": (cs, 0, wvs, v_s)}[which]
        rows = packed_rows(base + i * SUB, SUB)

        def product(r):
            w = rhs[r] if tl is None or i not in cfg["bgblocks"] else tl.bg.tie(rhs[r])
            m = jnp.dot(_unpack(lhs[r, rows, :]), _unpack(w), preferred_element_type=F32)
            if tl is not None:
                tl.issue(SUB * rhs.shape[1] // 256, [m[SUB // 2 - 8:SUB // 2], m[SUB - 8:SUB]])
            return m

        c = _block_product(product)
        for a in range(2):
            if which == "q":
                q_s[pl.ds(pl.multiple_of(i * BLK + a * SUB, SUB), SUB), :] = (
                    jnp.concatenate(c[a], axis=1) * (B_DH ** -0.5 * LOG2E)).astype(BF16)
            else:
                for head in range(2):
                    dst[head, packed_rows(i * BLK + a * SUB, SUB), :] = _pack(c[a][head])

    def head_rows(ref, h, r0, r1):
        return _unpack(ref[h, r0 // 2:r1 // 2, :])

    def scores(h, i, tl):
        def nt(a, b):
            return lax.dot_general(a, b, (((1,), (1,)), ((), ())), preferred_element_type=F32)
        row = lax.broadcasted_iota(jnp.int32, (SUB, SUB), 0)
        col = lax.broadcasted_iota(jnp.int32, (SUB, SUB), 1)
        r0 = i * BLK
        full = nt(q_s[r0:r0 + BLK, h * B_DH:(h + 1) * B_DH], head_rows(k_s, h, 0, r0)) if i else None
        if i:
            tl.issue(BLK * i // 2, [full[t % BLK:t % BLK + 8, t // BLK * LANES:(t // BLK + 1) * LANES]
                                    for t in range(56, BLK * i // 2, 64)])
        diag = []
        for a in range(2):
            d = nt(q_s[r0 + a * SUB:r0 + (a + 1) * SUB, h * B_DH:(h + 1) * B_DH],
                   head_rows(k_s, h, r0, r0 + (a + 1) * SUB))
            tl.issue(32 * (a + 1), [d])
            last = jnp.where(col <= row, d[:, a * SUB:], NEG)
            diag.append(jnp.concatenate([d[:, :SUB], last], axis=1) if a else last)
        return full, diag, tl.now

    def softmax(i, sc, tl, h):
        full, diag, t0 = sc
        nf = i * BLK
        lo, hi = tl.pace[h]
        span = tl.now - t0
        step = tl.pch
        pf, pd, inv = [], [], []
        for a in range(2):
            s = diag[a]
            if full is not None:
                s = jnp.concatenate([full[a * SUB:(a + 1) * SUB], s], axis=1)
            m = jnp.max(s, axis=1, keepdims=True)
            if step:
                m = jnp.concatenate([
                    tl.after(t0 + span * (lo + (hi - lo) * (a * SUB + c) / BLK), m[c:c + step])
                    for c in range(0, SUB, step)], axis=0)
            p = jnp.exp2(s - m)
            if i >= cfg["sum16"]:
                p = p.astype(BF16)
            inv.append(_reciprocal(jnp.sum(p.astype(F32), axis=1, keepdims=True)))
            if full is not None:
                pf.append(p[:, :nf])
            pd.append(p[:, nf:])
        return (jnp.concatenate(pf, axis=0) if pf else None), pd, inv

    def context(h, i, sm, tl):
        def pv(a, b):
            return jnp.dot(a.astype(BF16), b, preferred_element_type=F32)
        pf, pd, inv = sm
        r0 = i * BLK
        of = None
        for k0 in range(0, r0, cfg["pvk"]):
            k1 = min(k0 + cfg["pvk"], r0)
            words = v_s[h, k0 // 2:k1 // 2, :]
            if tl.bgpv and i in cfg["bgblocks_last"]:
                words = jnp.concatenate([tl.bg.tie(words[t:t + 64]) for t in range(0, words.shape[0], 64)], axis=0)
            part = pv(pf[:, k0:k1], _unpack(words))
            of = part if of is None else of + part
            tl.issue((k1 - k0) // 2, [of[t:t + 8] for t in range(56, BLK, 64)])
        out = []
        for a in range(2):
            o = pv(pd[a], head_rows(v_s, h, r0, r0 + (a + 1) * SUB))
            tl.issue(32 * (a + 1), [o])
            if of is not None:
                o = o + of[a * SUB:(a + 1) * SUB]
            out.append(o * inv[a])
        return out

    def stream_work(j, inner_part=True, outer_part=True):
        slot = j % 2

        def qkv(part):
            groups = [_heads_to_lanes([
                wqkv_raw[slot, k, :, part * DM + a * LANES:part * DM + (a + 1) * LANES]
                for a in range(8)]) for k in range(2)]
            rows = packed_rows(2 * POOL_QKV + part * HALF + j * (HALF // PAIRS), HALF // PAIRS)
            for a in range(4):
                for r, op in enumerate(_operand_sums(lambda k, n: _unpack(groups[k][4 * n + a]), B_TERMS)):
                    op = _pack(op)
                    pool[r, rows, a * LANES:(a + 1) * LANES] = op
                    yield op

        def two_level(block, dst, row0, cols):
            for r, inner in enumerate(_operand_sums2(block, B_TERMS)):
                for t, op in enumerate(inner()):
                    op = _pack(op)
                    dst[7 * r + t, packed_rows(row0, 32), cols] = op
                    yield op

        def out_a():
            c0 = j % 2 * LANES if isinstance(j, int) else pl.multiple_of(j % 2 * LANES, LANES)
            row0 = ((j >> 1 & 1) * 4 + (j >> 2)) * A_HEADS
            return two_level(lambda k, n: _word_half(woa_raw[slot, k % 2, :, pl.ds(n * 256 + c0, LANES)], k // 2),
                             woas, row0, pl.ds(c0, LANES))

        def out_b(r0, c0):
            return two_level(lambda k, n: _unpack(
                wob_raw[slot, k, r0 // 2:r0 // 2 + 16, n * 256 + c0:n * 256 + c0 + LANES]),
                wobs, j * 64 + r0, slice(c0, c0 + LANES))

        for n in range(4):
            if outer_part:
                yield from out_b(n // 2 * 32, n % 2 * LANES)
            if inner_part and n < 3:
                yield from qkv(n)
        if outer_part:
            yield from out_a()

    only = cfg.get("only")
    wk0, wv0, wq0 = pair_copies(0)
    _start([wk0, c_copy(0), wv0, c_copy(1)])
    early = cfg["early"]

    ks, qs = cfg["kstep"], cfg["qstep"]

    def first_kv(n, carry):
        blocks = [n * ks + t for t in range(ks)]
        _wait([c_copy(i) for i in blocks])
        for i in blocks:
            @pl.when(i + 2 < NBLK)
            def _():
                c_copy(i + 2).start()

            @pl.when(i >= NBLK - early)
            def _():
                xb_copy(i - (NBLK - early)).start()

        for i in blocks:
            prepare_inputs(i, c_raw, cs, 0)
        for i in blocks:
            project(i, "k")
            project(i, "v")
        return carry

    def first_q(n, carry):
        blocks = [n * qs + t for t in range(qs)]
        _wait([xb_copy(i) for i in blocks])
        for i in blocks:
            @pl.when(i + early < NBLK)
            def _():
                xb_copy(i + early).start()

            @pl.when(i == cfg["nextat"])
            def _():
                _start(pair_copies(1) + stream_copies(0))

        for i in blocks:
            prepare_inputs(i, xb_raw, pool, 2 * POOL_X)
        for i in blocks:
            project(i, "q")
        return carry

    with jax.named_scope("prologue"):
        if not only:
            with jax.named_scope("w0"):
                wk0.wait()
            prepare_pair_weights(0, "k")
            wv0.wait()
            wq0.start()
            prepare_pair_weights(0, "v")
            with jax.named_scope("kv"):
                lax.fori_loop(0, NBLK // ks, first_kv, 0)
            wq0.wait()
            prepare_pair_weights(0, "q")
            with jax.named_scope("q"):
                lax.fori_loop(0, NBLK // qs, first_q, 0)
    _start(stream_copies(1))
    _start(pair_copies(2))

    def head_pair(j, project_next):
        _wait(stream_copies(j))
        if project_next:
            _wait(pair_copies(j + 1))
            prepare_pair_weights(j + 1)
        else:
            xa_copy(0).start()
            xa_copy(1).start()
        tl = _Timeline(j < 0)
        tl.pace, tl.pch = (cfg["pace"], cfg["pch"]) if project_next else (cfg["pace_last"], cfg["pch_last"])
        tl.bg = _Background(j < 0)
        tl.bg.add(stream_work(j, True, project_next),
                  329 / (21 * len(cfg["bgblocks"])) if project_next else cfg["bgrate_last"])
        tl.bgpv = not project_next
        proj = (lambda i, which: project(i, which, tl)) if project_next else (lambda i, which: None)
        sc, o = {}, {}

        def finish_head(h, i):
            o[h, i] = context(h, i, softmax(i, sc.pop((h, i)), tl, h), tl)
            if (1 - h, i) in o:
                for a in range(2):
                    ctx[j, i * BLK + a * SUB:i * BLK + (a + 1) * SUB, :] = (
                        jnp.concatenate([o[0, i][a], o[1, i][a]], axis=1).astype(BF16))

        for i in range(NBLK - 1, -1, -1):
            order = cfg["order"] if project_next else cfg["order_last"]
            for tok in order[i] if isinstance(order, dict) else order:
                if tok[0] == "s":
                    sc[int(tok[1]), i] = scores(int(tok[1]), i, tl)
                elif tok[0] == "c":
                    finish_head(int(tok[1]), i)
                elif tok[0] == "C":
                    if (int(tok[1]), i + 1) in sc:
                        finish_head(int(tok[1]), i + 1)
                elif tok == "q":
                    proj(i, "q")
                elif i + 1 < NBLK:
                    proj(i + 1, tok)
        for h, i in sorted(sc):
            finish_head(h, i)
        proj(0, "k")
        proj(0, "v")
        tl.bg.finish()
        if project_next:
            @pl.when(j + 3 < PAIRS)
            def _():
                _start(pair_copies(j + 3))

            @pl.when(j + 2 < PAIRS)
            def _():
                _start(stream_copies(j + 2))

    def pair_step(j, carry):
        with jax.named_scope("group"):
            head_pair(j, True)
        return carry

    with jax.named_scope("phase1"):
        if only in (None, "p1"):
            lax.fori_loop(0, PAIRS - 1, pair_step, 0)
    with jax.named_scope("lastgroup"):
        if only == "p1" or only == "last":
            def keep(n, carry):
                obuf.bitcast(U32)[0, 0:8, 0:LANES] = (pltpu.bitcast(ctx[n, 0:16, 0:LANES], U32) | pltpu.bitcast(q_s[pl.ds(pl.multiple_of(n * 16, 16), 16), 0:LANES], U32) | pool[n, 0:8, 0:LANES] | wobs[n, 0:8, 0:LANES] | woas[n, 0:8, 0:LANES]
                                                      | k_s[n % 2, 0:8, :] | v_s[n % 2, 0:8, :])
                return carry
        if only == "last":
            lax.fori_loop(PAIRS - 1, PAIRS, lambda j, c: (head_pair(j, False), c)[1], 0)
        if only == "p1" or only == "last":
            lax.fori_loop(0, 7, keep, 0)
        if only in ("p1", "p2", "last"):
            _wait(stream_copies(PAIRS - 1))
            xa_copy(0).start()
            xa_copy(1).start()
        else:
            lax.fori_loop(PAIRS - 1, PAIRS, lambda j, c: (head_pair(j, False), c)[1], 0)

    loc[0:16, BLK:BLK + HALO, :] = jnp.zeros((16, HALO, LANES), F32)

    def store_blocks(i, col0, c):
        for a, n in ((0, 0), (1, 0), (0, 1), (1, 1)):
            obuf[i % 2, a * SUB:(a + 1) * SUB, col0 + n * HALF:col0 + (n + 1) * HALF] = c[a][n].astype(BF16)
            if col0 == 0:
                out_copy(i, 2 * a + n).start()
        if col0:
            out_copy(i, 4).start()

    def row_block(i, carry):
        slot = i % 2
        xa_copy(i).wait()

        @pl.when(i >= 2)
        def _():
            _wait([out_copy(i - 2, part) for part in range(5)])

        loc[0:16, 0:HALO, :] = loc[0:16, BLK:BLK + HALO, :]
        zero = i // NBLK if cfg["opaque"] else 0
        xops = [op.astype(BF16) for op in _operand_sums(
            lambda a, k: xa_raw[slot, a * SUB:(a + 1) * SUB, k * HALF:(k + 1) * HALF], A_TERMS)]

        bg = _Background(i < 0)
        bg.add(stream_work(PAIRS - 1, False, True), cfg["bgrate2"])

        def lane_groups(part):
            r0 = POOL_QKV + part * HALF // 2
            c = _block_product(lambda r: jnp.dot(xops[r], _unpack(bg.tie(pool[r, r0:r0 + HALF // 2, :])),
                                                 preferred_element_type=F32))
            return lambda a, g: c[a][g // 4][:, (g % 4) * LANES:(g % 4 + 1) * LANES]

        marks = []

        def out_b():
            quarter = PAIRS // 4

            def block(a, k):
                rows = pl.ds(pl.multiple_of(i * BLK + a * (BLK // 4), BLK // 4), BLK // 4)
                return jnp.concatenate(
                    [ctx[j, rows, :] for j in range(k * quarter, (k + 1) * quarter)], axis=1).astype(F32)

            lhs = _operand_sums2(block, A_TERMS)

            def outer(r):
                ops = lhs[r]()

                def product(t):
                    step = DM // cfg["ksplit"]
                    acc = None
                    for k0 in range(0, DM, step):
                        part = jnp.dot(ops[t][:, k0:k0 + step].astype(BF16),
                                       _unpack(wobs[7 * r + t, k0 // 2:(k0 + step) // 2, :]),
                                       preferred_element_type=F32)
                        acc = part if acc is None else acc + part
                        marks.append(acc)
                    return acc

                return _join(_block_product(product))

            store_blocks(i, DM, _block_product(outer))

        for part in cfg["aorder"]:
            if part == "b":
                bg.finish()
                out_b()
                continue
            f = lane_groups(part)
            for a in range(2):
                for g in range(8):
                    loc[(LOC_Q, LOC_K, LOC_V)[part] + g, HALO + a * SUB:HALO + (a + 1) * SUB, :] = f(a, g)

        ch = cfg["cha"]

        stages = cfg["stages"]
        total = stages * BLK // ch
        count = [0]

        def paced(values):
            lo, hi = cfg["gate"]
            mark = marks[int((lo + (hi - lo) * count[0] / (total - 1)) * (len(marks) - 1))]
            count[0] += 1
            return [jnp.where(i < 0, mark[0:ch, 0:LANES], t) for t in values]

        def attend(c0):
            def rows(base, g, w):
                b0 = HALO + c0 - A_DIL * w
                return loc[zero + base + g, b0:b0 + ch, :]

            q0 = [rows(LOC_Q, g, 0) for g in range(8)]
            logits = []
            half = max(stages // 2, 1)
            for w in range(A_WIN):
                if w % (A_WIN // half) == 0:
                    q = paced(q0)
                acc = q[0] * rows(LOC_K, 0, w)
                for g in range(1, 8):
                    acc = acc + q[g] * rows(LOC_K, g, w)
                acc = acc + pltpu.roll(acc, 2 * A_HEADS, 1)
                acc = acc + pltpu.roll(acc, A_HEADS, 1)
                if c0 < A_DIL * w:
                    pos = i * BLK + c0 + lax.broadcasted_iota(jnp.int32, (ch, LANES), 0)
                    acc = jnp.where(pos >= A_DIL * w, acc, NEG * A_DH ** 0.5)
                logits.append(acc)
            m = functools.reduce(jnp.maximum, logits)
            ps = [jnp.exp2((l - m) * (A_DH ** -0.5 * LOG2E)) for l in logits]
            inv = _reciprocal(functools.reduce(lambda a, b: a + b, ps))
            ps = [p * inv for p in ps]
            out = []
            for g in range(8):
                if stages > 1 and g % (8 // half) == 0:
                    pg = paced(ps)
                elif stages == 1:
                    pg = ps
                out.append(functools.reduce(lambda a, b: a + b, [pg[w] * rows(LOC_V, g, w) for w in range(A_WIN)]))
            return out

        quarters = [[] for _ in range(4)]
        for c0 in range(0, BLK // 4, ch):
            for a in range(4):
                quarters[a].append(jnp.concatenate(attend(a * (BLK // 4) + c0), axis=1))
        quarters = [jnp.concatenate(t, axis=0) for t in quarters]
        lhs = _operand_sums2(lambda a, k: quarters[a][:, k * 256:(k + 1) * 256], A_TERMS)

        def outer(r):
            ops = lhs[r]()
            return _join(_block_product(lambda t: jnp.dot(
                ops[t].astype(BF16), _unpack(woas[7 * r + t]), preferred_element_type=F32)))

        store_blocks(i, 0, _block_product(outer))

        @pl.when(i + 2 < NBLK)
        def _():
            xa_copy(i + 2).start()

        return carry

    def row_step(i, carry):
        with jax.named_scope("rowblk"):
            return row_block(i, carry)

    with jax.named_scope("phase2"):
        if only in (None, "p2"):
            lax.fori_loop(0, NBLK, row_step, 0)
    with jax.named_scope("tail"):
        _wait([out_copy(i, part) for i in (NBLK - 2, NBLK - 1) for part in range(5)])


DEFAULT_CFG = dict(cha=16, opaque=False, nsplit=4, ksplit=4, gate=(0, 0.88), stages=4, pace=((0, 0.7), (0.2, 0.8)), pch=0, bgblocks=(6, 5, 4, 3, 2, 1), bgblocks_last=(7, 6, 5, 4, 3, 2, 1), bgrate_last=1, bgrate2=14, pch_last=0, pace_last=((0, 0.7), (0.2, 0.8)), jobslots_last=[(3, 1, 1), (2, 1, 1), (3, 0, 1), (2, 0, 1), (1, 0, 1), (1, 1, 1), (3, 0, 0), (2, 0, 0), (2, 1, 0)], sum16=0, early=4, kstep=1, qstep=1, nextat=4, sumgate=False, wch=32, wspan=0, pvk=1024, jobslots=[(5, 1, 1), (4, 0, 0), (3, 1, 0), (5, 0, 1), (5, 0, 0), (4, 1, 1), (3, 0, 0), (2, 1, 0)], order={0: ('s0', 'k', 's1', 'v', 'c0', 'q', 'c1'), 1: ('s0', 'k', 's1', 'v', 'c0', 'q', 'c1'), 2: ('s0', 'k', 's1', 'v', 'c0', 'q', 'c1'), 3: ('s0', 's1', 'k', 'q', 'c0', 'v', 'c1'), 4: ('s0', 's1', 'k', 'v', 'c0', 'q', 'c1'), 5: ('s0', 'k', 's1', 'q', 'c0', 'v', 'c1'), 6: ('s0', 's1', 'k', 'c0', 'v', 'c1', 'q'), 7: ('s0', 's1', 'k', 'c0', 'v', 'c1', 'q')}, order_last=('s0', 'C0', 's1', 'C1'),
                   pieces=(6, 5, 4, 3, 6, 5, 4, 3), aorder=(1, 0, 2, "b"), nobc=True)


def build(cfg=None):
    cfg = dict(DEFAULT_CFG, **(cfg or {}))
    vmem = pltpu.VMEM

    def fn(A_x, A_wqkv, A_wo, B_x, B_c_kv, B_w_q, B_w_uk, B_w_uv, B_w_o):
        out = pl.pallas_call(
            functools.partial(_kernel, cfg=cfg),
            out_shape=jax.ShapeDtypeStruct((S, 2 * DM), BF16),
            in_specs=[pl.BlockSpec(memory_space=pl.ANY)] * 9,
            out_specs=pl.BlockSpec(memory_space=pl.ANY),
            scratch_shapes=[
                vmem((NBLK, BLK, DM), BF16),
                vmem((NBLK, BLK, B_DC), BF16),
                vmem((7, POOL_ROWS, HALF), U32),
                vmem((7, S // 4, B_DC // 2), U32),
                vmem((2, DM, B_DH), U32),
                vmem((2, B_DC, B_DH), U32),
                vmem((2, B_DC, B_DH), U32),
                vmem((7, DM // 4, B_DH), U32),
                vmem((7, B_DC // 4, B_DH), U32),
                vmem((7, B_DC // 4, B_DH), U32),
                vmem((S, 2 * B_DH), BF16),
                vmem((2, S // 2, B_DH), U32),
                vmem((2, S // 2, B_DH), U32),
                vmem((PAIRS, S, 2 * B_DH), BF16),
                vmem((49, DM // 2, DM // 4), U32),
                vmem((49, DM // 8, DM // 4), U32),
                vmem((2, 2, HALF // PAIRS // 2, 3 * DM), U32),
                vmem((2, 2, A_HEADS, DM), U32),
                vmem((2, 4, 32, DM), U32),
                vmem((2, BLK, DM), BF16),
                vmem((LOC_PANELS, HALO + BLK, LANES), F32),
                vmem((2, BLK, 2 * DM), BF16),
                pltpu.SemaphoreType.DMA((2, NBLK)),
                pltpu.SemaphoreType.DMA((2, 3)),
                pltpu.SemaphoreType.DMA((2, 9)),
                pltpu.SemaphoreType.DMA((2,)),
                pltpu.SemaphoreType.DMA((2, 5)),
            ],
            compiler_params=pltpu.CompilerParams(vmem_limit_bytes=124 * 2 ** 20, flags=cfg.get("flags"),
                                                 disable_bounds_checks=cfg.get("nobc", False)),
            name="fused_local_and_latent_attention",
        )(A_x.reshape(S, DM), A_wqkv, A_wo.reshape(A_HEADS, A_DH, DM), B_x.reshape(S, DM), B_c_kv.reshape(S, B_DC),
          B_w_q, B_w_uk, B_w_uv, B_w_o.reshape(B_HEADS * B_DH, DM))
        return out.reshape(1, S, 2 * DM)

    return jax.jit(fn)


@jax.jit
def pallas_concat_heads__sliding_local_dilated__compressed_kv_cla__prompt_kernel(
    A_x: jax.Array,
    A_wqkv: jax.Array,
    A_wo: jax.Array,
    B_x: jax.Array,
    B_c_kv: jax.Array,
    B_w_q: jax.Array,
    B_w_uk: jax.Array,
    B_w_uv: jax.Array,
    B_w_o: jax.Array,
):
    return build(dict())(A_x, A_wqkv, A_wo, B_x, B_c_kv, B_w_q, B_w_uk, B_w_uv, B_w_o)
```

```python
import functools
import itertools

import jax
import jax.numpy as jnp
from jax import lax
import jax.experimental.pallas as pl
import jax.experimental.pallas.tpu as pltpu

S = 2048
DM = 1024
HALF = DM // 2
LANES = 128
A_HEADS, A_DH, A_WIN, A_DIL = 32, 32, 8, 2
HALO = 16
B_HEADS, B_DH, B_DC = 32, 128, 512
PAIRS = B_HEADS // 2

BLK = 256
SUB = BLK // 2
NBLK = S // BLK

LOG2E = 1.4426950408889634
NEG = -1e9
F32, BF16, U32 = jnp.float32, jnp.bfloat16, jnp.uint32

A_TERMS = (((1, 0, 0), (1, 1, 1)), ((1, 1, 0), (1, 1, 1)), ((1, 0, 0),), ((1, 1, 1),),
           ((1, 0, 0), (1, 0, 1)), ((1, 1, 0), (-1, 0, 0)), ((1, 0, 1), (-1, 1, 1)))
B_TERMS = (((1, 0, 0), (1, 1, 1)), ((1, 0, 0),), ((1, 0, 1), (-1, 1, 1)), ((1, 1, 0), (-1, 0, 0)),
           ((1, 1, 1),), ((1, 0, 0), (1, 0, 1)), ((1, 1, 0), (1, 1, 1)))
C_TERMS = (((1, 0, 0), (1, 1, 1)), ((1, 1, 0), (-1, 1, 1)), ((1, 0, 1), (1, 1, 1)), ((1, 0, 0), (1, 1, 0)),
           ((-1, 0, 0), (1, 0, 1)), ((1, 1, 1),), ((1, 0, 0),))

POOL_X = 0
POOL_QKV = POOL_X + S // 4
POOL_ROWS = POOL_QKV + 3 * HALF // 2
LOC_K, LOC_V, LOC_Q, LOC_PANELS = 0, 8, 16, 24


def _pack(x):
    return pltpu.bitcast(x.astype(BF16), U32)


def _unpack(x):
    return pltpu.bitcast(x, BF16)


def _operand_sums(block, terms):
    blocks = [[block(i, j) for j in range(2)] for i in range(2)]
    out = []
    for (_, i, j), *rest in terms:
        acc = blocks[i][j]
        for sign, i, j in rest:
            a, b = acc.astype(F32), blocks[i][j].astype(F32)
            acc = a + b if sign > 0 else a - b
        out.append(acc)
    return out


def _block_product(product, order=(0, 3, 4, 6, 1, 2, 5)):
    c = [[None, None], [None, None]]
    for r in order:
        m = product(r)
        for sign, i, j in C_TERMS[r]:
            if c[i][j] is None:
                c[i][j] = m if sign > 0 else -m
            else:
                c[i][j] = c[i][j] + m if sign > 0 else c[i][j] - m
    return c


def _operand_sums2(block, terms):
    outer = [[_operand_sums(lambda i, j: block(2 * i + a, 2 * j + b), terms) for b in range(2)] for a in range(2)]
    return [functools.partial(_operand_sums, lambda a, b, r=r: outer[a][b][r], terms) for r in range(7)]


def _join(c):
    return jnp.concatenate([jnp.concatenate(row, axis=1) for row in c], axis=0)


def _heads_to_lanes(groups):
    lane = lax.broadcasted_iota(jnp.int32, groups[0].shape, 1)
    groups = list(groups)
    for group_bit, lane_bit in ((2, 4), (1, 3), (0, 2), (2, 6), (2, 1), (1, 5), (1, 0)):
        shift = 1 << lane_bit
        low = (lane & shift) == 0
        for g in range(8):
            if g >> group_bit & 1:
                continue
            x, y = groups[g], groups[g | 1 << group_bit]
            groups[g] = jnp.where(low, x, pltpu.roll(y, shift, 1))
            groups[g | 1 << group_bit] = jnp.where(low, pltpu.roll(x, LANES - shift, 1), y)
    return [groups[(g & 1) << 2 | (g >> 2) << 1 | (g >> 1 & 1)] for g in range(8)]


def _word_half(word, hi):
    return pltpu.bitcast(word & U32(0xFFFF0000) if hi else word << 16, F32)


def _reciprocal(x):
    r = pl.reciprocal(x, approx=True)
    return r * (2.0 - x * r)


class _Timeline:
    def __init__(self, never):
        self.never, self.now, self.marks = never, 0.0, []

    def issue(self, cycles, results):
        for n, value in enumerate(results):
            self.marks.append((self.now + cycles * (n + 1) / len(results), value))
        self.now += cycles

    def after(self, cycle, value):
        ready = [v for t, v in self.marks if t <= cycle]
        if not ready:
            return value
        mark = ready[-1][0:8, 0:value.shape[1]]
        if value.shape[0] > 8:
            mark = jnp.concatenate([mark] * (value.shape[0] // 8), axis=0)
        return jnp.where(self.never, mark, value)


class _Background:
    def __init__(self, never):
        self.never, self.pending, self.credit, self.rate = never, iter(()), 0.0, 0.0

    def add(self, pieces, rate):
        self.pending, self.rate = itertools.chain(self.pending, pieces), rate

    def tie(self, words):
        self.credit += self.rate
        due = list(itertools.islice(self.pending, int(self.credit)))
        self.credit -= int(self.credit)
        if not due:
            return words
        due = [pltpu.bitcast(d, U32) for d in due]
        mark = functools.reduce(jnp.bitwise_or, [
            d[r:r + 8, c:c + LANES] for d in due for r in range(0, d.shape[0], 8) for c in range(0, d.shape[1], LANES)])
        top = jnp.where(self.never, mark, words[:8, :LANES])
        if words.shape[1] > LANES:
            top = jnp.concatenate([top, words[:8, LANES:]], axis=1)
        return jnp.concatenate([top, words[8:]], axis=0)

    def finish(self):
        for _ in self.pending:
            pass


def _start(copies):
    for cp in copies:
        cp.start()


def _wait(copies):
    for cp in copies:
        cp.wait()


def _kernel(xa_hbm, wqkv_hbm, woa_hbm, xb_hbm, c_hbm, wq_hbm, wuk_hbm, wuv_hbm, wob_hbm,
            out_hbm,
            xb_raw, c_raw, pool, cs, wq_raw, wuk_raw, wuv_raw, wqs, wks, wvs,
            q_s, k_s, v_s, ctx, wobs, woas,
            wqkv_raw, woa_raw, wob_raw, xa_raw, loc, obuf,
            sem_x, sem_w, sem_s, sem_a, sem_o, *, cfg):
    wq_u = wq_hbm.bitcast(U32)
    wuk_u = wuk_hbm.bitcast(U32)
    wuv_u = wuv_hbm.bitcast(U32)
    wqkv_u = wqkv_hbm.bitcast(U32)
    wob_u = wob_hbm.bitcast(U32)
    woa_u = woa_hbm.bitcast(U32)

    def pair_copies(j, which=(0, 1, 2)):
        ends = ((wuk_u, wuk_raw), (wuv_u, wuv_raw), (wq_u, wq_raw))
        return [pltpu.make_async_copy(ends[n][0].at[:, j, :], ends[n][1].at[j % 2], sem_w.at[j % 2, n])
                for n in which]

    def stream_copies(j):
        slot = j % 2
        rows = HALF // PAIRS
        cps = []
        for k in range(2):
            cps.append(pltpu.make_async_copy(
                wqkv_u.at[packed_rows(k * HALF + j * rows, rows), :], wqkv_raw.at[slot, k], sem_s.at[slot, k]))
        for k in range(2):
            word = (j >> 1 & 1) | k << 1 | (j >> 2) << 2
            cps.append(pltpu.make_async_copy(woa_u.at[:, word, :], woa_raw.at[slot, k], sem_s.at[slot, 7 + k]))
        for k in range(4):
            cps.append(pltpu.make_async_copy(
                wob_u.at[packed_rows(k * DM + j * 64, 64), :], wob_raw.at[slot, k], sem_s.at[slot, 3 + k]))
        return cps

    def c_copy(i):
        rows = pl.ds(pl.multiple_of(i * BLK, BLK), BLK)
        return pltpu.make_async_copy(c_hbm.at[rows, :], c_raw.at[i], sem_x.at[0, i])

    def xb_copy(i):
        rows = pl.ds(pl.multiple_of(i * BLK, BLK), BLK)
        return pltpu.make_async_copy(xb_hbm.at[rows, :], xb_raw.at[i], sem_x.at[1, i])

    def xa_copy(i):
        rows = pl.ds(pl.multiple_of(i * BLK, BLK), BLK)
        return pltpu.make_async_copy(xa_hbm.at[rows, :], xa_raw.at[i % 2], sem_a.at[i % 2])

    def out_copy(i, part):
        r0, nr, c0, nc = (0, BLK, DM, DM) if part == 4 else (part // 2 * SUB, SUB, part % 2 * HALF, HALF)
        rows = pl.ds(pl.multiple_of(i * BLK + r0, SUB), nr)
        return pltpu.make_async_copy(obuf.at[i % 2, r0:r0 + nr, c0:c0 + nc], out_hbm.at[rows, c0:c0 + nc],
                                     sem_o.at[i % 2, part])

    def packed_rows(start, size):
        if isinstance(start, int):
            return pl.ds(start // 2, size // 2)
        return pl.ds(pl.multiple_of(start // 2, size // 2), size // 2)

    def prepare_pair_weights(j, which="qkv"):
        slot = j % 2
        for name in which:
            raw, dst = {"q": (wq_raw, wqs), "k": (wuk_raw, wks), "v": (wuv_raw, wvs)}[name]
            depth = raw.shape[1] // 2
            for r0 in range(0, depth, 32):
                words = [raw[slot, k * depth + r0:k * depth + r0 + 32, :] for k in range(2)]
                for r, op in enumerate(_operand_sums(lambda k, head: _word_half(words[k], head), B_TERMS)):
                    dst[r, r0 // 2:r0 // 2 + 16, :] = _pack(op)

    def prepare_inputs(i, raw, dst, base):
        width = raw.shape[2] // 2
        ops = _operand_sums(lambda a, k: raw[i, a * SUB:(a + 1) * SUB, k * width:(k + 1) * width], A_TERMS)
        ops = [_pack(op) for op in ops]
        for r, op in enumerate(ops):
            dst[r, packed_rows(base + i * SUB, SUB), :] = op
        return ops

    def project(i, which, tl=None, ops=None):
        lhs, base, rhs, dst = {"q": (pool, 2 * POOL_X, wqs, q_s), "k": (cs, 0, wks, k_s),
                               "v": (cs, 0, wvs, v_s)}[which]
        rows = packed_rows(base + i * SUB, SUB)

        def product(r):
            w = rhs[r] if tl is None or i not in cfg["bgblocks"] else tl.bg.tie(rhs[r])
            m = jnp.dot(_unpack(lhs[r, rows, :] if ops is None else ops[r]), _unpack(w), preferred_element_type=F32)
            if tl is not None:
                tl.issue(SUB * rhs.shape[1] // 256, [m[SUB // 2 - 8:SUB // 2], m[SUB - 8:SUB]])
            return m

        c = _block_product(product, cfg["o_p" + which])
        for a in range(2):
            if which == "q":
                q_s[pl.ds(pl.multiple_of(i * BLK + a * SUB, SUB), SUB), :] = (
                    jnp.concatenate(c[a], axis=1) * (B_DH ** -0.5 * LOG2E)).astype(BF16)
            else:
                for head in range(2):
                    dst[head, packed_rows(i * BLK + a * SUB, SUB), :] = _pack(c[a][head])

    def head_rows(ref, h, r0, r1):
        return _unpack(ref[h, r0 // 2:r1 // 2, :])

    def scores(h, i, tl):
        def nt(a, b):
            return lax.dot_general(a, b, (((1,), (1,)), ((), ())), preferred_element_type=F32)
        row = lax.broadcasted_iota(jnp.int32, (SUB, SUB), 0)
        col = lax.broadcasted_iota(jnp.int32, (SUB, SUB), 1)
        r0 = i * BLK
        full = nt(q_s[r0:r0 + BLK, h * B_DH:(h + 1) * B_DH], head_rows(k_s, h, 0, r0)) if i else None
        if i:
            tl.issue(BLK * i // 2, [full[t % BLK:t % BLK + 8, t // BLK * LANES:(t // BLK + 1) * LANES]
                                    for t in range(56, BLK * i // 2, 64)])
        diag = []
        for a in range(2):
            d = nt(q_s[r0 + a * SUB:r0 + (a + 1) * SUB, h * B_DH:(h + 1) * B_DH],
                   head_rows(k_s, h, r0, r0 + (a + 1) * SUB))
            tl.issue(32 * (a + 1), [d])
            last = jnp.where(col <= row, d[:, a * SUB:], NEG)
            diag.append(jnp.concatenate([d[:, :SUB], last], axis=1) if a else last)
        return full, diag, tl.now

    def softmax(i, sc, tl, h):
        full, diag, t0 = sc
        nf = i * BLK
        lo, hi = tl.pace[h]
        span = tl.now - t0
        step = tl.pch
        pf, pd, inv = [], [], []
        for a in range(2):
            s = diag[a]
            if full is not None:
                s = jnp.concatenate([full[a * SUB:(a + 1) * SUB], s], axis=1)
            m = jnp.max(s, axis=1, keepdims=True)
            if step:
                m = jnp.concatenate([
                    tl.after(t0 + span * (lo + (hi - lo) * (a * SUB + c) / BLK), m[c:c + step])
                    for c in range(0, SUB, step)], axis=0)
            p = jnp.exp2(s - m)
            if i >= cfg["sum16"]:
                p = p.astype(BF16)
            inv.append(_reciprocal(jnp.sum(p.astype(F32), axis=1, keepdims=True)))
            if full is not None:
                pf.append(p[:, :nf])
            pd.append(p[:, nf:])
        return (jnp.concatenate(pf, axis=0) if pf else None), pd, inv

    def context(h, i, sm, tl):
        def pv(a, b):
            return jnp.dot(a.astype(BF16), b, preferred_element_type=F32)
        pf, pd, inv = sm
        r0 = i * BLK
        of = None
        for k0 in range(0, r0, tl.pvk):
            k1 = min(k0 + tl.pvk, r0)
            words = v_s[h, k0 // 2:k1 // 2, :]
            if tl.bgpv and i in cfg["bgblocks_last"]:
                words = jnp.concatenate([tl.bg.tie(words[t:t + 64]) for t in range(0, words.shape[0], 64)], axis=0)
            part = pv(pf[:, k0:k1], _unpack(words))
            of = part if of is None else of + part
            tl.issue((k1 - k0) // 2, [of[t:t + 8] for t in range(56, BLK, 64)])
        out = []
        for a in range(2):
            o = pv(pd[a], head_rows(v_s, h, r0, r0 + (a + 1) * SUB))
            tl.issue(32 * (a + 1), [o])
            if of is not None:
                o = o + of[a * SUB:(a + 1) * SUB]
            out.append(o * inv[a])
        return out

    def stream_work(j, inner_part=True, outer_part=True):
        slot = j % 2

        def qkv(part):
            groups = [_heads_to_lanes([
                wqkv_raw[slot, k, :, part * DM + a * LANES:part * DM + (a + 1) * LANES]
                for a in range(8)]) for k in range(2)]
            rows = packed_rows(2 * POOL_QKV + part * HALF + j * (HALF // PAIRS), HALF // PAIRS)
            for a in range(4):
                for r, op in enumerate(_operand_sums(lambda k, n: _unpack(groups[k][4 * n + a]), B_TERMS)):
                    op = _pack(op)
                    pool[r, rows, a * LANES:(a + 1) * LANES] = op
                    yield op

        def two_level(block, dst, row0, cols):
            for r, inner in enumerate(_operand_sums2(block, B_TERMS)):
                for t, op in enumerate(inner()):
                    op = _pack(op)
                    dst[7 * r + t, packed_rows(row0, 32), cols] = op
                    yield op

        def out_a():
            c0 = j % 2 * LANES if isinstance(j, int) else pl.multiple_of(j % 2 * LANES, LANES)
            row0 = ((j >> 1 & 1) * 4 + (j >> 2)) * A_HEADS
            return two_level(lambda k, n: _word_half(woa_raw[slot, k % 2, :, pl.ds(n * 256 + c0, LANES)], k // 2),
                             woas, row0, pl.ds(c0, LANES))

        def out_b(r0, c0):
            return two_level(lambda k, n: _unpack(
                wob_raw[slot, k, r0 // 2:r0 // 2 + 16, n * 256 + c0:n * 256 + c0 + LANES]),
                wobs, j * 64 + r0, slice(c0, c0 + LANES))

        for n in cfg["joborder" if inner_part else "joborder2"]:
            if n < 4 and outer_part:
                yield from out_b(n // 2 * 32, n % 2 * LANES)
            elif n == 4 and outer_part:
                yield from out_a()
            elif n > 4 and inner_part:
                yield from qkv(n - 5)

    only = cfg.get("only")
    named = {"wk": lambda: pair_copies(0, (0,)), "wv": lambda: pair_copies(0, (1,)), "wq": lambda: pair_copies(0, (2,)),
             "p1": lambda: pair_copies(1), "s0": lambda: stream_copies(0)}

    def request(names):
        for name in names:
            if name in named:
                _start(named[name]())
            else:
                (c_copy if name[0] == "c" else xb_copy)(int(name[1])).start()

    def first_steps(copy, work, plan):
        step = NBLK // len(plan)

        def body(n, carry):
            blocks = [n * step + t for t in range(step)]
            _wait([copy(i) for i in blocks])
            for at, names in enumerate(plan):
                if names:
                    pl.when(n == at)(functools.partial(request, names))
            for i in blocks:
                work(i)
            return carry

        lax.fori_loop(0, len(plan), body, 0)

    def first_kv(i):
        ops = prepare_inputs(i, c_raw, cs, 0)
        project(i, "k", ops=ops)
        project(i, "v", ops=ops)

    def first_q(i):
        project(i, "q", ops=prepare_inputs(i, xb_raw, pool, 2 * POOL_X))

    with jax.named_scope("prologue"):
        if not only:
            request(cfg["plan0"])
            with jax.named_scope("w0"):
                _wait(pair_copies(0, (0,)))
            request(cfg["plan1"])
            prepare_pair_weights(0, "k")
            _wait(pair_copies(0, (1,)))
            prepare_pair_weights(0, "v")
            with jax.named_scope("kv"):
                first_steps(c_copy, first_kv, cfg["plan_kv"])
            _wait(pair_copies(0, (2,)))
            prepare_pair_weights(0, "q")
            with jax.named_scope("q"):
                first_steps(xb_copy, first_q, cfg["plan_q"])
    _wait(pair_copies(1) + stream_copies(0))
    _start(pair_copies(2) + stream_copies(1))

    def head_pair(j, project_next):
        if project_next:
            prepare_pair_weights(j + 1)
        else:
            xa_copy(0).start()
            xa_copy(1).start()
        tl = _Timeline(j < 0)
        tl.pace, tl.pch = (cfg["pace"], cfg["pch"]) if project_next else (cfg["pace_last"], cfg["pch_last"])
        tl.bg = _Background(j < 0)
        tl.bg.add(stream_work(j, True, project_next),
                  329 / (21 * len(cfg["bgblocks"])) if project_next else cfg["bgrate_last"])
        tl.bgpv = not project_next
        tl.pvk = cfg["pvk"] if project_next else cfg["pvk_last"]
        proj = (lambda i, which: project(i, which, tl)) if project_next else (lambda i, which: None)
        sc, o = {}, {}

        def finish_head(h, i):
            o[h, i] = context(h, i, softmax(i, sc.pop((h, i)), tl, h), tl)
            if (1 - h, i) in o:
                for a in range(2):
                    ctx[j, i * BLK + a * SUB:i * BLK + (a + 1) * SUB, :] = (
                        jnp.concatenate([o[0, i][a], o[1, i][a]], axis=1).astype(BF16))

        for i in range(NBLK - 1, -1, -1):
            order = cfg["order"] if project_next else cfg["order_last"]
            for tok in order[i] if isinstance(order, dict) else order:
                if tok[0] == "s":
                    sc[int(tok[1]), i] = scores(int(tok[1]), i, tl)
                elif tok[0] == "c":
                    finish_head(int(tok[1]), i)
                elif tok[0] == "C":
                    if (int(tok[1]), i + 1) in sc:
                        finish_head(int(tok[1]), i + 1)
                elif tok == "q":
                    proj(i, "q")
                elif i + 1 < NBLK:
                    proj(i + 1, tok)
        for h, i in sorted(sc):
            finish_head(h, i)
        proj(0, "k")
        proj(0, "v")
        tl.bg.finish()
        if project_next:
            _wait(stream_copies(j + 1))

            @pl.when(j + 2 < PAIRS)
            def _():
                _wait(pair_copies(j + 2))

            @pl.when(j + 3 < PAIRS)
            def _():
                _start(pair_copies(j + 3))

            @pl.when(j + 2 < PAIRS)
            def _():
                _start(stream_copies(j + 2))

    def pair_step(j, carry):
        with jax.named_scope("group"):
            head_pair(j, True)
        return carry

    with jax.named_scope("phase1"):
        if only in (None, "p1"):
            lax.fori_loop(0, PAIRS - 1, pair_step, 0)
    with jax.named_scope("lastgroup"):
        if only == "p1" or only == "last":
            def keep(n, carry):
                obuf.bitcast(U32)[0, 0:8, 0:LANES] = (pltpu.bitcast(ctx[n, 0:16, 0:LANES], U32) | pltpu.bitcast(q_s[pl.ds(pl.multiple_of(n * 16, 16), 16), 0:LANES], U32) | pool[n, 0:8, 0:LANES] | wobs[n, 0:8, 0:LANES] | woas[n, 0:8, 0:LANES]
                                                      | k_s[n % 2, 0:8, :] | v_s[n % 2, 0:8, :])
                return carry
        if only == "last":
            lax.fori_loop(PAIRS - 1, PAIRS, lambda j, c: (head_pair(j, False), c)[1], 0)
        if only == "p1" or only == "last":
            lax.fori_loop(0, 7, keep, 0)
        if only in ("p1", "p2", "last"):
            _wait(stream_copies(PAIRS - 1))
            xa_copy(0).start()
            xa_copy(1).start()
        else:
            lax.fori_loop(PAIRS - 1, PAIRS, lambda j, c: (head_pair(j, False), c)[1], 0)

    loc[0:16, BLK:BLK + HALO, :] = jnp.zeros((16, HALO, LANES), F32)

    def store_blocks(i, col0, c):
        for a, n in ((0, 0), (1, 0), (0, 1), (1, 1)):
            obuf[i % 2, a * SUB:(a + 1) * SUB, col0 + n * HALF:col0 + (n + 1) * HALF] = c[a][n].astype(BF16)
            if col0 == 0:
                out_copy(i, 2 * a + n).start()
        if col0:
            out_copy(i, 4).start()

    def row_block(i, carry):
        slot = i % 2
        xa_copy(i).wait()

        @pl.when(i >= 2)
        def _():
            _wait([out_copy(i - 2, part) for part in range(5)])

        loc[0:16, 0:HALO, :] = loc[0:16, BLK:BLK + HALO, :]
        zero = i // NBLK if cfg["opaque"] else 0
        xops = [op.astype(BF16) for op in _operand_sums(
            lambda a, k: xa_raw[slot, a * SUB:(a + 1) * SUB, k * HALF:(k + 1) * HALF], A_TERMS)]

        bg = _Background(i < 0)
        bg.add(stream_work(PAIRS - 1, False, True), cfg["bgrate2"])

        def lane_groups(part):
            r0 = POOL_QKV + part * HALF // 2
            c = _block_product(lambda r: jnp.dot(xops[r], _unpack(bg.tie(pool[r, r0:r0 + HALF // 2, :])),
                                                 preferred_element_type=F32), cfg["o_a"])
            return lambda a, g: c[a][g // 4][:, (g % 4) * LANES:(g % 4 + 1) * LANES]

        marks = []

        def out_b():
            quarter = PAIRS // 4

            def block(a, k):
                rows = pl.ds(pl.multiple_of(i * BLK + a * (BLK // 4), BLK // 4), BLK // 4)
                return jnp.concatenate(
                    [ctx[j, rows, :] for j in range(k * quarter, (k + 1) * quarter)], axis=1).astype(F32)

            lhs = _operand_sums2(block, A_TERMS)

            def outer(r):
                ops = lhs[r]()

                def product(t):
                    step = DM // cfg["ksplit"]
                    acc = None
                    for k0 in range(0, DM, step):
                        part = jnp.dot(ops[t][:, k0:k0 + step].astype(BF16),
                                       _unpack(wobs[7 * r + t, k0 // 2:(k0 + step) // 2, :]),
                                       preferred_element_type=F32)
                        acc = part if acc is None else acc + part
                        marks.append(acc)
                    return acc

                return _join(_block_product(product, cfg["o_bi"]))

            store_blocks(i, DM, _block_product(outer, cfg["o_bo"]))

        for part in cfg["aorder"]:
            if part == "b":
                bg.finish()
                out_b()
                continue
            f = lane_groups(part)
            for a in range(2):
                for g in range(8):
                    loc[(LOC_Q, LOC_K, LOC_V)[part] + g, HALO + a * SUB:HALO + (a + 1) * SUB, :] = f(a, g)

        ch = cfg["cha"]

        stages = cfg["stages"]
        total = stages * BLK // ch
        count = [0]

        def paced(values):
            lo, hi = cfg["gate"]
            mark = marks[int((lo + (hi - lo) * count[0] / (total - 1)) * (len(marks) - 1))]
            count[0] += 1
            return [jnp.where(i < 0, mark[0:ch, 0:LANES], t) for t in values]

        def attend(c0):
            def rows(base, g, w):
                b0 = HALO + c0 - A_DIL * w
                return loc[zero + base + g, b0:b0 + ch, :]

            q0 = [rows(LOC_Q, g, 0) for g in range(8)]
            logits = []
            half = max(stages // 2, 1)
            for w in range(A_WIN):
                if w % (A_WIN // half) == 0:
                    q = paced(q0)
                acc = q[0] * rows(LOC_K, 0, w)
                for g in range(1, 8):
                    acc = acc + q[g] * rows(LOC_K, g, w)
                acc = acc + pltpu.roll(acc, 2 * A_HEADS, 1)
                acc = acc + pltpu.roll(acc, A_HEADS, 1)
                if c0 < A_DIL * w:
                    pos = i * BLK + c0 + lax.broadcasted_iota(jnp.int32, (ch, LANES), 0)
                    acc = jnp.where(pos >= A_DIL * w, acc, NEG * A_DH ** 0.5)
                logits.append(acc)
            m = functools.reduce(jnp.maximum, logits)
            ps = [jnp.exp2((l - m) * (A_DH ** -0.5 * LOG2E)) for l in logits]
            inv = _reciprocal(functools.reduce(lambda a, b: a + b, ps))
            ps = [p * inv for p in ps]
            out = []
            for g in range(8):
                if stages > 1 and g % (8 // half) == 0:
                    pg = paced(ps)
                elif stages == 1:
                    pg = ps
                out.append(functools.reduce(lambda a, b: a + b, [pg[w] * rows(LOC_V, g, w) for w in range(A_WIN)]))
            return out

        quarters = [[] for _ in range(4)]
        for c0 in range(0, BLK // 4, ch):
            for a in range(4):
                quarters[a].append(jnp.concatenate(attend(a * (BLK // 4) + c0), axis=1))
        quarters = [jnp.concatenate(t, axis=0) for t in quarters]
        lhs = _operand_sums2(lambda a, k: quarters[a][:, k * 256:(k + 1) * 256], A_TERMS)

        def outer(r):
            ops = lhs[r]()
            return _join(_block_product(lambda t: jnp.dot(
                ops[t].astype(BF16), _unpack(woas[7 * r + t]), preferred_element_type=F32), cfg["o_ai"]))

        store_blocks(i, 0, _block_product(outer, cfg["o_ao"]))

        @pl.when(i + 2 < NBLK)
        def _():
            xa_copy(i + 2).start()

        return carry

    def row_step(i, carry):
        with jax.named_scope("rowblk"):
            return row_block(i, carry)

    with jax.named_scope("phase2"):
        if only in (None, "p2"):
            lax.fori_loop(0, NBLK, row_step, 0)
    with jax.named_scope("tail"):
        _wait([out_copy(i, part) for i in (NBLK - 2, NBLK - 1) for part in range(5)])


DEFAULT_CFG = dict(cha=16, opaque=False, nsplit=4, ksplit=4, gate=(0, 0.88), stages=4, pace=((0, 0.7), (0.2, 0.8)), pch=0, bgblocks=(6, 5, 4, 3, 2, 1), bgblocks_last=(7, 6, 5, 4, 3, 2, 1), bgrate_last=1, bgrate2=14, joborder=(0, 5, 1, 6, 2, 7, 3, 4),
                   **{"o_" + n: (0, 3, 4, 6, 1, 2, 5) for n in ("pq", "pk", "pv", "a", "bi", "bo", "ai", "ao")},
                   pch_last=0, pace_last=((0, 0.7), (0.2, 0.8)), jobslots_last=[(3, 1, 1), (2, 1, 1), (3, 0, 1), (2, 0, 1), (1, 0, 1), (1, 1, 1), (3, 0, 0), (2, 0, 0), (2, 1, 0)], sum16=0, plan0=("wk", "c0", "wv", "c1"), plan1=("c2", "c3"),
                   plan_kv=(("c4", "c5", "c6", "c7"), ("wq", "x0"), ("x1", "x2"), ("x3", "x4")),
                   plan_q=(("x5", "x6"), ("x7", "p1"), ("s0",), ()), sumgate=False, wch=32, wspan=0, pvk=1024, jobslots=[(5, 1, 1), (4, 0, 0), (3, 1, 0), (5, 0, 1), (5, 0, 0), (4, 1, 1), (3, 0, 0), (2, 1, 0)], order={0: ('s0', 'k', 's1', 'v', 'c0', 'q', 'c1'), 1: ('s0', 'k', 's1', 'v', 'c0', 'q', 'c1'), 2: ('s0', 'k', 's1', 'v', 'c0', 'q', 'c1'), 3: ('s0', 's1', 'k', 'q', 'c0', 'v', 'c1'), 4: ('s0', 's1', 'k', 'v', 'c0', 'q', 'c1'), 5: ('s0', 'k', 's1', 'q', 'c0', 'v', 'c1'), 6: ('s0', 's1', 'k', 'c0', 'v', 'c1', 'q'), 7: ('s0', 's1', 'k', 'c0', 'v', 'c1', 'q')}, order_last=('s0', 'C0', 's1', 'C1'),
                   pieces=(6, 5, 4, 3, 6, 5, 4, 3), aorder=(1, 0, 2, "b"), nobc=True)


DEFAULT_CFG.update({'order_last': ('s0', 'C0', 's1', 'C1'), 'bgblocks_last': (7, 5, 4, 3, 2, 0), 'bgrate_last': 1, 'pch_last': 0, 'pace_last': ((0, 0.7), (0.2, 0.9)), 'pvk_last': 1024, 'ksplit': 4, 'stages': 8, 'gate': (0, 0.92), 'cha': 16, 'bgrate2': 12, 'aorder': (0, 1, 2, 'b'), 'o_a': (0, 3, 4, 6, 1, 2, 5), 'o_bi': (3, 1, 2, 4, 0, 6, 5), 'o_bo': (3, 0, 1, 5, 2, 4, 6), 'o_ai': (2, 5, 0, 1, 3, 6, 4), 'o_ao': (0, 3, 4, 6, 1, 2, 5), 'joborder2': (3, 7, 1, 0, 2, 6, 5, 4), 'order': {0: ('s0', 'k', 's1', 'v', 'c0', 'q', 'c1'), 1: ('k', 's0', 'v', 's1', 'c0', 'q', 'c1'), 2: ('s0', 'k', 's1', 'v', 'c0', 'q', 'c1'), 3: ('s0', 's1', 'k', 'q', 'c0', 'v', 'c1'), 4: ('s0', 's1', 'k', 'q', 'c0', 'v', 'c1'), 5: ('s0', 's1', 'k', 'q', 'c0', 'v', 'c1'), 6: ('s0', 's1', 'k', 'v', 'c0', 'q', 'c1'), 7: ('s0', 's1', 'k', 'c0', 'q', 'c1', 'v')}, 'bgblocks': (6, 5, 4, 3, 2, 1), 'pvk': 512, 'joborder': (0, 5, 6, 1, 2, 7, 3, 4), 'o_pq': (3, 1, 0, 6, 4, 2, 5), 'o_pk': (0, 3, 4, 6, 1, 2, 5), 'o_pv': (5, 2, 0, 4, 6, 3, 1), 'pch': 16, 'pace': ((0, 0.6), (0.2, 0.8))})


def build(cfg=None):
    cfg = dict(DEFAULT_CFG, **(cfg or {}))
    vmem = pltpu.VMEM

    def fn(A_x, A_wqkv, A_wo, B_x, B_c_kv, B_w_q, B_w_uk, B_w_uv, B_w_o):
        out = pl.pallas_call(
            functools.partial(_kernel, cfg=cfg),
            out_shape=jax.ShapeDtypeStruct((S, 2 * DM), BF16),
            in_specs=[pl.BlockSpec(memory_space=pl.ANY)] * 9,
            out_specs=pl.BlockSpec(memory_space=pl.ANY),
            scratch_shapes=[
                vmem((NBLK, BLK, DM), BF16),
                vmem((NBLK, BLK, B_DC), BF16),
                vmem((7, POOL_ROWS, HALF), U32),
                vmem((7, S // 4, B_DC // 2), U32),
                vmem((2, DM, B_DH), U32),
                vmem((2, B_DC, B_DH), U32),
                vmem((2, B_DC, B_DH), U32),
                vmem((7, DM // 4, B_DH), U32),
                vmem((7, B_DC // 4, B_DH), U32),
                vmem((7, B_DC // 4, B_DH), U32),
                vmem((S, 2 * B_DH), BF16),
                vmem((2, S // 2, B_DH), U32),
                vmem((2, S // 2, B_DH), U32),
                vmem((PAIRS, S, 2 * B_DH), BF16),
                vmem((49, DM // 2, DM // 4), U32),
                vmem((49, DM // 8, DM // 4), U32),
                vmem((2, 2, HALF // PAIRS // 2, 3 * DM), U32),
                vmem((2, 2, A_HEADS, DM), U32),
                vmem((2, 4, 32, DM), U32),
                vmem((2, BLK, DM), BF16),
                vmem((LOC_PANELS, HALO + BLK, LANES), F32),
                vmem((2, BLK, 2 * DM), BF16),
                pltpu.SemaphoreType.DMA((2, NBLK)),
                pltpu.SemaphoreType.DMA((2, 3)),
                pltpu.SemaphoreType.DMA((2, 9)),
                pltpu.SemaphoreType.DMA((2,)),
                pltpu.SemaphoreType.DMA((2, 5)),
            ],
            compiler_params=pltpu.CompilerParams(vmem_limit_bytes=124 * 2 ** 20, flags=cfg.get("flags"),
                                                 disable_bounds_checks=cfg.get("nobc", False)),
            name="fused_local_and_latent_attention",
        )(A_x.reshape(S, DM), A_wqkv, A_wo.reshape(A_HEADS, A_DH, DM), B_x.reshape(S, DM), B_c_kv.reshape(S, B_DC),
          B_w_q, B_w_uk, B_w_uv, B_w_o.reshape(B_HEADS * B_DH, DM))
        return out.reshape(1, S, 2 * DM)

    return jax.jit(fn)


@jax.jit
def pallas_concat_heads__sliding_local_dilated__compressed_kv_cla__prompt_kernel(
    A_x: jax.Array,
    A_wqkv: jax.Array,
    A_wo: jax.Array,
    B_x: jax.Array,
    B_c_kv: jax.Array,
    B_w_q: jax.Array,
    B_w_uk: jax.Array,
    B_w_uv: jax.Array,
    B_w_o: jax.Array,
):
    return build(dict())(A_x, A_wqkv, A_wo, B_x, B_c_kv, B_w_q, B_w_uk, B_w_uv, B_w_o)
```

```python
import functools
import itertools

import jax
import jax.numpy as jnp
from jax import lax
import jax.experimental.pallas as pl
import jax.experimental.pallas.tpu as pltpu

S = 2048
DM = 1024
HALF = DM // 2
LANES = 128
A_HEADS, A_DH, A_WIN, A_DIL = 32, 32, 8, 2
HALO = 16
B_HEADS, B_DH, B_DC = 32, 128, 512
PAIRS = B_HEADS // 2

BLK = 256
SUB = BLK // 2
NBLK = S // BLK

LOG2E = 1.4426950408889634
NEG = -1e9
F32, BF16, U32 = jnp.float32, jnp.bfloat16, jnp.uint32

A_TERMS = (((1, 0, 0), (1, 1, 1)), ((1, 1, 0), (1, 1, 1)), ((1, 0, 0),), ((1, 1, 1),),
           ((1, 0, 0), (1, 0, 1)), ((1, 1, 0), (-1, 0, 0)), ((1, 0, 1), (-1, 1, 1)))
B_TERMS = (((1, 0, 0), (1, 1, 1)), ((1, 0, 0),), ((1, 0, 1), (-1, 1, 1)), ((1, 1, 0), (-1, 0, 0)),
           ((1, 1, 1),), ((1, 0, 0), (1, 0, 1)), ((1, 1, 0), (1, 1, 1)))
C_TERMS = (((1, 0, 0), (1, 1, 1)), ((1, 1, 0), (-1, 1, 1)), ((1, 0, 1), (1, 1, 1)), ((1, 0, 0), (1, 1, 0)),
           ((-1, 0, 0), (1, 0, 1)), ((1, 1, 1),), ((1, 0, 0),))

POOL_X = 0
POOL_QKV = POOL_X + S // 4
POOL_ROWS = POOL_QKV + 3 * HALF // 2
LOC_K, LOC_V, LOC_Q, LOC_PANELS = 0, 8, 16, 24


def _pack(x):
    return pltpu.bitcast(x.astype(BF16), U32)


def _unpack(x):
    return pltpu.bitcast(x, BF16)


def _operand_sums(block, terms):
    blocks = [[block(i, j) for j in range(2)] for i in range(2)]
    out = []
    for (_, i, j), *rest in terms:
        acc = blocks[i][j]
        for sign, i, j in rest:
            a, b = acc.astype(F32), blocks[i][j].astype(F32)
            acc = a + b if sign > 0 else a - b
        out.append(acc)
    return out


def _block_product(product, order=(0, 3, 4, 6, 1, 2, 5)):
    c = [[None, None], [None, None]]
    for r in order:
        m = product(r)
        for sign, i, j in C_TERMS[r]:
            if c[i][j] is None:
                c[i][j] = m if sign > 0 else -m
            else:
                c[i][j] = c[i][j] + m if sign > 0 else c[i][j] - m
    return c


def _operand_sums2(block, terms):
    outer = [[_operand_sums(lambda i, j: block(2 * i + a, 2 * j + b), terms) for b in range(2)] for a in range(2)]
    return [functools.partial(_operand_sums, lambda a, b, r=r: outer[a][b][r], terms) for r in range(7)]


def _join(c):
    return jnp.concatenate([jnp.concatenate(row, axis=1) for row in c], axis=0)


def _heads_to_lanes(groups):
    lane = lax.broadcasted_iota(jnp.int32, groups[0].shape, 1)
    groups = list(groups)
    for group_bit, lane_bit in ((2, 4), (1, 3), (0, 2), (2, 6), (2, 1), (1, 5), (1, 0)):
        shift = 1 << lane_bit
        low = (lane & shift) == 0
        for g in range(8):
            if g >> group_bit & 1:
                continue
            x, y = groups[g], groups[g | 1 << group_bit]
            groups[g] = jnp.where(low, x, pltpu.roll(y, shift, 1))
            groups[g | 1 << group_bit] = jnp.where(low, pltpu.roll(x, LANES - shift, 1), y)
    return [groups[(g & 1) << 2 | (g >> 2) << 1 | (g >> 1 & 1)] for g in range(8)]


def _word_half(word, hi):
    return pltpu.bitcast(word & U32(0xFFFF0000) if hi else word << 16, F32)


def _reciprocal(x):
    r = pl.reciprocal(x, approx=True)
    return r * (2.0 - x * r)


class _Timeline:
    def __init__(self, never):
        self.never, self.now, self.marks = never, 0.0, []

    def issue(self, cycles, results):
        for n, value in enumerate(results):
            self.marks.append((self.now + cycles * (n + 1) / len(results), value))
        self.now += cycles

    def after(self, cycle, value):
        ready = [v for t, v in self.marks if t <= cycle]
        if not ready:
            return value
        mark = ready[-1][0:8, 0:value.shape[1]]
        if value.shape[0] > 8:
            mark = jnp.concatenate([mark] * (value.shape[0] // 8), axis=0)
        return jnp.where(self.never, mark, value)


class _Background:
    def __init__(self, never):
        self.never, self.pending, self.credit, self.rate = never, iter(()), 0.0, 0.0

    def add(self, pieces, rate):
        self.pending, self.rate = itertools.chain(self.pending, pieces), rate

    def tie(self, words):
        self.credit += self.rate
        due = list(itertools.islice(self.pending, int(self.credit)))
        self.credit -= int(self.credit)
        if not due:
            return words
        due = [pltpu.bitcast(d, U32) for d in due]
        mark = functools.reduce(jnp.bitwise_or, [
            d[r:r + 8, c:c + LANES] for d in due for r in range(0, d.shape[0], 8) for c in range(0, d.shape[1], LANES)])
        top = jnp.where(self.never, mark, words[:8, :LANES])
        if words.shape[1] > LANES:
            top = jnp.concatenate([top, words[:8, LANES:]], axis=1)
        return jnp.concatenate([top, words[8:]], axis=0)

    def finish(self):
        for _ in self.pending:
            pass


def _start(copies):
    for cp in copies:
        cp.start()


def _wait(copies):
    for cp in copies:
        cp.wait()


def _kernel(xa_hbm, wqkv_hbm, woa_hbm, xb_hbm, c_hbm, wq_hbm, wuk_hbm, wuv_hbm, wob_hbm,
            out_hbm,
            xb_raw, c_raw, pool, cs, wq_raw, wuk_raw, wuv_raw, wqs, wks, wvs,
            q_s, k_s, v_s, ctx, wobs, woas,
            wqkv_raw, woa_raw, wob_raw, xa_raw, loc, obuf,
            sem_x, sem_w, sem_s, sem_a, sem_o, *, cfg):
    wq_u = wq_hbm.bitcast(U32)
    wuk_u = wuk_hbm.bitcast(U32)
    wuv_u = wuv_hbm.bitcast(U32)
    woa_u = woa_hbm.bitcast(U32)

    def pair_copies(j, which=(0, 1, 2)):
        ends = ((wuk_u, wuk_raw), (wuv_u, wuv_raw), (wq_u, wq_raw))
        return [pltpu.make_async_copy(ends[n][0].at[:, j, :], ends[n][1].at[j % 2], sem_w.at[j % 2, n])
                for n in which]

    def stream_copies(j):
        slot = j % 2
        rows = HALF // PAIRS
        cps = []
        for k in range(2):
            cps.append(pltpu.make_async_copy(
                wqkv_hbm.at[row_range(k * HALF + j * rows, rows), :], wqkv_raw.at[slot, k], sem_s.at[slot, k]))
        for k in range(2):
            word = (j >> 1 & 1) | k << 1 | (j >> 2) << 2
            cps.append(pltpu.make_async_copy(woa_u.at[:, word, :], woa_raw.at[slot, k], sem_s.at[slot, 7 + k]))
        for k in range(4):
            cps.append(pltpu.make_async_copy(
                wob_hbm.at[row_range(k * DM + j * 64, 64), :], wob_raw.at[slot, k], sem_s.at[slot, 3 + k]))
        return cps

    def c_copy(n):
        rows = pl.ds(pl.multiple_of(n * 2 * BLK, 2 * BLK), 2 * BLK)
        return pltpu.make_async_copy(c_hbm.at[rows, :], c_raw.at[rows, :], sem_x.at[0, n])

    def xb_copy(n):
        rows = pl.ds(pl.multiple_of(n * 2 * BLK, 2 * BLK), 2 * BLK)
        return pltpu.make_async_copy(xb_hbm.at[rows, :], xb_raw.at[rows, :], sem_x.at[1, n])

    def xa_copy(i):
        rows = pl.ds(pl.multiple_of(i * BLK, BLK), BLK)
        return pltpu.make_async_copy(xa_hbm.at[rows, :], xa_raw.at[i % 2], sem_a.at[i % 2])

    def out_copy(i, part):
        r0, nr, c0, nc = (0, BLK, DM, DM) if part == 4 else (part // 2 * SUB, SUB, part % 2 * HALF, HALF)
        rows = pl.ds(pl.multiple_of(i * BLK + r0, SUB), nr)
        return pltpu.make_async_copy(obuf.at[i % 2, r0:r0 + nr, c0:c0 + nc], out_hbm.at[rows, c0:c0 + nc],
                                     sem_o.at[i % 2, part])

    def row_range(start, size):
        return pl.ds(start if isinstance(start, int) else pl.multiple_of(start, size), size)

    def packed_rows(start, size):
        if isinstance(start, int):
            return pl.ds(start // 2, size // 2)
        return pl.ds(pl.multiple_of(start // 2, size // 2), size // 2)

    def prepare_pair_weights(j, which="qkv"):
        slot = j % 2
        for name in which:
            raw, dst = {"q": (wq_raw, wqs), "k": (wuk_raw, wks), "v": (wuv_raw, wvs)}[name]
            depth = raw.shape[1] // 2
            for r0 in range(0, depth, 32):
                words = [raw[slot, k * depth + r0:k * depth + r0 + 32, :] for k in range(2)]
                for r, op in enumerate(_operand_sums(lambda k, head: _word_half(words[k], head), B_TERMS)):
                    dst[r, r0 // 2:r0 // 2 + 16, :] = _pack(op)

    def prepare_inputs(i, raw, dst, base):
        width = raw.shape[1] // 2
        ops = _operand_sums(lambda a, k: raw[pl.ds(pl.multiple_of(i * BLK + a * SUB, SUB), SUB),
                                             k * width:(k + 1) * width], A_TERMS)
        ops = [_pack(op) for op in ops]
        for r, op in enumerate(ops):
            dst[r, packed_rows(base + i * SUB, SUB), :] = op
        return ops

    def project(i, which, tl=None, ops=None):
        lhs, base, rhs, dst = {"q": (pool, 2 * POOL_X, wqs, q_s), "k": (cs, 0, wks, k_s),
                               "v": (cs, 0, wvs, v_s)}[which]
        rows = packed_rows(base + i * SUB, SUB)

        def product(r):
            w = rhs[r] if tl is None or i not in cfg["bgblocks"] else tl.bg.tie(rhs[r])
            m = jnp.dot(_unpack(lhs[r, rows, :] if ops is None else ops[r]), _unpack(w), preferred_element_type=F32)
            if tl is not None:
                tl.issue(SUB * rhs.shape[1] // 256, [m[SUB // 2 - 8:SUB // 2], m[SUB - 8:SUB]])
            return m

        c = _block_product(product, cfg["o_p" + which])
        for a in range(2):
            if which == "q":
                q_s[pl.ds(pl.multiple_of(i * BLK + a * SUB, SUB), SUB), :] = (
                    jnp.concatenate(c[a], axis=1) * (B_DH ** -0.5 * LOG2E)).astype(BF16)
            else:
                for head in range(2):
                    dst[head, packed_rows(i * BLK + a * SUB, SUB), :] = _pack(c[a][head])

    def head_rows(ref, h, r0, r1):
        return _unpack(ref[h, r0 // 2:r1 // 2, :])

    def scores(h, i, tl):
        def nt(a, b):
            return lax.dot_general(a, b, (((1,), (1,)), ((), ())), preferred_element_type=F32)
        row = lax.broadcasted_iota(jnp.int32, (SUB, SUB), 0)
        col = lax.broadcasted_iota(jnp.int32, (SUB, SUB), 1)
        r0 = i * BLK
        full = nt(q_s[r0:r0 + BLK, h * B_DH:(h + 1) * B_DH], head_rows(k_s, h, 0, r0)) if i else None
        if i:
            tl.issue(BLK * i // 2, [full[t % BLK:t % BLK + 8, t // BLK * LANES:(t // BLK + 1) * LANES]
                                    for t in range(56, BLK * i // 2, 64)])
        diag = []
        for a in range(2):
            d = nt(q_s[r0 + a * SUB:r0 + (a + 1) * SUB, h * B_DH:(h + 1) * B_DH],
                   head_rows(k_s, h, r0, r0 + (a + 1) * SUB))
            tl.issue(32 * (a + 1), [d])
            last = jnp.where(col <= row, d[:, a * SUB:], NEG)
            diag.append(jnp.concatenate([d[:, :SUB], last], axis=1) if a else last)
        return full, diag, tl.now

    def softmax(i, sc, tl, h):
        full, diag, t0 = sc
        nf = i * BLK
        lo, hi = tl.pace[h]
        span = tl.now - t0
        step = tl.pch
        pf, pd, inv = [], [], []
        for a in range(2):
            s = diag[a]
            if full is not None:
                s = jnp.concatenate([full[a * SUB:(a + 1) * SUB], s], axis=1)
            m = jnp.max(s, axis=1, keepdims=True)
            if step:
                m = jnp.concatenate([
                    tl.after(t0 + span * (lo + (hi - lo) * (a * SUB + c) / BLK), m[c:c + step])
                    for c in range(0, SUB, step)], axis=0)
            p = jnp.exp2(s - m)
            if i >= cfg["sum16"]:
                p = p.astype(BF16)
            inv.append(_reciprocal(jnp.sum(p.astype(F32), axis=1, keepdims=True)))
            if full is not None:
                pf.append(p[:, :nf])
            pd.append(p[:, nf:])
        return (jnp.concatenate(pf, axis=0) if pf else None), pd, inv

    def context(h, i, sm, tl):
        def pv(a, b):
            return jnp.dot(a.astype(BF16), b, preferred_element_type=F32)
        pf, pd, inv = sm
        r0 = i * BLK
        of = None
        for k0 in range(0, r0, tl.pvk):
            k1 = min(k0 + tl.pvk, r0)
            words = v_s[h, k0 // 2:k1 // 2, :]
            if tl.bgpv and i in cfg["bgblocks_last"]:
                words = jnp.concatenate([tl.bg.tie(words[t:t + 64]) for t in range(0, words.shape[0], 64)], axis=0)
            part = pv(pf[:, k0:k1], _unpack(words))
            of = part if of is None else of + part
            tl.issue((k1 - k0) // 2, [of[t:t + 8] for t in range(56, BLK, 64)])
        out = []
        for a in range(2):
            o = pv(pd[a], head_rows(v_s, h, r0, r0 + (a + 1) * SUB))
            tl.issue(32 * (a + 1), [o])
            if of is not None:
                o = o + of[a * SUB:(a + 1) * SUB]
            out.append(o * inv[a])
        return out

    def stream_work(j, inner_part=True, outer_part=True):
        slot = j % 2

        def qkv(part):
            groups = [_heads_to_lanes([
                _pack(wqkv_raw[slot, k, :, part * DM + a * LANES:part * DM + (a + 1) * LANES])
                for a in range(8)]) for k in range(2)]
            rows = packed_rows(2 * POOL_QKV + part * HALF + j * (HALF // PAIRS), HALF // PAIRS)
            for a in range(4):
                for r, op in enumerate(_operand_sums(lambda k, n: _unpack(groups[k][4 * n + a]), B_TERMS)):
                    op = _pack(op)
                    pool[r, rows, a * LANES:(a + 1) * LANES] = op
                    yield op

        def two_level(block, dst, row0, cols):
            for r, inner in enumerate(_operand_sums2(block, B_TERMS)):
                for t, op in enumerate(inner()):
                    op = _pack(op)
                    dst[7 * r + t, packed_rows(row0, 32), cols] = op
                    yield op

        def out_a():
            c0 = j % 2 * LANES if isinstance(j, int) else pl.multiple_of(j % 2 * LANES, LANES)
            row0 = ((j >> 1 & 1) * 4 + (j >> 2)) * A_HEADS
            return two_level(lambda k, n: _word_half(woa_raw[slot, k % 2, :, pl.ds(n * 256 + c0, LANES)], k // 2),
                             woas, row0, pl.ds(c0, LANES))

        def out_b(r0, c0):
            return two_level(lambda k, n: wob_raw[slot, k, r0:r0 + 32, n * 256 + c0:n * 256 + c0 + LANES],
                             wobs, j * 64 + r0, slice(c0, c0 + LANES))

        for n in cfg["joborder" if inner_part else "joborder2"]:
            if n < 4 and outer_part:
                yield from out_b(n // 2 * 32, n % 2 * LANES)
            elif n == 4 and outer_part:
                yield from out_a()
            elif n > 4 and inner_part:
                yield from qkv(n - 5)

    only = cfg.get("only")
    named = {"wk": lambda: pair_copies(0, (0,)), "wv": lambda: pair_copies(0, (1,)), "wq": lambda: pair_copies(0, (2,)),
             "p1": lambda: pair_copies(1), "s0": lambda: stream_copies(0)}

    def request(names):
        for name in names:
            if name in named:
                _start(named[name]())
            else:
                (c_copy if name[0] == "c" else xb_copy)(int(name[1])).start()

    def first_steps(copy, work, plan):
        def body(n, carry):
            blocks = [2 * n, 2 * n + 1]
            copy(n).wait()
            for at, names in enumerate(plan):
                if names:
                    pl.when(n == at)(functools.partial(request, names))
            for i in blocks:
                work(i)
            return carry

        lax.fori_loop(0, len(plan), body, 0)

    def first_kv(i):
        ops = prepare_inputs(i, c_raw, cs, 0)
        project(i, "k", ops=ops)
        project(i, "v", ops=ops)

    def first_q(i):
        project(i, "q", ops=prepare_inputs(i, xb_raw, pool, 2 * POOL_X))

    with jax.named_scope("prologue"):
        if not only:
            request(cfg["plan0"])
            with jax.named_scope("w0"):
                _wait(pair_copies(0, (0,)))
            request(cfg["plan1"])
            prepare_pair_weights(0, "k")
            _wait(pair_copies(0, (1,)))
            prepare_pair_weights(0, "v")
            with jax.named_scope("kv"):
                first_steps(c_copy, first_kv, cfg["plan_kv"])
            _wait(pair_copies(0, (2,)))
            prepare_pair_weights(0, "q")
            with jax.named_scope("q"):
                first_steps(xb_copy, first_q, cfg["plan_q"])
    _wait(pair_copies(1) + stream_copies(0))
    _start(pair_copies(2) + stream_copies(1))

    def head_pair(j, project_next):
        if project_next:
            prepare_pair_weights(j + 1)
        else:
            xa_copy(0).start()
            xa_copy(1).start()
        tl = _Timeline(j < 0)
        tl.pace, tl.pch = (cfg["pace"], cfg["pch"]) if project_next else (cfg["pace_last"], cfg["pch_last"])
        tl.bg = _Background(j < 0)
        tl.bg.add(stream_work(j, True, project_next),
                  329 / (21 * len(cfg["bgblocks"])) if project_next else cfg["bgrate_last"])
        tl.bgpv = not project_next
        tl.pvk = cfg["pvk"] if project_next else cfg["pvk_last"]
        proj = (lambda i, which: project(i, which, tl)) if project_next else (lambda i, which: None)
        sc, o = {}, {}

        def finish_head(h, i):
            o[h, i] = context(h, i, softmax(i, sc.pop((h, i)), tl, h), tl)
            if (1 - h, i) in o:
                for a in range(2):
                    ctx[j, i * BLK + a * SUB:i * BLK + (a + 1) * SUB, :] = (
                        jnp.concatenate([o[0, i][a], o[1, i][a]], axis=1).astype(BF16))

        for i in range(NBLK - 1, -1, -1):
            order = cfg["order"] if project_next else cfg["order_last"]
            for tok in order[i] if isinstance(order, dict) else order:
                if tok[0] == "s":
                    sc[int(tok[1]), i] = scores(int(tok[1]), i, tl)
                elif tok[0] == "c":
                    finish_head(int(tok[1]), i)
                elif tok[0] == "C":
                    if (int(tok[1]), i + 1) in sc:
                        finish_head(int(tok[1]), i + 1)
                elif tok == "q":
                    proj(i, "q")
                elif i + 1 < NBLK:
                    proj(i + 1, tok)
        for h, i in sorted(sc):
            finish_head(h, i)
        proj(0, "k")
        proj(0, "v")
        tl.bg.finish()
        if project_next:
            _wait(stream_copies(j + 1))

            @pl.when(j + 2 < PAIRS)
            def _():
                _wait(pair_copies(j + 2))

            @pl.when(j + 3 < PAIRS)
            def _():
                _start(pair_copies(j + 3))

            @pl.when(j + 2 < PAIRS)
            def _():
                _start(stream_copies(j + 2))

    def pair_step(j, carry):
        with jax.named_scope("group"):
            head_pair(j, True)
        return carry

    with jax.named_scope("phase1"):
        if only in (None, "p1"):
            lax.fori_loop(0, PAIRS - 1, pair_step, 0)
    with jax.named_scope("lastgroup"):
        if only == "p1" or only == "last":
            def keep(n, carry):
                obuf.bitcast(U32)[0, 0:8, 0:LANES] = (pltpu.bitcast(ctx[n, 0:16, 0:LANES], U32) | pltpu.bitcast(q_s[pl.ds(pl.multiple_of(n * 16, 16), 16), 0:LANES], U32) | pool[n, 0:8, 0:LANES] | wobs[n, 0:8, 0:LANES] | woas[n, 0:8, 0:LANES]
                                                      | k_s[n % 2, 0:8, :] | v_s[n % 2, 0:8, :])
                return carry
        if only == "last":
            lax.fori_loop(PAIRS - 1, PAIRS, lambda j, c: (head_pair(j, False), c)[1], 0)
        if only == "p1" or only == "last":
            lax.fori_loop(0, 7, keep, 0)
        if only in ("p1", "p2", "last"):
            _wait(stream_copies(PAIRS - 1))
            xa_copy(0).start()
            xa_copy(1).start()
        else:
            lax.fori_loop(PAIRS - 1, PAIRS, lambda j, c: (head_pair(j, False), c)[1], 0)

    loc[0:16, BLK:BLK + HALO, :] = jnp.zeros((16, HALO, LANES), F32)

    def store_blocks(i, col0, c):
        for a, n in ((0, 0), (1, 0), (0, 1), (1, 1)):
            obuf[i % 2, a * SUB:(a + 1) * SUB, col0 + n * HALF:col0 + (n + 1) * HALF] = c[a][n].astype(BF16)
            if col0 == 0:
                out_copy(i, 2 * a + n).start()
        if col0:
            out_copy(i, 4).start()

    def row_block(i, carry):
        slot = i % 2
        xa_copy(i).wait()

        @pl.when(i >= 2)
        def _():
            _wait([out_copy(i - 2, part) for part in range(5)])

        loc[0:16, 0:HALO, :] = loc[0:16, BLK:BLK + HALO, :]
        zero = i // NBLK if cfg["opaque"] else 0
        xops = [op.astype(BF16) for op in _operand_sums(
            lambda a, k: xa_raw[slot, a * SUB:(a + 1) * SUB, k * HALF:(k + 1) * HALF], A_TERMS)]

        bg = _Background(i < 0)
        bg.add(stream_work(PAIRS - 1, False, True), cfg["bgrate2"])

        def lane_groups(part):
            r0 = POOL_QKV + part * HALF // 2
            c = _block_product(lambda r: jnp.dot(xops[r], _unpack(bg.tie(pool[r, r0:r0 + HALF // 2, :])),
                                                 preferred_element_type=F32), cfg["o_a"])
            return lambda a, g: c[a][g // 4][:, (g % 4) * LANES:(g % 4 + 1) * LANES]

        marks = []

        def out_b():
            quarter = PAIRS // 4

            def block(a, k):
                rows = pl.ds(pl.multiple_of(i * BLK + a * (BLK // 4), BLK // 4), BLK // 4)
                return jnp.concatenate(
                    [ctx[j, rows, :] for j in range(k * quarter, (k + 1) * quarter)], axis=1).astype(F32)

            lhs = _operand_sums2(block, A_TERMS)

            def outer(r):
                ops = lhs[r]()

                def product(t):
                    step = DM // cfg["ksplit"]
                    acc = None
                    for k0 in range(0, DM, step):
                        part = jnp.dot(ops[t][:, k0:k0 + step].astype(BF16),
                                       _unpack(wobs[7 * r + t, k0 // 2:(k0 + step) // 2, :]),
                                       preferred_element_type=F32)
                        acc = part if acc is None else acc + part
                        marks.append(acc)
                    return acc

                return _join(_block_product(product, cfg["o_bi"]))

            store_blocks(i, DM, _block_product(outer, cfg["o_bo"]))

        for part in cfg["aorder"]:
            if part == "b":
                bg.finish()
                out_b()
                continue
            f = lane_groups(part)
            for a in range(2):
                for g in range(8):
                    loc[(LOC_Q, LOC_K, LOC_V)[part] + g, HALO + a * SUB:HALO + (a + 1) * SUB, :] = f(a, g)

        ch = cfg["cha"]

        stages = cfg["stages"]
        total = stages * BLK // ch
        count = [0]

        def paced(values):
            lo, hi = cfg["gate"]
            mark = marks[int((lo + (hi - lo) * count[0] / (total - 1)) * (len(marks) - 1))]
            count[0] += 1
            return [jnp.where(i < 0, mark[0:ch, 0:LANES], t) for t in values]

        def attend(c0):
            def rows(base, g, w):
                b0 = HALO + c0 - A_DIL * w
                return loc[zero + base + g, b0:b0 + ch, :]

            q0 = [rows(LOC_Q, g, 0) for g in range(8)]
            logits = []
            half = max(stages // 2, 1)
            for w in range(A_WIN):
                if w % (A_WIN // half) == 0:
                    q = paced(q0)
                acc = q[0] * rows(LOC_K, 0, w)
                for g in range(1, 8):
                    acc = acc + q[g] * rows(LOC_K, g, w)
                acc = acc + pltpu.roll(acc, 2 * A_HEADS, 1)
                acc = acc + pltpu.roll(acc, A_HEADS, 1)
                if c0 < A_DIL * w:
                    pos = i * BLK + c0 + lax.broadcasted_iota(jnp.int32, (ch, LANES), 0)
                    acc = jnp.where(pos >= A_DIL * w, acc, NEG * A_DH ** 0.5)
                logits.append(acc)
            m = functools.reduce(jnp.maximum, logits)
            ps = [jnp.exp2((l - m) * (A_DH ** -0.5 * LOG2E)) for l in logits]
            inv = _reciprocal(functools.reduce(lambda a, b: a + b, ps))
            ps = [p * inv for p in ps]
            out = []
            for g in range(8):
                if stages > 1 and g % (8 // half) == 0:
                    pg = paced(ps)
                elif stages == 1:
                    pg = ps
                out.append(functools.reduce(lambda a, b: a + b, [pg[w] * rows(LOC_V, g, w) for w in range(A_WIN)]))
            return out

        quarters = [[] for _ in range(4)]
        for c0 in range(0, BLK // 4, ch):
            for a in range(4):
                quarters[a].append(jnp.concatenate(attend(a * (BLK // 4) + c0), axis=1))
        quarters = [jnp.concatenate(t, axis=0) for t in quarters]
        lhs = _operand_sums2(lambda a, k: quarters[a][:, k * 256:(k + 1) * 256], A_TERMS)

        def outer(r):
            ops = lhs[r]()
            return _join(_block_product(lambda t: jnp.dot(
                ops[t].astype(BF16), _unpack(woas[7 * r + t]), preferred_element_type=F32), cfg["o_ai"]))

        store_blocks(i, 0, _block_product(outer, cfg["o_ao"]))

        @pl.when(i + 2 < NBLK)
        def _():
            xa_copy(i + 2).start()

        return carry

    def row_step(i, carry):
        with jax.named_scope("rowblk"):
            return row_block(i, carry)

    with jax.named_scope("phase2"):
        if only in (None, "p2"):
            lax.fori_loop(0, NBLK, row_step, 0)
    with jax.named_scope("tail"):
        _wait([out_copy(i, part) for i in (NBLK - 2, NBLK - 1) for part in range(5)])


DEFAULT_CFG = dict(cha=16, opaque=False, nsplit=4, ksplit=4, gate=(0, 0.88), stages=4, pace=((0, 0.7), (0.2, 0.8)), pch=0, bgblocks=(6, 5, 4, 3, 2, 1), bgblocks_last=(7, 6, 5, 4, 3, 2, 1), bgrate_last=1, bgrate2=14, joborder=(0, 5, 1, 6, 2, 7, 3, 4),
                   **{"o_" + n: (0, 3, 4, 6, 1, 2, 5) for n in ("pq", "pk", "pv", "a", "bi", "bo", "ai", "ao")},
                   pch_last=0, pace_last=((0, 0.7), (0.2, 0.8)), jobslots_last=[(3, 1, 1), (2, 1, 1), (3, 0, 1), (2, 0, 1), (1, 0, 1), (1, 1, 1), (3, 0, 0), (2, 0, 0), (2, 1, 0)], sum16=0, plan0=("wk", "c0", "wv", "c1"), plan1=("c2", "c3"),
                   plan_kv=(("c4", "c5", "c6", "c7"), ("wq", "x0"), ("x1", "x2"), ("x3", "x4")),
                   plan_q=(("x5", "x6"), ("x7", "p1"), ("s0",), ()), sumgate=False, wch=32, wspan=0, pvk=1024, jobslots=[(5, 1, 1), (4, 0, 0), (3, 1, 0), (5, 0, 1), (5, 0, 0), (4, 1, 1), (3, 0, 0), (2, 1, 0)], order={0: ('s0', 'k', 's1', 'v', 'c0', 'q', 'c1'), 1: ('s0', 'k', 's1', 'v', 'c0', 'q', 'c1'), 2: ('s0', 'k', 's1', 'v', 'c0', 'q', 'c1'), 3: ('s0', 's1', 'k', 'q', 'c0', 'v', 'c1'), 4: ('s0', 's1', 'k', 'v', 'c0', 'q', 'c1'), 5: ('s0', 'k', 's1', 'q', 'c0', 'v', 'c1'), 6: ('s0', 's1', 'k', 'c0', 'v', 'c1', 'q'), 7: ('s0', 's1', 'k', 'c0', 'v', 'c1', 'q')}, order_last=('s0', 'C0', 's1', 'C1'),
                   pieces=(6, 5, 4, 3, 6, 5, 4, 3), aorder=(1, 0, 2, "b"), nobc=True)


DEFAULT_CFG.update({'order_last': ('s0', 'C0', 's1', 'C1'), 'bgblocks_last': (7, 5, 4, 3, 2, 0), 'bgrate_last': 1, 'pch_last': 0, 'pace_last': ((0, 0.7), (0.2, 0.9)), 'pvk_last': 1024, 'ksplit': 4, 'stages': 8, 'gate': (0, 0.92), 'cha': 16, 'bgrate2': 12, 'aorder': (0, 1, 2, 'b'), 'o_a': (0, 3, 4, 6, 1, 2, 5), 'o_bi': (3, 1, 2, 4, 0, 6, 5), 'o_bo': (3, 0, 1, 5, 2, 4, 6), 'o_ai': (2, 5, 0, 1, 3, 6, 4), 'o_ao': (0, 3, 4, 6, 1, 2, 5), 'joborder2': (3, 7, 1, 0, 2, 6, 5, 4), 'order': {0: ('s0', 'k', 's1', 'v', 'c0', 'q', 'c1'), 1: ('k', 's0', 'v', 's1', 'c0', 'q', 'c1'), 2: ('s0', 'k', 's1', 'v', 'c0', 'q', 'c1'), 3: ('s0', 's1', 'k', 'q', 'c0', 'v', 'c1'), 4: ('s0', 's1', 'k', 'q', 'c0', 'v', 'c1'), 5: ('s0', 's1', 'k', 'q', 'c0', 'v', 'c1'), 6: ('s0', 's1', 'k', 'v', 'c0', 'q', 'c1'), 7: ('s0', 's1', 'k', 'c0', 'q', 'c1', 'v')}, 'bgblocks': (6, 5, 4, 3, 2, 1), 'pvk': 512, 'joborder': (0, 5, 6, 1, 2, 7, 3, 4), 'o_pq': (3, 1, 0, 6, 4, 2, 5), 'o_pk': (0, 3, 4, 6, 1, 2, 5), 'o_pv': (5, 2, 0, 4, 6, 3, 1), 'pch': 16, 'pace': ((0, 0.6), (0.2, 0.8))})


DEFAULT_CFG.update(plan0=("wk", "wv", "c0"), plan1=("c1", "c2", "c3", "wq", "x0"),
                   plan_kv=((), ("x1", "x2"), ("x3",), ("p1",)), plan_q=(("s0",), (), (), ()))


def build(cfg=None):
    cfg = dict(DEFAULT_CFG, **(cfg or {}))
    vmem = pltpu.VMEM

    def fn(A_x, A_wqkv, A_wo, B_x, B_c_kv, B_w_q, B_w_uk, B_w_uv, B_w_o):
        out = pl.pallas_call(
            functools.partial(_kernel, cfg=cfg),
            out_shape=jax.ShapeDtypeStruct((S, 2 * DM), BF16),
            in_specs=[pl.BlockSpec(memory_space=pl.ANY)] * 9,
            out_specs=pl.BlockSpec(memory_space=pl.ANY),
            scratch_shapes=[
                vmem((S, DM), BF16),
                vmem((S, B_DC), BF16),
                vmem((7, POOL_ROWS, HALF), U32),
                vmem((7, S // 4, B_DC // 2), U32),
                vmem((2, DM, B_DH), U32),
                vmem((2, B_DC, B_DH), U32),
                vmem((2, B_DC, B_DH), U32),
                vmem((7, DM // 4, B_DH), U32),
                vmem((7, B_DC // 4, B_DH), U32),
                vmem((7, B_DC // 4, B_DH), U32),
                vmem((S, 2 * B_DH), BF16),
                vmem((2, S // 2, B_DH), U32),
                vmem((2, S // 2, B_DH), U32),
                vmem((PAIRS, S, 2 * B_DH), BF16),
                vmem((49, DM // 2, DM // 4), U32),
                vmem((49, DM // 8, DM // 4), U32),
                vmem((2, 2, HALF // PAIRS, 3 * DM), BF16),
                vmem((2, 2, A_HEADS, DM), U32),
                vmem((2, 4, 64, DM), BF16),
                vmem((2, BLK, DM), BF16),
                vmem((LOC_PANELS, HALO + BLK, LANES), F32),
                vmem((2, BLK, 2 * DM), BF16),
                pltpu.SemaphoreType.DMA((2, NBLK // 2)),
                pltpu.SemaphoreType.DMA((2, 3)),
                pltpu.SemaphoreType.DMA((2, 9)),
                pltpu.SemaphoreType.DMA((2,)),
                pltpu.SemaphoreType.DMA((2, 5)),
            ],
            compiler_params=pltpu.CompilerParams(vmem_limit_bytes=124 * 2 ** 20, flags=cfg.get("flags"),
                                                 disable_bounds_checks=cfg.get("nobc", False)),
            name="fused_local_and_latent_attention",
        )(A_x.reshape(S, DM), A_wqkv, A_wo.reshape(A_HEADS, A_DH, DM), B_x.reshape(S, DM), B_c_kv.reshape(S, B_DC),
          B_w_q, B_w_uk, B_w_uv, B_w_o.reshape(B_HEADS * B_DH, DM))
        return out.reshape(1, S, 2 * DM)

    return jax.jit(fn)


@jax.jit
def pallas_concat_heads__sliding_local_dilated__compressed_kv_cla__prompt_kernel(
    A_x: jax.Array,
    A_wqkv: jax.Array,
    A_wo: jax.Array,
    B_x: jax.Array,
    B_c_kv: jax.Array,
    B_w_q: jax.Array,
    B_w_uk: jax.Array,
    B_w_uv: jax.Array,
    B_w_o: jax.Array,
):
    return build(dict())(A_x, A_wqkv, A_wo, B_x, B_c_kv, B_w_q, B_w_uk, B_w_uv, B_w_o)
```

```python
import functools
import itertools

import jax
import jax.numpy as jnp
from jax import lax
import jax.experimental.pallas as pl
import jax.experimental.pallas.tpu as pltpu

S = 2048
DM = 1024
HALF = DM // 2
LANES = 128
A_HEADS, A_DH, A_WIN, A_DIL = 32, 32, 8, 2
HALO = 16
B_HEADS, B_DH, B_DC = 32, 128, 512
PAIRS = B_HEADS // 2

BLK = 256
SUB = BLK // 2
NBLK = S // BLK

LOG2E = 1.4426950408889634
NEG = -1e9
F32, BF16, U32 = jnp.float32, jnp.bfloat16, jnp.uint32

A_TERMS = (((1, 0, 0), (1, 1, 1)), ((1, 1, 0), (1, 1, 1)), ((1, 0, 0),), ((1, 1, 1),),
           ((1, 0, 0), (1, 0, 1)), ((1, 1, 0), (-1, 0, 0)), ((1, 0, 1), (-1, 1, 1)))
B_TERMS = (((1, 0, 0), (1, 1, 1)), ((1, 0, 0),), ((1, 0, 1), (-1, 1, 1)), ((1, 1, 0), (-1, 0, 0)),
           ((1, 1, 1),), ((1, 0, 0), (1, 0, 1)), ((1, 1, 0), (1, 1, 1)))
C_TERMS = (((1, 0, 0), (1, 1, 1)), ((1, 1, 0), (-1, 1, 1)), ((1, 0, 1), (1, 1, 1)), ((1, 0, 0), (1, 1, 0)),
           ((-1, 0, 0), (1, 0, 1)), ((1, 1, 1),), ((1, 0, 0),))

POOL_X = 0
POOL_QKV = POOL_X + S // 4
POOL_ROWS = POOL_QKV + 2 * HALF // 2
LOC_K, LOC_V, LOC_Q, LOC_PANELS = 0, 8, 16, 24


def _pack(x):
    return pltpu.bitcast(x.astype(BF16), U32)


def _unpack(x):
    return pltpu.bitcast(x, BF16)


def _operand_sums(block, terms):
    blocks = [[block(i, j) for j in range(2)] for i in range(2)]
    out = []
    for (_, i, j), *rest in terms:
        acc = blocks[i][j]
        for sign, i, j in rest:
            a, b = acc.astype(F32), blocks[i][j].astype(F32)
            acc = a + b if sign > 0 else a - b
        out.append(acc)
    return out


def _block_product(product, order=(0, 3, 4, 6, 1, 2, 5), c=None):
    c = c or [[None, None], [None, None]]
    for r in order:
        m = product(r)
        for sign, i, j in C_TERMS[r]:
            if c[i][j] is None:
                c[i][j] = m if sign > 0 else -m
            else:
                c[i][j] = c[i][j] + m if sign > 0 else c[i][j] - m
    return c


def _operand_sums2(block, terms):
    outer = [[_operand_sums(lambda i, j: block(2 * i + a, 2 * j + b), terms) for b in range(2)] for a in range(2)]
    return [functools.partial(_operand_sums, lambda a, b, r=r: outer[a][b][r], terms) for r in range(7)]


def _join(c):
    return jnp.concatenate([jnp.concatenate(row, axis=1) for row in c], axis=0)


def _heads_to_lanes(groups):
    lane = lax.broadcasted_iota(jnp.int32, groups[0].shape, 1)
    groups = list(groups)
    for group_bit, lane_bit in ((2, 4), (1, 3), (0, 2), (2, 6), (2, 1), (1, 5), (1, 0)):
        shift = 1 << lane_bit
        low = (lane & shift) == 0
        for g in range(8):
            if g >> group_bit & 1:
                continue
            x, y = groups[g], groups[g | 1 << group_bit]
            groups[g] = jnp.where(low, x, pltpu.roll(y, shift, 1))
            groups[g | 1 << group_bit] = jnp.where(low, pltpu.roll(x, LANES - shift, 1), y)
    return [groups[(g & 1) << 2 | (g >> 2) << 1 | (g >> 1 & 1)] for g in range(8)]


def _word_half(word, hi):
    return pltpu.bitcast(word & U32(0xFFFF0000) if hi else word << 16, F32)


def _reciprocal(x):
    r = pl.reciprocal(x, approx=True)
    return r * (2.0 - x * r)


class _Timeline:
    def __init__(self, never):
        self.never, self.now, self.marks = never, 0.0, []

    def issue(self, cycles, results):
        for n, value in enumerate(results):
            self.marks.append((self.now + cycles * (n + 1) / len(results), value))
        self.now += cycles

    def after(self, cycle, value):
        ready = [v for t, v in self.marks if t <= cycle]
        if not ready:
            return value
        mark = ready[-1][0:8, 0:value.shape[1]]
        if value.shape[0] > 8:
            mark = jnp.concatenate([mark] * (value.shape[0] // 8), axis=0)
        return jnp.where(self.never, mark, value)


class _Background:
    def __init__(self, never):
        self.never, self.pending, self.credit, self.rate = never, iter(()), 0.0, 0.0

    def add(self, pieces, rate):
        self.pending, self.rate = itertools.chain(self.pending, pieces), rate

    def tie(self, words):
        self.credit += self.rate
        due = list(itertools.islice(self.pending, int(self.credit)))
        self.credit -= int(self.credit)
        if not due:
            return words
        due = [pltpu.bitcast(d, U32) for d in due]
        mark = functools.reduce(jnp.bitwise_or, [
            d[r:r + 8, c:c + LANES] for d in due for r in range(0, d.shape[0], 8) for c in range(0, d.shape[1], LANES)])
        top = jnp.where(self.never, mark, words[:8, :LANES])
        if words.shape[1] > LANES:
            top = jnp.concatenate([top, words[:8, LANES:]], axis=1)
        return jnp.concatenate([top, words[8:]], axis=0)

    def finish(self):
        for _ in self.pending:
            pass


def _start(copies):
    for cp in copies:
        cp.start()


def _wait(copies):
    for cp in copies:
        cp.wait()


def _kernel(xa_hbm, wqkv_hbm, woa_hbm, xb_hbm, c_hbm, wq_hbm, wuk_hbm, wuv_hbm, wob_hbm,
            out_hbm,
            xb_raw, c_raw, pool, cs, wq_raw, wuk_raw, wuv_raw, wqs, wks, cts,
            q_s, k_s, v_s, ctx, wobs, woas,
            wqkv_raw, wva_raw, wvas, woa_raw, wob_raw, xa_raw, loc, obuf,
            sem_x, sem_w, sem_s, sem_a, sem_o, *, cfg):
    wq_u = wq_hbm.bitcast(U32)
    wuk_u = wuk_hbm.bitcast(U32)
    wuv_u = wuv_hbm.bitcast(U32)
    woa_u = woa_hbm.bitcast(U32)

    def pair_copies(j, which=(0, 1, 2)):
        ends = ((wuk_u, wuk_raw), (wuv_u, wuv_raw), (wq_u, wq_raw))
        return [pltpu.make_async_copy(ends[n][0].at[:, j, :], ends[n][1].at[j % 2], sem_w.at[j % 2, n])
                for n in which]

    def stream_copies(j):
        slot = j % 2
        rows = HALF // PAIRS
        cps = []
        for k in range(2):
            cps.append(pltpu.make_async_copy(
                wqkv_hbm.at[row_range(k * HALF + j * rows, rows), 0:2 * DM], wqkv_raw.at[slot, k], sem_s.at[slot, k]))
        for k in range(4):
            cps.append(pltpu.make_async_copy(
                wqkv_hbm.at[row_range(k * 256 + j * 16, 16), 2 * DM:3 * DM], wva_raw.at[slot, k],
                sem_s.at[slot, 9 + k]))
        for k in range(2):
            word = (j >> 1 & 1) | k << 1 | (j >> 2) << 2
            cps.append(pltpu.make_async_copy(woa_u.at[:, word, :], woa_raw.at[slot, k], sem_s.at[slot, 7 + k]))
        for k in range(4):
            cps.append(pltpu.make_async_copy(
                wob_hbm.at[row_range(k * DM + j * 64, 64), :], wob_raw.at[slot, k], sem_s.at[slot, 3 + k]))
        return cps

    def c_copy(n):
        rows = pl.ds(pl.multiple_of(n * 2 * BLK, 2 * BLK), 2 * BLK)
        return pltpu.make_async_copy(c_hbm.at[rows, :], c_raw.at[rows, :], sem_x.at[0, n])

    def xb_copy(n):
        rows = pl.ds(pl.multiple_of(n * 2 * BLK, 2 * BLK), 2 * BLK)
        return pltpu.make_async_copy(xb_hbm.at[rows, :], xb_raw.at[rows, :], sem_x.at[1, n])

    def xa_copy(i):
        rows = pl.ds(pl.multiple_of(i * BLK, BLK), BLK)
        return pltpu.make_async_copy(xa_hbm.at[rows, :], xa_raw.at[i % 2], sem_a.at[i % 2])

    def out_copy(i, part):
        r0, nr, c0, nc = (0, BLK, DM, DM) if part == 4 else (part // 2 * SUB, SUB, part % 2 * HALF, HALF)
        rows = pl.ds(pl.multiple_of(i * BLK + r0, SUB), nr)
        return pltpu.make_async_copy(obuf.at[i % 2, r0:r0 + nr, c0:c0 + nc], out_hbm.at[rows, c0:c0 + nc],
                                     sem_o.at[i % 2, part])

    def row_range(start, size):
        return pl.ds(start if isinstance(start, int) else pl.multiple_of(start, size), size)

    def packed_rows(start, size):
        if isinstance(start, int):
            return pl.ds(start // 2, size // 2)
        return pl.ds(pl.multiple_of(start // 2, size // 2), size // 2)

    def prepare_pair_weights(j, which="qk"):
        slot = j % 2
        for name in which:
            raw, dst = {"q": (wq_raw, wqs), "k": (wuk_raw, wks)}[name]
            depth = raw.shape[1] // 2
            for r0 in range(0, depth, 32):
                words = [raw[slot, k * depth + r0:k * depth + r0 + 32, :] for k in range(2)]
                for r, op in enumerate(_operand_sums(lambda k, head: _word_half(words[k], head), B_TERMS)):
                    dst[r, r0 // 2:r0 // 2 + 16, :] = _pack(op)

    def value_weights(j):
        words = wuv_raw[j % 2].T

        def block(a, k):
            return _word_half(words[a % 2 * 64:(a % 2 + 1) * 64, k * LANES:(k + 1) * LANES], a // 2)

        return [[op.astype(BF16) for op in inner()] for inner in _operand_sums2(block, A_TERMS)]

    def prepare_latents(t):
        blocks = [[c_raw[row_range((4 * t + n) * LANES, LANES), k * LANES:(k + 1) * LANES].astype(F32).T
                   for n in range(4)] for k in range(4)]
        ops = [[_pack(op) for op in inner()] for inner in _operand_sums2(lambda k, n: blocks[k][n], B_TERMS)]
        for r in range(7):
            for u in range(7):
                cts[t, 7 * r + u] = ops[r][u]
        return ops

    def project_values(t, weights, tl=None, ops=None):
        def outer(r):
            def product(u):
                rhs = cts[t, 7 * r + u] if ops is None else ops[r][u]
                m = jnp.dot(weights[r][u], _unpack(rhs), preferred_element_type=F32)
                if tl is not None:
                    tl.issue(16, [m[-8:]])
                return m
            return _join(_block_product(product, cfg["o_wi"]))

        c = _block_product(outer, cfg["o_wo"][:cfg["vsplit"]])
        yield
        c = _block_product(outer, cfg["o_wo"][cfg["vsplit"]:], c)
        for head in range(2):
            for n in range(2):
                v_s[head, :, row_range((2 * t + n) * BLK, BLK)] = _pack(c[head][n])

    def prepare_inputs(i, raw, dst, base):
        width = raw.shape[1] // 2
        ops = _operand_sums(lambda a, k: raw[pl.ds(pl.multiple_of(i * BLK + a * SUB, SUB), SUB),
                                             k * width:(k + 1) * width], A_TERMS)
        ops = [_pack(op) for op in ops]
        for r, op in enumerate(ops):
            dst[r, packed_rows(base + i * SUB, SUB), :] = op
        return ops

    def project(i, which, tl=None, ops=None):
        lhs, base, rhs, dst = {"q": (pool, 2 * POOL_X, wqs, q_s), "k": (cs, 0, wks, k_s)}[which]
        rows = packed_rows(base + i * SUB, SUB)

        def product(r):
            w = rhs[r] if tl is None or i not in cfg["bgblocks"] else tl.bg.tie(rhs[r])
            m = jnp.dot(_unpack(lhs[r, rows, :] if ops is None else ops[r]), _unpack(w), preferred_element_type=F32)
            if tl is not None:
                tl.issue(SUB * rhs.shape[1] // 256, [m[SUB // 2 - 8:SUB // 2], m[SUB - 8:SUB]])
            return m

        c = _block_product(product, cfg["o_p" + which])
        for a in range(2):
            if which == "q":
                q_s[pl.ds(pl.multiple_of(i * BLK + a * SUB, SUB), SUB), :] = (
                    jnp.concatenate(c[a], axis=1) * (B_DH ** -0.5 * LOG2E)).astype(BF16)
            else:
                for head in range(2):
                    dst[head, packed_rows(i * BLK + a * SUB, SUB), :] = _pack(c[a][head])

    def head_rows(ref, h, r0, r1):
        return _unpack(ref[h, r0 // 2:r1 // 2, :])

    def scores(h, i, tl):
        def nt(a, b):
            return lax.dot_general(a, b, (((1,), (1,)), ((), ())), preferred_element_type=F32)
        row = lax.broadcasted_iota(jnp.int32, (SUB, SUB), 0)
        col = lax.broadcasted_iota(jnp.int32, (SUB, SUB), 1)
        r0 = i * BLK
        full = nt(q_s[r0:r0 + BLK, h * B_DH:(h + 1) * B_DH], head_rows(k_s, h, 0, r0)) if i else None
        if i:
            tl.issue(BLK * i // 2, [full[t % BLK:t % BLK + 8, t // BLK * LANES:(t // BLK + 1) * LANES]
                                    for t in range(56, BLK * i // 2, 64)])
        diag = []
        for a in range(2):
            d = nt(q_s[r0 + a * SUB:r0 + (a + 1) * SUB, h * B_DH:(h + 1) * B_DH],
                   head_rows(k_s, h, r0, r0 + (a + 1) * SUB))
            tl.issue(32 * (a + 1), [d])
            last = jnp.where(col <= row, d[:, a * SUB:], NEG)
            diag.append(jnp.concatenate([d[:, :SUB], last], axis=1) if a else last)
        return full, diag, tl.now

    def softmax(i, sc, tl, h):
        full, diag, t0 = sc
        nf = i * BLK
        lo, hi = tl.pace[h]
        span = tl.now - t0
        step = tl.pch
        pf, pd, inv = [], [], []
        for a in range(2):
            s = diag[a]
            if full is not None:
                s = jnp.concatenate([full[a * SUB:(a + 1) * SUB], s], axis=1)
            m = jnp.max(s, axis=1, keepdims=True)
            if step:
                m = jnp.concatenate([
                    tl.after(t0 + span * (lo + (hi - lo) * (a * SUB + c) / BLK), m[c:c + step])
                    for c in range(0, SUB, step)], axis=0)
            p = jnp.exp2(s - m)
            if i >= cfg["sum16"]:
                p = p.astype(BF16)
            inv.append(_reciprocal(jnp.sum(p.astype(F32), axis=1, keepdims=True)))
            if full is not None:
                pf.append(p[:, :nf])
            pd.append(p[:, nf:])
        return (jnp.concatenate(pf, axis=0) if pf else None), pd, inv

    def context(h, i, sm, tl):
        def pv(a, b):
            return lax.dot_general(a.astype(BF16), b, (((1,), (1,)), ((), ())), preferred_element_type=F32)
        pf, pd, inv = sm
        r0 = i * BLK
        of = None
        for k0 in range(0, r0, tl.pvk):
            k1 = min(k0 + tl.pvk, r0)
            words = v_s[h, :, k0:k1]
            if tl.bgpv and i in cfg["bgblocks_last"]:
                words = jnp.concatenate(
                    [tl.bg.tie(words[:, t:t + LANES]) for t in range(0, words.shape[1], LANES)], axis=1)
            part = pv(pf[:, k0:k1], _unpack(words))
            of = part if of is None else of + part
            tl.issue((k1 - k0) // 2, [of[t:t + 8] for t in range(56, BLK, 64)])
        out = []
        for a in range(2):
            o = pv(pd[a], _unpack(v_s[h, :, r0:r0 + (a + 1) * SUB]))
            tl.issue(32 * (a + 1), [o])
            if of is not None:
                o = o + of[a * SUB:(a + 1) * SUB]
            out.append(o * inv[a])
        return out

    def stream_work(j, inner_part=True, outer_part=True):
        slot = j % 2

        def qkv(part):
            groups = [_heads_to_lanes([
                _pack(wqkv_raw[slot, k, :, part * DM + a * LANES:part * DM + (a + 1) * LANES])
                for a in range(8)]) for k in range(2)]
            rows = packed_rows(2 * POOL_QKV + part * HALF + j * (HALF // PAIRS), HALF // PAIRS)
            for a in range(4):
                for r, op in enumerate(_operand_sums(lambda k, n: _unpack(groups[k][4 * n + a]), B_TERMS)):
                    op = _pack(op)
                    pool[r, rows, a * LANES:(a + 1) * LANES] = op
                    yield op

        def two_level(block, dst, row0, cols):
            for r, inner in enumerate(_operand_sums2(block, B_TERMS)):
                for t, op in enumerate(inner()):
                    op = _pack(op)
                    dst[7 * r + t, packed_rows(row0, 2 * op.shape[0]), cols] = op
                    yield op

        def value():
            groups = [_heads_to_lanes([_pack(wva_raw[slot, k, :, a * LANES:(a + 1) * LANES]) for a in range(8)])
                      for k in range(4)]
            return two_level(lambda k, n: _unpack(jnp.concatenate(groups[k][2 * n:2 * n + 2], axis=1)),
                             wvas, j * 16, slice(None))

        def out_a():
            c0 = j % 2 * LANES if isinstance(j, int) else pl.multiple_of(j % 2 * LANES, LANES)
            row0 = ((j >> 1 & 1) * 4 + (j >> 2)) * A_HEADS
            return two_level(lambda k, n: _word_half(woa_raw[slot, k % 2, :, pl.ds(n * 256 + c0, LANES)], k // 2),
                             woas, row0, pl.ds(c0, LANES))

        def out_b(r0, c0):
            return two_level(lambda k, n: wob_raw[slot, k, r0:r0 + 32, n * 256 + c0:n * 256 + c0 + LANES],
                             wobs, j * 64 + r0, slice(c0, c0 + LANES))

        for n in cfg["joborder" if inner_part else "joborder2"]:
            if n < 4 and outer_part:
                yield from out_b(n // 2 * 32, n % 2 * LANES)
            elif n == 4 and outer_part:
                yield from out_a()
            elif n > 4 and inner_part:
                yield from value() if n == 7 else qkv(n - 5)

    only = cfg.get("only")
    named = {"wk": lambda: pair_copies(0, (0,)), "wv": lambda: pair_copies(0, (1,)), "wq": lambda: pair_copies(0, (2,)),
             "p1": lambda: pair_copies(1), "s0": lambda: stream_copies(0)}

    def request(names):
        for name in names:
            if name in named:
                _start(named[name]())
            else:
                (c_copy if name[0] == "c" else xb_copy)(int(name[1])).start()

    def first_steps(copy, work, plan):
        def body(n, carry):
            blocks = [2 * n, 2 * n + 1]
            copy(n).wait()
            for at, names in enumerate(plan):
                if names:
                    pl.when(n == at)(functools.partial(request, names))
            work(n, blocks)
            return carry

        lax.fori_loop(0, len(plan), body, 0)

    def first_kv(weights, n, blocks):
        for i in blocks:
            project(i, "k", ops=prepare_inputs(i, c_raw, cs, 0))
        for _ in project_values(n, weights, ops=prepare_latents(n)):
            pass

    def first_q(n, blocks):
        for i in blocks:
            project(i, "q", ops=prepare_inputs(i, xb_raw, pool, 2 * POOL_X))

    with jax.named_scope("prologue"):
        if not only:
            request(cfg["plan0"])
            with jax.named_scope("w0"):
                _wait(pair_copies(0, (0,)))
            request(cfg["plan1"])
            prepare_pair_weights(0, "k")
            _wait(pair_copies(0, (1,)))
            with jax.named_scope("kv"):
                first_steps(c_copy, functools.partial(first_kv, value_weights(0)), cfg["plan_kv"])
            _wait(pair_copies(0, (2,)))
            prepare_pair_weights(0, "q")
            with jax.named_scope("q"):
                first_steps(xb_copy, first_q, cfg["plan_q"])
    _wait(pair_copies(1) + stream_copies(0))
    _start(pair_copies(2) + stream_copies(1))

    def head_pair(j, project_next):
        if project_next:
            prepare_pair_weights(j + 1)
            weights = value_weights(j + 1)
        else:
            xa_copy(0).start()
            xa_copy(1).start()
        tl = _Timeline(j < 0)
        tl.pace, tl.pch = (cfg["pace"], cfg["pch"]) if project_next else (cfg["pace_last"], cfg["pch_last"])
        tl.bg = _Background(j < 0)
        tl.bg.add(stream_work(j, True, project_next),
                  350 / (14 * len(cfg["bgblocks"])) if project_next else cfg["bgrate_last"])
        tl.bgpv = not project_next
        tl.pvk = cfg["pvk"] if project_next else cfg["pvk_last"]
        proj = (lambda i, which: project(i, which, tl)) if project_next else (lambda i, which: None)
        sc, o = {}, {}
        if project_next:
            values = [project_values(t, weights, tl) for t in range(NBLK // 2)]

        def finish_head(h, i):
            o[h, i] = context(h, i, softmax(i, sc.pop((h, i)), tl, h), tl)
            if (1 - h, i) in o:
                for a in range(2):
                    ctx[j, i * BLK + a * SUB:i * BLK + (a + 1) * SUB, :] = (
                        jnp.concatenate([o[0, i][a], o[1, i][a]], axis=1).astype(BF16))

        for i in range(NBLK - 1, -1, -1):
            order = cfg["order"] if project_next else cfg["order_last"]
            for tok in order[i] if isinstance(order, dict) else order:
                if tok[0] == "s":
                    sc[int(tok[1]), i] = scores(int(tok[1]), i, tl)
                elif tok[0] == "c":
                    finish_head(int(tok[1]), i)
                elif tok[0] == "C":
                    if (int(tok[1]), i + 1) in sc:
                        finish_head(int(tok[1]), i + 1)
                elif tok == "q":
                    proj(i, "q")
                elif tok == "v":
                    if i + 2 < NBLK:
                        next(values[i // 2 + 1], None)
                elif i + 1 < NBLK:
                    proj(i + 1, tok)
        for h, i in sorted(sc):
            finish_head(h, i)
        proj(0, "k")
        if project_next:
            for _ in values[0]:
                pass
        tl.bg.finish()
        if project_next:
            _wait(stream_copies(j + 1))

            @pl.when(j + 2 < PAIRS)
            def _():
                _wait(pair_copies(j + 2))

            @pl.when(j + 3 < PAIRS)
            def _():
                _start(pair_copies(j + 3))

            @pl.when(j + 2 < PAIRS)
            def _():
                _start(stream_copies(j + 2))

    def pair_step(j, carry):
        with jax.named_scope("group"):
            head_pair(j, True)
        return carry

    with jax.named_scope("phase1"):
        if only in (None, "p1"):
            lax.fori_loop(0, PAIRS - 1, pair_step, 0)
    with jax.named_scope("lastgroup"):
        if only == "p1" or only == "last":
            def keep(n, carry):
                obuf.bitcast(U32)[0, 0:8, 0:LANES] = (pltpu.bitcast(ctx[n, 0:16, 0:LANES], U32) | pltpu.bitcast(q_s[pl.ds(pl.multiple_of(n * 16, 16), 16), 0:LANES], U32) | pool[n, 0:8, 0:LANES] | wobs[n, 0:8, 0:LANES] | woas[n, 0:8, 0:LANES] | wvas[n, 0:8, 0:LANES]
                                                      | k_s[n % 2, 0:8, :] | v_s[n % 2, 0:8, 0:LANES])
                return carry
        if only == "last":
            lax.fori_loop(PAIRS - 1, PAIRS, lambda j, c: (head_pair(j, False), c)[1], 0)
        if only == "p1" or only == "last":
            lax.fori_loop(0, 7, keep, 0)
        if only in ("p1", "p2", "last"):
            _wait(stream_copies(PAIRS - 1))
            xa_copy(0).start()
            xa_copy(1).start()
        else:
            lax.fori_loop(PAIRS - 1, PAIRS, lambda j, c: (head_pair(j, False), c)[1], 0)

    loc[0:16, BLK:BLK + HALO, :] = jnp.zeros((16, HALO, LANES), F32)

    def store_blocks(i, col0, c):
        for a, n in ((0, 0), (1, 0), (0, 1), (1, 1)):
            obuf[i % 2, a * SUB:(a + 1) * SUB, col0 + n * HALF:col0 + (n + 1) * HALF] = c[a][n].astype(BF16)
            if col0 == 0:
                out_copy(i, 2 * a + n).start()
        if col0:
            out_copy(i, 4).start()

    def row_block(i, carry):
        slot = i % 2
        xa_copy(i).wait()

        @pl.when(i >= 2)
        def _():
            _wait([out_copy(i - 2, part) for part in range(5)])

        loc[0:16, 0:HALO, :] = loc[0:16, BLK:BLK + HALO, :]
        zero = i // NBLK if cfg["opaque"] else 0
        xsums = _operand_sums(
            lambda a, k: xa_raw[slot, a * SUB:(a + 1) * SUB, k * HALF:(k + 1) * HALF], A_TERMS)
        xops = [op.astype(BF16) for op in xsums]

        bg = _Background(i < 0)
        bg.add(stream_work(PAIRS - 1, False, True), cfg["bgrate2"])

        def lane_groups(part):
            if part == 2:
                def outer(r):
                    ops = _operand_sums(lambda a, k: xsums[r][64 * a:64 * (a + 1), 256 * k:256 * (k + 1)], A_TERMS)
                    return _join(_block_product(lambda t: jnp.dot(
                        ops[t].astype(BF16), _unpack(wvas[7 * r + t]), preferred_element_type=F32), cfg["o_vi"]))

                c = _block_product(outer, cfg["o_vo"])
                return lambda a, g: c[a][g // 4][:, (g % 4) * LANES:(g % 4 + 1) * LANES]
            r0 = POOL_QKV + part * HALF // 2
            c = _block_product(lambda r: jnp.dot(xops[r], _unpack(bg.tie(pool[r, r0:r0 + HALF // 2, :])),
                                                 preferred_element_type=F32), cfg["o_a"])
            return lambda a, g: c[a][g // 4][:, (g % 4) * LANES:(g % 4 + 1) * LANES]

        marks = []

        def out_b():
            quarter = PAIRS // 4

            def block(a, k):
                rows = pl.ds(pl.multiple_of(i * BLK + a * (BLK // 4), BLK // 4), BLK // 4)
                return jnp.concatenate(
                    [ctx[j, rows, :] for j in range(k * quarter, (k + 1) * quarter)], axis=1).astype(F32)

            lhs = _operand_sums2(block, A_TERMS)

            def outer(r):
                ops = lhs[r]()

                def product(t):
                    step = DM // cfg["ksplit"]
                    acc = None
                    for k0 in range(0, DM, step):
                        part = jnp.dot(ops[t][:, k0:k0 + step].astype(BF16),
                                       _unpack(wobs[7 * r + t, k0 // 2:(k0 + step) // 2, :]),
                                       preferred_element_type=F32)
                        acc = part if acc is None else acc + part
                        marks.append(acc)
                    return acc

                return _join(_block_product(product, cfg["o_bi"]))

            store_blocks(i, DM, _block_product(outer, cfg["o_bo"]))

        for part in cfg["aorder"]:
            if part == "b":
                bg.finish()
                out_b()
                continue
            f = lane_groups(part)
            for a in range(2):
                for g in range(8):
                    loc[(LOC_Q, LOC_K, LOC_V)[part] + g, HALO + a * SUB:HALO + (a + 1) * SUB, :] = f(a, g)

        ch = cfg["cha"]

        stages = cfg["stages"]
        total = stages * BLK // ch
        count = [0]

        def paced(values):
            lo, hi = cfg["gate"]
            mark = marks[int((lo + (hi - lo) * count[0] / (total - 1)) * (len(marks) - 1))]
            count[0] += 1
            return [jnp.where(i < 0, mark[0:ch, 0:LANES], t) for t in values]

        def attend(c0):
            def rows(base, g, w):
                b0 = HALO + c0 - A_DIL * w
                return loc[zero + base + g, b0:b0 + ch, :]

            q0 = [rows(LOC_Q, g, 0) for g in range(8)]
            logits = []
            half = max(stages // 2, 1)
            for w in range(A_WIN):
                if w % (A_WIN // half) == 0:
                    q = paced(q0)
                acc = q[0] * rows(LOC_K, 0, w)
                for g in range(1, 8):
                    acc = acc + q[g] * rows(LOC_K, g, w)
                acc = acc + pltpu.roll(acc, 2 * A_HEADS, 1)
                acc = acc + pltpu.roll(acc, A_HEADS, 1)
                if c0 < A_DIL * w:
                    pos = i * BLK + c0 + lax.broadcasted_iota(jnp.int32, (ch, LANES), 0)
                    acc = jnp.where(pos >= A_DIL * w, acc, NEG * A_DH ** 0.5)
                logits.append(acc)
            m = functools.reduce(jnp.maximum, logits)
            ps = [jnp.exp2((l - m) * (A_DH ** -0.5 * LOG2E)) for l in logits]
            inv = _reciprocal(functools.reduce(lambda a, b: a + b, ps))
            ps = [p * inv for p in ps]
            out = []
            for g in range(8):
                if stages > 1 and g % (8 // half) == 0:
                    pg = paced(ps)
                elif stages == 1:
                    pg = ps
                out.append(functools.reduce(lambda a, b: a + b, [pg[w] * rows(LOC_V, g, w) for w in range(A_WIN)]))
            return out

        quarters = [[] for _ in range(4)]
        for c0 in range(0, BLK // 4, ch):
            for a in range(4):
                quarters[a].append(jnp.concatenate(attend(a * (BLK // 4) + c0), axis=1))
        quarters = [jnp.concatenate(t, axis=0) for t in quarters]
        lhs = _operand_sums2(lambda a, k: quarters[a][:, k * 256:(k + 1) * 256], A_TERMS)

        def outer(r):
            ops = lhs[r]()
            return _join(_block_product(lambda t: jnp.dot(
                ops[t].astype(BF16), _unpack(woas[7 * r + t]), preferred_element_type=F32), cfg["o_ai"]))

        store_blocks(i, 0, _block_product(outer, cfg["o_ao"]))

        @pl.when(i + 2 < NBLK)
        def _():
            xa_copy(i + 2).start()

        return carry

    def row_step(i, carry):
        with jax.named_scope("rowblk"):
            return row_block(i, carry)

    with jax.named_scope("phase2"):
        if only in (None, "p2"):
            lax.fori_loop(0, NBLK, row_step, 0)
    with jax.named_scope("tail"):
        _wait([out_copy(i, part) for i in (NBLK - 2, NBLK - 1) for part in range(5)])


DEFAULT_CFG = dict(cha=16, opaque=False, nsplit=4, ksplit=4, gate=(0, 0.88), stages=4, pace=((0, 0.7), (0.2, 0.8)), pch=0, bgblocks=(6, 5, 4, 3, 2, 1), bgblocks_last=(7, 6, 5, 4, 3, 2, 1), bgrate_last=1, bgrate2=14, joborder=(0, 5, 1, 6, 2, 7, 3, 4),
                   **{"o_" + n: (0, 3, 4, 6, 1, 2, 5) for n in ("pq", "pk", "pv", "a", "bi", "bo", "ai", "ao")},
                   pch_last=0, pace_last=((0, 0.7), (0.2, 0.8)), jobslots_last=[(3, 1, 1), (2, 1, 1), (3, 0, 1), (2, 0, 1), (1, 0, 1), (1, 1, 1), (3, 0, 0), (2, 0, 0), (2, 1, 0)], sum16=0, plan0=("wk", "c0", "wv", "c1"), plan1=("c2", "c3"),
                   plan_kv=(("c4", "c5", "c6", "c7"), ("wq", "x0"), ("x1", "x2"), ("x3", "x4")),
                   plan_q=(("x5", "x6"), ("x7", "p1"), ("s0",), ()), sumgate=False, wch=32, wspan=0, pvk=1024, jobslots=[(5, 1, 1), (4, 0, 0), (3, 1, 0), (5, 0, 1), (5, 0, 0), (4, 1, 1), (3, 0, 0), (2, 1, 0)], order={0: ('s0', 'k', 's1', 'v', 'c0', 'q', 'c1'), 1: ('s0', 'k', 's1', 'v', 'c0', 'q', 'c1'), 2: ('s0', 'k', 's1', 'v', 'c0', 'q', 'c1'), 3: ('s0', 's1', 'k', 'q', 'c0', 'v', 'c1'), 4: ('s0', 's1', 'k', 'v', 'c0', 'q', 'c1'), 5: ('s0', 'k', 's1', 'q', 'c0', 'v', 'c1'), 6: ('s0', 's1', 'k', 'c0', 'v', 'c1', 'q'), 7: ('s0', 's1', 'k', 'c0', 'v', 'c1', 'q')}, order_last=('s0', 'C0', 's1', 'C1'),
                   pieces=(6, 5, 4, 3, 6, 5, 4, 3), aorder=(1, 0, 2, "b"), nobc=True)


DEFAULT_CFG.update({'order_last': ('s0', 'C0', 's1', 'C1'), 'bgblocks_last': (7, 5, 4, 3, 2, 0), 'bgrate_last': 1, 'pch_last': 0, 'pace_last': ((0, 0.7), (0.2, 0.9)), 'pvk_last': 1024, 'ksplit': 4, 'stages': 8, 'gate': (0, 0.92), 'cha': 16, 'bgrate2': 12, 'aorder': (0, 1, 2, 'b'), 'o_a': (0, 3, 4, 6, 1, 2, 5), 'o_bi': (3, 1, 2, 4, 0, 6, 5), 'o_bo': (3, 0, 1, 5, 2, 4, 6), 'o_ai': (2, 5, 0, 1, 3, 6, 4), 'o_ao': (0, 3, 4, 6, 1, 2, 5), 'joborder2': (3, 7, 1, 0, 2, 6, 5, 4), 'order': {0: ('s0', 'k', 's1', 'v', 'c0', 'q', 'c1'), 1: ('k', 's0', 'v', 's1', 'c0', 'q', 'c1'), 2: ('s0', 'k', 's1', 'v', 'c0', 'q', 'c1'), 3: ('s0', 's1', 'k', 'q', 'c0', 'v', 'c1'), 4: ('s0', 's1', 'k', 'q', 'c0', 'v', 'c1'), 5: ('s0', 's1', 'k', 'q', 'c0', 'v', 'c1'), 6: ('s0', 's1', 'k', 'v', 'c0', 'q', 'c1'), 7: ('s0', 's1', 'k', 'c0', 'q', 'c1', 'v')}, 'bgblocks': (6, 5, 4, 3, 2, 1), 'pvk': 512, 'joborder': (0, 5, 6, 1, 2, 7, 3, 4), 'o_pq': (3, 1, 0, 6, 4, 2, 5), 'o_pk': (0, 3, 4, 6, 1, 2, 5), 'o_pv': (5, 2, 0, 4, 6, 3, 1), 'pch': 16, 'pace': ((0, 0.6), (0.2, 0.8))})


DEFAULT_CFG.update(plan0=("wk", "wv", "c0"), plan1=("c1", "c2", "c3", "wq", "x0"),
                   plan_kv=((), ("x1", "x2"), ("x3",), ("p1",)), plan_q=(("s0",), (), (), ()))


DEFAULT_CFG.update(o_vi=(0, 3, 4, 6, 1, 2, 5), o_vo=(0, 3, 4, 6, 1, 2, 5), bgrate2=18)


DEFAULT_CFG.update({'ksplit': 8, 'stages': 8, 'gate': (0, 0.92), 'cha': 16, 'bgrate2': 16, 'aorder': (2, 1, 0, 'b'), 'o_a': (0, 3, 4, 6, 1, 2, 5), 'o_bi': (3, 1, 2, 4, 0, 6, 5), 'o_bo': (2, 5, 0, 1, 3, 6, 4), 'o_ai': (5, 2, 0, 4, 6, 3, 1), 'o_ao': (0, 3, 4, 6, 1, 2, 5), 'joborder2': (0, 7, 1, 3, 2, 6, 5, 4), 'o_vi': (3, 1, 0, 6, 4, 2, 5), 'o_vo': (3, 1, 2, 4, 0, 6, 5)})
DEFAULT_CFG.update(o_wi=(0, 3, 4, 6, 1, 2, 5), o_wo=(0, 3, 4, 6, 1, 2, 5), vsplit=3)


DEFAULT_CFG.update({'order_last': ('s0', 'C0', 's1', 'C1'), 'bgblocks_last': (6, 5, 4, 3, 2, 0), 'bgrate_last': 0.5, 'pch_last': 0, 'pace_last': ((0, 0.6), (0.2, 0.9)), 'pvk_last': 512, 'order': {0: ('s0', 'k', 's1', 'c0', 'v', 'q', 'c1'), 1: ('s0', 'k', 's1', 'q', 'c0', 'v', 'c1'), 2: ('s0', 's1', 'k', 'c0', 'q', 'c1', 'v'), 3: ('s0', 's1', 'c0', 'k', 'q', 'c1', 'v'), 4: ('s0', 'v', 's1', 'k', 'c0', 'q', 'c1'), 5: ('k', 's0', 'v', 's1', 'c0', 'q', 'c1'), 6: ('s0', 's1', 'k', 'v', 'c0', 'q', 'c1'), 7: ('s0', 's1', 'k', 'v', 'c0', 'q', 'c1')}, 'bgblocks': (6, 5, 4, 3, 2, 1), 'pvk': 1024, 'joborder': (4, 5, 6, 1, 0, 7, 3, 2), 'o_pq': (2, 0, 4, 3, 6, 1, 5), 'o_pk': (6, 0, 3, 4, 1, 2, 5), 'o_wi': (0, 5, 1, 2, 3, 4, 6), 'o_wo': (2, 4, 0, 3, 6, 1, 5), 'vsplit': 3, 'pch': 16, 'pace': ((0, 0.6), (0.2, 0.9))})


def build(cfg=None):
    cfg = dict(DEFAULT_CFG, **(cfg or {}))
    vmem = pltpu.VMEM

    def fn(A_x, A_wqkv, A_wo, B_x, B_c_kv, B_w_q, B_w_uk, B_w_uv, B_w_o):
        out = pl.pallas_call(
            functools.partial(_kernel, cfg=cfg),
            out_shape=jax.ShapeDtypeStruct((S, 2 * DM), BF16),
            in_specs=[pl.BlockSpec(memory_space=pl.ANY)] * 9,
            out_specs=pl.BlockSpec(memory_space=pl.ANY),
            scratch_shapes=[
                vmem((S, DM), BF16),
                vmem((S, B_DC), BF16),
                vmem((7, POOL_ROWS, HALF), U32),
                vmem((7, S // 4, B_DC // 2), U32),
                vmem((2, DM, B_DH), U32),
                vmem((2, B_DC, B_DH), U32),
                vmem((2, B_DC, B_DH), U32),
                vmem((7, DM // 4, B_DH), U32),
                vmem((7, B_DC // 4, B_DH), U32),
                vmem((NBLK // 2, 49, LANES // 2, LANES), U32),
                vmem((S, 2 * B_DH), BF16),
                vmem((2, S // 2, B_DH), U32),
                vmem((2, B_DH // 2, S), U32),
                vmem((PAIRS, S, 2 * B_DH), BF16),
                vmem((49, DM // 2, DM // 4), U32),
                vmem((49, DM // 8, DM // 4), U32),
                vmem((2, 2, HALF // PAIRS, 2 * DM), BF16),
                vmem((2, 4, 16, DM), BF16),
                vmem((49, DM // 8, DM // 4), U32),
                vmem((2, 2, A_HEADS, DM), U32),
                vmem((2, 4, 64, DM), BF16),
                vmem((2, BLK, DM), BF16),
                vmem((LOC_PANELS, HALO + BLK, LANES), F32),
                vmem((2, BLK, 2 * DM), BF16),
                pltpu.SemaphoreType.DMA((2, NBLK // 2)),
                pltpu.SemaphoreType.DMA((2, 3)),
                pltpu.SemaphoreType.DMA((2, 13)),
                pltpu.SemaphoreType.DMA((2,)),
                pltpu.SemaphoreType.DMA((2, 5)),
            ],
            compiler_params=pltpu.CompilerParams(vmem_limit_bytes=124 * 2 ** 20, flags=cfg.get("flags"),
                                                 disable_bounds_checks=cfg.get("nobc", False)),
            name="fused_local_and_latent_attention",
        )(A_x.reshape(S, DM), A_wqkv, A_wo.reshape(A_HEADS, A_DH, DM), B_x.reshape(S, DM), B_c_kv.reshape(S, B_DC),
          B_w_q, B_w_uk, B_w_uv, B_w_o.reshape(B_HEADS * B_DH, DM))
        return out.reshape(1, S, 2 * DM)

    return jax.jit(fn)


@jax.jit
def pallas_concat_heads__sliding_local_dilated__compressed_kv_cla__prompt_kernel(
    A_x: jax.Array,
    A_wqkv: jax.Array,
    A_wo: jax.Array,
    B_x: jax.Array,
    B_c_kv: jax.Array,
    B_w_q: jax.Array,
    B_w_uk: jax.Array,
    B_w_uv: jax.Array,
    B_w_o: jax.Array,
):
    return build(dict())(A_x, A_wqkv, A_wo, B_x, B_c_kv, B_w_q, B_w_uk, B_w_uv, B_w_o)
```

```python
import functools
import itertools

import jax
import jax.numpy as jnp
from jax import lax
import jax.experimental.pallas as pl
import jax.experimental.pallas.tpu as pltpu

S = 2048
DM = 1024
HALF = DM // 2
LANES = 128
A_HEADS, A_DH, A_WIN, A_DIL = 32, 32, 8, 2
HALO = 16
B_HEADS, B_DH, B_DC = 32, 128, 512
PAIRS = B_HEADS // 2

BLK = 256
SUB = BLK // 2
NBLK = S // BLK

LOG2E = 1.4426950408889634
NEG = -1e9
F32, BF16, U32 = jnp.float32, jnp.bfloat16, jnp.uint32

A_TERMS = (((1, 0, 0), (1, 1, 1)), ((1, 1, 0), (1, 1, 1)), ((1, 0, 0),), ((1, 1, 1),),
           ((1, 0, 0), (1, 0, 1)), ((1, 1, 0), (-1, 0, 0)), ((1, 0, 1), (-1, 1, 1)))
B_TERMS = (((1, 0, 0), (1, 1, 1)), ((1, 0, 0),), ((1, 0, 1), (-1, 1, 1)), ((1, 1, 0), (-1, 0, 0)),
           ((1, 1, 1),), ((1, 0, 0), (1, 0, 1)), ((1, 1, 0), (1, 1, 1)))
C_TERMS = (((1, 0, 0), (1, 1, 1)), ((1, 1, 0), (-1, 1, 1)), ((1, 0, 1), (1, 1, 1)), ((1, 0, 0), (1, 1, 0)),
           ((-1, 0, 0), (1, 0, 1)), ((1, 1, 1),), ((1, 0, 0),))

POOL_X = 0
POOL_QKV = POOL_X + S // 4
POOL_ROWS = POOL_QKV + 2 * HALF // 2
LOC_K, LOC_V, LOC_Q, LOC_PANELS = 0, 8, 16, 24


def _pack(x):
    return pltpu.bitcast(x.astype(BF16), U32)


def _unpack(x):
    return pltpu.bitcast(x, BF16)


def _operand_sums(block, terms):
    blocks = [[block(i, j) for j in range(2)] for i in range(2)]
    out = []
    for (_, i, j), *rest in terms:
        acc = blocks[i][j]
        for sign, i, j in rest:
            a, b = acc.astype(F32), blocks[i][j].astype(F32)
            acc = a + b if sign > 0 else a - b
        out.append(acc)
    return out


def _block_product(product, order=(0, 3, 4, 6, 1, 2, 5), c=None):
    c = c or [[None, None], [None, None]]
    for r in order:
        m = product(r)
        for sign, i, j in C_TERMS[r]:
            if c[i][j] is None:
                c[i][j] = m if sign > 0 else -m
            else:
                c[i][j] = c[i][j] + m if sign > 0 else c[i][j] - m
    return c


def _operand_sums2(block, terms):
    outer = [[_operand_sums(lambda i, j: block(2 * i + a, 2 * j + b), terms) for b in range(2)] for a in range(2)]
    return [functools.partial(_operand_sums, lambda a, b, r=r: outer[a][b][r], terms) for r in range(7)]


def _join(c):
    return jnp.concatenate([jnp.concatenate(row, axis=1) for row in c], axis=0)


def _heads_to_lanes(groups):
    lane = lax.broadcasted_iota(jnp.int32, groups[0].shape, 1)
    groups = list(groups)
    for group_bit, lane_bit in ((2, 4), (1, 3), (0, 2), (2, 6), (2, 1), (1, 5), (1, 0)):
        shift = 1 << lane_bit
        low = (lane & shift) == 0
        for g in range(8):
            if g >> group_bit & 1:
                continue
            x, y = groups[g], groups[g | 1 << group_bit]
            groups[g] = jnp.where(low, x, pltpu.roll(y, shift, 1))
            groups[g | 1 << group_bit] = jnp.where(low, pltpu.roll(x, LANES - shift, 1), y)
    return [groups[(g & 1) << 2 | (g >> 2) << 1 | (g >> 1 & 1)] for g in range(8)]


def _word_half(word, hi):
    return pltpu.bitcast(word & U32(0xFFFF0000) if hi else word << 16, F32)


def _reciprocal(x):
    r = pl.reciprocal(x, approx=True)
    return r * (2.0 - x * r)


class _Timeline:
    def __init__(self, never):
        self.never, self.now, self.marks = never, 0.0, []

    def issue(self, cycles, results):
        for n, value in enumerate(results):
            self.marks.append((self.now + cycles * (n + 1) / len(results), value))
        self.now += cycles

    def after(self, cycle, value):
        ready = [v for t, v in self.marks if t <= cycle]
        if not ready:
            return value
        mark = ready[-1][0:8, 0:value.shape[1]]
        if value.shape[0] > 8:
            mark = jnp.concatenate([mark] * (value.shape[0] // 8), axis=0)
        return jnp.where(self.never, mark, value)


class _Background:
    def __init__(self, never):
        self.never, self.pending, self.credit, self.rate = never, iter(()), 0.0, 0.0

    def add(self, pieces, rate):
        self.pending, self.rate = itertools.chain(self.pending, pieces), rate

    def tie(self, words):
        self.credit += self.rate
        due = list(itertools.islice(self.pending, int(self.credit)))
        self.credit -= int(self.credit)
        if not due:
            return words
        due = [pltpu.bitcast(d, U32) for d in due]
        mark = functools.reduce(jnp.bitwise_or, [
            d[r:r + 8, c:c + LANES] for d in due for r in range(0, d.shape[0], 8) for c in range(0, d.shape[1], LANES)])
        top = jnp.where(self.never, mark, words[:8, :LANES])
        if words.shape[1] > LANES:
            top = jnp.concatenate([top, words[:8, LANES:]], axis=1)
        return jnp.concatenate([top, words[8:]], axis=0)

    def finish(self):
        for _ in self.pending:
            pass


def _start(copies):
    for cp in copies:
        cp.start()


def _wait(copies):
    for cp in copies:
        cp.wait()


def _kernel(xa_hbm, wqkv_hbm, woa_hbm, xb_hbm, c_hbm, wq_hbm, wuk_hbm, wuv_hbm, wob_hbm,
            out_hbm,
            xb_raw, c_raw, pool, cs, wq_raw, wuk_raw, wuv_raw, wqs, wks, cts,
            q_s, k_s, v_s, ctx, wobs, woas,
            wqkv_raw, wva_raw, wvas, woa_raw, wob_raw, xa_raw, loc, obuf,
            sem_x, sem_w, sem_s, sem_a, sem_o, *, cfg):
    wq_u = wq_hbm.bitcast(U32)
    wuk_u = wuk_hbm.bitcast(U32)
    wuv_u = wuv_hbm.bitcast(U32)
    woa_u = woa_hbm.bitcast(U32)

    def pair_copies(j, which=(0, 1, 2)):
        ends = ((wuk_u, wuk_raw), (wuv_u, wuv_raw), (wq_u, wq_raw))
        return [pltpu.make_async_copy(ends[n][0].at[:, j, :], ends[n][1].at[j % 2], sem_w.at[j % 2, n])
                for n in which]

    def stream_copies(j):
        slot = j % 2
        rows = HALF // PAIRS
        cps = []
        for k in range(2):
            cps.append(pltpu.make_async_copy(
                wqkv_hbm.at[row_range(k * HALF + j * rows, rows), 0:2 * DM], wqkv_raw.at[slot, k], sem_s.at[slot, k]))
        for k in range(4):
            cps.append(pltpu.make_async_copy(
                wqkv_hbm.at[row_range(k * 256 + j * 16, 16), 2 * DM:3 * DM], wva_raw.at[slot, k],
                sem_s.at[slot, 9 + k]))
        for k in range(2):
            word = (j >> 1 & 1) | k << 1 | (j >> 2) << 2
            cps.append(pltpu.make_async_copy(woa_u.at[:, word, :], woa_raw.at[slot, k], sem_s.at[slot, 7 + k]))
        for k in range(4):
            cps.append(pltpu.make_async_copy(
                wob_hbm.at[row_range(k * DM + j * 64, 64), :], wob_raw.at[slot, k], sem_s.at[slot, 3 + k]))
        return cps

    def c_copy(n):
        rows = pl.ds(pl.multiple_of(n * 2 * BLK, 2 * BLK), 2 * BLK)
        return pltpu.make_async_copy(c_hbm.at[rows, :], c_raw.at[rows, :], sem_x.at[0, n])

    def xb_copy(n):
        rows = pl.ds(pl.multiple_of(n * 2 * BLK, 2 * BLK), 2 * BLK)
        return pltpu.make_async_copy(xb_hbm.at[rows, :], xb_raw.at[rows, :], sem_x.at[1, n])

    def xa_copy(i):
        rows = pl.ds(pl.multiple_of(i * BLK, BLK), BLK)
        return pltpu.make_async_copy(xa_hbm.at[rows, :], xa_raw.at[i % 2], sem_a.at[i % 2])

    def out_copy(i, part):
        r0, nr, c0, nc = (0, BLK, DM, DM) if part == 4 else (part // 2 * SUB, SUB, part % 2 * HALF, HALF)
        rows = pl.ds(pl.multiple_of(i * BLK + r0, SUB), nr)
        return pltpu.make_async_copy(obuf.at[i % 2, r0:r0 + nr, c0:c0 + nc], out_hbm.at[rows, c0:c0 + nc],
                                     sem_o.at[i % 2, part])

    def row_range(start, size):
        return pl.ds(start if isinstance(start, int) else pl.multiple_of(start, size), size)

    def packed_rows(start, size):
        if isinstance(start, int):
            return pl.ds(start // 2, size // 2)
        return pl.ds(pl.multiple_of(start // 2, size // 2), size // 2)

    def prepare_pair_weights(j, which="qk"):
        slot = j % 2
        for name in which:
            raw, dst = {"q": (wq_raw, wqs), "k": (wuk_raw, wks)}[name]
            depth = raw.shape[1] // 2
            for r0 in range(0, depth, 32):
                words = [raw[slot, k * depth + r0:k * depth + r0 + 32, :] for k in range(2)]
                for r, op in enumerate(_operand_sums(lambda k, head: _word_half(words[k], head), B_TERMS)):
                    dst[r, r0 // 2:r0 // 2 + 16, :] = _pack(op)

    def value_weights(j):
        words = wuv_raw[j % 2].T

        def block(a, k):
            return _word_half(words[a % 2 * 64:(a % 2 + 1) * 64, k * LANES:(k + 1) * LANES], a // 2)

        return [[op.astype(BF16) for op in inner()] for inner in _operand_sums2(block, A_TERMS)]

    def prepare_latents(t):
        blocks = [[c_raw[row_range((4 * t + n) * LANES, LANES), k * LANES:(k + 1) * LANES].astype(F32).T
                   for n in range(4)] for k in range(4)]
        ops = [[_pack(op) for op in inner()] for inner in _operand_sums2(lambda k, n: blocks[k][n], B_TERMS)]
        for r in range(7):
            for u in range(7):
                cts[t, 7 * r + u] = ops[r][u]
        return ops

    def project_values(t, weights, stream=None, ops=None):
        def outer(r):
            def product(u):
                rhs = cts[t, 7 * r + u] if ops is None else ops[r][u]
                m = jnp.dot(weights[r][u], _unpack(rhs), preferred_element_type=F32)
                if stream is not None:
                    stream.issue(16, [m[-8:]])
                return m
            return _join(_block_product(product, cfg["o_wi"]))

        c = _block_product(outer, cfg["o_wo"][:cfg["vsplit"]])
        yield
        c = _block_product(outer, cfg["o_wo"][cfg["vsplit"]:], c)
        for head in range(2):
            for n in range(2):
                v_s[head, :, row_range((2 * t + n) * BLK, BLK)] = _pack(c[head][n])

    def prepare_inputs(i, raw, dst, base):
        width = raw.shape[1] // 2
        ops = _operand_sums(lambda a, k: raw[pl.ds(pl.multiple_of(i * BLK + a * SUB, SUB), SUB),
                                             k * width:(k + 1) * width], A_TERMS)
        ops = [_pack(op) for op in ops]
        for r, op in enumerate(ops):
            dst[r, packed_rows(base + i * SUB, SUB), :] = op
        return ops

    def project(i, which, stream=None, ops=None):
        lhs, base, rhs, dst = {"q": (pool, 2 * POOL_X, wqs, q_s), "k": (cs, 0, wks, k_s)}[which]
        rows = packed_rows(base + i * SUB, SUB)

        def product(r):
            w = rhs[r] if stream is None or i not in cfg["bgblocks"] else stream.bg.tie(rhs[r])
            m = jnp.dot(_unpack(lhs[r, rows, :] if ops is None else ops[r]), _unpack(w), preferred_element_type=F32)
            if stream is not None:
                stream.issue(SUB * rhs.shape[1] // 256, [m[SUB // 2 - 8:SUB // 2], m[SUB - 8:SUB]])
            return m

        c = _block_product(product, cfg["o_p" + which])
        for a in range(2):
            if which == "q":
                q_s[pl.ds(pl.multiple_of(i * BLK + a * SUB, SUB), SUB), :] = (
                    jnp.concatenate(c[a], axis=1) * (B_DH ** -0.5 * LOG2E)).astype(BF16)
            else:
                for head in range(2):
                    dst[head, packed_rows(i * BLK + a * SUB, SUB), :] = _pack(c[a][head])

    def head_rows(ref, h, r0, r1):
        return _unpack(ref[h, r0 // 2:r1 // 2, :])

    def scores(h, i, stream):
        def nt(a, b):
            return lax.dot_general(a, b, (((1,), (1,)), ((), ())), preferred_element_type=F32)
        row = lax.broadcasted_iota(jnp.int32, (SUB, SUB), 0)
        col = lax.broadcasted_iota(jnp.int32, (SUB, SUB), 1)
        r0 = i * BLK
        full = nt(q_s[r0:r0 + BLK, h * B_DH:(h + 1) * B_DH], head_rows(k_s, h, 0, r0)) if i else None
        if i:
            stream.issue(BLK * i // 2, [full[t % BLK:t % BLK + 8, t // BLK * LANES:(t // BLK + 1) * LANES]
                                    for t in range(56, BLK * i // 2, 64)])
        diag = []
        for a in range(2):
            d = nt(q_s[r0 + a * SUB:r0 + (a + 1) * SUB, h * B_DH:(h + 1) * B_DH],
                   head_rows(k_s, h, r0, r0 + (a + 1) * SUB))
            stream.issue(32 * (a + 1), [d])
            last = jnp.where(col <= row, d[:, a * SUB:], NEG)
            diag.append(jnp.concatenate([d[:, :SUB], last], axis=1) if a else last)
        return full, diag, stream.now

    def softmax(i, sc, stream, h):
        full, diag, t0 = sc
        nf = i * BLK
        lo, hi = stream.pace[h]
        span = stream.now - t0
        step = stream.pch
        pf, pd, inv = [], [], []
        for a in range(2):
            s = diag[a]
            if full is not None:
                s = jnp.concatenate([full[a * SUB:(a + 1) * SUB], s], axis=1)
            m = jnp.max(s, axis=1, keepdims=True)
            if step:
                m = jnp.concatenate([
                    stream.after(t0 + span * (lo + (hi - lo) * (a * SUB + c) / BLK), m[c:c + step])
                    for c in range(0, SUB, step)], axis=0)
            p = jnp.exp2(s - m)
            if i >= cfg["sum16"]:
                p = p.astype(BF16)
            inv.append(_reciprocal(jnp.sum(p.astype(F32), axis=1, keepdims=True)))
            if full is not None:
                pf.append(p[:, :nf])
            pd.append(p[:, nf:])
        return (jnp.concatenate(pf, axis=0) if pf else None), pd, inv

    def context(h, i, sm, stream):
        def pv(a, b):
            return lax.dot_general(a.astype(BF16), b, (((1,), (1,)), ((), ())), preferred_element_type=F32)
        pf, pd, inv = sm
        r0 = i * BLK
        of = None
        for k0 in range(0, r0, stream.pvk):
            k1 = min(k0 + stream.pvk, r0)
            words = v_s[h, :, k0:k1]
            if stream.bgpv and i in cfg["bgblocks_last"]:
                words = jnp.concatenate(
                    [stream.bg.tie(words[:, t:t + LANES]) for t in range(0, words.shape[1], LANES)], axis=1)
            part = pv(pf[:, k0:k1], _unpack(words))
            of = part if of is None else of + part
            stream.issue((k1 - k0) // 2, [of[t:t + 8] for t in range(56, BLK, 64)])
        out = []
        for a in range(2):
            o = pv(pd[a], _unpack(v_s[h, :, r0:r0 + (a + 1) * SUB]))
            stream.issue(32 * (a + 1), [o])
            if of is not None:
                o = o + of[a * SUB:(a + 1) * SUB]
            out.append(o * inv[a])
        return out

    def stream_work(j, inner_part=True, outer_part=True):
        slot = j % 2

        def qkv(part):
            groups = [_heads_to_lanes([
                _pack(wqkv_raw[slot, k, :, part * DM + a * LANES:part * DM + (a + 1) * LANES])
                for a in range(8)]) for k in range(2)]
            rows = packed_rows(2 * POOL_QKV + part * HALF + j * (HALF // PAIRS), HALF // PAIRS)
            for a in range(4):
                for r, op in enumerate(_operand_sums(lambda k, n: _unpack(groups[k][4 * n + a]), B_TERMS)):
                    op = _pack(op)
                    pool[r, rows, a * LANES:(a + 1) * LANES] = op
                    yield op

        def two_level(block, dst, row0, cols):
            for r, inner in enumerate(_operand_sums2(block, B_TERMS)):
                for t, op in enumerate(inner()):
                    op = _pack(op)
                    dst[7 * r + t, packed_rows(row0, 2 * op.shape[0]), cols] = op
                    yield op

        def value():
            groups = [_heads_to_lanes([_pack(wva_raw[slot, k, :, a * LANES:(a + 1) * LANES]) for a in range(8)])
                      for k in range(4)]
            return two_level(lambda k, n: _unpack(jnp.concatenate(groups[k][2 * n:2 * n + 2], axis=1)),
                             wvas, j * 16, slice(None))

        def out_a():
            c0 = j % 2 * LANES if isinstance(j, int) else pl.multiple_of(j % 2 * LANES, LANES)
            row0 = ((j >> 1 & 1) * 4 + (j >> 2)) * A_HEADS
            return two_level(lambda k, n: _word_half(woa_raw[slot, k % 2, :, pl.ds(n * 256 + c0, LANES)], k // 2),
                             woas, row0, pl.ds(c0, LANES))

        def out_b(r0, c0):
            return two_level(lambda k, n: wob_raw[slot, k, r0:r0 + 32, n * 256 + c0:n * 256 + c0 + LANES],
                             wobs, j * 64 + r0, slice(c0, c0 + LANES))

        for n in cfg["joborder" if inner_part else "joborder2"]:
            if n < 4 and outer_part:
                yield from out_b(n // 2 * 32, n % 2 * LANES)
            elif n == 4 and outer_part:
                yield from out_a()
            elif n > 4 and inner_part:
                yield from value() if n == 7 else qkv(n - 5)

    only = cfg.get("only")
    named = {"wk": lambda: pair_copies(0, (0,)), "wv": lambda: pair_copies(0, (1,)), "wq": lambda: pair_copies(0, (2,)),
             "p1": lambda: pair_copies(1), "s0": lambda: stream_copies(0)}

    def request(names):
        for name in names:
            if name in named:
                _start(named[name]())
            else:
                (c_copy if name[0] == "c" else xb_copy)(int(name[1])).start()

    def first_steps(copy, work, plan):
        def body(n, carry):
            blocks = [2 * n, 2 * n + 1]
            copy(n).wait()
            for at, names in enumerate(plan):
                if names:
                    pl.when(n == at)(functools.partial(request, names))
            work(n, blocks)
            return carry

        lax.fori_loop(0, len(plan), body, 0)

    def first_kv(weights, n, blocks):
        for i in blocks:
            project(i, "k", ops=prepare_inputs(i, c_raw, cs, 0))
        for _ in project_values(n, weights, ops=prepare_latents(n)):
            pass

    def first_q(n, blocks):
        for i in blocks:
            project(i, "q", ops=prepare_inputs(i, xb_raw, pool, 2 * POOL_X))

    with jax.named_scope("prologue"):
        if not only:
            request(cfg["plan0"])
            with jax.named_scope("w0"):
                _wait(pair_copies(0, (0,)))
            request(cfg["plan1"])
            prepare_pair_weights(0, "k")
            _wait(pair_copies(0, (1,)))
            with jax.named_scope("kv"):
                first_steps(c_copy, functools.partial(first_kv, value_weights(0)), cfg["plan_kv"])
            _wait(pair_copies(0, (2,)))
            prepare_pair_weights(0, "q")
            with jax.named_scope("q"):
                first_steps(xb_copy, first_q, cfg["plan_q"])
    _wait(pair_copies(1) + stream_copies(0))
    _start(pair_copies(2) + stream_copies(1))

    def head_pair(j, project_next):
        if project_next:
            prepare_pair_weights(j + 1)
            weights = value_weights(j + 1)
        else:
            xa_copy(0).start()
            xa_copy(1).start()
        stream = _Timeline(j < 0)
        stream.pace, stream.pch = (cfg["pace"], cfg["pch"]) if project_next else (cfg["pace_last"], cfg["pch_last"])
        stream.bg = _Background(j < 0)
        stream.bg.add(stream_work(j, True, project_next),
                  350 / (14 * len(cfg["bgblocks"])) if project_next else cfg["bgrate_last"])
        stream.bgpv = not project_next
        stream.pvk = cfg["pvk"] if project_next else cfg["pvk_last"]
        proj = (lambda i, which: project(i, which, stream)) if project_next else (lambda i, which: None)
        sc, o = {}, {}
        if project_next:
            values = [project_values(t, weights, stream) for t in range(NBLK // 2)]

        def finish_head(h, i):
            o[h, i] = context(h, i, softmax(i, sc.pop((h, i)), stream, h), stream)
            if (1 - h, i) in o:
                for a in range(2):
                    ctx[j, i * BLK + a * SUB:i * BLK + (a + 1) * SUB, :] = (
                        jnp.concatenate([o[0, i][a], o[1, i][a]], axis=1).astype(BF16))

        for i in range(NBLK - 1, -1, -1):
            order = cfg["order"] if project_next else cfg["order_last"]
            for tok in order[i] if isinstance(order, dict) else order:
                if tok[0] == "s":
                    sc[int(tok[1]), i] = scores(int(tok[1]), i, stream)
                elif tok[0] == "c":
                    finish_head(int(tok[1]), i)
                elif tok[0] == "C":
                    if (int(tok[1]), i + 1) in sc:
                        finish_head(int(tok[1]), i + 1)
                elif tok == "q":
                    proj(i, "q")
                elif tok == "v":
                    if i + 2 < NBLK:
                        next(values[i // 2 + 1], None)
                elif i + 1 < NBLK:
                    proj(i + 1, tok)
        for h, i in sorted(sc):
            finish_head(h, i)
        proj(0, "k")
        if project_next:
            for _ in values[0]:
                pass
        stream.bg.finish()
        if project_next:
            _wait(stream_copies(j + 1))

            @pl.when(j + 2 < PAIRS)
            def _():
                _wait(pair_copies(j + 2))

            @pl.when(j + 3 < PAIRS)
            def _():
                _start(pair_copies(j + 3))

            @pl.when(j + 2 < PAIRS)
            def _():
                _start(stream_copies(j + 2))

    def pair_step(j, carry):
        with jax.named_scope("group"):
            head_pair(j, True)
        return carry

    with jax.named_scope("phase1"):
        if only in (None, "p1"):
            lax.fori_loop(0, PAIRS - 1, pair_step, 0)
    with jax.named_scope("lastgroup"):
        if only == "p1" or only == "last":
            def keep(n, carry):
                obuf.bitcast(U32)[0, 0:8, 0:LANES] = (pltpu.bitcast(ctx[n, 0:16, 0:LANES], U32) | pltpu.bitcast(q_s[pl.ds(pl.multiple_of(n * 16, 16), 16), 0:LANES], U32) | pool[n, 0:8, 0:LANES] | wobs[n, 0:8, 0:LANES] | woas[n, 0:8, 0:LANES] | wvas[n, 0:8, 0:LANES]
                                                      | k_s[n % 2, 0:8, :] | v_s[n % 2, 0:8, 0:LANES])
                return carry
        if only == "last":
            lax.fori_loop(PAIRS - 1, PAIRS, lambda j, c: (head_pair(j, False), c)[1], 0)
        if only == "p1" or only == "last":
            lax.fori_loop(0, 7, keep, 0)
        if only in ("p1", "p2", "last"):
            _wait(stream_copies(PAIRS - 1))
            xa_copy(0).start()
            xa_copy(1).start()
        else:
            lax.fori_loop(PAIRS - 1, PAIRS, lambda j, c: (head_pair(j, False), c)[1], 0)

    loc[0:16, BLK:BLK + HALO, :] = jnp.zeros((16, HALO, LANES), F32)

    def store_blocks(i, col0, c):
        for a, n in ((0, 0), (1, 0), (0, 1), (1, 1)):
            obuf[i % 2, a * SUB:(a + 1) * SUB, col0 + n * HALF:col0 + (n + 1) * HALF] = c[a][n].astype(BF16)
            if col0 == 0:
                out_copy(i, 2 * a + n).start()
        if col0:
            out_copy(i, 4).start()

    def row_block(i, carry):
        slot = i % 2
        xa_copy(i).wait()

        @pl.when(i >= 2)
        def _():
            _wait([out_copy(i - 2, part) for part in range(5)])

        loc[0:16, 0:HALO, :] = loc[0:16, BLK:BLK + HALO, :]
        zero = i // NBLK if cfg["opaque"] else 0
        xsums = _operand_sums(
            lambda a, k: xa_raw[slot, a * SUB:(a + 1) * SUB, k * HALF:(k + 1) * HALF], A_TERMS)
        xops = [op.astype(BF16) for op in xsums]

        bg = _Background(i < 0)
        bg.add(stream_work(PAIRS - 1, False, True), cfg["bgrate2"])

        def lane_groups(part):
            if part == 2:
                def outer(r):
                    ops = _operand_sums(lambda a, k: xsums[r][64 * a:64 * (a + 1), 256 * k:256 * (k + 1)], A_TERMS)
                    return _join(_block_product(lambda t: jnp.dot(
                        ops[t].astype(BF16), _unpack(wvas[7 * r + t]), preferred_element_type=F32), cfg["o_vi"]))

                c = _block_product(outer, cfg["o_vo"])
                return lambda a, g: c[a][g // 4][:, (g % 4) * LANES:(g % 4 + 1) * LANES]
            r0 = POOL_QKV + part * HALF // 2
            c = _block_product(lambda r: jnp.dot(xops[r], _unpack(bg.tie(pool[r, r0:r0 + HALF // 2, :])),
                                                 preferred_element_type=F32), cfg["o_a"])
            return lambda a, g: c[a][g // 4][:, (g % 4) * LANES:(g % 4 + 1) * LANES]

        marks = []

        def out_b():
            quarter = PAIRS // 4

            def block(a, k):
                rows = pl.ds(pl.multiple_of(i * BLK + a * (BLK // 4), BLK // 4), BLK // 4)
                return jnp.concatenate(
                    [ctx[j, rows, :] for j in range(k * quarter, (k + 1) * quarter)], axis=1).astype(F32)

            lhs = _operand_sums2(block, A_TERMS)

            def outer(r):
                ops = lhs[r]()

                def product(t):
                    step = DM // cfg["ksplit"]
                    acc = None
                    for k0 in range(0, DM, step):
                        part = jnp.dot(ops[t][:, k0:k0 + step].astype(BF16),
                                       _unpack(wobs[7 * r + t, k0 // 2:(k0 + step) // 2, :]),
                                       preferred_element_type=F32)
                        acc = part if acc is None else acc + part
                        marks.append(acc)
                    return acc

                return _join(_block_product(product, cfg["o_bi"]))

            store_blocks(i, DM, _block_product(outer, cfg["o_bo"]))

        for part in cfg["aorder"]:
            if part == "b":
                bg.finish()
                out_b()
                continue
            f = lane_groups(part)
            for a in range(2):
                for g in range(8):
                    loc[(LOC_Q, LOC_K, LOC_V)[part] + g, HALO + a * SUB:HALO + (a + 1) * SUB, :] = f(a, g)

        ch = cfg["cha"]

        stages = cfg["stages"]
        total = stages * BLK // ch
        count = [0]

        def paced(values):
            lo, hi = cfg["gate"]
            mark = marks[int((lo + (hi - lo) * count[0] / (total - 1)) * (len(marks) - 1))]
            count[0] += 1
            return [jnp.where(i < 0, mark[0:ch, 0:LANES], t) for t in values]

        def attend(c0):
            def rows(base, g, w):
                b0 = HALO + c0 - A_DIL * w
                return loc[zero + base + g, b0:b0 + ch, :]

            q0 = [rows(LOC_Q, g, 0) for g in range(8)]
            logits = []
            half = max(stages // 2, 1)
            for w in range(A_WIN):
                if w % (A_WIN // half) == 0:
                    q = paced(q0)
                acc = q[0] * rows(LOC_K, 0, w)
                for g in range(1, 8):
                    acc = acc + q[g] * rows(LOC_K, g, w)
                acc = acc + pltpu.roll(acc, 2 * A_HEADS, 1)
                acc = acc + pltpu.roll(acc, A_HEADS, 1)
                if c0 < A_DIL * w:
                    pos = i * BLK + c0 + lax.broadcasted_iota(jnp.int32, (ch, LANES), 0)
                    acc = jnp.where(pos >= A_DIL * w, acc, NEG * A_DH ** 0.5)
                logits.append(acc)
            m = functools.reduce(jnp.maximum, logits)
            ps = [jnp.exp2((l - m) * (A_DH ** -0.5 * LOG2E)) for l in logits]
            inv = _reciprocal(functools.reduce(lambda a, b: a + b, ps))
            ps = [p * inv for p in ps]
            out = []
            for g in range(8):
                if stages > 1 and g % (8 // half) == 0:
                    pg = paced(ps)
                elif stages == 1:
                    pg = ps
                out.append(functools.reduce(lambda a, b: a + b, [pg[w] * rows(LOC_V, g, w) for w in range(A_WIN)]))
            return out

        quarters = [[] for _ in range(4)]
        for c0 in range(0, BLK // 4, ch):
            for a in range(4):
                quarters[a].append(jnp.concatenate(attend(a * (BLK // 4) + c0), axis=1))
        quarters = [jnp.concatenate(t, axis=0) for t in quarters]
        lhs = _operand_sums2(lambda a, k: quarters[a][:, k * 256:(k + 1) * 256], A_TERMS)

        def outer(r):
            ops = lhs[r]()
            return _join(_block_product(lambda t: jnp.dot(
                ops[t].astype(BF16), _unpack(woas[7 * r + t]), preferred_element_type=F32), cfg["o_ai"]))

        store_blocks(i, 0, _block_product(outer, cfg["o_ao"]))

        @pl.when(i + 2 < NBLK)
        def _():
            xa_copy(i + 2).start()

        return carry

    def row_step(i, carry):
        with jax.named_scope("rowblk"):
            return row_block(i, carry)

    with jax.named_scope("phase2"):
        if only in (None, "p2"):
            lax.fori_loop(0, NBLK, row_step, 0)
    with jax.named_scope("tail"):
        _wait([out_copy(i, part) for i in (NBLK - 2, NBLK - 1) for part in range(5)])


DEFAULT_CFG = dict(cha=16, opaque=False, nsplit=4, ksplit=4, gate=(0, 0.88), stages=4, pace=((0, 0.7), (0.2, 0.8)), pch=0, bgblocks=(6, 5, 4, 3, 2, 1), bgblocks_last=(7, 6, 5, 4, 3, 2, 1), bgrate_last=1, bgrate2=14, joborder=(0, 5, 1, 6, 2, 7, 3, 4),
                   **{"o_" + n: (0, 3, 4, 6, 1, 2, 5) for n in ("pq", "pk", "pv", "a", "bi", "bo", "ai", "ao")},
                   pch_last=0, pace_last=((0, 0.7), (0.2, 0.8)), jobslots_last=[(3, 1, 1), (2, 1, 1), (3, 0, 1), (2, 0, 1), (1, 0, 1), (1, 1, 1), (3, 0, 0), (2, 0, 0), (2, 1, 0)], sum16=0, plan0=("wk", "c0", "wv", "c1"), plan1=("c2", "c3"),
                   plan_kv=(("c4", "c5", "c6", "c7"), ("wq", "x0"), ("x1", "x2"), ("x3", "x4")),
                   plan_q=(("x5", "x6"), ("x7", "p1"), ("s0",), ()), sumgate=False, wch=32, wspan=0, pvk=1024, jobslots=[(5, 1, 1), (4, 0, 0), (3, 1, 0), (5, 0, 1), (5, 0, 0), (4, 1, 1), (3, 0, 0), (2, 1, 0)], order={0: ('s0', 'k', 's1', 'v', 'c0', 'q', 'c1'), 1: ('s0', 'k', 's1', 'v', 'c0', 'q', 'c1'), 2: ('s0', 'k', 's1', 'v', 'c0', 'q', 'c1'), 3: ('s0', 's1', 'k', 'q', 'c0', 'v', 'c1'), 4: ('s0', 's1', 'k', 'v', 'c0', 'q', 'c1'), 5: ('s0', 'k', 's1', 'q', 'c0', 'v', 'c1'), 6: ('s0', 's1', 'k', 'c0', 'v', 'c1', 'q'), 7: ('s0', 's1', 'k', 'c0', 'v', 'c1', 'q')}, order_last=('s0', 'C0', 's1', 'C1'),
                   pieces=(6, 5, 4, 3, 6, 5, 4, 3), aorder=(1, 0, 2, "b"), nobc=True)


DEFAULT_CFG.update({'order_last': ('s0', 'C0', 's1', 'C1'), 'bgblocks_last': (7, 5, 4, 3, 2, 0), 'bgrate_last': 1, 'pch_last': 0, 'pace_last': ((0, 0.7), (0.2, 0.9)), 'pvk_last': 1024, 'ksplit': 4, 'stages': 8, 'gate': (0, 0.92), 'cha': 16, 'bgrate2': 12, 'aorder': (0, 1, 2, 'b'), 'o_a': (0, 3, 4, 6, 1, 2, 5), 'o_bi': (3, 1, 2, 4, 0, 6, 5), 'o_bo': (3, 0, 1, 5, 2, 4, 6), 'o_ai': (2, 5, 0, 1, 3, 6, 4), 'o_ao': (0, 3, 4, 6, 1, 2, 5), 'joborder2': (3, 7, 1, 0, 2, 6, 5, 4), 'order': {0: ('s0', 'k', 's1', 'v', 'c0', 'q', 'c1'), 1: ('k', 's0', 'v', 's1', 'c0', 'q', 'c1'), 2: ('s0', 'k', 's1', 'v', 'c0', 'q', 'c1'), 3: ('s0', 's1', 'k', 'q', 'c0', 'v', 'c1'), 4: ('s0', 's1', 'k', 'q', 'c0', 'v', 'c1'), 5: ('s0', 's1', 'k', 'q', 'c0', 'v', 'c1'), 6: ('s0', 's1', 'k', 'v', 'c0', 'q', 'c1'), 7: ('s0', 's1', 'k', 'c0', 'q', 'c1', 'v')}, 'bgblocks': (6, 5, 4, 3, 2, 1), 'pvk': 512, 'joborder': (0, 5, 6, 1, 2, 7, 3, 4), 'o_pq': (3, 1, 0, 6, 4, 2, 5), 'o_pk': (0, 3, 4, 6, 1, 2, 5), 'o_pv': (5, 2, 0, 4, 6, 3, 1), 'pch': 16, 'pace': ((0, 0.6), (0.2, 0.8))})


DEFAULT_CFG.update(plan0=("wk", "wv", "c0"), plan1=("c1", "c2", "c3", "wq", "x0"),
                   plan_kv=((), ("x1", "x2"), ("x3",), ("p1",)), plan_q=(("s0",), (), (), ()))


DEFAULT_CFG.update(o_vi=(0, 3, 4, 6, 1, 2, 5), o_vo=(0, 3, 4, 6, 1, 2, 5), bgrate2=18)


DEFAULT_CFG.update({'ksplit': 8, 'stages': 8, 'gate': (0, 0.92), 'cha': 16, 'bgrate2': 16, 'aorder': (2, 1, 0, 'b'), 'o_a': (0, 3, 4, 6, 1, 2, 5), 'o_bi': (3, 1, 2, 4, 0, 6, 5), 'o_bo': (2, 5, 0, 1, 3, 6, 4), 'o_ai': (5, 2, 0, 4, 6, 3, 1), 'o_ao': (0, 3, 4, 6, 1, 2, 5), 'joborder2': (0, 7, 1, 3, 2, 6, 5, 4), 'o_vi': (3, 1, 0, 6, 4, 2, 5), 'o_vo': (3, 1, 2, 4, 0, 6, 5)})
DEFAULT_CFG.update(o_wi=(0, 3, 4, 6, 1, 2, 5), o_wo=(0, 3, 4, 6, 1, 2, 5), vsplit=3)


DEFAULT_CFG.update({'order_last': ('s0', 'C0', 's1', 'C1'), 'bgblocks_last': (6, 5, 4, 3, 2, 0), 'bgrate_last': 0.5, 'pch_last': 0, 'pace_last': ((0, 0.6), (0.2, 0.9)), 'pvk_last': 512, 'order': {0: ('s0', 'k', 's1', 'c0', 'v', 'q', 'c1'), 1: ('s0', 'k', 's1', 'q', 'c0', 'v', 'c1'), 2: ('s0', 's1', 'k', 'c0', 'q', 'c1', 'v'), 3: ('s0', 's1', 'c0', 'k', 'q', 'c1', 'v'), 4: ('s0', 'v', 's1', 'k', 'c0', 'q', 'c1'), 5: ('k', 's0', 'v', 's1', 'c0', 'q', 'c1'), 6: ('s0', 's1', 'k', 'v', 'c0', 'q', 'c1'), 7: ('s0', 's1', 'k', 'v', 'c0', 'q', 'c1')}, 'bgblocks': (6, 5, 4, 3, 2, 1), 'pvk': 1024, 'joborder': (4, 5, 6, 1, 0, 7, 3, 2), 'o_pq': (2, 0, 4, 3, 6, 1, 5), 'o_pk': (6, 0, 3, 4, 1, 2, 5), 'o_wi': (0, 5, 1, 2, 3, 4, 6), 'o_wo': (2, 4, 0, 3, 6, 1, 5), 'vsplit': 3, 'pch': 16, 'pace': ((0, 0.6), (0.2, 0.9))})


def build(cfg=None):
    cfg = dict(DEFAULT_CFG, **(cfg or {}))
    vmem = pltpu.VMEM

    def fn(A_x, A_wqkv, A_wo, B_x, B_c_kv, B_w_q, B_w_uk, B_w_uv, B_w_o):
        out = pl.pallas_call(
            functools.partial(_kernel, cfg=cfg),
            out_shape=jax.ShapeDtypeStruct((S, 2 * DM), BF16),
            in_specs=[pl.BlockSpec(memory_space=pl.ANY)] * 9,
            out_specs=pl.BlockSpec(memory_space=pl.ANY),
            scratch_shapes=[
                vmem((S, DM), BF16),
                vmem((S, B_DC), BF16),
                vmem((7, POOL_ROWS, HALF), U32),
                vmem((7, S // 4, B_DC // 2), U32),
                vmem((2, DM, B_DH), U32),
                vmem((2, B_DC, B_DH), U32),
                vmem((2, B_DC, B_DH), U32),
                vmem((7, DM // 4, B_DH), U32),
                vmem((7, B_DC // 4, B_DH), U32),
                vmem((NBLK // 2, 49, LANES // 2, LANES), U32),
                vmem((S, 2 * B_DH), BF16),
                vmem((2, S // 2, B_DH), U32),
                vmem((2, B_DH // 2, S), U32),
                vmem((PAIRS, S, 2 * B_DH), BF16),
                vmem((49, DM // 2, DM // 4), U32),
                vmem((49, DM // 8, DM // 4), U32),
                vmem((2, 2, HALF // PAIRS, 2 * DM), BF16),
                vmem((2, 4, 16, DM), BF16),
                vmem((49, DM // 8, DM // 4), U32),
                vmem((2, 2, A_HEADS, DM), U32),
                vmem((2, 4, 64, DM), BF16),
                vmem((2, BLK, DM), BF16),
                vmem((LOC_PANELS, HALO + BLK, LANES), F32),
                vmem((2, BLK, 2 * DM), BF16),
                pltpu.SemaphoreType.DMA((2, NBLK // 2)),
                pltpu.SemaphoreType.DMA((2, 3)),
                pltpu.SemaphoreType.DMA((2, 13)),
                pltpu.SemaphoreType.DMA((2,)),
                pltpu.SemaphoreType.DMA((2, 5)),
            ],
            compiler_params=pltpu.CompilerParams(vmem_limit_bytes=124 * 2 ** 20, flags=cfg.get("flags"),
                                                 disable_bounds_checks=cfg.get("nobc", False)),
            name="fused_local_and_latent_attention",
        )(A_x.reshape(S, DM), A_wqkv, A_wo.reshape(A_HEADS, A_DH, DM), B_x.reshape(S, DM), B_c_kv.reshape(S, B_DC),
          B_w_q, B_w_uk, B_w_uv, B_w_o.reshape(B_HEADS * B_DH, DM))
        return out.reshape(1, S, 2 * DM)

    return jax.jit(fn)


@jax.jit
def pallas_concat_heads__sliding_local_dilated__compressed_kv_cla__prompt_kernel(
    A_x: jax.Array,
    A_wqkv: jax.Array,
    A_wo: jax.Array,
    B_x: jax.Array,
    B_c_kv: jax.Array,
    B_w_q: jax.Array,
    B_w_uk: jax.Array,
    B_w_uv: jax.Array,
    B_w_o: jax.Array,
):
    return build(dict())(A_x, A_wqkv, A_wo, B_x, B_c_kv, B_w_q, B_w_uk, B_w_uv, B_w_o)
```

```python
import functools
import itertools

import jax
import jax.numpy as jnp
from jax import lax
import jax.experimental.pallas as pl
import jax.experimental.pallas.tpu as pltpu

S = 2048
DM = 1024
HALF, QUARTER = DM // 2, DM // 4
LANES = 128
A_HEADS, A_DH, A_WIN, A_DIL = 32, 32, 8, 2
HALO = 16
B_HEADS, B_DH, B_DC = 32, 128, 512
PAIRS = B_HEADS // 2

BLK = 256
SUB = BLK // 2
NBLK = S // BLK

LOG2E = 1.4426950408889634
NEG = -1e9
F32, BF16, U32 = jnp.float32, jnp.bfloat16, jnp.uint32

A_TERMS = (((1, 0, 0), (1, 1, 1)), ((1, 1, 0), (1, 1, 1)), ((1, 0, 0),), ((1, 1, 1),),
           ((1, 0, 0), (1, 0, 1)), ((1, 1, 0), (-1, 0, 0)), ((1, 0, 1), (-1, 1, 1)))
B_TERMS = (((1, 0, 0), (1, 1, 1)), ((1, 0, 0),), ((1, 0, 1), (-1, 1, 1)), ((1, 1, 0), (-1, 0, 0)),
           ((1, 1, 1),), ((1, 0, 0), (1, 0, 1)), ((1, 1, 0), (1, 1, 1)))
C_TERMS = (((1, 0, 0), (1, 1, 1)), ((1, 1, 0), (-1, 1, 1)), ((1, 0, 1), (1, 1, 1)), ((1, 0, 0), (1, 1, 0)),
           ((-1, 0, 0), (1, 0, 1)), ((1, 1, 1),), ((1, 0, 0),))

LOC_K, LOC_V, LOC_Q = 0, 8, 16

PAIR_STEPS = (
    ("s0", "k", "s1", "c0", "v", "q", "c1"),
    ("s0", "k", "s1", "q", "c0", "v", "c1"),
    ("s0", "s1", "k", "c0", "q", "c1", "v"),
    ("s0", "s1", "c0", "k", "q", "c1", "v"),
    ("s0", "v", "s1", "k", "c0", "q", "c1"),
    ("k", "s0", "v", "s1", "c0", "q", "c1"),
    ("s0", "s1", "k", "v", "c0", "q", "c1"),
    ("s0", "s1", "k", "v", "c0", "q", "c1"),
)
LAST_PAIR_STEPS = (
    (0, 7), (0, 1), (0, 0), (1, 7), (0, 6), (1, 0), (1, 6), (1, 1),
    (0, 5), (1, 5), (0, 4), (1, 2), (0, 2), (0, 3), (1, 4), (1, 3),
)
LAST_PAIR_LAG = 3
PRODUCT_ORDER = {
    "q": (2, 0, 4, 3, 6, 1, 5),
    "k": (6, 0, 3, 4, 1, 2, 5),
    "v inner": (0, 5, 1, 2, 3, 4, 6),
    "v outer": (2, 4, 0, 3, 6, 1, 5),
    "local qk": (0, 3, 4, 6, 1, 2, 5),
    "local v inner": (3, 1, 0, 6, 4, 2, 5),
    "local v outer": (3, 1, 2, 4, 0, 6, 5),
    "out b inner": (3, 1, 2, 4, 0, 6, 5),
    "out b outer": (2, 5, 0, 1, 3, 6, 4),
    "out a inner": (5, 2, 0, 4, 6, 3, 1),
    "out a outer": (0, 3, 4, 6, 1, 2, 5),
}
VALUE_SPLIT = 3
SOFTMAX_ROWS, SOFTMAX_PACE = 16, ((0, 0.6), (0.2, 0.9))
CONTEXT_KEYS, LAST_CONTEXT_KEYS = 1024, 2048
SLICE_JOBS, SLICE_BLOCKS = (4, 5, 6, 1, 0, 7, 3, 2), (6, 5, 4, 3, 2, 1)
LAST_SLICE_BLOCKS, LAST_SLICE_RATE = (6, 5, 4, 2, 0), 0.7
FINAL_JOBS, FINAL_RATE = (0, 1, 3, 2, 4), 16
LOCAL_PARTS, LOCAL_ROWS, LOCAL_STAGES, LOCAL_PACE = (2, 1, 0), 16, 8, (0, 0.92)
OUTPUT_DEPTH = DM // 8


def _pack(x):
    return pltpu.bitcast(x.astype(BF16), U32)


def _unpack(x):
    return pltpu.bitcast(x, BF16)


def _word_half(word, hi):
    return pltpu.bitcast(word & U32(0xFFFF0000) if hi else word << 16, F32)


def _dot(a, b):
    return jnp.dot(a, b, preferred_element_type=F32)


def _dot_nt(a, b):
    return lax.dot_general(a, b, (((1,), (1,)), ((), ())), preferred_element_type=F32)


def _reciprocal(x):
    r = pl.reciprocal(x, approx=True)
    return r * (2.0 - x * r)


def _operand_sums(block, terms):
    blocks = [[block(i, j) for j in range(2)] for i in range(2)]
    out = []
    for (_, i, j), *rest in terms:
        acc = blocks[i][j]
        for sign, i, j in rest:
            a, b = acc.astype(F32), blocks[i][j].astype(F32)
            acc = a + b if sign > 0 else a - b
        out.append(acc)
    return out


def _operand_sums2(block, terms):
    outer = [[_operand_sums(lambda i, j: block(2 * i + a, 2 * j + b), terms) for b in range(2)]
             for a in range(2)]
    return [functools.partial(_operand_sums, lambda a, b, r=r: outer[a][b][r], terms) for r in range(7)]


def _block_product(product, order, c=None):
    c = c or [[None, None], [None, None]]
    for r in order:
        m = product(r)
        for sign, i, j in C_TERMS[r]:
            if c[i][j] is None:
                c[i][j] = m if sign > 0 else -m
            else:
                c[i][j] = c[i][j] + m if sign > 0 else c[i][j] - m
    return c


def _join(c):
    return jnp.concatenate([jnp.concatenate(row, axis=1) for row in c], axis=0)


def _heads_to_lanes(groups):
    lane = lax.broadcasted_iota(jnp.int32, groups[0].shape, 1)
    groups = list(groups)
    for group_bit, lane_bit in ((2, 4), (1, 3), (0, 2), (2, 6), (2, 1), (1, 5), (1, 0)):
        shift = 1 << lane_bit
        low = (lane & shift) == 0
        for g in range(8):
            if g >> group_bit & 1:
                continue
            x, y = groups[g], groups[g | 1 << group_bit]
            groups[g] = jnp.where(low, x, pltpu.roll(y, shift, 1))
            groups[g | 1 << group_bit] = jnp.where(low, pltpu.roll(x, LANES - shift, 1), y)
    return [groups[(g & 1) << 2 | (g >> 2) << 1 | (g >> 1 & 1)] for g in range(8)]


class _Timeline:
    def __init__(self, never):
        self.never, self.now, self.marks = never, 0.0, []

    def issue(self, cycles, results):
        for n, value in enumerate(results):
            self.marks.append((self.now + cycles * (n + 1) / len(results), value))
        self.now += cycles

    def after(self, cycle, value):
        ready = [v for t, v in self.marks if t <= cycle]
        if not ready:
            return value
        mark = ready[-1][0:8, 0:value.shape[1]]
        if value.shape[0] > 8:
            mark = jnp.concatenate([mark] * (value.shape[0] // 8), axis=0)
        return jnp.where(self.never, mark, value)


class _Background:
    def __init__(self, never, pieces, rate):
        self.never, self.pending, self.rate, self.credit = never, pieces, rate, 0.0

    def tie(self, words):
        self.credit += self.rate
        due = [pltpu.bitcast(d, U32) for d in itertools.islice(self.pending, int(self.credit))]
        self.credit -= int(self.credit)
        if not due:
            return words
        mark = functools.reduce(jnp.bitwise_or, [
            d[r:r + 8, c:c + LANES]
            for d in due for r in range(0, d.shape[0], 8) for c in range(0, d.shape[1], LANES)])
        top = jnp.where(self.never, mark, words[:8, :LANES])
        if words.shape[1] > LANES:
            top = jnp.concatenate([top, words[:8, LANES:]], axis=1)
        return jnp.concatenate([top, words[8:]], axis=0)

    def finish(self):
        for _ in self.pending:
            pass


def _start(copies):
    for copy in copies:
        copy.start()


def _wait(copies):
    for copy in copies:
        copy.wait()


def _rows(start, size):
    return pl.ds(start if isinstance(start, int) else pl.multiple_of(start, size), size)


def _packed_rows(start, size):
    return _rows(start // 2, size // 2)


def _kernel(xa_hbm, wqkv_hbm, woa_hbm, xb_hbm, c_hbm, wq_hbm, wuk_hbm, wuv_hbm, wob_hbm,
            out_hbm,
            xb_raw, c_raw, wq_raw, wuk_raw, wuv_raw,
            x_sums, c_sums, ct_sums, wq_sums, wk_sums,
            q_s, k_s, vt_s, ctx,
            wqk_raw, wva_raw, woa_raw, wob_raw,
            wqk_sums, wva_sums, woa_sums, wob_sums,
            xa_raw, loc, obuf,
            sem_in, sem_pair, sem_slice, sem_xa, sem_out):
    wq_words, wuk_words, wuv_words = wq_hbm.bitcast(U32), wuk_hbm.bitcast(U32), wuv_hbm.bitcast(U32)
    woa_words = woa_hbm.bitcast(U32)

    def pair_copies(j, which=(0, 1, 2)):
        ends = ((wuk_words, wuk_raw), (wuv_words, wuv_raw), (wq_words, wq_raw))
        return [pltpu.make_async_copy(ends[n][0].at[:, j, :], ends[n][1].at[j % 2], sem_pair.at[j % 2, n])
                for n in which]

    def slice_copies(j):
        slot = j % 2
        ends = [(wqkv_hbm.at[_rows(k * HALF + j * 32, 32), 0:2 * DM], wqk_raw.at[slot, k]) for k in range(2)]
        ends += [(wqkv_hbm.at[_rows(k * QUARTER + j * 16, 16), 2 * DM:3 * DM], wva_raw.at[slot, k])
                 for k in range(4)]
        ends += [(woa_words.at[:, (j >> 1 & 1) | k << 1 | (j >> 2) << 2, :], woa_raw.at[slot, k])
                 for k in range(2)]
        ends += [(wob_hbm.at[_rows(k * DM + j * 64, 64), :], wob_raw.at[slot, k]) for k in range(4)]
        return [pltpu.make_async_copy(src, dst, sem_slice.at[slot]) for src, dst in ends]

    def latent_copy(n):
        rows = _rows(n * 2 * BLK, 2 * BLK)
        return pltpu.make_async_copy(c_hbm.at[rows, :], c_raw.at[rows, :], sem_in.at[0, n])

    def xb_copy(n):
        rows = _rows(n * 2 * BLK, 2 * BLK)
        return pltpu.make_async_copy(xb_hbm.at[rows, :], xb_raw.at[rows, :], sem_in.at[1, n])

    def xa_copy(i):
        return pltpu.make_async_copy(xa_hbm.at[_rows(i * BLK, BLK), :], xa_raw.at[i % 2], sem_xa.at[i % 2])

    def out_copy(i, part):
        r0, nr, c0, nc = (0, BLK, DM, DM) if part == 4 else (part // 2 * SUB, SUB, part % 2 * HALF, HALF)
        return pltpu.make_async_copy(obuf.at[i % 2, r0:r0 + nr, c0:c0 + nc],
                                     out_hbm.at[_rows(i * BLK + r0, nr), c0:c0 + nc], sem_out.at[i % 2])

    def prepare_weights(j, raw, dst):
        slot, depth = j % 2, raw.shape[1] // 2
        for r0 in range(0, depth, 32):
            words = [raw[slot, k * depth + r0:k * depth + r0 + 32, :] for k in range(2)]
            for r, op in enumerate(_operand_sums(lambda k, head: _word_half(words[k], head), B_TERMS)):
                dst[r, r0 // 2:r0 // 2 + 16, :] = _pack(op)

    def prepare_inputs(i, raw, dst):
        width = raw.shape[1] // 2
        ops = _operand_sums(
            lambda a, k: raw[_rows(i * BLK + a * SUB, SUB), k * width:(k + 1) * width], A_TERMS)
        ops = [_pack(op) for op in ops]
        for r, op in enumerate(ops):
            dst[r, _packed_rows(i * SUB, SUB), :] = op
        return ops

    def project(i, which, line=None, background=None, ops=None):
        lhs, rhs = (x_sums, wq_sums) if which == "q" else (c_sums, wk_sums)
        rows = _packed_rows(i * SUB, SUB)

        def product(r):
            w = rhs[r] if background is None else background.tie(rhs[r])
            m = _dot(_unpack(lhs[r, rows, :] if ops is None else ops[r]), _unpack(w))
            if line is not None:
                line.issue(SUB * rhs.shape[1] // 256, [m[SUB // 2 - 8:SUB // 2], m[SUB - 8:SUB]])
            return m

        c = _block_product(product, PRODUCT_ORDER[which])
        for a in range(2):
            if which == "q":
                q_s[_rows(i * BLK + a * SUB, SUB), :] = (
                    jnp.concatenate(c[a], axis=1) * (B_DH ** -0.5 * LOG2E)).astype(BF16)
            else:
                for head in range(2):
                    k_s[head, _packed_rows(i * BLK + a * SUB, SUB), :] = _pack(c[a][head])

    def value_weights(j):
        words = wuv_raw[j % 2].T

        def block(a, k):
            return _word_half(words[a % 2 * 64:(a % 2 + 1) * 64, k * LANES:(k + 1) * LANES], a // 2)

        return [[op.astype(BF16) for op in inner()] for inner in _operand_sums2(block, A_TERMS)]

    def prepare_latents(t):
        blocks = [[c_raw[_rows((4 * t + n) * LANES, LANES), k * LANES:(k + 1) * LANES].astype(F32).T
                   for n in range(4)] for k in range(4)]
        ops = [[_pack(op) for op in inner()] for inner in _operand_sums2(lambda k, n: blocks[k][n], B_TERMS)]
        for r in range(7):
            for u in range(7):
                ct_sums[t, 7 * r + u] = ops[r][u]
        return ops

    def project_values(t, weights, line=None, ops=None):
        def outer(r):
            def product(u):
                m = _dot(weights[r][u], _unpack(ct_sums[t, 7 * r + u] if ops is None else ops[r][u]))
                if line is not None:
                    line.issue(16, [m[-8:]])
                return m
            return _join(_block_product(product, PRODUCT_ORDER["v inner"]))

        c = _block_product(outer, PRODUCT_ORDER["v outer"][:VALUE_SPLIT])
        yield
        c = _block_product(outer, PRODUCT_ORDER["v outer"][VALUE_SPLIT:], c)
        for head in range(2):
            for n in range(2):
                vt_s[head, :, _rows((2 * t + n) * BLK, BLK)] = _pack(c[head][n])

    def scores(h, i, line):
        row = lax.broadcasted_iota(jnp.int32, (SUB, SUB), 0)
        col = lax.broadcasted_iota(jnp.int32, (SUB, SUB), 1)
        r0, cols = i * BLK, slice(h * B_DH, (h + 1) * B_DH)
        past = None
        if i:
            past = _dot_nt(q_s[r0:r0 + BLK, cols], _unpack(k_s[h, 0:r0 // 2, :]))
            line.issue(r0 // 2, [past[t % BLK:t % BLK + 8, t // BLK * LANES:(t // BLK + 1) * LANES]
                                 for t in range(56, r0 // 2, 64)])
        diagonal = []
        for a in range(2):
            d = _dot_nt(q_s[r0 + a * SUB:r0 + (a + 1) * SUB, cols],
                        _unpack(k_s[h, r0 // 2:(r0 + (a + 1) * SUB) // 2, :]))
            line.issue(32 * (a + 1), [d])
            last = jnp.where(col <= row, d[:, a * SUB:], NEG)
            diagonal.append(jnp.concatenate([d[:, :SUB], last], axis=1) if a else last)
        return past, diagonal, line.now

    def softmax(i, scored, line, pace):
        past, diagonal, t0 = scored
        span = line.now - t0
        p_past, p_diagonal, inverse = [], [], []
        for a in range(2):
            s = diagonal[a]
            if past is not None:
                s = jnp.concatenate([past[a * SUB:(a + 1) * SUB], s], axis=1)
            m = jnp.max(s, axis=1, keepdims=True)
            if pace is not None:
                lo, hi = pace
                m = jnp.concatenate([
                    line.after(t0 + span * (lo + (hi - lo) * (a * SUB + c) / BLK), m[c:c + SOFTMAX_ROWS])
                    for c in range(0, SUB, SOFTMAX_ROWS)], axis=0)
            p = jnp.exp2(s - m).astype(BF16)
            inverse.append(_reciprocal(jnp.sum(p.astype(F32), axis=1, keepdims=True)))
            if past is not None:
                p_past.append(p[:, :i * BLK])
            p_diagonal.append(p[:, i * BLK:])
        return (jnp.concatenate(p_past, axis=0) if p_past else None), p_diagonal, inverse

    def context(h, i, weights, line, keys, background):
        p_past, p_diagonal, inverse = weights
        r0 = i * BLK
        past = None
        for k0 in range(0, r0, keys):
            k1 = min(k0 + keys, r0)
            words = vt_s[h, :, k0:k1]
            if background is not None:
                words = jnp.concatenate(
                    [background.tie(words[:, t:t + LANES]) for t in range(0, k1 - k0, LANES)], axis=1)
            part = _dot_nt(p_past[:, k0:k1], _unpack(words))
            past = part if past is None else past + part
            line.issue((k1 - k0) // 2, [past[t:t + 8] for t in range(56, BLK, 64)])
        out = []
        for a in range(2):
            o = _dot_nt(p_diagonal[a], _unpack(vt_s[h, :, r0:r0 + (a + 1) * SUB]))
            line.issue(32 * (a + 1), [o])
            if past is not None:
                o = o + past[a * SUB:(a + 1) * SUB]
            out.append(o * inverse[a])
        return out

    def slice_work(j, jobs):
        slot = j % 2

        def query_or_key(part):
            groups = [_heads_to_lanes([
                _pack(wqk_raw[slot, k, :, part * DM + a * LANES:part * DM + (a + 1) * LANES])
                for a in range(8)]) for k in range(2)]
            rows = _packed_rows(part * HALF + j * 32, 32)
            for a in range(4):
                for r, op in enumerate(_operand_sums(lambda k, n: _unpack(groups[k][4 * n + a]), B_TERMS)):
                    op = _pack(op)
                    wqk_sums[r, rows, a * LANES:(a + 1) * LANES] = op
                    yield op

        def two_levels(block, dst, row0, cols):
            for r, inner in enumerate(_operand_sums2(block, B_TERMS)):
                for u, op in enumerate(inner()):
                    op = _pack(op)
                    dst[7 * r + u, _packed_rows(row0, 2 * op.shape[0]), cols] = op
                    yield op

        def value():
            groups = [_heads_to_lanes([_pack(wva_raw[slot, k, :, a * LANES:(a + 1) * LANES]) for a in range(8)])
                      for k in range(4)]
            return two_levels(lambda k, n: _unpack(jnp.concatenate(groups[k][2 * n:2 * n + 2], axis=1)),
                              wva_sums, j * 16, slice(None))

        def output_a():
            return two_levels(
                lambda k, n: _word_half(woa_raw[slot, k % 2, :, _rows(n * QUARTER + j % 2 * LANES, LANES)], k // 2),
                woa_sums, ((j >> 1 & 1) * 4 + (j >> 2)) * A_HEADS, _rows(j % 2 * LANES, LANES))

        def output_b(r0, c0):
            return two_levels(
                lambda k, n: wob_raw[slot, k, r0:r0 + 32, n * QUARTER + c0:n * QUARTER + c0 + LANES],
                wob_sums, j * 64 + r0, slice(c0, c0 + LANES))

        for n in jobs:
            if n < 4:
                yield from output_b(n // 2 * 32, n % 2 * LANES)
            elif n == 4:
                yield from output_a()
            else:
                yield from value() if n == 7 else query_or_key(n - 5)

    def first_steps(copy, work, requests):
        def step(n, carry):
            copy(n).wait()
            for at, copies in requests:
                pl.when(n == at)(lambda: _start(copies()))
            work(n)
            return carry

        lax.fori_loop(0, NBLK // 2, step, 0)

    def first_keys_and_values(weights, n):
        for i in (2 * n, 2 * n + 1):
            project(i, "k", ops=prepare_inputs(i, c_raw, c_sums))
        for _ in project_values(n, weights, ops=prepare_latents(n)):
            pass

    def first_queries(n):
        for i in (2 * n, 2 * n + 1):
            project(i, "q", ops=prepare_inputs(i, xb_raw, x_sums))

    _start(pair_copies(0, (0, 1)) + [latent_copy(0)])
    _wait(pair_copies(0, (0,)))
    _start([latent_copy(1), latent_copy(2), latent_copy(3)] + pair_copies(0, (2,)) + [xb_copy(0)])
    prepare_weights(0, wuk_raw, wk_sums)
    _wait(pair_copies(0, (1,)))
    first_steps(latent_copy, functools.partial(first_keys_and_values, value_weights(0)),
                ((1, lambda: [xb_copy(1), xb_copy(2)]), (2, lambda: [xb_copy(3)]), (3, lambda: pair_copies(1))))
    _wait(pair_copies(0, (2,)))
    prepare_weights(0, wq_raw, wq_sums)
    first_steps(xb_copy, first_queries, ((0, lambda: slice_copies(0)),))
    _wait(pair_copies(1) + slice_copies(0))
    _start(pair_copies(2) + slice_copies(1))

    def attention_steps(j, line, pace, keys, background):
        scored, done = {}, {}

        def begin(h, i):
            scored[h, i] = scores(h, i, line)

        def finish(h, i):
            weights = softmax(i, scored.pop((h, i)), line, pace and pace[h])
            done[h, i] = context(h, i, weights, line, keys, background(i))
            if (1 - h, i) in done:
                for a in range(2):
                    ctx[j, i * BLK + a * SUB:i * BLK + (a + 1) * SUB, :] = (
                        jnp.concatenate([done[0, i][a], done[1, i][a]], axis=1).astype(BF16))

        return begin, finish

    def head_pair(j, carry):
        prepare_weights(j + 1, wq_raw, wq_sums)
        prepare_weights(j + 1, wuk_raw, wk_sums)
        weights = value_weights(j + 1)
        line = _Timeline(j < 0)
        background = _Background(j < 0, slice_work(j, SLICE_JOBS), 350 / (14 * len(SLICE_BLOCKS)))
        values = [project_values(t, weights, line) for t in range(NBLK // 2)]
        begin, finish = attention_steps(j, line, SOFTMAX_PACE, CONTEXT_KEYS, lambda i: None)
        for i in range(NBLK - 1, -1, -1):
            for what in PAIR_STEPS[i]:
                if what[0] == "s":
                    begin(int(what[1]), i)
                elif what[0] == "c":
                    finish(int(what[1]), i)
                elif what == "q":
                    project(i, "q", line, background if i in SLICE_BLOCKS else None)
                elif what == "v":
                    if i + 2 < NBLK:
                        next(values[i // 2 + 1], None)
                elif i + 1 < NBLK:
                    project(i + 1, "k", line, background if i + 1 in SLICE_BLOCKS else None)
        project(0, "k", line, background if 0 in SLICE_BLOCKS else None)
        for _ in values[0]:
            pass
        background.finish()

        _wait(slice_copies(j + 1))
        pl.when(j + 2 < PAIRS)(lambda: _wait(pair_copies(j + 2)))
        pl.when(j + 3 < PAIRS)(lambda: _start(pair_copies(j + 3)))
        pl.when(j + 2 < PAIRS)(lambda: _start(slice_copies(j + 2)))
        return carry

    def last_head_pair(j, carry):
        _start([xa_copy(0), xa_copy(1)])
        line = _Timeline(j < 0)
        background = _Background(j < 0, slice_work(j, [n for n in SLICE_JOBS if n > 4]), LAST_SLICE_RATE)
        begin, finish = attention_steps(j, line, None, LAST_CONTEXT_KEYS,
                                        lambda i: background if i in LAST_SLICE_BLOCKS else None)
        for n, (h, i) in enumerate(LAST_PAIR_STEPS):
            begin(h, i)
            if n >= LAST_PAIR_LAG:
                finish(*LAST_PAIR_STEPS[n - LAST_PAIR_LAG])
        for h, i in LAST_PAIR_STEPS[-LAST_PAIR_LAG:]:
            finish(h, i)
        background.finish()
        return carry

    lax.fori_loop(0, PAIRS - 1, head_pair, 0)
    lax.fori_loop(PAIRS - 1, PAIRS, last_head_pair, 0)

    def store_blocks(i, col0, c):
        for a, n in ((0, 0), (1, 0), (0, 1), (1, 1)):
            obuf[i % 2, a * SUB:(a + 1) * SUB, col0 + n * HALF:col0 + (n + 1) * HALF] = c[a][n].astype(BF16)
            if col0 == 0:
                out_copy(i, 2 * a + n).start()
        if col0:
            out_copy(i, 4).start()

    def row_block(i, carry):
        xa_copy(i).wait()
        pl.when(i >= 2)(lambda: _wait([out_copy(i - 2, part) for part in range(5)]))
        loc[0:LOC_Q, 0:HALO, :] = loc[0:LOC_Q, BLK:BLK + HALO, :]

        x_ops = _operand_sums(
            lambda a, k: xa_raw[i % 2, a * SUB:(a + 1) * SUB, k * HALF:(k + 1) * HALF], A_TERMS)
        x_rounded = [op.astype(BF16) for op in x_ops]
        background = _Background(i < 0, slice_work(PAIRS - 1, FINAL_JOBS), FINAL_RATE)
        for part in LOCAL_PARTS:
            if part == 2:
                def value_product(r):
                    ops = _operand_sums(
                        lambda a, k: x_ops[r][64 * a:64 * (a + 1), QUARTER * k:QUARTER * (k + 1)], A_TERMS)
                    return _join(_block_product(
                        lambda u: _dot(ops[u].astype(BF16), _unpack(wva_sums[7 * r + u])),
                        PRODUCT_ORDER["local v inner"]))

                c = _block_product(value_product, PRODUCT_ORDER["local v outer"])
            else:
                rows = slice(part * HALF // 2, (part + 1) * HALF // 2)
                c = _block_product(lambda r: _dot(x_rounded[r], _unpack(background.tie(wqk_sums[r, rows, :]))),
                                   PRODUCT_ORDER["local qk"])
            for a in range(2):
                for g in range(8):
                    loc[(LOC_Q, LOC_K, LOC_V)[part] + g, HALO + a * SUB:HALO + (a + 1) * SUB, :] = (
                        c[a][g // 4][:, (g % 4) * LANES:(g % 4 + 1) * LANES])
        background.finish()

        def context_block(a, k):
            rows = _rows(i * BLK + a * (BLK // 4), BLK // 4)
            return jnp.concatenate(
                [ctx[j, rows, :] for j in range(k * PAIRS // 4, (k + 1) * PAIRS // 4)], axis=1).astype(F32)

        context_ops = _operand_sums2(context_block, A_TERMS)
        marks = []

        def output_product(r):
            ops = context_ops[r]()

            def product(u):
                acc = None
                for k0 in range(0, DM, OUTPUT_DEPTH):
                    part = _dot(ops[u][:, k0:k0 + OUTPUT_DEPTH].astype(BF16),
                                _unpack(wob_sums[7 * r + u, k0 // 2:(k0 + OUTPUT_DEPTH) // 2, :]))
                    acc = part if acc is None else acc + part
                    marks.append(acc)
                return acc

            return _join(_block_product(product, PRODUCT_ORDER["out b inner"]))

        store_blocks(i, DM, _block_product(output_product, PRODUCT_ORDER["out b outer"]))

        ticks = itertools.count()
        last_tick = LOCAL_STAGES * BLK // LOCAL_ROWS - 1

        def paced(values):
            lo, hi = LOCAL_PACE
            mark = marks[int((lo + (hi - lo) * next(ticks) / last_tick) * (len(marks) - 1))]
            return [jnp.where(i < 0, mark[0:LOCAL_ROWS, 0:LANES], v) for v in values]

        def attend(c0):
            def shifted(base, g, w):
                r0 = HALO + c0 - A_DIL * w
                return loc[base + g, r0:r0 + LOCAL_ROWS, :]

            every = 16 // LOCAL_STAGES
            queries = [shifted(LOC_Q, g, 0) for g in range(8)]
            logits = []
            for w in range(A_WIN):
                if w % every == 0:
                    q = paced(queries)
                acc = q[0] * shifted(LOC_K, 0, w)
                for g in range(1, 8):
                    acc = acc + q[g] * shifted(LOC_K, g, w)
                acc = acc + pltpu.roll(acc, 2 * A_HEADS, 1)
                acc = acc + pltpu.roll(acc, A_HEADS, 1)
                if c0 < A_DIL * w:
                    pos = i * BLK + c0 + lax.broadcasted_iota(jnp.int32, (LOCAL_ROWS, LANES), 0)
                    acc = jnp.where(pos >= A_DIL * w, acc, NEG * A_DH ** 0.5)
                logits.append(acc)
            m = functools.reduce(jnp.maximum, logits)
            p = [jnp.exp2((l - m) * (A_DH ** -0.5 * LOG2E)) for l in logits]
            inverse = _reciprocal(functools.reduce(jnp.add, p))
            p = [t * inverse for t in p]
            out = []
            for g in range(8):
                if g % every == 0:
                    weights = paced(p)
                out.append(functools.reduce(
                    jnp.add, [weights[w] * shifted(LOC_V, g, w) for w in range(A_WIN)]))
            return out

        quarters = [[] for _ in range(4)]
        for c0 in range(0, BLK // 4, LOCAL_ROWS):
            for a in range(4):
                quarters[a].append(jnp.concatenate(attend(a * (BLK // 4) + c0), axis=1))
        quarters = [jnp.concatenate(rows, axis=0) for rows in quarters]

        local_ops = _operand_sums2(lambda a, k: quarters[a][:, k * QUARTER:(k + 1) * QUARTER], A_TERMS)

        def local_product(r):
            ops = local_ops[r]()
            return _join(_block_product(
                lambda u: _dot(ops[u].astype(BF16), _unpack(woa_sums[7 * r + u])), PRODUCT_ORDER["out a inner"]))

        store_blocks(i, 0, _block_product(local_product, PRODUCT_ORDER["out a outer"]))
        pl.when(i + 2 < NBLK)(lambda: xa_copy(i + 2).start())
        return carry

    loc[0:LOC_Q, BLK:BLK + HALO, :] = jnp.zeros((LOC_Q, HALO, LANES), F32)
    lax.fori_loop(0, NBLK, row_block, 0)
    _wait([out_copy(i, part) for i in (NBLK - 2, NBLK - 1) for part in range(5)])


@jax.jit
def pallas_concat_heads__sliding_local_dilated__compressed_kv_cla__prompt_kernel(
    A_x: jax.Array,
    A_wqkv: jax.Array,
    A_wo: jax.Array,
    B_x: jax.Array,
    B_c_kv: jax.Array,
    B_w_q: jax.Array,
    B_w_uk: jax.Array,
    B_w_uv: jax.Array,
    B_w_o: jax.Array,
):
    vmem, sems = pltpu.VMEM, pltpu.SemaphoreType.DMA
    out = pl.pallas_call(
        _kernel,
        out_shape=jax.ShapeDtypeStruct((S, 2 * DM), BF16),
        in_specs=[pl.BlockSpec(memory_space=pl.ANY)] * 9,
        out_specs=pl.BlockSpec(memory_space=pl.ANY),
        scratch_shapes=[
            vmem((S, DM), BF16),
            vmem((S, B_DC), BF16),
            vmem((2, DM, B_DH), U32),
            vmem((2, B_DC, B_DH), U32),
            vmem((2, B_DC, B_DH), U32),
            vmem((7, S // 4, HALF), U32),
            vmem((7, S // 4, B_DC // 2), U32),
            vmem((NBLK // 2, 49, LANES // 2, LANES), U32),
            vmem((7, DM // 4, B_DH), U32),
            vmem((7, B_DC // 4, B_DH), U32),
            vmem((S, 2 * B_DH), BF16),
            vmem((2, S // 2, B_DH), U32),
            vmem((2, B_DH // 2, S), U32),
            vmem((PAIRS, S, 2 * B_DH), BF16),
            vmem((2, 2, 32, 2 * DM), BF16),
            vmem((2, 4, 16, DM), BF16),
            vmem((2, 2, A_HEADS, DM), U32),
            vmem((2, 4, 64, DM), BF16),
            vmem((7, HALF, HALF), U32),
            vmem((49, QUARTER // 2, QUARTER), U32),
            vmem((49, QUARTER // 2, QUARTER), U32),
            vmem((49, DM // 2, QUARTER), U32),
            vmem((2, BLK, DM), BF16),
            vmem((LOC_Q + 8, HALO + BLK, LANES), F32),
            vmem((2, BLK, 2 * DM), BF16),
            sems((2, NBLK // 2)), sems((2, 3)), sems((2,)), sems((2,)), sems((2,)),
        ],
        compiler_params=pltpu.CompilerParams(vmem_limit_bytes=120 * 2 ** 20, disable_bounds_checks=True),
        name="local_and_latent_attention",
    )(A_x.reshape(S, DM), A_wqkv, A_wo.reshape(A_HEADS, A_DH, DM), B_x.reshape(S, DM),
      B_c_kv.reshape(S, B_DC), B_w_q, B_w_uk, B_w_uv, B_w_o.reshape(B_HEADS * B_DH, DM))
    return out.reshape(1, S, 2 * DM)
```

```python
import functools
import itertools

import jax
import jax.numpy as jnp
from jax import lax
import jax.experimental.pallas as pl
import jax.experimental.pallas.tpu as pltpu

S = 2048
DM = 1024
HALF, QUARTER = DM // 2, DM // 4
LANES = 128
A_HEADS, A_DH, A_WIN, A_DIL = 32, 32, 8, 2
HALO = 16
B_HEADS, B_DH, B_DC = 32, 128, 512
PAIRS = B_HEADS // 2

BLK = 256
SUB = BLK // 2
NBLK = S // BLK

LOG2E = 1.4426950408889634
NEG = -1e9
F32, BF16, U32 = jnp.float32, jnp.bfloat16, jnp.uint32

A_TERMS = (((1, 0, 0), (1, 1, 1)), ((1, 1, 0), (1, 1, 1)), ((1, 0, 0),), ((1, 1, 1),),
           ((1, 0, 0), (1, 0, 1)), ((1, 1, 0), (-1, 0, 0)), ((1, 0, 1), (-1, 1, 1)))
B_TERMS = (((1, 0, 0), (1, 1, 1)), ((1, 0, 0),), ((1, 0, 1), (-1, 1, 1)), ((1, 1, 0), (-1, 0, 0)),
           ((1, 1, 1),), ((1, 0, 0), (1, 0, 1)), ((1, 1, 0), (1, 1, 1)))
C_TERMS = (((1, 0, 0), (1, 1, 1)), ((1, 1, 0), (-1, 1, 1)), ((1, 0, 1), (1, 1, 1)), ((1, 0, 0), (1, 1, 0)),
           ((-1, 0, 0), (1, 0, 1)), ((1, 1, 1),), ((1, 0, 0),))

HK_A, HK_B, HK_C = zip(
    (((1, 0, 0), (-1, 0, 1), (-1, 2, 0)), ((1, 0, 0), (-1, 0, 1)), ((1, 0, 0),)),
    (((1, 0, 0), (-1, 0, 2), (-1, 1, 0)), ((1, 0, 1),), ((1, 0, 0), (1, 0, 1))),
    (((1, 0, 3), (1, 1, 1), (-1, 1, 0), (-1, 1, 3), (-1, 2, 1)), ((1, 1, 0),), ((1, 1, 0),)),
    (((1, 1, 1), (1, 3, 0), (-1, 0, 1), (-1, 1, 2), (-1, 3, 1)), ((1, 1, 1),), ((1, 1, 1),)),
    (((1, 1, 0), (-1, 0, 3)), ((1, 0, 0), (1, 1, 0)), ((1, 0, 0), (1, 0, 1), (1, 1, 0), (1, 1, 1))),
    (((1, 0, 1), (-1, 3, 0)), ((1, 0, 1), (1, 1, 1), (-1, 0, 0), (-1, 1, 0)), ((1, 0, 1), (1, 1, 1))),
    (((1, 0, 1), (-1, 1, 0)), ((1, 0, 0), (1, 1, 0), (-1, 0, 1)), ((1, 0, 0), (1, 0, 1), (1, 1, 1))),
    (((1, 3, 0), (1, 3, 3), (-1, 0, 3), (-1, 2, 3), (-1, 3, 1)), ((1, 3, 0), (-1, 3, 1)), ((1, 3, 0),)),
    (((1, 0, 3), (1, 3, 3), (-1, 1, 3), (-1, 3, 0), (-1, 3, 2)), ((1, 3, 1),), ((1, 3, 0), (1, 3, 1))),
    (((1, 0, 3),), ((1, 0, 0), (1, 1, 0), (1, 3, 0)), ((1, 0, 0), (1, 1, 0), (1, 3, 0))),
    (((1, 3, 0),), ((1, 0, 1), (1, 1, 1), (1, 3, 1)), ((1, 0, 1), (1, 1, 1), (1, 3, 1))),
    (((1, 0, 3), (-1, 3, 0)), ((1, 0, 0), (1, 1, 0), (1, 3, 1)), ((1, 0, 1), (1, 1, 1), (-1, 3, 0))),
    (((1, 1, 3), (-1, 0, 3)), ((1, 1, 0), (1, 3, 0)), ((1, 1, 0), (1, 1, 1), (1, 3, 0), (1, 3, 1))),
    (((1, 3, 1), (-1, 3, 0)), ((1, 1, 1), (1, 3, 1), (-1, 1, 0), (-1, 3, 0)), ((1, 1, 1), (1, 3, 1))),
    (((1, 0, 3), (1, 3, 1), (-1, 1, 3), (-1, 3, 0)),
     ((1, 1, 0), (1, 3, 0), (-1, 3, 1)), ((1, 1, 1), (1, 3, 0), (1, 3, 1))),
    (((1, 2, 2), (-1, 1, 2), (-1, 2, 0), (-1, 2, 3)), ((1, 2, 0),), ((1, 2, 0), (1, 2, 1))),
    (((1, 2, 2), (-1, 0, 2), (-1, 2, 1), (-1, 3, 2)), ((1, 2, 1), (-1, 2, 0)), ((1, 2, 1),)),
    (((1, 2, 0),), ((1, 0, 0), (1, 2, 0)), ((1, 0, 0), (1, 2, 0))),
    (((1, 0, 2),), ((1, 0, 1), (1, 2, 1)), ((1, 0, 1), (1, 2, 1))),
    (((1, 0, 2), (-1, 2, 0)), ((1, 0, 1), (1, 2, 0)), ((1, 0, 0), (-1, 2, 1))),
    (((1, 2, 1),), ((1, 1, 0), (1, 2, 0), (-1, 1, 1), (-1, 2, 1)), ((1, 1, 0), (1, 2, 0))),
    (((1, 1, 2),), ((1, 1, 1), (1, 2, 1)), ((1, 1, 0), (1, 1, 1), (1, 2, 0), (1, 2, 1))),
    (((1, 2, 1), (-1, 1, 2)), ((1, 1, 1), (1, 2, 1), (-1, 2, 0)), ((1, 1, 0), (1, 2, 0), (1, 2, 1))),
    (((1, 2, 3),), ((1, 2, 0), (1, 3, 0)), ((1, 2, 0), (1, 3, 0))),
    (((1, 3, 2),), ((1, 2, 1), (1, 3, 1)), ((1, 2, 1), (1, 3, 1))),
    (((1, 2, 3), (-1, 3, 2)), ((1, 2, 0), (1, 3, 1)), ((1, 2, 1), (-1, 3, 0))),
)

LOC_K, LOC_V, LOC_Q = 0, 8, 16

PAIR_STEPS = (
    ("s0", "k", "s1", "c0", "v", "q", "c1"),
    ("s0", "s1", "q", "c0", "k", "v", "c1"),
    ("s0", "s1", "k", "c0", "q", "c1", "v"),
    ("s0", "s1", "c0", "k", "q", "c1", "v"),
    ("s0", "v", "s1", "k", "c0", "q", "c1"),
    ("s0", "s1", "k", "c0", "q", "c1", "v"),
    ("s0", "s1", "k", "v", "c0", "q", "c1"),
    ("s0", "s1", "k", "c0", "v", "c1", "q"),
)
LAST_PAIR_STEPS = (
    (0, 7), (0, 1), (0, 0), (1, 7), (0, 6), (1, 0), (1, 6), (1, 1),
    (0, 5), (1, 5), (0, 4), (1, 2), (0, 2), (0, 3), (1, 4), (1, 3),
)
LAST_PAIR_LAG = 3
PRODUCT_ORDER = {
    "q": (1, 3, 0, 2, 4, 5, 11, 6, 7, 8, 9, 10, 12, 13, 14, 15, 16, 17, 18, 19, 20, 21, 22, 23, 24, 25),
    "k": (6, 0, 3, 4, 1, 2, 5),
    "v inner": (5, 2, 0, 4, 6, 3, 1),
    "v outer": (2, 4, 0, 3, 6, 1, 5),
    "local qk": (0, 3, 4, 6, 1, 2, 5),
    "local v inner": (3, 1, 0, 6, 4, 2, 5),
    "local v outer": (3, 1, 2, 4, 0, 6, 5),
    "out b inner": (3, 1, 2, 4, 0, 6, 5),
    "out b outer": (2, 5, 0, 1, 3, 6, 4),
    "out a inner": (5, 2, 0, 4, 6, 3, 1),
    "out a outer": (0, 3, 4, 6, 1, 2, 5),
}
VALUE_SPLIT = 3
CONTEXT_KEYS, LAST_CONTEXT_KEYS = 1024, 2048
SLICE_JOBS, SLICE_BLOCKS = (4, 5, 6, 1, 3, 7, 0, 2), (6, 5, 4, 3, 2, 1)
LAST_SLICE_BLOCKS, LAST_SLICE_RATE = (6, 5, 4, 2, 0), 0.7
FINAL_JOBS, FINAL_RATE = (0, 1, 3, 2, 4), 16
LOCAL_PARTS, LOCAL_ROWS, LOCAL_STAGES, LOCAL_PACE = (2, 1, 0), 16, 8, (0, 0.92)
OUTPUT_DEPTH = DM // 8


def _pack(x):
    return pltpu.bitcast(x.astype(BF16), U32)


def _unpack(x):
    return pltpu.bitcast(x, BF16)


def _word_half(word, hi):
    return pltpu.bitcast(word & U32(0xFFFF0000) if hi else word << 16, F32)


def _dot(a, b):
    return jnp.dot(a, b, preferred_element_type=F32)


def _dot_nt(a, b):
    return lax.dot_general(a, b, (((1,), (1,)), ((), ())), preferred_element_type=F32)


def _reciprocal(x):
    r = pl.reciprocal(x, approx=True)
    return r * (2.0 - x * r)


def _operand_sums(block, terms, shape=(2, 2)):
    blocks = [[block(i, j) for j in range(shape[1])] for i in range(shape[0])]
    out = []
    for (_, i, j), *rest in terms:
        acc = blocks[i][j]
        for sign, i, j in rest:
            a, b = acc.astype(F32), blocks[i][j].astype(F32)
            acc = a + b if sign > 0 else a - b
        out.append(acc)
    return out


def _operand_sums2(block, terms):
    outer = [[_operand_sums(lambda i, j: block(2 * i + a, 2 * j + b), terms) for b in range(2)]
             for a in range(2)]
    return [functools.partial(_operand_sums, lambda a, b, r=r: outer[a][b][r], terms) for r in range(7)]


def _block_product(product, order, c=None, terms=C_TERMS):
    c = c or [[None, None], [None, None]]
    for r in order:
        m = product(r)
        for sign, i, j in terms[r]:
            if c[i][j] is None:
                c[i][j] = m if sign > 0 else -m
            else:
                c[i][j] = c[i][j] + m if sign > 0 else c[i][j] - m
    return c


def _join(c):
    return jnp.concatenate([jnp.concatenate(row, axis=1) for row in c], axis=0)


def _heads_to_lanes(groups):
    lane = lax.broadcasted_iota(jnp.int32, groups[0].shape, 1)
    groups = list(groups)
    for group_bit, lane_bit in ((2, 4), (1, 3), (0, 2), (2, 6), (2, 1), (1, 5), (1, 0)):
        shift = 1 << lane_bit
        low = (lane & shift) == 0
        for g in range(8):
            if g >> group_bit & 1:
                continue
            x, y = groups[g], groups[g | 1 << group_bit]
            groups[g] = jnp.where(low, x, pltpu.roll(y, shift, 1))
            groups[g | 1 << group_bit] = jnp.where(low, pltpu.roll(x, LANES - shift, 1), y)
    return [groups[(g & 1) << 2 | (g >> 2) << 1 | (g >> 1 & 1)] for g in range(8)]


class _Background:
    def __init__(self, never, pieces, rate):
        self.never, self.pending, self.rate, self.credit = never, pieces, rate, 0.0

    def tie(self, words):
        self.credit += self.rate
        due = [pltpu.bitcast(d, U32) for d in itertools.islice(self.pending, int(self.credit))]
        self.credit -= int(self.credit)
        if not due:
            return words
        mark = functools.reduce(jnp.bitwise_or, [
            d[r:r + 8, c:c + LANES]
            for d in due for r in range(0, d.shape[0], 8) for c in range(0, d.shape[1], LANES)])
        top = jnp.where(self.never, mark, words[:8, :LANES])
        if words.shape[1] > LANES:
            top = jnp.concatenate([top, words[:8, LANES:]], axis=1)
        return jnp.concatenate([top, words[8:]], axis=0)

    def finish(self):
        for _ in self.pending:
            pass


def _start(copies):
    for copy in copies:
        copy.start()


def _wait(copies):
    for copy in copies:
        copy.wait()


def _rows(start, size):
    return pl.ds(start if isinstance(start, int) else pl.multiple_of(start, size), size)


def _packed_rows(start, size):
    return _rows(start // 2, size // 2)


def _kernel(xa_hbm, wqkv_hbm, woa_hbm, xb_hbm, c_hbm, wq_hbm, wuk_hbm, wuv_hbm, wob_hbm,
            out_hbm,
            xb_raw, c_raw, wq_raw, wuk_raw, wuv_raw,
            x_sums, c_sums, ct_sums, wq_sums, wk_sums,
            q_s, k_s, vt_s, ctx,
            wqk_raw, wva_raw, woa_raw, wob_raw,
            wqk_sums, wva_sums, woa_sums, wob_sums,
            xa_raw, loc, obuf,
            sem_in, sem_pair, sem_slice, sem_xa, sem_out):
    wq_words, wuk_words, wuv_words = wq_hbm.bitcast(U32), wuk_hbm.bitcast(U32), wuv_hbm.bitcast(U32)
    woa_words = woa_hbm.bitcast(U32)

    def pair_copies(j, which=(0, 1, 2)):
        ends = ((wuk_words, wuk_raw), (wuv_words, wuv_raw), (wq_words, wq_raw))
        return [pltpu.make_async_copy(ends[n][0].at[:, j, :], ends[n][1].at[j % 2], sem_pair.at[j % 2, n])
                for n in which]

    def slice_copies(j):
        slot = j % 2
        ends = [(wqkv_hbm.at[_rows(k * HALF + j * 32, 32), 0:2 * DM], wqk_raw.at[slot, k]) for k in range(2)]
        ends += [(wqkv_hbm.at[_rows(k * QUARTER + j * 16, 16), 2 * DM:3 * DM], wva_raw.at[slot, k])
                 for k in range(4)]
        ends += [(woa_words.at[:, (j >> 1 & 1) | k << 1 | (j >> 2) << 2, :], woa_raw.at[slot, k])
                 for k in range(2)]
        ends += [(wob_hbm.at[_rows(k * DM + j * 64, 64), :], wob_raw.at[slot, k]) for k in range(4)]
        return [pltpu.make_async_copy(src, dst, sem_slice.at[slot]) for src, dst in ends]

    def latent_copy(n):
        rows = _rows(n * 2 * BLK, 2 * BLK)
        return pltpu.make_async_copy(c_hbm.at[rows, :], c_raw.at[rows, :], sem_in.at[0, n])

    def xb_copy(n):
        rows = _rows(n * 2 * BLK, 2 * BLK)
        return pltpu.make_async_copy(xb_hbm.at[rows, :], xb_raw.at[rows, :], sem_in.at[1, n])

    def xa_copy(i):
        return pltpu.make_async_copy(xa_hbm.at[_rows(i * BLK, BLK), :], xa_raw.at[i % 2], sem_xa.at[i % 2])

    def out_copy(i, part):
        r0, nr, c0, nc = (0, BLK, DM, DM) if part == 4 else (part // 2 * SUB, SUB, part % 2 * HALF, HALF)
        return pltpu.make_async_copy(obuf.at[i % 2, r0:r0 + nr, c0:c0 + nc],
                                     out_hbm.at[_rows(i * BLK + r0, nr), c0:c0 + nc], sem_out.at[i % 2])

    def prepare_weights(j, raw, dst, terms, parts):
        slot, depth = j % 2, raw.shape[1] // parts
        for r0 in range(0, depth, 32):
            words = [raw[slot, k * depth + r0:k * depth + r0 + 32, :] for k in range(parts)]
            for r, op in enumerate(_operand_sums(lambda k, head: _word_half(words[k], head), terms, (parts, 2))):
                dst[r, r0 // 2:r0 // 2 + 16, :] = _pack(op)

    def prepare_inputs(i, raw, dst, terms, parts):
        rows, width = BLK // parts, raw.shape[1] // parts
        ops = _operand_sums(lambda a, k: raw[_rows(i * BLK + a * rows, rows), k * width:(k + 1) * width],
                            terms, (parts, parts))
        ops = [_pack(op) for op in ops]
        for r, op in enumerate(ops):
            dst[r, _packed_rows(i * rows, rows), :] = op
        return ops

    def project_queries(i, background=None, ops=None):
        def product(r):
            w = wq_sums[r] if background is None else background.tie(wq_sums[r])
            return _dot(_unpack(x_sums[r, _packed_rows(i * 64, 64), :] if ops is None else ops[r]), _unpack(w))

        c = _block_product(product, PRODUCT_ORDER["q"], [[None, None] for _ in range(4)], HK_C)
        for a in range(4):
            q_s[_rows(i * BLK + a * 64, 64), :] = (
                jnp.concatenate(c[a], axis=1) * (B_DH ** -0.5 * LOG2E)).astype(BF16)

    def project_keys(i, background=None, ops=None):
        def product(r):
            w = wk_sums[r] if background is None else background.tie(wk_sums[r])
            return _dot(_unpack(c_sums[r, _packed_rows(i * SUB, SUB), :] if ops is None else ops[r]), _unpack(w))

        c = _block_product(product, PRODUCT_ORDER["k"])
        for a in range(2):
            for head in range(2):
                k_s[head, _packed_rows(i * BLK + a * SUB, SUB), :] = _pack(c[a][head])

    def value_weights(j):
        words = wuv_raw[j % 2].T

        def block(a, k):
            return _word_half(words[a % 2 * 64:(a % 2 + 1) * 64, k * LANES:(k + 1) * LANES], a // 2)

        return [[op.astype(BF16) for op in inner()] for inner in _operand_sums2(block, A_TERMS)]

    def prepare_latents(t):
        blocks = [[c_raw[_rows((4 * t + n) * LANES, LANES), k * LANES:(k + 1) * LANES].astype(F32).T
                   for n in range(4)] for k in range(4)]
        ops = [[_pack(op) for op in inner()] for inner in _operand_sums2(lambda k, n: blocks[k][n], B_TERMS)]
        for r in range(7):
            for u in range(7):
                ct_sums[t, 7 * r + u] = ops[r][u]
        return ops

    def project_values(t, weights, ops=None):
        def outer(r):
            return _join(_block_product(
                lambda u: _dot(weights[r][u], _unpack(ct_sums[t, 7 * r + u] if ops is None else ops[r][u])),
                PRODUCT_ORDER["v inner"]))

        c = _block_product(outer, PRODUCT_ORDER["v outer"][:VALUE_SPLIT])
        yield
        c = _block_product(outer, PRODUCT_ORDER["v outer"][VALUE_SPLIT:], c)
        for head in range(2):
            for n in range(2):
                vt_s[head, :, _rows((2 * t + n) * BLK, BLK)] = _pack(c[head][n])

    def scores(h, i):
        row = lax.broadcasted_iota(jnp.int32, (SUB, SUB), 0)
        col = lax.broadcasted_iota(jnp.int32, (SUB, SUB), 1)
        r0, cols = i * BLK, slice(h * B_DH, (h + 1) * B_DH)
        past = _dot_nt(q_s[r0:r0 + BLK, cols], _unpack(k_s[h, 0:r0 // 2, :])) if i else None
        diagonal = []
        for a in range(2):
            d = _dot_nt(q_s[r0 + a * SUB:r0 + (a + 1) * SUB, cols],
                        _unpack(k_s[h, r0 // 2:(r0 + (a + 1) * SUB) // 2, :]))
            last = jnp.where(col <= row, d[:, a * SUB:], NEG)
            diagonal.append(jnp.concatenate([d[:, :SUB], last], axis=1) if a else last)
        return past, diagonal

    def softmax(i, past, diagonal):
        p_past, p_diagonal, inverse = [], [], []
        for a in range(2):
            s = diagonal[a]
            if past is not None:
                s = jnp.concatenate([past[a * SUB:(a + 1) * SUB], s], axis=1)
            p = jnp.exp2(s - jnp.max(s, axis=1, keepdims=True)).astype(BF16)
            inverse.append(_reciprocal(jnp.sum(p.astype(F32), axis=1, keepdims=True)))
            if past is not None:
                p_past.append(p[:, :i * BLK])
            p_diagonal.append(p[:, i * BLK:])
        return (jnp.concatenate(p_past, axis=0) if p_past else None), p_diagonal, inverse

    def context(h, i, weights, keys, background):
        p_past, p_diagonal, inverse = weights
        r0 = i * BLK
        past = None
        for k0 in range(0, r0, keys):
            k1 = min(k0 + keys, r0)
            words = vt_s[h, :, k0:k1]
            if background is not None:
                words = jnp.concatenate(
                    [background.tie(words[:, t:t + LANES]) for t in range(0, k1 - k0, LANES)], axis=1)
            part = _dot_nt(p_past[:, k0:k1], _unpack(words))
            past = part if past is None else past + part
        out = []
        for a in range(2):
            o = _dot_nt(p_diagonal[a], _unpack(vt_s[h, :, r0:r0 + (a + 1) * SUB]))
            if past is not None:
                o = o + past[a * SUB:(a + 1) * SUB]
            out.append(o * inverse[a])
        return out

    def slice_work(j, jobs):
        slot = j % 2

        def query_or_key(part):
            groups = [_heads_to_lanes([
                _pack(wqk_raw[slot, k, :, part * DM + a * LANES:part * DM + (a + 1) * LANES])
                for a in range(8)]) for k in range(2)]
            rows = _packed_rows(part * HALF + j * 32, 32)
            for a in range(4):
                for r, op in enumerate(_operand_sums(lambda k, n: _unpack(groups[k][4 * n + a]), B_TERMS)):
                    op = _pack(op)
                    wqk_sums[r, rows, a * LANES:(a + 1) * LANES] = op
                    yield op

        def two_levels(block, dst, row0, cols):
            for r, inner in enumerate(_operand_sums2(block, B_TERMS)):
                for u, op in enumerate(inner()):
                    op = _pack(op)
                    dst[7 * r + u, _packed_rows(row0, 2 * op.shape[0]), cols] = op
                    yield op

        def value():
            groups = [_heads_to_lanes([_pack(wva_raw[slot, k, :, a * LANES:(a + 1) * LANES]) for a in range(8)])
                      for k in range(4)]
            return two_levels(lambda k, n: _unpack(jnp.concatenate(groups[k][2 * n:2 * n + 2], axis=1)),
                              wva_sums, j * 16, slice(None))

        def output_a():
            return two_levels(
                lambda k, n: _word_half(woa_raw[slot, k % 2, :, _rows(n * QUARTER + j % 2 * LANES, LANES)], k // 2),
                woa_sums, ((j >> 1 & 1) * 4 + (j >> 2)) * A_HEADS, _rows(j % 2 * LANES, LANES))

        def output_b(r0, c0):
            return two_levels(
                lambda k, n: wob_raw[slot, k, r0:r0 + 32, n * QUARTER + c0:n * QUARTER + c0 + LANES],
                wob_sums, j * 64 + r0, slice(c0, c0 + LANES))

        for n in jobs:
            if n < 4:
                yield from output_b(n // 2 * 32, n % 2 * LANES)
            elif n == 4:
                yield from output_a()
            else:
                yield from value() if n == 7 else query_or_key(n - 5)

    def first_steps(copy, work, requests):
        def step(n, carry):
            copy(n).wait()
            for at, copies in requests:
                pl.when(n == at)(lambda: _start(copies()))
            work(n)
            return carry

        lax.fori_loop(0, NBLK // 2, step, 0)

    def first_keys_and_values(weights, n):
        for i in (2 * n, 2 * n + 1):
            project_keys(i, ops=prepare_inputs(i, c_raw, c_sums, A_TERMS, 2))
        for _ in project_values(n, weights, ops=prepare_latents(n)):
            pass

    def first_queries(n):
        for i in (2 * n, 2 * n + 1):
            project_queries(i, ops=prepare_inputs(i, xb_raw, x_sums, HK_A, 4))

    _start(pair_copies(0, (0, 1)) + [latent_copy(0)])
    _wait(pair_copies(0, (0,)))
    _start([latent_copy(1), latent_copy(2), latent_copy(3)] + pair_copies(0, (2,)) + [xb_copy(0)])
    prepare_weights(0, wuk_raw, wk_sums, B_TERMS, 2)
    _wait(pair_copies(0, (1,)))
    first_steps(latent_copy, functools.partial(first_keys_and_values, value_weights(0)),
                ((1, lambda: [xb_copy(1), xb_copy(2)]), (2, lambda: [xb_copy(3)]), (3, lambda: pair_copies(1))))
    _wait(pair_copies(0, (2,)))
    prepare_weights(0, wq_raw, wq_sums, HK_B, 4)
    first_steps(xb_copy, first_queries, ((0, lambda: slice_copies(0)),))
    _wait(pair_copies(1) + slice_copies(0))
    _start(pair_copies(2) + slice_copies(1))

    def attention_steps(j, keys, background):
        scored, done = {}, {}

        def begin(h, i):
            scored[h, i] = scores(h, i)

        def finish(h, i):
            done[h, i] = context(h, i, softmax(i, *scored.pop((h, i))), keys, background(i))
            if (1 - h, i) in done:
                for a in range(2):
                    ctx[j, i * BLK + a * SUB:i * BLK + (a + 1) * SUB, :] = (
                        jnp.concatenate([done[0, i][a], done[1, i][a]], axis=1).astype(BF16))

        return begin, finish

    def head_pair(j, carry):
        prepare_weights(j + 1, wq_raw, wq_sums, HK_B, 4)
        prepare_weights(j + 1, wuk_raw, wk_sums, B_TERMS, 2)
        weights = value_weights(j + 1)
        background = _Background(j < 0, slice_work(j, SLICE_JOBS), 350 / (33 * len(SLICE_BLOCKS)))
        values = [project_values(t, weights) for t in range(NBLK // 2)]
        begin, finish = attention_steps(j, CONTEXT_KEYS, lambda i: None)
        for i in range(NBLK - 1, -1, -1):
            for what in PAIR_STEPS[i]:
                if what[0] == "s":
                    begin(int(what[1]), i)
                elif what[0] == "c":
                    finish(int(what[1]), i)
                elif what == "q":
                    project_queries(i, background if i in SLICE_BLOCKS else None)
                elif what == "v":
                    if i + 2 < NBLK:
                        next(values[i // 2 + 1], None)
                elif i + 1 < NBLK:
                    project_keys(i + 1, background if i + 1 in SLICE_BLOCKS else None)
        project_keys(0, background if 0 in SLICE_BLOCKS else None)
        for _ in values[0]:
            pass
        background.finish()

        _wait(slice_copies(j + 1))
        pl.when(j + 2 < PAIRS)(lambda: _wait(pair_copies(j + 2)))
        pl.when(j + 3 < PAIRS)(lambda: _start(pair_copies(j + 3)))
        pl.when(j + 2 < PAIRS)(lambda: _start(slice_copies(j + 2)))
        return carry

    def last_head_pair(j, carry):
        _start([xa_copy(0), xa_copy(1)])
        background = _Background(j < 0, slice_work(j, [n for n in SLICE_JOBS if n > 4]), LAST_SLICE_RATE)
        begin, finish = attention_steps(j, LAST_CONTEXT_KEYS,
                                        lambda i: background if i in LAST_SLICE_BLOCKS else None)
        for n, (h, i) in enumerate(LAST_PAIR_STEPS):
            begin(h, i)
            if n >= LAST_PAIR_LAG:
                finish(*LAST_PAIR_STEPS[n - LAST_PAIR_LAG])
        for h, i in LAST_PAIR_STEPS[-LAST_PAIR_LAG:]:
            finish(h, i)
        background.finish()
        return carry

    lax.fori_loop(0, PAIRS - 1, head_pair, 0)
    lax.fori_loop(PAIRS - 1, PAIRS, last_head_pair, 0)

    def store_blocks(i, col0, c):
        for a, n in ((0, 0), (1, 0), (0, 1), (1, 1)):
            obuf[i % 2, a * SUB:(a + 1) * SUB, col0 + n * HALF:col0 + (n + 1) * HALF] = c[a][n].astype(BF16)
            if col0 == 0:
                out_copy(i, 2 * a + n).start()
        if col0:
            out_copy(i, 4).start()

    def row_block(i, carry):
        xa_copy(i).wait()
        pl.when(i >= 2)(lambda: _wait([out_copy(i - 2, part) for part in range(5)]))
        loc[0:LOC_Q, 0:HALO, :] = loc[0:LOC_Q, BLK:BLK + HALO, :]

        x_ops = _operand_sums(
            lambda a, k: xa_raw[i % 2, a * SUB:(a + 1) * SUB, k * HALF:(k + 1) * HALF], A_TERMS)
        x_rounded = [op.astype(BF16) for op in x_ops]
        background = _Background(i < 0, slice_work(PAIRS - 1, FINAL_JOBS), FINAL_RATE)
        for part in LOCAL_PARTS:
            if part == 2:
                def value_product(r):
                    ops = _operand_sums(
                        lambda a, k: x_ops[r][64 * a:64 * (a + 1), QUARTER * k:QUARTER * (k + 1)], A_TERMS)
                    return _join(_block_product(
                        lambda u: _dot(ops[u].astype(BF16), _unpack(wva_sums[7 * r + u])),
                        PRODUCT_ORDER["local v inner"]))

                c = _block_product(value_product, PRODUCT_ORDER["local v outer"])
            else:
                rows = slice(part * HALF // 2, (part + 1) * HALF // 2)
                c = _block_product(lambda r: _dot(x_rounded[r], _unpack(background.tie(wqk_sums[r, rows, :]))),
                                   PRODUCT_ORDER["local qk"])
            for a in range(2):
                for g in range(8):
                    loc[(LOC_Q, LOC_K, LOC_V)[part] + g, HALO + a * SUB:HALO + (a + 1) * SUB, :] = (
                        c[a][g // 4][:, (g % 4) * LANES:(g % 4 + 1) * LANES])
        background.finish()

        def context_block(a, k):
            rows = _rows(i * BLK + a * (BLK // 4), BLK // 4)
            return jnp.concatenate(
                [ctx[j, rows, :] for j in range(k * PAIRS // 4, (k + 1) * PAIRS // 4)], axis=1).astype(F32)

        context_ops = _operand_sums2(context_block, A_TERMS)
        marks = []

        def output_product(r):
            ops = context_ops[r]()

            def product(u):
                acc = None
                for k0 in range(0, DM, OUTPUT_DEPTH):
                    part = _dot(ops[u][:, k0:k0 + OUTPUT_DEPTH].astype(BF16),
                                _unpack(wob_sums[7 * r + u, k0 // 2:(k0 + OUTPUT_DEPTH) // 2, :]))
                    acc = part if acc is None else acc + part
                    marks.append(acc)
                return acc

            return _join(_block_product(product, PRODUCT_ORDER["out b inner"]))

        store_blocks(i, DM, _block_product(output_product, PRODUCT_ORDER["out b outer"]))

        ticks = itertools.count()
        last_tick = LOCAL_STAGES * BLK // LOCAL_ROWS - 1

        def paced(values):
            lo, hi = LOCAL_PACE
            mark = marks[int((lo + (hi - lo) * next(ticks) / last_tick) * (len(marks) - 1))]
            return [jnp.where(i < 0, mark[0:LOCAL_ROWS, 0:LANES], v) for v in values]

        def attend(c0):
            def shifted(base, g, w):
                r0 = HALO + c0 - A_DIL * w
                return loc[base + g, r0:r0 + LOCAL_ROWS, :]

            every = 16 // LOCAL_STAGES
            queries = [shifted(LOC_Q, g, 0) for g in range(8)]
            logits = []
            for w in range(A_WIN):
                if w % every == 0:
                    q = paced(queries)
                acc = q[0] * shifted(LOC_K, 0, w)
                for g in range(1, 8):
                    acc = acc + q[g] * shifted(LOC_K, g, w)
                acc = acc + pltpu.roll(acc, 2 * A_HEADS, 1)
                acc = acc + pltpu.roll(acc, A_HEADS, 1)
                if c0 < A_DIL * w:
                    pos = i * BLK + c0 + lax.broadcasted_iota(jnp.int32, (LOCAL_ROWS, LANES), 0)
                    acc = jnp.where(pos >= A_DIL * w, acc, NEG * A_DH ** 0.5)
                logits.append(acc)
            m = functools.reduce(jnp.maximum, logits)
            p = [jnp.exp2((l - m) * (A_DH ** -0.5 * LOG2E)) for l in logits]
            inverse = _reciprocal(functools.reduce(jnp.add, p))
            p = [t * inverse for t in p]
            out = []
            for g in range(8):
                if g % every == 0:
                    weights = paced(p)
                out.append(functools.reduce(
                    jnp.add, [weights[w] * shifted(LOC_V, g, w) for w in range(A_WIN)]))
            return out

        quarters = [[] for _ in range(4)]
        for c0 in range(0, BLK // 4, LOCAL_ROWS):
            for a in range(4):
                quarters[a].append(jnp.concatenate(attend(a * (BLK // 4) + c0), axis=1))
        quarters = [jnp.concatenate(rows, axis=0) for rows in quarters]

        local_ops = _operand_sums2(lambda a, k: quarters[a][:, k * QUARTER:(k + 1) * QUARTER], A_TERMS)

        def local_product(r):
            ops = local_ops[r]()
            return _join(_block_product(
                lambda u: _dot(ops[u].astype(BF16), _unpack(woa_sums[7 * r + u])), PRODUCT_ORDER["out a inner"]))

        store_blocks(i, 0, _block_product(local_product, PRODUCT_ORDER["out a outer"]))
        pl.when(i + 2 < NBLK)(lambda: xa_copy(i + 2).start())
        return carry

    loc[0:LOC_Q, BLK:BLK + HALO, :] = jnp.zeros((LOC_Q, HALO, LANES), F32)
    lax.fori_loop(0, NBLK, row_block, 0)
    _wait([out_copy(i, part) for i in (NBLK - 2, NBLK - 1) for part in range(5)])


@jax.jit
def pallas_concat_heads__sliding_local_dilated__compressed_kv_cla__prompt_kernel(
    A_x: jax.Array,
    A_wqkv: jax.Array,
    A_wo: jax.Array,
    B_x: jax.Array,
    B_c_kv: jax.Array,
    B_w_q: jax.Array,
    B_w_uk: jax.Array,
    B_w_uv: jax.Array,
    B_w_o: jax.Array,
):
    vmem, sems = pltpu.VMEM, pltpu.SemaphoreType.DMA
    out = pl.pallas_call(
        _kernel,
        out_shape=jax.ShapeDtypeStruct((S, 2 * DM), BF16),
        in_specs=[pl.BlockSpec(memory_space=pl.ANY)] * 9,
        out_specs=pl.BlockSpec(memory_space=pl.ANY),
        scratch_shapes=[
            vmem((S, DM), BF16),
            vmem((S, B_DC), BF16),
            vmem((2, DM, B_DH), U32),
            vmem((2, B_DC, B_DH), U32),
            vmem((2, B_DC, B_DH), U32),
            vmem((26, S // 8, QUARTER), U32),
            vmem((7, S // 4, B_DC // 2), U32),
            vmem((NBLK // 2, 49, LANES // 2, LANES), U32),
            vmem((26, DM // 8, B_DH), U32),
            vmem((7, B_DC // 4, B_DH), U32),
            vmem((S, 2 * B_DH), BF16),
            vmem((2, S // 2, B_DH), U32),
            vmem((2, B_DH // 2, S), U32),
            vmem((PAIRS, S, 2 * B_DH), BF16),
            vmem((2, 2, 32, 2 * DM), BF16),
            vmem((2, 4, 16, DM), BF16),
            vmem((2, 2, A_HEADS, DM), U32),
            vmem((2, 4, 64, DM), BF16),
            vmem((7, HALF, HALF), U32),
            vmem((49, QUARTER // 2, QUARTER), U32),
            vmem((49, QUARTER // 2, QUARTER), U32),
            vmem((49, DM // 2, QUARTER), U32),
            vmem((2, BLK, DM), BF16),
            vmem((LOC_Q + 8, HALO + BLK, LANES), F32),
            vmem((2, BLK, 2 * DM), BF16),
            sems((2, NBLK // 2)), sems((2, 3)), sems((2,)), sems((2,)), sems((2,)),
        ],
        compiler_params=pltpu.CompilerParams(vmem_limit_bytes=120 * 2 ** 20, disable_bounds_checks=True),
        name="local_and_latent_attention",
    )(A_x.reshape(S, DM), A_wqkv, A_wo.reshape(A_HEADS, A_DH, DM), B_x.reshape(S, DM),
      B_c_kv.reshape(S, B_DC), B_w_q, B_w_uk, B_w_uv, B_w_o.reshape(B_HEADS * B_DH, DM))
    return out.reshape(1, S, 2 * DM)
```

```python
import functools
import itertools

import jax
import jax.numpy as jnp
from jax import lax
import jax.experimental.pallas as pl
import jax.experimental.pallas.tpu as pltpu

S = 2048
DM = 1024
HALF, QUARTER = DM // 2, DM // 4
LANES = 128
A_HEADS, A_DH, A_WIN, A_DIL = 32, 32, 8, 2
HALO = 16
B_HEADS, B_DH, B_DC = 32, 128, 512
PAIRS = B_HEADS // 2

BLK = 256
SUB = BLK // 2
NBLK = S // BLK

LOG2E = 1.4426950408889634
NEG = -1e9
F32, BF16, U32 = jnp.float32, jnp.bfloat16, jnp.uint32

A_TERMS = (((1, 0, 0), (1, 1, 1)), ((1, 1, 0), (1, 1, 1)), ((1, 0, 0),), ((1, 1, 1),),
           ((1, 0, 0), (1, 0, 1)), ((1, 1, 0), (-1, 0, 0)), ((1, 0, 1), (-1, 1, 1)))
B_TERMS = (((1, 0, 0), (1, 1, 1)), ((1, 0, 0),), ((1, 0, 1), (-1, 1, 1)), ((1, 1, 0), (-1, 0, 0)),
           ((1, 1, 1),), ((1, 0, 0), (1, 0, 1)), ((1, 1, 0), (1, 1, 1)))
C_TERMS = (((1, 0, 0), (1, 1, 1)), ((1, 1, 0), (-1, 1, 1)), ((1, 0, 1), (1, 1, 1)), ((1, 0, 0), (1, 1, 0)),
           ((-1, 0, 0), (1, 0, 1)), ((1, 1, 1),), ((1, 0, 0),))

HK_A, HK_B, HK_C = zip(
    (((1, 0, 0), (-1, 0, 1), (-1, 2, 0)), ((1, 0, 0), (-1, 0, 1)), ((1, 0, 0),)),
    (((1, 0, 0), (-1, 0, 2), (-1, 1, 0)), ((1, 0, 1),), ((1, 0, 0), (1, 0, 1))),
    (((1, 0, 3), (1, 1, 1), (-1, 1, 0), (-1, 1, 3), (-1, 2, 1)), ((1, 1, 0),), ((1, 1, 0),)),
    (((1, 1, 1), (1, 3, 0), (-1, 0, 1), (-1, 1, 2), (-1, 3, 1)), ((1, 1, 1),), ((1, 1, 1),)),
    (((1, 1, 0), (-1, 0, 3)), ((1, 0, 0), (1, 1, 0)), ((1, 0, 0), (1, 0, 1), (1, 1, 0), (1, 1, 1))),
    (((1, 0, 1), (-1, 3, 0)), ((1, 0, 1), (1, 1, 1), (-1, 0, 0), (-1, 1, 0)), ((1, 0, 1), (1, 1, 1))),
    (((1, 0, 1), (-1, 1, 0)), ((1, 0, 0), (1, 1, 0), (-1, 0, 1)), ((1, 0, 0), (1, 0, 1), (1, 1, 1))),
    (((1, 3, 0), (1, 3, 3), (-1, 0, 3), (-1, 2, 3), (-1, 3, 1)), ((1, 3, 0), (-1, 3, 1)), ((1, 3, 0),)),
    (((1, 0, 3), (1, 3, 3), (-1, 1, 3), (-1, 3, 0), (-1, 3, 2)), ((1, 3, 1),), ((1, 3, 0), (1, 3, 1))),
    (((1, 0, 3),), ((1, 0, 0), (1, 1, 0), (1, 3, 0)), ((1, 0, 0), (1, 1, 0), (1, 3, 0))),
    (((1, 3, 0),), ((1, 0, 1), (1, 1, 1), (1, 3, 1)), ((1, 0, 1), (1, 1, 1), (1, 3, 1))),
    (((1, 0, 3), (-1, 3, 0)), ((1, 0, 0), (1, 1, 0), (1, 3, 1)), ((1, 0, 1), (1, 1, 1), (-1, 3, 0))),
    (((1, 1, 3), (-1, 0, 3)), ((1, 1, 0), (1, 3, 0)), ((1, 1, 0), (1, 1, 1), (1, 3, 0), (1, 3, 1))),
    (((1, 3, 1), (-1, 3, 0)), ((1, 1, 1), (1, 3, 1), (-1, 1, 0), (-1, 3, 0)), ((1, 1, 1), (1, 3, 1))),
    (((1, 0, 3), (1, 3, 1), (-1, 1, 3), (-1, 3, 0)),
     ((1, 1, 0), (1, 3, 0), (-1, 3, 1)), ((1, 1, 1), (1, 3, 0), (1, 3, 1))),
    (((1, 2, 2), (-1, 1, 2), (-1, 2, 0), (-1, 2, 3)), ((1, 2, 0),), ((1, 2, 0), (1, 2, 1))),
    (((1, 2, 2), (-1, 0, 2), (-1, 2, 1), (-1, 3, 2)), ((1, 2, 1), (-1, 2, 0)), ((1, 2, 1),)),
    (((1, 2, 0),), ((1, 0, 0), (1, 2, 0)), ((1, 0, 0), (1, 2, 0))),
    (((1, 0, 2),), ((1, 0, 1), (1, 2, 1)), ((1, 0, 1), (1, 2, 1))),
    (((1, 0, 2), (-1, 2, 0)), ((1, 0, 1), (1, 2, 0)), ((1, 0, 0), (-1, 2, 1))),
    (((1, 2, 1),), ((1, 1, 0), (1, 2, 0), (-1, 1, 1), (-1, 2, 1)), ((1, 1, 0), (1, 2, 0))),
    (((1, 1, 2),), ((1, 1, 1), (1, 2, 1)), ((1, 1, 0), (1, 1, 1), (1, 2, 0), (1, 2, 1))),
    (((1, 2, 1), (-1, 1, 2)), ((1, 1, 1), (1, 2, 1), (-1, 2, 0)), ((1, 1, 0), (1, 2, 0), (1, 2, 1))),
    (((1, 2, 3),), ((1, 2, 0), (1, 3, 0)), ((1, 2, 0), (1, 3, 0))),
    (((1, 3, 2),), ((1, 2, 1), (1, 3, 1)), ((1, 2, 1), (1, 3, 1))),
    (((1, 2, 3), (-1, 3, 2)), ((1, 2, 0), (1, 3, 1)), ((1, 2, 1), (-1, 3, 0))),
)

LOC_K, LOC_V, LOC_Q = 0, 8, 16

PAIR_STEPS = (
    ("s0", "v", "s1", "k", "c0", "q", "c1"),
    ("s0", "s1", "q", "c0", "v", "c1", "k"),
    ("s0", "s1", "k", "c0", "q", "c1", "v"),
    ("s0", "s1", "c0", "k", "q", "c1", "v"),
    ("s0", "v", "s1", "k", "c0", "q", "c1"),
    ("s0", "s1", "k", "c0", "q", "c1", "v"),
    ("s0", "k", "s1", "c0", "q", "c1", "v"),
    ("s0", "s1", "k", "c0", "v", "c1", "q"),
)
LAST_PAIR_STEPS = (
    (0, 7), (0, 1), (0, 0), (1, 7), (0, 6), (1, 0), (1, 6), (1, 1),
    (0, 5), (1, 5), (0, 4), (1, 2), (0, 2), (0, 3), (1, 4), (1, 3),
)
LAST_PAIR_LAG = 3
PRODUCT_ORDER = {
    "q": (1, 3, 0, 2, 9, 4, 11, 7, 8, 10, 12, 5, 13, 6, 14, 20, 15, 16, 22, 17, 18, 19, 24, 21, 23, 25),
    "k": (6, 0, 3, 4, 2, 5, 1),
    "v inner": (0, 5, 2, 4, 6, 3, 1),
    "v outer": (3, 0, 4, 6, 1, 2, 5),
    "local qk": (0, 3, 6, 4, 2, 1, 5),
    "local v inner": (3, 1, 0, 6, 4, 2, 5),
    "local v outer": (0, 3, 4, 6, 1, 2, 5),
    "out b inner": (3, 1, 2, 4, 0, 6, 5),
    "out b outer": (2, 5, 0, 1, 3, 6, 4),
    "out a inner": (6, 5, 2, 0, 4, 3, 1),
    "out a outer": (0, 3, 4, 6, 1, 2, 5),
}
VALUE_SPLIT = 2
CONTEXT_KEYS, LAST_CONTEXT_KEYS = 1024, 2048
SLICE_JOBS, SLICE_BLOCKS = (4, 5, 6, 1, 0, 7, 3, 2), (6, 5, 4, 3, 2, 1)
LAST_SLICE_BLOCKS, LAST_SLICE_RATE = (6, 5, 4, 2, 0), 0.7
EARLY_SCORES, EARLY_CONTEXT, EARLY_RATE = ((0, 6), (0, 7), (1, 6)), (6, 7), 2
Q_DELAY = (7,)
FINAL_JOBS, FINAL_RATE = (2, 1, 3, 0, 4), 14
LOCAL_PARTS, LOCAL_ROWS, LOCAL_STAGES, LOCAL_PACE = (2, 1, 0), 16, 16, (0, 0.92)
OUTPUT_DEPTH = 128


def _pack(x):
    return pltpu.bitcast(x.astype(BF16), U32)


def _unpack(x):
    return pltpu.bitcast(x, BF16)


def _word_half(word, hi):
    return pltpu.bitcast(word & U32(0xFFFF0000) if hi else word << 16, F32)


def _dot(a, b):
    return jnp.dot(a, b, preferred_element_type=F32)


def _dot_nt(a, b):
    return lax.dot_general(a, b, (((1,), (1,)), ((), ())), preferred_element_type=F32)


def _reciprocal(x):
    r = pl.reciprocal(x, approx=True)
    return r * (2.0 - x * r)


def _operand_sums(block, terms, shape=(2, 2)):
    blocks = [[block(i, j) for j in range(shape[1])] for i in range(shape[0])]
    out = []
    for (_, i, j), *rest in terms:
        acc = blocks[i][j]
        for sign, i, j in rest:
            a, b = acc.astype(F32), blocks[i][j].astype(F32)
            acc = a + b if sign > 0 else a - b
        out.append(acc)
    return out


def _operand_sums2(block, terms):
    outer = [[_operand_sums(lambda i, j: block(2 * i + a, 2 * j + b), terms) for b in range(2)]
             for a in range(2)]
    return [functools.partial(_operand_sums, lambda a, b, r=r: outer[a][b][r], terms) for r in range(7)]


def _block_product(product, order, c=None, terms=C_TERMS):
    c = c or [[None, None], [None, None]]
    for r in order:
        m = product(r)
        for sign, i, j in terms[r]:
            if c[i][j] is None:
                c[i][j] = m if sign > 0 else -m
            else:
                c[i][j] = c[i][j] + m if sign > 0 else c[i][j] - m
    return c


def _join(c):
    return jnp.concatenate([jnp.concatenate(row, axis=1) for row in c], axis=0)


def _heads_to_lanes(groups):
    lane = lax.broadcasted_iota(jnp.int32, groups[0].shape, 1)
    groups = list(groups)
    for group_bit, lane_bit in ((2, 4), (1, 3), (0, 2), (2, 6), (2, 1), (1, 5), (1, 0)):
        shift = 1 << lane_bit
        low = (lane & shift) == 0
        for g in range(8):
            if g >> group_bit & 1:
                continue
            x, y = groups[g], groups[g | 1 << group_bit]
            groups[g] = jnp.where(low, x, pltpu.roll(y, shift, 1))
            groups[g | 1 << group_bit] = jnp.where(low, pltpu.roll(x, LANES - shift, 1), y)
    return [groups[(g & 1) << 2 | (g >> 2) << 1 | (g >> 1 & 1)] for g in range(8)]


class _Background:
    def __init__(self, never, pieces, rate):
        self.never, self.pending, self.rate, self.credit = never, pieces, rate, 0.0

    def tie(self, words):
        self.credit += self.rate
        due = [pltpu.bitcast(d, U32) for d in itertools.islice(self.pending, int(self.credit))]
        self.credit -= int(self.credit)
        if not due:
            return words
        mark = functools.reduce(jnp.bitwise_or, [
            d[r:r + 8, c:c + LANES]
            for d in due for r in range(0, d.shape[0], 8) for c in range(0, d.shape[1], LANES)])
        top = jnp.where(self.never, mark, words[:8, :LANES])
        if words.shape[1] > LANES:
            top = jnp.concatenate([top, words[:8, LANES:]], axis=1)
        return jnp.concatenate([top, words[8:]], axis=0)

    def tie_tiles(self, words, axis, size):
        return jnp.concatenate([self.tie(lax.slice_in_dim(words, t, t + size, axis=axis))
                                for t in range(0, words.shape[axis], size)], axis=axis)


def _finish(generator):
    for _ in generator:
        pass


def _start(copies):
    for copy in copies:
        copy.start()


def _wait(copies):
    for copy in copies:
        copy.wait()


def _rows(start, size):
    return pl.ds(start if isinstance(start, int) else pl.multiple_of(start, size), size)


def _packed_rows(start, size):
    return _rows(start // 2, size // 2)


def _kernel(xa_hbm, wqkv_hbm, woa_hbm, xb_hbm, c_hbm, wq_hbm, wuk_hbm, wuv_hbm, wob_hbm,
            out_hbm,
            xb_raw, c_raw, wq_raw, wuk_raw, wuv_raw,
            x_sums, c_sums, ct_sums, wq_sums, wk_sums,
            q_s, k_s, vt_s, ctx,
            wqk_raw, wva_raw, woa_raw, wob_raw,
            wqk_sums, wva_sums, woa_sums, wob_sums,
            xa_raw, loc, obuf,
            sem_in, sem_pair, sem_slice, sem_xa, sem_out):
    wq_words, wuk_words, wuv_words = wq_hbm.bitcast(U32), wuk_hbm.bitcast(U32), wuv_hbm.bitcast(U32)
    woa_words = woa_hbm.bitcast(U32)

    def pair_copies(j, which=(0, 1, 2)):
        ends = ((wuk_words, wuk_raw), (wuv_words, wuv_raw), (wq_words, wq_raw))
        return [pltpu.make_async_copy(ends[n][0].at[:, j, :], ends[n][1].at[j % 2], sem_pair.at[j % 2, n])
                for n in which]

    def slice_copies(j):
        slot = j % 2
        ends = [(wqkv_hbm.at[_rows(k * HALF + j * 32, 32), 0:2 * DM], wqk_raw.at[slot, k]) for k in range(2)]
        ends += [(wqkv_hbm.at[_rows(k * QUARTER + j * 16, 16), 2 * DM:3 * DM], wva_raw.at[slot, k])
                 for k in range(4)]
        ends += [(woa_words.at[:, (j >> 1 & 1) | k << 1 | (j >> 2) << 2, :], woa_raw.at[slot, k])
                 for k in range(2)]
        ends += [(wob_hbm.at[_rows(k * DM + j * 64, 64), :], wob_raw.at[slot, k]) for k in range(4)]
        return [pltpu.make_async_copy(src, dst, sem_slice.at[slot]) for src, dst in ends]

    def latent_copy(n):
        rows = _rows(n * 2 * BLK, 2 * BLK)
        return pltpu.make_async_copy(c_hbm.at[rows, :], c_raw.at[rows, :], sem_in.at[0, n])

    def xb_copy(n):
        rows = _rows(n * 2 * BLK, 2 * BLK)
        return pltpu.make_async_copy(xb_hbm.at[rows, :], xb_raw.at[rows, :], sem_in.at[1, n])

    def xa_copy(i):
        return pltpu.make_async_copy(xa_hbm.at[_rows(i * BLK, BLK), :], xa_raw.at[i % 2], sem_xa.at[i % 2])

    def out_copy(i, part):
        r0, nr, c0, nc = (0, BLK, DM, DM) if part == 4 else (part // 2 * SUB, SUB, part % 2 * HALF, HALF)
        return pltpu.make_async_copy(obuf.at[i % 2, r0:r0 + nr, c0:c0 + nc],
                                     out_hbm.at[_rows(i * BLK + r0, nr), c0:c0 + nc], sem_out.at[i % 2])

    def prepare_weights(j, raw, dst, terms, parts):
        slot, depth = j % 2, raw.shape[1] // parts
        for r0 in range(0, depth, 32):
            words = [raw[slot, k * depth + r0:k * depth + r0 + 32, :] for k in range(parts)]
            for r, op in enumerate(_operand_sums(lambda k, head: _word_half(words[k], head), terms, (parts, 2))):
                op = _pack(op)
                dst[r, r0 // 2:r0 // 2 + 16, :] = op
                yield op

    def prepare_inputs(i, raw, dst, terms, parts):
        rows, width = BLK // parts, raw.shape[1] // parts
        ops = _operand_sums(lambda a, k: raw[_rows(i * BLK + a * rows, rows), k * width:(k + 1) * width],
                            terms, (parts, parts))
        ops = [_pack(op) for op in ops]
        for r, op in enumerate(ops):
            dst[r, _packed_rows(i * rows, rows), :] = op
        return ops

    def project_queries(i, background=None, ops=None):
        def product(r):
            w = wq_sums[r] if background is None else background.tie(wq_sums[r])
            return _dot(_unpack(x_sums[r, _packed_rows(i * 64, 64), :] if ops is None else ops[r]), _unpack(w))

        c = _block_product(product, PRODUCT_ORDER["q"], [[None, None] for _ in range(4)], HK_C)
        for a in range(4):
            q_s[_rows(i * BLK + a * 64, 64), :] = (
                jnp.concatenate(c[a], axis=1) * (B_DH ** -0.5 * LOG2E)).astype(BF16)

    def project_keys(i, background=None, ops=None):
        def product(r):
            w = wk_sums[r] if background is None else background.tie(wk_sums[r])
            return _dot(_unpack(c_sums[r, _packed_rows(i * SUB, SUB), :] if ops is None else ops[r]), _unpack(w))

        c = _block_product(product, PRODUCT_ORDER["k"])
        for a in range(2):
            for head in range(2):
                k_s[head, _packed_rows(i * BLK + a * SUB, SUB), :] = _pack(c[a][head])

    def value_weights(j):
        words = wuv_raw[j % 2].T

        def block(a, k):
            return _word_half(words[a % 2 * 64:(a % 2 + 1) * 64, k * LANES:(k + 1) * LANES], a // 2)

        return [[op.astype(BF16) for op in inner()] for inner in _operand_sums2(block, A_TERMS)]

    def prepare_latents(t):
        blocks = [[c_raw[_rows((4 * t + n) * LANES, LANES), k * LANES:(k + 1) * LANES].astype(F32).T
                   for n in range(4)] for k in range(4)]
        ops = [[_pack(op) for op in inner()] for inner in _operand_sums2(lambda k, n: blocks[k][n], B_TERMS)]
        for r in range(7):
            for u in range(7):
                ct_sums[t, 7 * r + u] = ops[r][u]
        return ops

    def project_values(t, weights, ops=None):
        def outer(r):
            return _join(_block_product(
                lambda u: _dot(weights[r][u], _unpack(ct_sums[t, 7 * r + u] if ops is None else ops[r][u])),
                PRODUCT_ORDER["v inner"]))

        c = _block_product(outer, PRODUCT_ORDER["v outer"][:VALUE_SPLIT])
        yield
        c = _block_product(outer, PRODUCT_ORDER["v outer"][VALUE_SPLIT:], c)
        for head in range(2):
            for n in range(2):
                vt_s[head, :, _rows((2 * t + n) * BLK, BLK)] = _pack(c[head][n])

    def scores(h, i, background):
        row = lax.broadcasted_iota(jnp.int32, (SUB, SUB), 0)
        col = lax.broadcasted_iota(jnp.int32, (SUB, SUB), 1)
        r0, cols = i * BLK, slice(h * B_DH, (h + 1) * B_DH)
        past = None
        if i:
            words = k_s[h, 0:r0 // 2, :]
            if background is not None:
                words = background.tie_tiles(words, 0, LANES // 2)
            past = _dot_nt(q_s[r0:r0 + BLK, cols], _unpack(words))
        diagonal = []
        for a in range(2):
            d = _dot_nt(q_s[r0 + a * SUB:r0 + (a + 1) * SUB, cols],
                        _unpack(k_s[h, r0 // 2:(r0 + (a + 1) * SUB) // 2, :]))
            last = jnp.where(col <= row, d[:, a * SUB:], NEG)
            diagonal.append(jnp.concatenate([d[:, :SUB], last], axis=1) if a else last)
        return past, diagonal

    def softmax(i, past, diagonal):
        p_past, p_diagonal, inverse = [], [], []
        for a in range(2):
            s = diagonal[a]
            if past is not None:
                s = jnp.concatenate([past[a * SUB:(a + 1) * SUB], s], axis=1)
            p = jnp.exp2(s - jnp.max(s, axis=1, keepdims=True)).astype(BF16)
            inverse.append(_reciprocal(jnp.sum(p.astype(F32), axis=1, keepdims=True)))
            if past is not None:
                p_past.append(p[:, :i * BLK])
            p_diagonal.append(p[:, i * BLK:])
        return (jnp.concatenate(p_past, axis=0) if p_past else None), p_diagonal, inverse

    def context(h, i, weights, keys, background):
        p_past, p_diagonal, inverse = weights
        r0 = i * BLK
        past = None
        for k0 in range(0, r0, keys):
            k1 = min(k0 + keys, r0)
            words = vt_s[h, :, k0:k1]
            if background is not None:
                words = background.tie_tiles(words, 1, LANES)
            part = _dot_nt(p_past[:, k0:k1], _unpack(words))
            past = part if past is None else past + part
        out = []
        for a in range(2):
            o = _dot_nt(p_diagonal[a], _unpack(vt_s[h, :, r0:r0 + (a + 1) * SUB]))
            if past is not None:
                o = o + past[a * SUB:(a + 1) * SUB]
            out.append(o * inverse[a])
        return out

    def slice_work(j, jobs):
        slot = j % 2

        def query_or_key(part):
            groups = [_heads_to_lanes([
                _pack(wqk_raw[slot, k, :, part * DM + a * LANES:part * DM + (a + 1) * LANES])
                for a in range(8)]) for k in range(2)]
            rows = _packed_rows(part * HALF + j * 32, 32)
            for a in range(4):
                for r, op in enumerate(_operand_sums(lambda k, n: _unpack(groups[k][4 * n + a]), B_TERMS)):
                    op = _pack(op)
                    wqk_sums[r, rows, a * LANES:(a + 1) * LANES] = op
                    yield op

        def two_levels(block, dst, row0, cols):
            for r, inner in enumerate(_operand_sums2(block, B_TERMS)):
                for u, op in enumerate(inner()):
                    op = _pack(op)
                    dst[7 * r + u, _packed_rows(row0, 2 * op.shape[0]), cols] = op
                    yield op

        def value():
            groups = [_heads_to_lanes([_pack(wva_raw[slot, k, :, a * LANES:(a + 1) * LANES]) for a in range(8)])
                      for k in range(4)]
            return two_levels(lambda k, n: _unpack(jnp.concatenate(groups[k][2 * n:2 * n + 2], axis=1)),
                              wva_sums, j * 16, slice(None))

        def output_a():
            return two_levels(
                lambda k, n: _word_half(woa_raw[slot, k % 2, :, _rows(n * QUARTER + j % 2 * LANES, LANES)], k // 2),
                woa_sums, ((j >> 1 & 1) * 4 + (j >> 2)) * A_HEADS, _rows(j % 2 * LANES, LANES))

        def output_b(r0, c0):
            return two_levels(
                lambda k, n: wob_raw[slot, k, r0:r0 + 32, n * QUARTER + c0:n * QUARTER + c0 + LANES],
                wob_sums, j * 64 + r0, slice(c0, c0 + LANES))

        for n in jobs:
            if n < 4:
                yield from output_b(n // 2 * 32, n % 2 * LANES)
            elif n == 4:
                yield from output_a()
            else:
                yield from value() if n == 7 else query_or_key(n - 5)

    def first_steps(copy, work, requests):
        def step(n, carry):
            copy(n).wait()
            for at, copies in requests:
                pl.when(n == at)(lambda: _start(copies()))
            work(n)
            return carry

        lax.fori_loop(0, NBLK // 2, step, 0)

    def first_keys_and_values(weights, n):
        for i in (2 * n, 2 * n + 1):
            project_keys(i, ops=prepare_inputs(i, c_raw, c_sums, A_TERMS, 2))
        _finish(project_values(n, weights, ops=prepare_latents(n)))

    def first_queries(n):
        for i in (2 * n, 2 * n + 1):
            project_queries(i, ops=prepare_inputs(i, xb_raw, x_sums, HK_A, 4))

    _start(pair_copies(0, (0, 1)) + [latent_copy(0)])
    _wait(pair_copies(0, (0,)))
    _start([latent_copy(1), latent_copy(2), latent_copy(3)] + pair_copies(0, (2,)) + [xb_copy(0)])
    _finish(prepare_weights(0, wuk_raw, wk_sums, B_TERMS, 2))
    _wait(pair_copies(0, (1,)))
    first_steps(latent_copy, functools.partial(first_keys_and_values, value_weights(0)),
                ((1, lambda: [xb_copy(1), xb_copy(2)]), (2, lambda: [xb_copy(3)]), (3, lambda: pair_copies(1))))
    _wait(pair_copies(0, (2,)))
    _finish(prepare_weights(0, wq_raw, wq_sums, HK_B, 4))
    first_steps(xb_copy, first_queries, ((0, lambda: slice_copies(0)),))
    _wait(pair_copies(1) + slice_copies(0))
    _start(pair_copies(2) + slice_copies(1))

    def attention_steps(j, keys, beside_scores, background):
        scored, done = {}, {}

        def begin(h, i):
            scored[h, i] = scores(h, i, beside_scores(h, i))

        def finish(h, i):
            done[h, i] = context(h, i, softmax(i, *scored.pop((h, i))), keys, background(i))
            if (1 - h, i) in done:
                for a in range(2):
                    ctx[j, i * BLK + a * SUB:i * BLK + (a + 1) * SUB, :] = (
                        jnp.concatenate([done[0, i][a], done[1, i][a]], axis=1).astype(BF16))

        return begin, finish

    def head_pair(j, carry):
        early = _Background(j < 0, itertools.chain(prepare_weights(j + 1, wq_raw, wq_sums, HK_B, 4),
                                                   prepare_weights(j + 1, wuk_raw, wk_sums, B_TERMS, 2)), EARLY_RATE)
        weights = value_weights(j + 1)
        background = _Background(j < 0, slice_work(j, SLICE_JOBS), 350 / (33 * len(SLICE_BLOCKS)))
        values = [project_values(t, weights) for t in range(NBLK // 2)]
        begin, finish = attention_steps(
            j, CONTEXT_KEYS, lambda h, i: early if (h, i) in EARLY_SCORES else None,
            lambda i: early if i in EARLY_CONTEXT else None)
        for i in range(NBLK - 1, -1, -1):
            for what in PAIR_STEPS[i]:
                if what[0] == "s":
                    begin(int(what[1]), i)
                elif what[0] == "c":
                    finish(int(what[1]), i)
                elif what == "q":
                    for n in [i + 1] * (i + 1 in Q_DELAY) + [i] * (i not in Q_DELAY):
                        _finish(early.pending)
                        project_queries(n, background if n in SLICE_BLOCKS else None)
                elif what == "v":
                    if i + 2 < NBLK:
                        next(values[i // 2 + 1], None)
                elif i + 1 < NBLK:
                    _finish(early.pending)
                    project_keys(i + 1, background if i + 1 in SLICE_BLOCKS else None)
        if 0 in Q_DELAY:
            project_queries(0, background if 0 in SLICE_BLOCKS else None)
        project_keys(0, background if 0 in SLICE_BLOCKS else None)
        _finish(values[0])
        _finish(background.pending)

        _wait(slice_copies(j + 1))
        pl.when(j + 2 < PAIRS)(lambda: _wait(pair_copies(j + 2)))
        pl.when(j + 3 < PAIRS)(lambda: _start(pair_copies(j + 3)))
        pl.when(j + 2 < PAIRS)(lambda: _start(slice_copies(j + 2)))
        return carry

    def last_head_pair(j, carry):
        _start([xa_copy(0), xa_copy(1)])
        background = _Background(j < 0, slice_work(j, [n for n in SLICE_JOBS if n > 4]), LAST_SLICE_RATE)
        begin, finish = attention_steps(j, LAST_CONTEXT_KEYS, lambda h, i: None,
                                        lambda i: background if i in LAST_SLICE_BLOCKS else None)
        for n, (h, i) in enumerate(LAST_PAIR_STEPS):
            begin(h, i)
            if n >= LAST_PAIR_LAG:
                finish(*LAST_PAIR_STEPS[n - LAST_PAIR_LAG])
        for h, i in LAST_PAIR_STEPS[-LAST_PAIR_LAG:]:
            finish(h, i)
        _finish(background.pending)
        return carry

    lax.fori_loop(0, PAIRS - 1, head_pair, 0)
    lax.fori_loop(PAIRS - 1, PAIRS, last_head_pair, 0)

    def store_blocks(i, col0, c):
        for a, n in ((0, 0), (1, 0), (0, 1), (1, 1)):
            obuf[i % 2, a * SUB:(a + 1) * SUB, col0 + n * HALF:col0 + (n + 1) * HALF] = c[a][n].astype(BF16)
            if col0 == 0:
                out_copy(i, 2 * a + n).start()
        if col0:
            out_copy(i, 4).start()

    def row_block(i, carry):
        xa_copy(i).wait()
        pl.when(i >= 2)(lambda: _wait([out_copy(i - 2, part) for part in range(5)]))
        loc[0:LOC_Q, 0:HALO, :] = loc[0:LOC_Q, BLK:BLK + HALO, :]

        x_ops = _operand_sums(
            lambda a, k: xa_raw[i % 2, a * SUB:(a + 1) * SUB, k * HALF:(k + 1) * HALF], A_TERMS)
        x_rounded = [op.astype(BF16) for op in x_ops]
        background = _Background(i < 0, slice_work(PAIRS - 1, FINAL_JOBS), FINAL_RATE)
        for part in LOCAL_PARTS:
            if part == 2:
                def value_product(r):
                    ops = _operand_sums(
                        lambda a, k: x_ops[r][64 * a:64 * (a + 1), QUARTER * k:QUARTER * (k + 1)], A_TERMS)
                    return _join(_block_product(
                        lambda u: _dot(ops[u].astype(BF16), _unpack(wva_sums[7 * r + u])),
                        PRODUCT_ORDER["local v inner"]))

                c = _block_product(value_product, PRODUCT_ORDER["local v outer"])
            else:
                rows = slice(part * HALF // 2, (part + 1) * HALF // 2)
                c = _block_product(lambda r: _dot(x_rounded[r], _unpack(background.tie(wqk_sums[r, rows, :]))),
                                   PRODUCT_ORDER["local qk"])
            for a in range(2):
                for g in range(8):
                    loc[(LOC_Q, LOC_K, LOC_V)[part] + g, HALO + a * SUB:HALO + (a + 1) * SUB, :] = (
                        c[a][g // 4][:, (g % 4) * LANES:(g % 4 + 1) * LANES])
        _finish(background.pending)

        def context_block(a, k):
            rows = _rows(i * BLK + a * (BLK // 4), BLK // 4)
            return jnp.concatenate(
                [ctx[j, rows, :] for j in range(k * PAIRS // 4, (k + 1) * PAIRS // 4)], axis=1).astype(F32)

        context_ops = _operand_sums2(context_block, A_TERMS)
        marks = []

        def output_product(r):
            ops = context_ops[r]()

            def product(u):
                acc = None
                for k0 in range(0, DM, OUTPUT_DEPTH):
                    part = _dot(ops[u][:, k0:k0 + OUTPUT_DEPTH].astype(BF16),
                                _unpack(wob_sums[7 * r + u, k0 // 2:(k0 + OUTPUT_DEPTH) // 2, :]))
                    acc = part if acc is None else acc + part
                    marks.append(acc)
                return acc

            return _join(_block_product(product, PRODUCT_ORDER["out b inner"]))

        store_blocks(i, DM, _block_product(output_product, PRODUCT_ORDER["out b outer"]))

        ticks = itertools.count()
        last_tick = LOCAL_STAGES * BLK // LOCAL_ROWS - 1

        def paced(values):
            lo, hi = LOCAL_PACE
            mark = marks[int((lo + (hi - lo) * next(ticks) / last_tick) * (len(marks) - 1))]
            return [jnp.where(i < 0, mark[0:LOCAL_ROWS, 0:LANES], v) for v in values]

        def attend(c0):
            def shifted(base, g, w):
                r0 = HALO + c0 - A_DIL * w
                return loc[base + g, r0:r0 + LOCAL_ROWS, :]

            every = 16 // LOCAL_STAGES
            queries = [shifted(LOC_Q, g, 0) for g in range(8)]
            logits = []
            for w in range(A_WIN):
                if w % every == 0:
                    q = paced(queries)
                acc = q[0] * shifted(LOC_K, 0, w)
                for g in range(1, 8):
                    acc = acc + q[g] * shifted(LOC_K, g, w)
                acc = acc + pltpu.roll(acc, 2 * A_HEADS, 1)
                acc = acc + pltpu.roll(acc, A_HEADS, 1)
                if c0 < A_DIL * w:
                    pos = i * BLK + c0 + lax.broadcasted_iota(jnp.int32, (LOCAL_ROWS, LANES), 0)
                    acc = jnp.where(pos >= A_DIL * w, acc, NEG * A_DH ** 0.5)
                logits.append(acc)
            m = functools.reduce(jnp.maximum, logits)
            p = [jnp.exp2((l - m) * (A_DH ** -0.5 * LOG2E)) for l in logits]
            inverse = _reciprocal(functools.reduce(jnp.add, p))
            p = [t * inverse for t in p]
            out = []
            for g in range(8):
                if g % every == 0:
                    weights = paced(p)
                out.append(functools.reduce(
                    jnp.add, [weights[w] * shifted(LOC_V, g, w) for w in range(A_WIN)]))
            return out

        quarters = [[] for _ in range(4)]
        for c0 in range(0, BLK // 4, LOCAL_ROWS):
            for a in range(4):
                quarters[a].append(jnp.concatenate(attend(a * (BLK // 4) + c0), axis=1))
        quarters = [jnp.concatenate(rows, axis=0) for rows in quarters]

        local_ops = _operand_sums2(lambda a, k: quarters[a][:, k * QUARTER:(k + 1) * QUARTER], A_TERMS)

        def local_product(r):
            ops = local_ops[r]()
            return _join(_block_product(
                lambda u: _dot(ops[u].astype(BF16), _unpack(woa_sums[7 * r + u])), PRODUCT_ORDER["out a inner"]))

        store_blocks(i, 0, _block_product(local_product, PRODUCT_ORDER["out a outer"]))
        pl.when(i + 2 < NBLK)(lambda: xa_copy(i + 2).start())
        return carry

    loc[0:LOC_Q, BLK:BLK + HALO, :] = jnp.zeros((LOC_Q, HALO, LANES), F32)
    lax.fori_loop(0, NBLK, row_block, 0)
    _wait([out_copy(i, part) for i in (NBLK - 2, NBLK - 1) for part in range(5)])


@jax.jit
def pallas_concat_heads__sliding_local_dilated__compressed_kv_cla__prompt_kernel(
    A_x: jax.Array,
    A_wqkv: jax.Array,
    A_wo: jax.Array,
    B_x: jax.Array,
    B_c_kv: jax.Array,
    B_w_q: jax.Array,
    B_w_uk: jax.Array,
    B_w_uv: jax.Array,
    B_w_o: jax.Array,
):
    vmem, sems = pltpu.VMEM, pltpu.SemaphoreType.DMA
    out = pl.pallas_call(
        _kernel,
        out_shape=jax.ShapeDtypeStruct((S, 2 * DM), BF16),
        in_specs=[pl.BlockSpec(memory_space=pl.ANY)] * 9,
        out_specs=pl.BlockSpec(memory_space=pl.ANY),
        scratch_shapes=[
            vmem((S, DM), BF16),
            vmem((S, B_DC), BF16),
            vmem((2, DM, B_DH), U32),
            vmem((2, B_DC, B_DH), U32),
            vmem((2, B_DC, B_DH), U32),
            vmem((26, S // 8, QUARTER), U32),
            vmem((7, S // 4, B_DC // 2), U32),
            vmem((NBLK // 2, 49, LANES // 2, LANES), U32),
            vmem((26, DM // 8, B_DH), U32),
            vmem((7, B_DC // 4, B_DH), U32),
            vmem((S, 2 * B_DH), BF16),
            vmem((2, S // 2, B_DH), U32),
            vmem((2, B_DH // 2, S), U32),
            vmem((PAIRS, S, 2 * B_DH), BF16),
            vmem((2, 2, 32, 2 * DM), BF16),
            vmem((2, 4, 16, DM), BF16),
            vmem((2, 2, A_HEADS, DM), U32),
            vmem((2, 4, 64, DM), BF16),
            vmem((7, HALF, HALF), U32),
            vmem((49, QUARTER // 2, QUARTER), U32),
            vmem((49, QUARTER // 2, QUARTER), U32),
            vmem((49, DM // 2, QUARTER), U32),
            vmem((2, BLK, DM), BF16),
            vmem((LOC_Q + 8, HALO + BLK, LANES), F32),
            vmem((2, BLK, 2 * DM), BF16),
            sems((2, NBLK // 2)), sems((2, 3)), sems((2,)), sems((2,)), sems((2,)),
        ],
        compiler_params=pltpu.CompilerParams(vmem_limit_bytes=120 * 2 ** 20, disable_bounds_checks=True),
        name="local_and_latent_attention",
    )(A_x.reshape(S, DM), A_wqkv, A_wo.reshape(A_HEADS, A_DH, DM), B_x.reshape(S, DM),
      B_c_kv.reshape(S, B_DC), B_w_q, B_w_uk, B_w_uv, B_w_o.reshape(B_HEADS * B_DH, DM))
    return out.reshape(1, S, 2 * DM)
```

```python
import functools
import itertools

import jax
import jax.numpy as jnp
from jax import lax
import jax.experimental.pallas as pl
import jax.experimental.pallas.tpu as pltpu

S = 2048
DM = 1024
HALF, QUARTER = DM // 2, DM // 4
LANES = 128
A_HEADS, A_DH, A_WIN, A_DIL = 32, 32, 8, 2
HALO = 16
B_HEADS, B_DH, B_DC = 32, 128, 512
PAIRS = B_HEADS // 2

BLK = 256
SUB = BLK // 2
NBLK = S // BLK

LOG2E = 1.4426950408889634
NEG = -1e9
F32, BF16, U32 = jnp.float32, jnp.bfloat16, jnp.uint32

A_TERMS = (((1, 0, 0), (1, 1, 1)), ((1, 1, 0), (1, 1, 1)), ((1, 0, 0),), ((1, 1, 1),),
           ((1, 0, 0), (1, 0, 1)), ((1, 1, 0), (-1, 0, 0)), ((1, 0, 1), (-1, 1, 1)))
B_TERMS = (((1, 0, 0), (1, 1, 1)), ((1, 0, 0),), ((1, 0, 1), (-1, 1, 1)), ((1, 1, 0), (-1, 0, 0)),
           ((1, 1, 1),), ((1, 0, 0), (1, 0, 1)), ((1, 1, 0), (1, 1, 1)))
C_TERMS = (((1, 0, 0), (1, 1, 1)), ((1, 1, 0), (-1, 1, 1)), ((1, 0, 1), (1, 1, 1)), ((1, 0, 0), (1, 1, 0)),
           ((-1, 0, 0), (1, 0, 1)), ((1, 1, 1),), ((1, 0, 0),))

HK_A, HK_B, HK_C = zip(
    (((1, 0, 0), (-1, 0, 1), (-1, 2, 0)), ((1, 0, 0), (-1, 0, 1)), ((1, 0, 0),)),
    (((1, 0, 0), (-1, 0, 2), (-1, 1, 0)), ((1, 0, 1),), ((1, 0, 0), (1, 0, 1))),
    (((1, 0, 3), (1, 1, 1), (-1, 1, 0), (-1, 1, 3), (-1, 2, 1)), ((1, 1, 0),), ((1, 1, 0),)),
    (((1, 1, 1), (1, 3, 0), (-1, 0, 1), (-1, 1, 2), (-1, 3, 1)), ((1, 1, 1),), ((1, 1, 1),)),
    (((1, 1, 0), (-1, 0, 3)), ((1, 0, 0), (1, 1, 0)), ((1, 0, 0), (1, 0, 1), (1, 1, 0), (1, 1, 1))),
    (((1, 0, 1), (-1, 3, 0)), ((1, 0, 1), (1, 1, 1), (-1, 0, 0), (-1, 1, 0)), ((1, 0, 1), (1, 1, 1))),
    (((1, 0, 1), (-1, 1, 0)), ((1, 0, 0), (1, 1, 0), (-1, 0, 1)), ((1, 0, 0), (1, 0, 1), (1, 1, 1))),
    (((1, 3, 0), (1, 3, 3), (-1, 0, 3), (-1, 2, 3), (-1, 3, 1)), ((1, 3, 0), (-1, 3, 1)), ((1, 3, 0),)),
    (((1, 0, 3), (1, 3, 3), (-1, 1, 3), (-1, 3, 0), (-1, 3, 2)), ((1, 3, 1),), ((1, 3, 0), (1, 3, 1))),
    (((1, 0, 3),), ((1, 0, 0), (1, 1, 0), (1, 3, 0)), ((1, 0, 0), (1, 1, 0), (1, 3, 0))),
    (((1, 3, 0),), ((1, 0, 1), (1, 1, 1), (1, 3, 1)), ((1, 0, 1), (1, 1, 1), (1, 3, 1))),
    (((1, 0, 3), (-1, 3, 0)), ((1, 0, 0), (1, 1, 0), (1, 3, 1)), ((1, 0, 1), (1, 1, 1), (-1, 3, 0))),
    (((1, 1, 3), (-1, 0, 3)), ((1, 1, 0), (1, 3, 0)), ((1, 1, 0), (1, 1, 1), (1, 3, 0), (1, 3, 1))),
    (((1, 3, 1), (-1, 3, 0)), ((1, 1, 1), (1, 3, 1), (-1, 1, 0), (-1, 3, 0)), ((1, 1, 1), (1, 3, 1))),
    (((1, 0, 3), (1, 3, 1), (-1, 1, 3), (-1, 3, 0)),
     ((1, 1, 0), (1, 3, 0), (-1, 3, 1)), ((1, 1, 1), (1, 3, 0), (1, 3, 1))),
    (((1, 2, 2), (-1, 1, 2), (-1, 2, 0), (-1, 2, 3)), ((1, 2, 0),), ((1, 2, 0), (1, 2, 1))),
    (((1, 2, 2), (-1, 0, 2), (-1, 2, 1), (-1, 3, 2)), ((1, 2, 1), (-1, 2, 0)), ((1, 2, 1),)),
    (((1, 2, 0),), ((1, 0, 0), (1, 2, 0)), ((1, 0, 0), (1, 2, 0))),
    (((1, 0, 2),), ((1, 0, 1), (1, 2, 1)), ((1, 0, 1), (1, 2, 1))),
    (((1, 0, 2), (-1, 2, 0)), ((1, 0, 1), (1, 2, 0)), ((1, 0, 0), (-1, 2, 1))),
    (((1, 2, 1),), ((1, 1, 0), (1, 2, 0), (-1, 1, 1), (-1, 2, 1)), ((1, 1, 0), (1, 2, 0))),
    (((1, 1, 2),), ((1, 1, 1), (1, 2, 1)), ((1, 1, 0), (1, 1, 1), (1, 2, 0), (1, 2, 1))),
    (((1, 2, 1), (-1, 1, 2)), ((1, 1, 1), (1, 2, 1), (-1, 2, 0)), ((1, 1, 0), (1, 2, 0), (1, 2, 1))),
    (((1, 2, 3),), ((1, 2, 0), (1, 3, 0)), ((1, 2, 0), (1, 3, 0))),
    (((1, 3, 2),), ((1, 2, 1), (1, 3, 1)), ((1, 2, 1), (1, 3, 1))),
    (((1, 2, 3), (-1, 3, 2)), ((1, 2, 0), (1, 3, 1)), ((1, 2, 1), (-1, 3, 0))),
)

LOC_K, LOC_V, LOC_Q = 0, 8, 16

PAIR_STEPS = (
    ("s0", "v", "s1", "k", "c0", "q", "c1"),
    ("s0", "s1", "q", "c0", "v", "c1", "k"),
    ("s0", "s1", "k", "c0", "q", "c1", "v"),
    ("s0", "s1", "c0", "k", "q", "c1", "v"),
    ("s0", "v", "s1", "k", "c0", "q", "c1"),
    ("s0", "s1", "k", "c0", "q", "c1", "v"),
    ("s0", "k", "s1", "c0", "q", "c1", "v"),
    ("s0", "s1", "k", "c0", "v", "c1", "q"),
)
LAST_PAIR_STEPS = (
    (0, 7), (0, 1), (0, 0), (1, 7), (0, 6), (1, 0), (1, 6), (1, 1),
    (0, 5), (1, 5), (0, 4), (1, 2), (0, 2), (0, 3), (1, 4), (1, 3),
)
LAST_PAIR_LAG = 3
PRODUCT_ORDER = {
    "q": (1, 3, 0, 2, 9, 4, 11, 7, 8, 10, 12, 5, 13, 6, 14, 20, 15, 16, 22, 17, 18, 19, 24, 21, 23, 25),
    "k": (6, 0, 3, 4, 2, 5, 1),
    "v inner": (0, 5, 2, 4, 6, 3, 1),
    "v outer": (3, 0, 4, 6, 1, 2, 5),
    "local qk": (0, 3, 6, 4, 2, 1, 5),
    "local v inner": (3, 1, 0, 6, 4, 2, 5),
    "local v outer": (0, 3, 4, 6, 1, 2, 5),
    "out b inner": (3, 1, 2, 4, 0, 6, 5),
    "out b outer": (2, 5, 0, 1, 3, 6, 4),
    "out a inner": (6, 5, 2, 0, 4, 3, 1),
    "out a outer": (0, 3, 4, 6, 1, 2, 5),
}
VALUE_SPLIT = 2
CONTEXT_KEYS, LAST_CONTEXT_KEYS = 1024, 2048
SLICE_JOBS, SLICE_BLOCKS = (4, 5, 6, 1, 0, 7, 3, 2), (6, 5, 4, 3, 2, 1)
LAST_SLICE_BLOCKS, LAST_SLICE_RATE = (6, 5, 4, 2, 0), 0.7
EARLY_SCORES, EARLY_CONTEXT, EARLY_RATE = ((0, 6), (0, 7), (1, 6)), (6, 7), 2
Q_DELAY = (7,)
FINAL_JOBS, FINAL_RATE = (2, 1, 3, 0, 4), 14
LOCAL_PARTS, LOCAL_ROWS, LOCAL_STAGES, LOCAL_PACE = (2, 1, 0), 16, 16, (0, 0.92)
OUTPUT_DEPTH = 128


def _pack(x):
    return pltpu.bitcast(x.astype(BF16), U32)


def _unpack(x):
    return pltpu.bitcast(x, BF16)


def _word_half(word, hi):
    return pltpu.bitcast(word & U32(0xFFFF0000) if hi else word << 16, F32)


def _dot(a, b):
    return jnp.dot(a, b, preferred_element_type=F32)


def _dot_nt(a, b):
    return lax.dot_general(a, b, (((1,), (1,)), ((), ())), preferred_element_type=F32)


def _reciprocal(x):
    r = pl.reciprocal(x, approx=True)
    return r * (2.0 - x * r)


def _operand_sums(block, terms, shape=(2, 2)):
    blocks = [[block(i, j) for j in range(shape[1])] for i in range(shape[0])]
    out = []
    for (_, i, j), *rest in terms:
        acc = blocks[i][j]
        for sign, i, j in rest:
            a, b = acc.astype(F32), blocks[i][j].astype(F32)
            acc = a + b if sign > 0 else a - b
        out.append(acc)
    return out


def _operand_sums2(block, terms):
    outer = [[_operand_sums(lambda i, j: block(2 * i + a, 2 * j + b), terms) for b in range(2)]
             for a in range(2)]
    return [functools.partial(_operand_sums, lambda a, b, r=r: outer[a][b][r], terms) for r in range(7)]


def _block_product(product, order, c=None, terms=C_TERMS):
    c = c or [[None, None], [None, None]]
    for r in order:
        m = product(r)
        for sign, i, j in terms[r]:
            if c[i][j] is None:
                c[i][j] = m if sign > 0 else -m
            else:
                c[i][j] = c[i][j] + m if sign > 0 else c[i][j] - m
    return c


def _join(c):
    return jnp.concatenate([jnp.concatenate(row, axis=1) for row in c], axis=0)


def _heads_to_lanes(groups):
    lane = lax.broadcasted_iota(jnp.int32, groups[0].shape, 1)
    groups = list(groups)
    for group_bit, lane_bit in ((2, 4), (1, 3), (0, 2), (2, 6), (2, 1), (1, 5), (1, 0)):
        shift = 1 << lane_bit
        low = (lane & shift) == 0
        for g in range(8):
            if g >> group_bit & 1:
                continue
            x, y = groups[g], groups[g | 1 << group_bit]
            groups[g] = jnp.where(low, x, pltpu.roll(y, shift, 1))
            groups[g | 1 << group_bit] = jnp.where(low, pltpu.roll(x, LANES - shift, 1), y)
    return [groups[(g & 1) << 2 | (g >> 2) << 1 | (g >> 1 & 1)] for g in range(8)]


class _Background:
    def __init__(self, never, pieces, rate):
        self.never, self.pending, self.rate, self.credit = never, pieces, rate, 0.0

    def tie(self, words):
        self.credit += self.rate
        due = [pltpu.bitcast(d, U32) for d in itertools.islice(self.pending, int(self.credit))]
        self.credit -= int(self.credit)
        if not due:
            return words
        mark = functools.reduce(jnp.bitwise_or, [
            d[r:r + 8, c:c + LANES]
            for d in due for r in range(0, d.shape[0], 8) for c in range(0, d.shape[1], LANES)])
        top = jnp.where(self.never, mark, words[:8, :LANES])
        if words.shape[1] > LANES:
            top = jnp.concatenate([top, words[:8, LANES:]], axis=1)
        return jnp.concatenate([top, words[8:]], axis=0)

    def tie_tiles(self, words, axis, size):
        return jnp.concatenate([self.tie(lax.slice_in_dim(words, t, t + size, axis=axis))
                                for t in range(0, words.shape[axis], size)], axis=axis)


def _finish(generator):
    for _ in generator:
        pass


def _start(copies):
    for copy in copies:
        copy.start()


def _wait(copies):
    for copy in copies:
        copy.wait()


def _rows(start, size):
    return pl.ds(start if isinstance(start, int) else pl.multiple_of(start, size), size)


def _packed_rows(start, size):
    return _rows(start // 2, size // 2)


def _kernel(xa_hbm, wqkv_halves, wqkv_quarters, woa_hbm, xb_hbm, c_hbm, wq_hbm, wuk_hbm, wuv_hbm, wob_quarters,
            out_hbm,
            xb_raw, c_raw, wq_raw, wuk_raw, wuv_raw,
            x_sums, c_sums, ct_sums, wq_sums, wk_sums,
            q_s, k_s, vt_s, ctx,
            wqk_raw, wva_raw, woa_raw, wob_raw,
            wqk_sums, wva_sums, woa_sums, wob_sums,
            xa_raw, loc, obuf,
            sem_in, sem_pair, sem_slice, sem_xa, sem_out):
    wq_words, wuk_words, wuv_words = wq_hbm.bitcast(U32), wuk_hbm.bitcast(U32), wuv_hbm.bitcast(U32)
    woa_words = woa_hbm.bitcast(U32)

    def pair_copies(j, which=(0, 1, 2)):
        ends = ((wuk_words, wuk_raw), (wuv_words, wuv_raw), (wq_words, wq_raw))
        return [pltpu.make_async_copy(ends[n][0].at[:, j, :], ends[n][1].at[j % 2], sem_pair.at[j % 2, n])
                for n in which]

    def slice_copies(j):
        slot = j % 2
        ends = [(wqkv_halves.at[:, _rows(j * 32, 32), 0:2 * DM], wqk_raw.at[slot]),
                (wqkv_quarters.at[:, _rows(j * 16, 16), 2 * DM:3 * DM], wva_raw.at[slot]),
                (wob_quarters.at[:, _rows(j * 64, 64), :], wob_raw.at[slot])]
        ends += [(woa_words.at[:, (j >> 1 & 1) | k << 1 | (j >> 2) << 2, :], woa_raw.at[slot, k])
                 for k in range(2)]
        return [pltpu.make_async_copy(src, dst, sem_slice.at[slot]) for src, dst in ends]

    def latent_copy(n):
        rows = _rows(n * 2 * BLK, 2 * BLK)
        return pltpu.make_async_copy(c_hbm.at[rows, :], c_raw.at[rows, :], sem_in.at[0, n])

    def xb_copy(n):
        rows = _rows(n * 2 * BLK, 2 * BLK)
        return pltpu.make_async_copy(xb_hbm.at[rows, :], xb_raw.at[rows, :], sem_in.at[1, n])

    def xa_copy(i):
        return pltpu.make_async_copy(xa_hbm.at[_rows(i * BLK, BLK), :], xa_raw.at[i % 2], sem_xa.at[i % 2])

    def out_copy(i, part):
        r0, nr, c0, nc = (0, BLK, DM, DM) if part == 4 else (part // 2 * SUB, SUB, part % 2 * HALF, HALF)
        return pltpu.make_async_copy(obuf.at[i % 2, r0:r0 + nr, c0:c0 + nc],
                                     out_hbm.at[_rows(i * BLK + r0, nr), c0:c0 + nc], sem_out.at[i % 2])

    def prepare_weights(j, raw, dst, terms, parts):
        slot, depth = j % 2, raw.shape[1] // parts
        for r0 in range(0, depth, 32):
            words = [raw[slot, k * depth + r0:k * depth + r0 + 32, :] for k in range(parts)]
            for r, op in enumerate(_operand_sums(lambda k, head: _word_half(words[k], head), terms, (parts, 2))):
                op = _pack(op)
                dst[r, r0 // 2:r0 // 2 + 16, :] = op
                yield op

    def prepare_inputs(i, raw, dst, terms, parts):
        rows, width = BLK // parts, raw.shape[1] // parts
        ops = _operand_sums(lambda a, k: raw[_rows(i * BLK + a * rows, rows), k * width:(k + 1) * width],
                            terms, (parts, parts))
        ops = [_pack(op) for op in ops]
        for r, op in enumerate(ops):
            dst[r, _packed_rows(i * rows, rows), :] = op
        return ops

    def project_queries(i, background=None, ops=None):
        def product(r):
            w = wq_sums[r] if background is None else background.tie(wq_sums[r])
            return _dot(_unpack(x_sums[r, _packed_rows(i * 64, 64), :] if ops is None else ops[r]), _unpack(w))

        c = _block_product(product, PRODUCT_ORDER["q"], [[None, None] for _ in range(4)], HK_C)
        for a in range(4):
            q_s[_rows(i * BLK + a * 64, 64), :] = (
                jnp.concatenate(c[a], axis=1) * (B_DH ** -0.5 * LOG2E)).astype(BF16)

    def project_keys(i, background=None, ops=None):
        def product(r):
            w = wk_sums[r] if background is None else background.tie(wk_sums[r])
            return _dot(_unpack(c_sums[r, _packed_rows(i * SUB, SUB), :] if ops is None else ops[r]), _unpack(w))

        c = _block_product(product, PRODUCT_ORDER["k"])
        for a in range(2):
            for head in range(2):
                k_s[head, _packed_rows(i * BLK + a * SUB, SUB), :] = _pack(c[a][head])

    def value_weights(j):
        words = wuv_raw[j % 2].T

        def block(a, k):
            return _word_half(words[a % 2 * 64:(a % 2 + 1) * 64, k * LANES:(k + 1) * LANES], a // 2)

        return [[op.astype(BF16) for op in inner()] for inner in _operand_sums2(block, A_TERMS)]

    def prepare_latents(t):
        blocks = [[c_raw[_rows((4 * t + n) * LANES, LANES), k * LANES:(k + 1) * LANES].astype(F32).T
                   for n in range(4)] for k in range(4)]
        ops = [[_pack(op) for op in inner()] for inner in _operand_sums2(lambda k, n: blocks[k][n], B_TERMS)]
        for r in range(7):
            for u in range(7):
                ct_sums[t, 7 * r + u] = ops[r][u]
        return ops

    def project_values(t, weights, ops=None):
        def outer(r):
            return _join(_block_product(
                lambda u: _dot(weights[r][u], _unpack(ct_sums[t, 7 * r + u] if ops is None else ops[r][u])),
                PRODUCT_ORDER["v inner"]))

        c = _block_product(outer, PRODUCT_ORDER["v outer"][:VALUE_SPLIT])
        yield
        c = _block_product(outer, PRODUCT_ORDER["v outer"][VALUE_SPLIT:], c)
        for head in range(2):
            for n in range(2):
                vt_s[head, :, _rows((2 * t + n) * BLK, BLK)] = _pack(c[head][n])

    def scores(h, i, background):
        row = lax.broadcasted_iota(jnp.int32, (SUB, SUB), 0)
        col = lax.broadcasted_iota(jnp.int32, (SUB, SUB), 1)
        r0, cols = i * BLK, slice(h * B_DH, (h + 1) * B_DH)
        past = None
        if i:
            words = k_s[h, 0:r0 // 2, :]
            if background is not None:
                words = background.tie_tiles(words, 0, LANES // 2)
            past = _dot_nt(q_s[r0:r0 + BLK, cols], _unpack(words))
        diagonal = []
        for a in range(2):
            d = _dot_nt(q_s[r0 + a * SUB:r0 + (a + 1) * SUB, cols],
                        _unpack(k_s[h, r0 // 2:(r0 + (a + 1) * SUB) // 2, :]))
            last = jnp.where(col <= row, d[:, a * SUB:], NEG)
            diagonal.append(jnp.concatenate([d[:, :SUB], last], axis=1) if a else last)
        return past, diagonal

    def softmax(i, past, diagonal):
        p_past, p_diagonal, inverse = [], [], []
        for a in range(2):
            s = diagonal[a]
            if past is not None:
                s = jnp.concatenate([past[a * SUB:(a + 1) * SUB], s], axis=1)
            p = jnp.exp2(s - jnp.max(s, axis=1, keepdims=True)).astype(BF16)
            inverse.append(_reciprocal(jnp.sum(p.astype(F32), axis=1, keepdims=True)))
            if past is not None:
                p_past.append(p[:, :i * BLK])
            p_diagonal.append(p[:, i * BLK:])
        return (jnp.concatenate(p_past, axis=0) if p_past else None), p_diagonal, inverse

    def context(h, i, weights, keys, background):
        p_past, p_diagonal, inverse = weights
        r0 = i * BLK
        past = None
        for k0 in range(0, r0, keys):
            k1 = min(k0 + keys, r0)
            words = vt_s[h, :, k0:k1]
            if background is not None:
                words = background.tie_tiles(words, 1, LANES)
            part = _dot_nt(p_past[:, k0:k1], _unpack(words))
            past = part if past is None else past + part
        out = []
        for a in range(2):
            o = _dot_nt(p_diagonal[a], _unpack(vt_s[h, :, r0:r0 + (a + 1) * SUB]))
            if past is not None:
                o = o + past[a * SUB:(a + 1) * SUB]
            out.append(o * inverse[a])
        return out

    def slice_work(j, jobs):
        slot = j % 2

        def query_or_key(part):
            groups = [_heads_to_lanes([
                _pack(wqk_raw[slot, k, :, part * DM + a * LANES:part * DM + (a + 1) * LANES])
                for a in range(8)]) for k in range(2)]
            rows = _packed_rows(part * HALF + j * 32, 32)
            for a in range(4):
                for r, op in enumerate(_operand_sums(lambda k, n: _unpack(groups[k][4 * n + a]), B_TERMS)):
                    op = _pack(op)
                    wqk_sums[r, rows, a * LANES:(a + 1) * LANES] = op
                    yield op

        def two_levels(block, dst, row0, cols):
            for r, inner in enumerate(_operand_sums2(block, B_TERMS)):
                for u, op in enumerate(inner()):
                    op = _pack(op)
                    dst[7 * r + u, _packed_rows(row0, 2 * op.shape[0]), cols] = op
                    yield op

        def value():
            groups = [_heads_to_lanes([_pack(wva_raw[slot, k, :, a * LANES:(a + 1) * LANES]) for a in range(8)])
                      for k in range(4)]
            return two_levels(lambda k, n: _unpack(jnp.concatenate(groups[k][2 * n:2 * n + 2], axis=1)),
                              wva_sums, j * 16, slice(None))

        def output_a():
            return two_levels(
                lambda k, n: _word_half(woa_raw[slot, k % 2, :, _rows(n * QUARTER + j % 2 * LANES, LANES)], k // 2),
                woa_sums, ((j >> 1 & 1) * 4 + (j >> 2)) * A_HEADS, _rows(j % 2 * LANES, LANES))

        def output_b(r0, c0):
            return two_levels(
                lambda k, n: wob_raw[slot, k, r0:r0 + 32, n * QUARTER + c0:n * QUARTER + c0 + LANES],
                wob_sums, j * 64 + r0, slice(c0, c0 + LANES))

        for n in jobs:
            if n < 4:
                yield from output_b(n // 2 * 32, n % 2 * LANES)
            elif n == 4:
                yield from output_a()
            else:
                yield from value() if n == 7 else query_or_key(n - 5)

    def first_steps(copy, work, requests):
        def step(n, carry):
            copy(n).wait()
            for at, copies in requests:
                pl.when(n == at)(lambda: _start(copies()))
            work(n)
            return carry

        lax.fori_loop(0, NBLK // 2, step, 0)

    def first_keys_and_values(weights, n):
        for i in (2 * n, 2 * n + 1):
            project_keys(i, ops=prepare_inputs(i, c_raw, c_sums, A_TERMS, 2))
        _finish(project_values(n, weights, ops=prepare_latents(n)))

    def first_queries(n):
        for i in (2 * n, 2 * n + 1):
            project_queries(i, ops=prepare_inputs(i, xb_raw, x_sums, HK_A, 4))

    _start(pair_copies(0, (0, 1)) + [latent_copy(0)])
    _wait(pair_copies(0, (0,)))
    _start([latent_copy(1), latent_copy(2), latent_copy(3)] + pair_copies(0, (2,)) + [xb_copy(0)])
    _finish(prepare_weights(0, wuk_raw, wk_sums, B_TERMS, 2))
    _wait(pair_copies(0, (1,)))
    first_steps(latent_copy, functools.partial(first_keys_and_values, value_weights(0)),
                ((1, lambda: [xb_copy(1), xb_copy(2)]), (2, lambda: [xb_copy(3)]), (3, lambda: pair_copies(1))))
    _wait(pair_copies(0, (2,)))
    _finish(prepare_weights(0, wq_raw, wq_sums, HK_B, 4))
    first_steps(xb_copy, first_queries, ((0, lambda: slice_copies(0)),))
    _wait(pair_copies(1) + slice_copies(0))
    _start(pair_copies(2) + slice_copies(1))

    def attention_steps(j, keys, beside_scores, background):
        scored, done = {}, {}

        def begin(h, i):
            scored[h, i] = scores(h, i, beside_scores(h, i))

        def finish(h, i):
            done[h, i] = context(h, i, softmax(i, *scored.pop((h, i))), keys, background(i))
            if (1 - h, i) in done:
                for a in range(2):
                    ctx[j, i * BLK + a * SUB:i * BLK + (a + 1) * SUB, :] = (
                        jnp.concatenate([done[0, i][a], done[1, i][a]], axis=1).astype(BF16))

        return begin, finish

    def head_pair(j, carry):
        early = _Background(j < 0, itertools.chain(prepare_weights(j + 1, wq_raw, wq_sums, HK_B, 4),
                                                   prepare_weights(j + 1, wuk_raw, wk_sums, B_TERMS, 2)), EARLY_RATE)
        weights = value_weights(j + 1)
        background = _Background(j < 0, slice_work(j, SLICE_JOBS), 350 / (33 * len(SLICE_BLOCKS)))
        values = [project_values(t, weights) for t in range(NBLK // 2)]
        begin, finish = attention_steps(
            j, CONTEXT_KEYS, lambda h, i: early if (h, i) in EARLY_SCORES else None,
            lambda i: early if i in EARLY_CONTEXT else None)
        for i in range(NBLK - 1, -1, -1):
            for what in PAIR_STEPS[i]:
                if what[0] == "s":
                    begin(int(what[1]), i)
                elif what[0] == "c":
                    finish(int(what[1]), i)
                elif what == "q":
                    for n in [i + 1] * (i + 1 in Q_DELAY) + [i] * (i not in Q_DELAY):
                        _finish(early.pending)
                        project_queries(n, background if n in SLICE_BLOCKS else None)
                elif what == "v":
                    if i + 2 < NBLK:
                        next(values[i // 2 + 1], None)
                elif i + 1 < NBLK:
                    _finish(early.pending)
                    project_keys(i + 1, background if i + 1 in SLICE_BLOCKS else None)
        if 0 in Q_DELAY:
            project_queries(0, background if 0 in SLICE_BLOCKS else None)
        project_keys(0, background if 0 in SLICE_BLOCKS else None)
        _finish(values[0])
        _finish(background.pending)

        _wait(slice_copies(j + 1))
        pl.when(j + 2 < PAIRS)(lambda: _wait(pair_copies(j + 2)))
        pl.when(j + 3 < PAIRS)(lambda: _start(pair_copies(j + 3)))
        pl.when(j + 2 < PAIRS)(lambda: _start(slice_copies(j + 2)))
        return carry

    def last_head_pair(j, carry):
        _start([xa_copy(0), xa_copy(1)])
        background = _Background(j < 0, slice_work(j, [n for n in SLICE_JOBS if n > 4]), LAST_SLICE_RATE)
        begin, finish = attention_steps(j, LAST_CONTEXT_KEYS, lambda h, i: None,
                                        lambda i: background if i in LAST_SLICE_BLOCKS else None)
        for n, (h, i) in enumerate(LAST_PAIR_STEPS):
            begin(h, i)
            if n >= LAST_PAIR_LAG:
                finish(*LAST_PAIR_STEPS[n - LAST_PAIR_LAG])
        for h, i in LAST_PAIR_STEPS[-LAST_PAIR_LAG:]:
            finish(h, i)
        _finish(background.pending)
        return carry

    lax.fori_loop(0, PAIRS - 1, head_pair, 0)
    lax.fori_loop(PAIRS - 1, PAIRS, last_head_pair, 0)

    def store_blocks(i, col0, c):
        for a, n in ((0, 0), (1, 0), (0, 1), (1, 1)):
            obuf[i % 2, a * SUB:(a + 1) * SUB, col0 + n * HALF:col0 + (n + 1) * HALF] = c[a][n].astype(BF16)
            if col0 == 0:
                out_copy(i, 2 * a + n).start()
        if col0:
            out_copy(i, 4).start()

    def row_block(i, carry):
        xa_copy(i).wait()
        pl.when(i >= 2)(lambda: _wait([out_copy(i - 2, part) for part in range(5)]))
        loc[0:LOC_Q, 0:HALO, :] = loc[0:LOC_Q, BLK:BLK + HALO, :]

        x_ops = _operand_sums(
            lambda a, k: xa_raw[i % 2, a * SUB:(a + 1) * SUB, k * HALF:(k + 1) * HALF], A_TERMS)
        x_rounded = [op.astype(BF16) for op in x_ops]
        background = _Background(i < 0, slice_work(PAIRS - 1, FINAL_JOBS), FINAL_RATE)
        for part in LOCAL_PARTS:
            if part == 2:
                def value_product(r):
                    ops = _operand_sums(
                        lambda a, k: x_ops[r][64 * a:64 * (a + 1), QUARTER * k:QUARTER * (k + 1)], A_TERMS)
                    return _join(_block_product(
                        lambda u: _dot(ops[u].astype(BF16), _unpack(wva_sums[7 * r + u])),
                        PRODUCT_ORDER["local v inner"]))

                c = _block_product(value_product, PRODUCT_ORDER["local v outer"])
            else:
                rows = slice(part * HALF // 2, (part + 1) * HALF // 2)
                c = _block_product(lambda r: _dot(x_rounded[r], _unpack(background.tie(wqk_sums[r, rows, :]))),
                                   PRODUCT_ORDER["local qk"])
            for a in range(2):
                for g in range(8):
                    loc[(LOC_Q, LOC_K, LOC_V)[part] + g, HALO + a * SUB:HALO + (a + 1) * SUB, :] = (
                        c[a][g // 4][:, (g % 4) * LANES:(g % 4 + 1) * LANES])
        _finish(background.pending)

        def context_block(a, k):
            rows = _rows(i * BLK + a * (BLK // 4), BLK // 4)
            return jnp.concatenate(
                [ctx[j, rows, :] for j in range(k * PAIRS // 4, (k + 1) * PAIRS // 4)], axis=1).astype(F32)

        context_ops = _operand_sums2(context_block, A_TERMS)
        marks = []

        def output_product(r):
            ops = context_ops[r]()

            def product(u):
                acc = None
                for k0 in range(0, DM, OUTPUT_DEPTH):
                    part = _dot(ops[u][:, k0:k0 + OUTPUT_DEPTH].astype(BF16),
                                _unpack(wob_sums[7 * r + u, k0 // 2:(k0 + OUTPUT_DEPTH) // 2, :]))
                    acc = part if acc is None else acc + part
                    marks.append(acc)
                return acc

            return _join(_block_product(product, PRODUCT_ORDER["out b inner"]))

        store_blocks(i, DM, _block_product(output_product, PRODUCT_ORDER["out b outer"]))

        ticks = itertools.count()
        last_tick = LOCAL_STAGES * BLK // LOCAL_ROWS - 1

        def paced(values):
            lo, hi = LOCAL_PACE
            mark = marks[int((lo + (hi - lo) * next(ticks) / last_tick) * (len(marks) - 1))]
            return [jnp.where(i < 0, mark[0:LOCAL_ROWS, 0:LANES], v) for v in values]

        def attend(c0):
            def shifted(base, g, w):
                r0 = HALO + c0 - A_DIL * w
                return loc[base + g, r0:r0 + LOCAL_ROWS, :]

            every = 16 // LOCAL_STAGES
            queries = [shifted(LOC_Q, g, 0) for g in range(8)]
            logits = []
            for w in range(A_WIN):
                if w % every == 0:
                    q = paced(queries)
                acc = q[0] * shifted(LOC_K, 0, w)
                for g in range(1, 8):
                    acc = acc + q[g] * shifted(LOC_K, g, w)
                acc = acc + pltpu.roll(acc, 2 * A_HEADS, 1)
                acc = acc + pltpu.roll(acc, A_HEADS, 1)
                if c0 < A_DIL * w:
                    pos = i * BLK + c0 + lax.broadcasted_iota(jnp.int32, (LOCAL_ROWS, LANES), 0)
                    acc = jnp.where(pos >= A_DIL * w, acc, NEG * A_DH ** 0.5)
                logits.append(acc)
            m = functools.reduce(jnp.maximum, logits)
            p = [jnp.exp2((l - m) * (A_DH ** -0.5 * LOG2E)) for l in logits]
            inverse = _reciprocal(functools.reduce(jnp.add, p))
            p = [t * inverse for t in p]
            out = []
            for g in range(8):
                if g % every == 0:
                    weights = paced(p)
                out.append(functools.reduce(
                    jnp.add, [weights[w] * shifted(LOC_V, g, w) for w in range(A_WIN)]))
            return out

        quarters = [[] for _ in range(4)]
        for c0 in range(0, BLK // 4, LOCAL_ROWS):
            for a in range(4):
                quarters[a].append(jnp.concatenate(attend(a * (BLK // 4) + c0), axis=1))
        quarters = [jnp.concatenate(rows, axis=0) for rows in quarters]

        local_ops = _operand_sums2(lambda a, k: quarters[a][:, k * QUARTER:(k + 1) * QUARTER], A_TERMS)

        def local_product(r):
            ops = local_ops[r]()
            return _join(_block_product(
                lambda u: _dot(ops[u].astype(BF16), _unpack(woa_sums[7 * r + u])), PRODUCT_ORDER["out a inner"]))

        store_blocks(i, 0, _block_product(local_product, PRODUCT_ORDER["out a outer"]))
        pl.when(i + 2 < NBLK)(lambda: xa_copy(i + 2).start())
        return carry

    loc[0:LOC_Q, BLK:BLK + HALO, :] = jnp.zeros((LOC_Q, HALO, LANES), F32)
    lax.fori_loop(0, NBLK, row_block, 0)
    _wait([out_copy(i, part) for i in (NBLK - 2, NBLK - 1) for part in range(5)])


@jax.jit
def pallas_concat_heads__sliding_local_dilated__compressed_kv_cla__prompt_kernel(
    A_x: jax.Array,
    A_wqkv: jax.Array,
    A_wo: jax.Array,
    B_x: jax.Array,
    B_c_kv: jax.Array,
    B_w_q: jax.Array,
    B_w_uk: jax.Array,
    B_w_uv: jax.Array,
    B_w_o: jax.Array,
):
    vmem, sems = pltpu.VMEM, pltpu.SemaphoreType.DMA
    out = pl.pallas_call(
        _kernel,
        out_shape=jax.ShapeDtypeStruct((S, 2 * DM), BF16),
        in_specs=[pl.BlockSpec(memory_space=pl.ANY)] * 10,
        out_specs=pl.BlockSpec(memory_space=pl.ANY),
        scratch_shapes=[
            vmem((S, DM), BF16),
            vmem((S, B_DC), BF16),
            vmem((2, DM, B_DH), U32),
            vmem((2, B_DC, B_DH), U32),
            vmem((2, B_DC, B_DH), U32),
            vmem((26, S // 8, QUARTER), U32),
            vmem((7, S // 4, B_DC // 2), U32),
            vmem((NBLK // 2, 49, LANES // 2, LANES), U32),
            vmem((26, DM // 8, B_DH), U32),
            vmem((7, B_DC // 4, B_DH), U32),
            vmem((S, 2 * B_DH), BF16),
            vmem((2, S // 2, B_DH), U32),
            vmem((2, B_DH // 2, S), U32),
            vmem((PAIRS, S, 2 * B_DH), BF16),
            vmem((2, 2, 32, 2 * DM), BF16),
            vmem((2, 4, 16, DM), BF16),
            vmem((2, 2, A_HEADS, DM), U32),
            vmem((2, 4, 64, DM), BF16),
            vmem((7, HALF, HALF), U32),
            vmem((49, QUARTER // 2, QUARTER), U32),
            vmem((49, QUARTER // 2, QUARTER), U32),
            vmem((49, DM // 2, QUARTER), U32),
            vmem((2, BLK, DM), BF16),
            vmem((LOC_Q + 8, HALO + BLK, LANES), F32),
            vmem((2, BLK, 2 * DM), BF16),
            sems((2, NBLK // 2)), sems((2, 3)), sems((2,)), sems((2,)), sems((2,)),
        ],
        compiler_params=pltpu.CompilerParams(vmem_limit_bytes=120 * 2 ** 20, disable_bounds_checks=True),
        name="local_and_latent_attention",
    )(A_x.reshape(S, DM), A_wqkv.reshape(2, HALF, 3 * DM), A_wqkv.reshape(4, QUARTER, 3 * DM),
      A_wo.reshape(A_HEADS, A_DH, DM), B_x.reshape(S, DM), B_c_kv.reshape(S, B_DC),
      B_w_q, B_w_uk, B_w_uv, B_w_o.reshape(4, DM, DM))
    return out.reshape(1, S, 2 * DM)
```

```python
import functools
import itertools

import jax
import jax.numpy as jnp
from jax import lax
import jax.experimental.pallas as pl
import jax.experimental.pallas.tpu as pltpu
import numpy as np

S = 2048
DM = 1024
HALF, QUARTER = DM // 2, DM // 4
LANES = 128
A_HEADS, A_DH, A_WIN, A_DIL = 32, 32, 8, 2
HALO = 16
B_HEADS, B_DH, B_DC = 32, 128, 512
PAIRS = B_HEADS // 2

BLK = 256
SUB = BLK // 2
NBLK = S // BLK

LOG2E = 1.4426950408889634
NEG = -1e9
F32, BF16, U32 = jnp.float32, jnp.bfloat16, jnp.uint32

A_TERMS = (((1, 0, 0), (1, 1, 1)), ((1, 1, 0), (1, 1, 1)), ((1, 0, 0),), ((1, 1, 1),),
           ((1, 0, 0), (1, 0, 1)), ((1, 1, 0), (-1, 0, 0)), ((1, 0, 1), (-1, 1, 1)))
B_TERMS = (((1, 0, 0), (1, 1, 1)), ((1, 0, 0),), ((1, 0, 1), (-1, 1, 1)), ((1, 1, 0), (-1, 0, 0)),
           ((1, 1, 1),), ((1, 0, 0), (1, 0, 1)), ((1, 1, 0), (1, 1, 1)))
C_TERMS = (((1, 0, 0), (1, 1, 1)), ((1, 1, 0), (-1, 1, 1)), ((1, 0, 1), (1, 1, 1)), ((1, 0, 0), (1, 1, 0)),
           ((-1, 0, 0), (1, 0, 1)), ((1, 1, 1),), ((1, 0, 0),))

HK_A, HK_B, HK_C = zip(
    (((1, 0, 0), (-1, 0, 1), (-1, 2, 0)), ((1, 0, 0), (-1, 0, 1)), ((1, 0, 0),)),
    (((1, 0, 0), (-1, 0, 2), (-1, 1, 0)), ((1, 0, 1),), ((1, 0, 0), (1, 0, 1))),
    (((1, 0, 3), (1, 1, 1), (-1, 1, 0), (-1, 1, 3), (-1, 2, 1)), ((1, 1, 0),), ((1, 1, 0),)),
    (((1, 1, 1), (1, 3, 0), (-1, 0, 1), (-1, 1, 2), (-1, 3, 1)), ((1, 1, 1),), ((1, 1, 1),)),
    (((1, 1, 0), (-1, 0, 3)), ((1, 0, 0), (1, 1, 0)), ((1, 0, 0), (1, 0, 1), (1, 1, 0), (1, 1, 1))),
    (((1, 0, 1), (-1, 3, 0)), ((1, 0, 1), (1, 1, 1), (-1, 0, 0), (-1, 1, 0)), ((1, 0, 1), (1, 1, 1))),
    (((1, 0, 1), (-1, 1, 0)), ((1, 0, 0), (1, 1, 0), (-1, 0, 1)), ((1, 0, 0), (1, 0, 1), (1, 1, 1))),
    (((1, 3, 0), (1, 3, 3), (-1, 0, 3), (-1, 2, 3), (-1, 3, 1)), ((1, 3, 0), (-1, 3, 1)), ((1, 3, 0),)),
    (((1, 0, 3), (1, 3, 3), (-1, 1, 3), (-1, 3, 0), (-1, 3, 2)), ((1, 3, 1),), ((1, 3, 0), (1, 3, 1))),
    (((1, 0, 3),), ((1, 0, 0), (1, 1, 0), (1, 3, 0)), ((1, 0, 0), (1, 1, 0), (1, 3, 0))),
    (((1, 3, 0),), ((1, 0, 1), (1, 1, 1), (1, 3, 1)), ((1, 0, 1), (1, 1, 1), (1, 3, 1))),
    (((1, 0, 3), (-1, 3, 0)), ((1, 0, 0), (1, 1, 0), (1, 3, 1)), ((1, 0, 1), (1, 1, 1), (-1, 3, 0))),
    (((1, 1, 3), (-1, 0, 3)), ((1, 1, 0), (1, 3, 0)), ((1, 1, 0), (1, 1, 1), (1, 3, 0), (1, 3, 1))),
    (((1, 3, 1), (-1, 3, 0)), ((1, 1, 1), (1, 3, 1), (-1, 1, 0), (-1, 3, 0)), ((1, 1, 1), (1, 3, 1))),
    (((1, 0, 3), (1, 3, 1), (-1, 1, 3), (-1, 3, 0)),
     ((1, 1, 0), (1, 3, 0), (-1, 3, 1)), ((1, 1, 1), (1, 3, 0), (1, 3, 1))),
    (((1, 2, 2), (-1, 1, 2), (-1, 2, 0), (-1, 2, 3)), ((1, 2, 0),), ((1, 2, 0), (1, 2, 1))),
    (((1, 2, 2), (-1, 0, 2), (-1, 2, 1), (-1, 3, 2)), ((1, 2, 1), (-1, 2, 0)), ((1, 2, 1),)),
    (((1, 2, 0),), ((1, 0, 0), (1, 2, 0)), ((1, 0, 0), (1, 2, 0))),
    (((1, 0, 2),), ((1, 0, 1), (1, 2, 1)), ((1, 0, 1), (1, 2, 1))),
    (((1, 0, 2), (-1, 2, 0)), ((1, 0, 1), (1, 2, 0)), ((1, 0, 0), (-1, 2, 1))),
    (((1, 2, 1),), ((1, 1, 0), (1, 2, 0), (-1, 1, 1), (-1, 2, 1)), ((1, 1, 0), (1, 2, 0))),
    (((1, 1, 2),), ((1, 1, 1), (1, 2, 1)), ((1, 1, 0), (1, 1, 1), (1, 2, 0), (1, 2, 1))),
    (((1, 2, 1), (-1, 1, 2)), ((1, 1, 1), (1, 2, 1), (-1, 2, 0)), ((1, 1, 0), (1, 2, 0), (1, 2, 1))),
    (((1, 2, 3),), ((1, 2, 0), (1, 3, 0)), ((1, 2, 0), (1, 3, 0))),
    (((1, 3, 2),), ((1, 2, 1), (1, 3, 1)), ((1, 2, 1), (1, 3, 1))),
    (((1, 2, 3), (-1, 3, 2)), ((1, 2, 0), (1, 3, 1)), ((1, 2, 1), (-1, 3, 0))),
)

LOC_K, LOC_V, LOC_Q = 0, 8, 16

PAIR_STEPS = (
    ("s0", "v", "s1", "k", "c0", "q", "c1"),
    ("s0", "s1", "q", "c0", "v", "c1", "k"),
    ("s0", "s1", "k", "c0", "q", "c1", "v"),
    ("s0", "s1", "c0", "k", "q", "c1", "v"),
    ("s0", "v", "s1", "k", "c0", "q", "c1"),
    ("s0", "s1", "k", "c0", "q", "c1", "v"),
    ("s0", "k", "s1", "c0", "q", "c1"),
    ("s0", "s1", "c0", "c1"),
)
LAST_PAIR_STEPS = (
    (0, 7), (1, 1), (0, 0), (1, 7), (0, 6), (1, 0), (1, 6), (0, 1),
    (0, 5), (1, 5), (0, 4), (1, 2), (0, 2), (1, 3), (1, 4), (0, 3),
)
LAST_PAIR_LAG = 3
PRODUCT_ORDER = {
    "q": (1, 3, 0, 2, 9, 4, 11, 7, 8, 10, 12, 5, 13, 6, 14, 20, 15, 16, 22, 17, 18, 19, 24, 21, 23, 25),
    "k": (6, 0, 3, 4, 2, 5, 1),
    "v inner": (0, 5, 2, 4, 6, 3, 1),
    "v outer": (3, 0, 4, 6, 1, 2, 5),
    "local qk": (0, 3, 6, 4, 2, 1, 5),
    "local v inner": (3, 1, 0, 6, 4, 2, 5),
    "local v outer": (0, 3, 4, 6, 1, 2, 5),
    "out b inner": (3, 1, 2, 4, 0, 6, 5),
    "out b outer": (2, 5, 0, 1, 3, 6, 4),
    "out a inner": (6, 5, 2, 0, 4, 3, 1),
    "out a outer": (0, 3, 4, 6, 1, 2, 5),
}
VALUE_SPLIT = 2
CONTEXT_KEYS, LAST_CONTEXT_KEYS = 1024, 2048
SLICE_JOBS, SLICE_BLOCKS = (4, 5, 6, 1, 0, 7, 3, 2), (6, 5, 4, 3, 2, 1)
LAST_SLICE_BLOCKS, LAST_SLICE_RATE = (6, 5, 4, 2, 0), 0.7
EARLY_SCORES, EARLY_CONTEXT, EARLY_RATE = ((0, 6), (0, 7), (1, 6)), (6, 7), 2
FINAL_JOBS, FINAL_RATE = (2, 1, 3, 0, 4), 14
LOCAL_PARTS, LOCAL_ROWS, LOCAL_STAGES, LOCAL_PACE = (2, 1, 0), 16, 16, (0, 0.92)
OUTPUT_DEPTH = 128


def _pack(x):
    return pltpu.bitcast(x.astype(BF16), U32)


def _unpack(x):
    return pltpu.bitcast(x, BF16)


def _word_half(word, hi):
    return pltpu.bitcast(word & np.uint32(0xFFFF0000) if hi else word << 16, F32)


def _dot(a, b):
    return jnp.dot(a, b, preferred_element_type=F32)


def _dot_nt(a, b):
    return lax.dot_general(a, b, (((1,), (1,)), ((), ())), preferred_element_type=F32)


def _reciprocal(x):
    r = pl.reciprocal(x, approx=True)
    return r * (2.0 - x * r)


def _operand_sums(block, terms, shape=(2, 2)):
    blocks = [[block(i, j) for j in range(shape[1])] for i in range(shape[0])]
    out = []
    for (_, i, j), *rest in terms:
        acc = blocks[i][j]
        for sign, i, j in rest:
            a, b = acc.astype(F32), blocks[i][j].astype(F32)
            acc = a + b if sign > 0 else a - b
        out.append(acc)
    return out


def _operand_sums2(block, terms):
    outer = [[_operand_sums(lambda i, j: block(2 * i + a, 2 * j + b), terms) for b in range(2)]
             for a in range(2)]
    return [functools.partial(_operand_sums, lambda a, b, r=r: outer[a][b][r], terms) for r in range(7)]


def _block_product(product, order, c=None, terms=C_TERMS):
    c = c or [[None, None], [None, None]]
    for r in order:
        m = product(r)
        for sign, i, j in terms[r]:
            if c[i][j] is None:
                c[i][j] = m if sign > 0 else -m
            else:
                c[i][j] = c[i][j] + m if sign > 0 else c[i][j] - m
    return c


def _join(c):
    return jnp.concatenate([jnp.concatenate(row, axis=1) for row in c], axis=0)


def _heads_to_lanes(groups):
    lane = lax.broadcasted_iota(jnp.int32, groups[0].shape, 1)
    groups = list(groups)
    for group_bit, lane_bit in ((2, 4), (1, 3), (0, 2), (2, 6), (2, 1), (1, 5), (1, 0)):
        shift = 1 << lane_bit
        low = (lane & shift) == 0
        for g in range(8):
            if g >> group_bit & 1:
                continue
            x, y = groups[g], groups[g | 1 << group_bit]
            groups[g] = jnp.where(low, x, pltpu.roll(y, shift, 1))
            groups[g | 1 << group_bit] = jnp.where(low, pltpu.roll(x, LANES - shift, 1), y)
    return [groups[(g & 1) << 2 | (g >> 2) << 1 | (g >> 1 & 1)] for g in range(8)]


class _Background:
    def __init__(self, never, pieces, rate):
        self.never, self.pending, self.rate, self.credit = never, pieces, rate, 0.0

    def tie(self, words):
        self.credit += self.rate
        due = [pltpu.bitcast(d, U32) for d in itertools.islice(self.pending, int(self.credit))]
        self.credit -= int(self.credit)
        if not due:
            return words
        mark = functools.reduce(jnp.bitwise_or, [
            d[r:r + 8, c:c + LANES]
            for d in due for r in range(0, d.shape[0], 8) for c in range(0, d.shape[1], LANES)])
        top = jnp.where(self.never, mark, words[:8, :LANES])
        if words.shape[1] > LANES:
            top = jnp.concatenate([top, words[:8, LANES:]], axis=1)
        return jnp.concatenate([top, words[8:]], axis=0)

    def tie_tiles(self, words, axis, size):
        return jnp.concatenate([self.tie(lax.slice_in_dim(words, t, t + size, axis=axis))
                                for t in range(0, words.shape[axis], size)], axis=axis)


def _finish(generator):
    for _ in generator:
        pass


def _start(copies):
    for copy in copies:
        copy.start()


def _wait(copies):
    for copy in copies:
        copy.wait()


def _rows(start, size):
    return pl.ds(start if isinstance(start, int) else pl.multiple_of(start, size), size)


def _packed_rows(start, size):
    return _rows(start // 2, size // 2)


def _kernel(xa_hbm, wqkv_halves, wqkv_quarters, woa_hbm, xb_hbm, c_hbm, wq_hbm, wuk_hbm, wuv_hbm, wob_quarters,
            out_hbm,
            xb_raw, c_raw, wq_raw, wuk_raw, wuv_raw,
            x_sums, c_sums, ct_sums, wq_sums, wk_sums,
            q_s, k_s, vt_s, ctx,
            wqk_raw, wva_raw, woa_raw, wob_raw,
            wqk_sums, wva_sums, woa_sums, wob_sums,
            xa_raw, loc, obuf,
            sem_in, sem_pair, sem_slice, sem_xa, sem_out):
    wq_words, wuk_words, wuv_words = wq_hbm.bitcast(U32), wuk_hbm.bitcast(U32), wuv_hbm.bitcast(U32)
    woa_words = woa_hbm.bitcast(U32)

    def pair_copies(j, which=(0, 1, 2)):
        ends = ((wuk_words, wuk_raw), (wuv_words, wuv_raw), (wq_words, wq_raw))
        return [pltpu.make_async_copy(ends[n][0].at[:, j, :], ends[n][1].at[j % 2], sem_pair.at[j % 2, n])
                for n in which]

    def slice_copies(j):
        slot = j % 2
        ends = [(wqkv_halves.at[:, _rows(j * 32, 32), 0:2 * DM], wqk_raw.at[slot]),
                (wqkv_quarters.at[:, _rows(j * 16, 16), 2 * DM:3 * DM], wva_raw.at[slot]),
                (wob_quarters.at[:, _rows(j * 64, 64), :], wob_raw.at[slot])]
        ends += [(woa_words.at[:, (j >> 1 & 1) | k << 1 | (j >> 2) << 2, :], woa_raw.at[slot, k])
                 for k in range(2)]
        return [pltpu.make_async_copy(src, dst, sem_slice.at[slot]) for src, dst in ends]

    def latent_copy(n):
        rows = _rows(n * 2 * BLK, 2 * BLK)
        return pltpu.make_async_copy(c_hbm.at[rows, :], c_raw.at[rows, :], sem_in.at[0, n])

    def xb_copy(n):
        rows = _rows(n * 2 * BLK, 2 * BLK)
        return pltpu.make_async_copy(xb_hbm.at[rows, :], xb_raw.at[rows, :], sem_in.at[1, n])

    def xa_copy(i):
        return pltpu.make_async_copy(xa_hbm.at[_rows(i * BLK, BLK), :], xa_raw.at[i % 2], sem_xa.at[i % 2])

    def out_copy(i, part):
        r0, nr, c0, nc = (0, BLK, DM, DM) if part == 4 else (part // 2 * SUB, SUB, part % 2 * HALF, HALF)
        return pltpu.make_async_copy(obuf.at[i % 2, r0:r0 + nr, c0:c0 + nc],
                                     out_hbm.at[_rows(i * BLK + r0, nr), c0:c0 + nc], sem_out.at[i % 2])

    def prepare_weights(j, raw, dst, terms, parts):
        slot, depth = j % 2, raw.shape[1] // parts
        for r0 in range(0, depth, 32):
            words = [raw[slot, k * depth + r0:k * depth + r0 + 32, :] for k in range(parts)]
            for r, op in enumerate(_operand_sums(lambda k, head: _word_half(words[k], head), terms, (parts, 2))):
                op = _pack(op)
                dst[r, r0 // 2:r0 // 2 + 16, :] = op
                yield op

    def prepare_inputs(i, raw, dst, terms, parts):
        rows, width = BLK // parts, raw.shape[1] // parts
        ops = _operand_sums(lambda a, k: raw[_rows(i * BLK + a * rows, rows), k * width:(k + 1) * width],
                            terms, (parts, parts))
        ops = [_pack(op) for op in ops]
        for r, op in enumerate(ops):
            dst[r, _packed_rows(i * rows, rows), :] = op
        return ops

    def project_queries(i, background=None, ops=None):
        def product(r):
            w = wq_sums[r] if background is None else background.tie(wq_sums[r])
            return _dot(_unpack(x_sums[r, _packed_rows(i * 64, 64), :] if ops is None else ops[r]), _unpack(w))

        c = _block_product(product, PRODUCT_ORDER["q"], [[None, None] for _ in range(4)], HK_C)
        for a in range(4):
            q_s[_rows(i * BLK + a * 64, 64), :] = (
                jnp.concatenate(c[a], axis=1) * (B_DH ** -0.5 * LOG2E)).astype(BF16)

    def project_keys(i, background=None, ops=None):
        def product(r):
            w = wk_sums[r] if background is None else background.tie(wk_sums[r])
            return _dot(_unpack(c_sums[r, _packed_rows(i * SUB, SUB), :] if ops is None else ops[r]), _unpack(w))

        c = _block_product(product, PRODUCT_ORDER["k"])
        for a in range(2):
            for head in range(2):
                k_s[head, _packed_rows(i * BLK + a * SUB, SUB), :] = _pack(c[a][head])

    def value_weights(j):
        words = wuv_raw[j % 2].T

        def block(a, k):
            return _word_half(words[a % 2 * 64:(a % 2 + 1) * 64, k * LANES:(k + 1) * LANES], a // 2)

        return [[op.astype(BF16) for op in inner()] for inner in _operand_sums2(block, A_TERMS)]

    def prepare_latents(t):
        blocks = [[c_raw[_rows((4 * t + n) * LANES, LANES), k * LANES:(k + 1) * LANES].astype(F32).T
                   for n in range(4)] for k in range(4)]
        ops = [[_pack(op) for op in inner()] for inner in _operand_sums2(lambda k, n: blocks[k][n], B_TERMS)]
        for r in range(7):
            for u in range(7):
                ct_sums[t, 7 * r + u] = ops[r][u]
        return ops

    def project_values(t, weights, ops=None):
        def outer(r):
            return _join(_block_product(
                lambda u: _dot(weights[r][u], _unpack(ct_sums[t, 7 * r + u] if ops is None else ops[r][u])),
                PRODUCT_ORDER["v inner"]))

        c = _block_product(outer, PRODUCT_ORDER["v outer"][:VALUE_SPLIT])
        yield
        c = _block_product(outer, PRODUCT_ORDER["v outer"][VALUE_SPLIT:], c)
        for head in range(2):
            for n in range(2):
                vt_s[head, :, _rows((2 * t + n) * BLK, BLK)] = _pack(c[head][n])

    def scores(h, i, background):
        row = lax.broadcasted_iota(jnp.int32, (SUB, SUB), 0)
        col = lax.broadcasted_iota(jnp.int32, (SUB, SUB), 1)
        r0, cols = i * BLK, slice(h * B_DH, (h + 1) * B_DH)
        past = None
        if i:
            words = k_s[h, 0:r0 // 2, :]
            if background is not None:
                words = background.tie_tiles(words, 0, LANES // 2)
            past = _dot_nt(q_s[r0:r0 + BLK, cols], _unpack(words))
        diagonal = []
        for a in range(2):
            d = _dot_nt(q_s[r0 + a * SUB:r0 + (a + 1) * SUB, cols],
                        _unpack(k_s[h, r0 // 2:(r0 + (a + 1) * SUB) // 2, :]))
            last = jnp.where(col <= row, d[:, a * SUB:], NEG)
            diagonal.append(jnp.concatenate([d[:, :SUB], last], axis=1) if a else last)
        return past, diagonal

    def softmax(i, past, diagonal):
        p_past, p_diagonal, inverse = [], [], []
        for a in range(2):
            s = diagonal[a]
            if past is not None:
                s = jnp.concatenate([past[a * SUB:(a + 1) * SUB], s], axis=1)
            p = jnp.exp2(s - jnp.max(s, axis=1, keepdims=True)).astype(BF16)
            inverse.append(_reciprocal(jnp.sum(p.astype(F32), axis=1, keepdims=True)))
            if past is not None:
                p_past.append(p[:, :i * BLK])
            p_diagonal.append(p[:, i * BLK:])
        return (jnp.concatenate(p_past, axis=0) if p_past else None), p_diagonal, inverse

    def context(h, i, weights, keys, background):
        p_past, p_diagonal, inverse = weights
        r0 = i * BLK
        past = None
        for k0 in range(0, r0, keys):
            k1 = min(k0 + keys, r0)
            words = vt_s[h, :, k0:k1]
            if background is not None:
                words = background.tie_tiles(words, 1, LANES)
            part = _dot_nt(p_past[:, k0:k1], _unpack(words))
            past = part if past is None else past + part
        out = []
        for a in range(2):
            o = _dot_nt(p_diagonal[a], _unpack(vt_s[h, :, r0:r0 + (a + 1) * SUB]))
            if past is not None:
                o = o + past[a * SUB:(a + 1) * SUB]
            out.append(o * inverse[a])
        return out

    def slice_work(j, jobs):
        slot = j % 2

        def query_or_key(part):
            groups = [_heads_to_lanes([
                _pack(wqk_raw[slot, k, :, part * DM + a * LANES:part * DM + (a + 1) * LANES])
                for a in range(8)]) for k in range(2)]
            rows = _packed_rows(part * HALF + j * 32, 32)
            for a in range(4):
                for r, op in enumerate(_operand_sums(lambda k, n: _unpack(groups[k][4 * n + a]), B_TERMS)):
                    op = _pack(op)
                    wqk_sums[r, rows, a * LANES:(a + 1) * LANES] = op
                    yield op

        def two_levels(block, dst, row0, cols):
            for r, inner in enumerate(_operand_sums2(block, B_TERMS)):
                for u, op in enumerate(inner()):
                    op = _pack(op)
                    dst[7 * r + u, _packed_rows(row0, 2 * op.shape[0]), cols] = op
                    yield op

        def value():
            groups = [_heads_to_lanes([_pack(wva_raw[slot, k, :, a * LANES:(a + 1) * LANES]) for a in range(8)])
                      for k in range(4)]
            return two_levels(lambda k, n: _unpack(jnp.concatenate(groups[k][2 * n:2 * n + 2], axis=1)),
                              wva_sums, j * 16, slice(None))

        def output_a():
            return two_levels(
                lambda k, n: _word_half(woa_raw[slot, k % 2, :, _rows(n * QUARTER + j % 2 * LANES, LANES)], k // 2),
                woa_sums, ((j >> 1 & 1) * 4 + (j >> 2)) * A_HEADS, _rows(j % 2 * LANES, LANES))

        def output_b(r0, c0):
            return two_levels(
                lambda k, n: wob_raw[slot, k, r0:r0 + 32, n * QUARTER + c0:n * QUARTER + c0 + LANES],
                wob_sums, j * 64 + r0, slice(c0, c0 + LANES))

        for n in jobs:
            if n < 4:
                yield from output_b(n // 2 * 32, n % 2 * LANES)
            elif n == 4:
                yield from output_a()
            else:
                yield from value() if n == 7 else query_or_key(n - 5)

    def first_steps(copy, work, requests):
        def step(n, carry):
            copy(n).wait()
            for at, copies in requests:
                pl.when(n == at)(lambda: _start(copies()))
            work(n)
            return carry

        lax.fori_loop(0, NBLK // 2, step, 0)

    def first_keys_and_values(weights, n):
        for i in (2 * n, 2 * n + 1):
            project_keys(i, ops=prepare_inputs(i, c_raw, c_sums, A_TERMS, 2))
        _finish(project_values(n, weights, ops=prepare_latents(n)))

    def first_queries(n):
        for i in (2 * n, 2 * n + 1):
            project_queries(i, ops=prepare_inputs(i, xb_raw, x_sums, HK_A, 4))

    _start(pair_copies(0, (0, 1)) + [latent_copy(0)])
    _wait(pair_copies(0, (0,)))
    _start([latent_copy(1), latent_copy(2), latent_copy(3)] + pair_copies(0, (2,)) + [xb_copy(0)])
    _finish(prepare_weights(0, wuk_raw, wk_sums, B_TERMS, 2))
    _wait(pair_copies(0, (1,)))
    first_steps(latent_copy, functools.partial(first_keys_and_values, value_weights(0)),
                ((1, lambda: [xb_copy(1), xb_copy(2)]), (2, lambda: [xb_copy(3)]), (3, lambda: pair_copies(1))))
    _wait(pair_copies(0, (2,)))
    _finish(prepare_weights(0, wq_raw, wq_sums, HK_B, 4))
    first_steps(xb_copy, first_queries, ((0, lambda: slice_copies(0)),))
    _wait(pair_copies(1) + slice_copies(0))
    _start(pair_copies(2) + slice_copies(1))

    def attention_steps(j, keys, beside_scores, background):
        scored, done = {}, {}

        def begin(h, i):
            scored[h, i] = scores(h, i, beside_scores(h, i))

        def finish(h, i):
            done[h, i] = context(h, i, softmax(i, *scored.pop((h, i))), keys, background(i))
            if (1 - h, i) in done:
                for a in range(2):
                    ctx[j, i * BLK + a * SUB:i * BLK + (a + 1) * SUB, :] = (
                        jnp.concatenate([done[0, i][a], done[1, i][a]], axis=1).astype(BF16))

        return begin, finish

    def head_pair(j, carry):
        early = _Background(j < 0, itertools.chain(prepare_weights(j + 1, wq_raw, wq_sums, HK_B, 4),
                                                   prepare_weights(j + 1, wuk_raw, wk_sums, B_TERMS, 2)), EARLY_RATE)
        weights = value_weights(j + 1)
        background = _Background(j < 0, slice_work(j, SLICE_JOBS), 350 / (33 * len(SLICE_BLOCKS)))
        values = [project_values(t, weights) for t in range(NBLK // 2)]
        begin, finish = attention_steps(
            j, CONTEXT_KEYS, lambda h, i: early if (h, i) in EARLY_SCORES else None,
            lambda i: early if i in EARLY_CONTEXT else None)
        for i in range(NBLK - 1, -1, -1):
            for what in PAIR_STEPS[i]:
                if what[0] == "s":
                    begin(int(what[1]), i)
                elif what[0] == "c":
                    finish(int(what[1]), i)
                elif what == "q":
                    _finish(early.pending)
                    for n in (i + 1, i) if i + 2 == NBLK else (i,):
                        project_queries(n, background if n in SLICE_BLOCKS else None)
                elif what == "v":
                    next(values[i // 2 + 1], None)
                else:
                    _finish(early.pending)
                    project_keys(i + 1, background if i + 1 in SLICE_BLOCKS else None)
        project_keys(0, background if 0 in SLICE_BLOCKS else None)
        _finish(values[0])
        _finish(background.pending)

        _wait(slice_copies(j + 1))
        pl.when(j + 2 < PAIRS)(lambda: _wait(pair_copies(j + 2)))
        pl.when(j + 3 < PAIRS)(lambda: _start(pair_copies(j + 3)))
        pl.when(j + 2 < PAIRS)(lambda: _start(slice_copies(j + 2)))
        return carry

    def last_head_pair(j, carry):
        _start([xa_copy(0), xa_copy(1)])
        background = _Background(j < 0, slice_work(j, [n for n in SLICE_JOBS if n > 4]), LAST_SLICE_RATE)
        begin, finish = attention_steps(j, LAST_CONTEXT_KEYS, lambda h, i: None,
                                        lambda i: background if i in LAST_SLICE_BLOCKS else None)
        for n, (h, i) in enumerate(LAST_PAIR_STEPS):
            begin(h, i)
            if n >= LAST_PAIR_LAG:
                finish(*LAST_PAIR_STEPS[n - LAST_PAIR_LAG])
        for h, i in LAST_PAIR_STEPS[-LAST_PAIR_LAG:]:
            finish(h, i)
        _finish(background.pending)
        return carry

    lax.fori_loop(0, PAIRS - 1, head_pair, 0)
    lax.fori_loop(PAIRS - 1, PAIRS, last_head_pair, 0)

    def store_blocks(i, col0, c):
        for a, n in ((0, 0), (1, 0), (0, 1), (1, 1)):
            obuf[i % 2, a * SUB:(a + 1) * SUB, col0 + n * HALF:col0 + (n + 1) * HALF] = c[a][n].astype(BF16)
            if col0 == 0:
                out_copy(i, 2 * a + n).start()
        if col0:
            out_copy(i, 4).start()

    def row_block(i, carry):
        xa_copy(i).wait()
        pl.when(i >= 2)(lambda: _wait([out_copy(i - 2, part) for part in range(5)]))
        loc[0:LOC_Q, 0:HALO, :] = loc[0:LOC_Q, BLK:BLK + HALO, :]

        x_ops = _operand_sums(
            lambda a, k: xa_raw[i % 2, a * SUB:(a + 1) * SUB, k * HALF:(k + 1) * HALF], A_TERMS)
        x_rounded = [op.astype(BF16) for op in x_ops]
        background = _Background(i < 0, slice_work(PAIRS - 1, FINAL_JOBS), FINAL_RATE)
        for part in LOCAL_PARTS:
            if part == 2:
                def value_product(r):
                    ops = _operand_sums(
                        lambda a, k: x_ops[r][64 * a:64 * (a + 1), QUARTER * k:QUARTER * (k + 1)], A_TERMS)
                    return _join(_block_product(
                        lambda u: _dot(ops[u].astype(BF16), _unpack(wva_sums[7 * r + u])),
                        PRODUCT_ORDER["local v inner"]))

                c = _block_product(value_product, PRODUCT_ORDER["local v outer"])
            else:
                rows = slice(part * HALF // 2, (part + 1) * HALF // 2)
                c = _block_product(lambda r: _dot(x_rounded[r], _unpack(background.tie(wqk_sums[r, rows, :]))),
                                   PRODUCT_ORDER["local qk"])
            for a in range(2):
                for g in range(8):
                    loc[(LOC_Q, LOC_K, LOC_V)[part] + g, HALO + a * SUB:HALO + (a + 1) * SUB, :] = (
                        c[a][g // 4][:, (g % 4) * LANES:(g % 4 + 1) * LANES])
        _finish(background.pending)

        def context_block(a, k):
            rows = _rows(i * BLK + a * (BLK // 4), BLK // 4)
            return jnp.concatenate(
                [ctx[j, rows, :] for j in range(k * PAIRS // 4, (k + 1) * PAIRS // 4)], axis=1).astype(F32)

        context_ops = _operand_sums2(context_block, A_TERMS)
        marks = []

        def output_product(r):
            ops = context_ops[r]()

            def product(u):
                acc = None
                for k0 in range(0, DM, OUTPUT_DEPTH):
                    part = _dot(ops[u][:, k0:k0 + OUTPUT_DEPTH].astype(BF16),
                                _unpack(wob_sums[7 * r + u, k0 // 2:(k0 + OUTPUT_DEPTH) // 2, :]))
                    acc = part if acc is None else acc + part
                    marks.append(acc)
                return acc

            return _join(_block_product(product, PRODUCT_ORDER["out b inner"]))

        store_blocks(i, DM, _block_product(output_product, PRODUCT_ORDER["out b outer"]))

        ticks = itertools.count()
        last_tick = LOCAL_STAGES * BLK // LOCAL_ROWS - 1

        def paced(values):
            lo, hi = LOCAL_PACE
            mark = marks[int((lo + (hi - lo) * next(ticks) / last_tick) * (len(marks) - 1))]
            return [jnp.where(i < 0, mark[0:LOCAL_ROWS, 0:LANES], v) for v in values]

        def attend(c0):
            def shifted(base, g, w):
                r0 = HALO + c0 - A_DIL * w
                return loc[base + g, r0:r0 + LOCAL_ROWS, :]

            every = 16 // LOCAL_STAGES
            queries = [shifted(LOC_Q, g, 0) for g in range(8)]
            logits = []
            for w in range(A_WIN):
                if w % every == 0:
                    q = paced(queries)
                acc = q[0] * shifted(LOC_K, 0, w)
                for g in range(1, 8):
                    acc = acc + q[g] * shifted(LOC_K, g, w)
                acc = acc + pltpu.roll(acc, 2 * A_HEADS, 1)
                acc = acc + pltpu.roll(acc, A_HEADS, 1)
                if c0 < A_DIL * w:
                    pos = i * BLK + c0 + lax.broadcasted_iota(jnp.int32, (LOCAL_ROWS, LANES), 0)
                    acc = jnp.where(pos >= A_DIL * w, acc, NEG * A_DH ** 0.5)
                logits.append(acc)
            m = functools.reduce(jnp.maximum, logits)
            p = [jnp.exp2((l - m) * (A_DH ** -0.5 * LOG2E)) for l in logits]
            inverse = _reciprocal(functools.reduce(jnp.add, p))
            p = [t * inverse for t in p]
            out = []
            for g in range(8):
                if g % every == 0:
                    weights = paced(p)
                out.append(functools.reduce(
                    jnp.add, [weights[w] * shifted(LOC_V, g, w) for w in range(A_WIN)]))
            return out

        quarters = [[] for _ in range(4)]
        for c0 in range(0, BLK // 4, LOCAL_ROWS):
            for a in range(4):
                quarters[a].append(jnp.concatenate(attend(a * (BLK // 4) + c0), axis=1))
        quarters = [jnp.concatenate(rows, axis=0) for rows in quarters]

        local_ops = _operand_sums2(lambda a, k: quarters[a][:, k * QUARTER:(k + 1) * QUARTER], A_TERMS)

        def local_product(r):
            ops = local_ops[r]()
            return _join(_block_product(
                lambda u: _dot(ops[u].astype(BF16), _unpack(woa_sums[7 * r + u])), PRODUCT_ORDER["out a inner"]))

        store_blocks(i, 0, _block_product(local_product, PRODUCT_ORDER["out a outer"]))
        pl.when(i + 2 < NBLK)(lambda: xa_copy(i + 2).start())
        return carry

    loc[0:LOC_Q, BLK:BLK + HALO, :] = jnp.zeros((LOC_Q, HALO, LANES), F32)
    lax.fori_loop(0, NBLK, row_block, 0)
    _wait([out_copy(i, part) for i in (NBLK - 2, NBLK - 1) for part in range(5)])


@jax.jit
def pallas_concat_heads__sliding_local_dilated__compressed_kv_cla__prompt_kernel(
    A_x: jax.Array,
    A_wqkv: jax.Array,
    A_wo: jax.Array,
    B_x: jax.Array,
    B_c_kv: jax.Array,
    B_w_q: jax.Array,
    B_w_uk: jax.Array,
    B_w_uv: jax.Array,
    B_w_o: jax.Array,
):
    vmem, sems = pltpu.VMEM, pltpu.SemaphoreType.DMA
    out = pl.pallas_call(
        _kernel,
        out_shape=jax.ShapeDtypeStruct((S, 2 * DM), BF16),
        in_specs=[pl.BlockSpec(memory_space=pl.ANY)] * 10,
        out_specs=pl.BlockSpec(memory_space=pl.ANY),
        scratch_shapes=[
            vmem((S, DM), BF16),
            vmem((S, B_DC), BF16),
            vmem((2, DM, B_DH), U32),
            vmem((2, B_DC, B_DH), U32),
            vmem((2, B_DC, B_DH), U32),
            vmem((26, S // 8, QUARTER), U32),
            vmem((7, S // 4, B_DC // 2), U32),
            vmem((NBLK // 2, 49, LANES // 2, LANES), U32),
            vmem((26, DM // 8, B_DH), U32),
            vmem((7, B_DC // 4, B_DH), U32),
            vmem((S, 2 * B_DH), BF16),
            vmem((2, S // 2, B_DH), U32),
            vmem((2, B_DH // 2, S), U32),
            vmem((PAIRS, S, 2 * B_DH), BF16),
            vmem((2, 2, 32, 2 * DM), BF16),
            vmem((2, 4, 16, DM), BF16),
            vmem((2, 2, A_HEADS, DM), U32),
            vmem((2, 4, 64, DM), BF16),
            vmem((7, HALF, HALF), U32),
            vmem((49, QUARTER // 2, QUARTER), U32),
            vmem((49, QUARTER // 2, QUARTER), U32),
            vmem((49, DM // 2, QUARTER), U32),
            vmem((2, BLK, DM), BF16),
            vmem((LOC_Q + 8, HALO + BLK, LANES), F32),
            vmem((2, BLK, 2 * DM), BF16),
            sems((2, NBLK // 2)), sems((2, 3)), sems((2,)), sems((2,)), sems((2,)),
        ],
        compiler_params=pltpu.CompilerParams(vmem_limit_bytes=124 * 2 ** 20, disable_bounds_checks=True),
        name="local_and_latent_attention",
    )(A_x.reshape(S, DM), A_wqkv.reshape(2, HALF, 3 * DM), A_wqkv.reshape(4, QUARTER, 3 * DM),
      A_wo.reshape(A_HEADS, A_DH, DM), B_x.reshape(S, DM), B_c_kv.reshape(S, B_DC),
      B_w_q, B_w_uk, B_w_uv, B_w_o.reshape(4, DM, DM))
    return out.reshape(1, S, 2 * DM)
```
